```python
import jax
import jax.numpy as jnp

def _softmax(x, axis=-1):
    return jax.nn.softmax(x, axis=axis)

def _gelu(x):
    return jax.nn.gelu(x, approximate=True)

def _silu(x):
    return jax.nn.silu(x)

def _sigmoid(x):
    return jax.nn.sigmoid(x)

def _layernorm(x, axis=-1, eps=1e-05):
    m = jnp.mean(x, axis=axis, keepdims=True)
    v = jnp.var(x, axis=axis, keepdims=True)
    return (x - m) / jnp.sqrt(v + eps)

def _scatter_add(tgt, idx, src, axis=0):
    return tgt.at[idx].add(src)

def _segment_sum(src, seg, n):
    return jax.ops.segment_sum(src, seg, n)

class _Rng:

    def __init__(self, key):
        self._k = key

    def _next(self):
        self._k, sub = jax.random.split(self._k)
        return sub

    def normal(self, shape):
        return jax.random.normal(self._next(), shape, dtype=jnp.bfloat16)

    def randint(self, lo, hi, shape):
        return jax.random.randint(self._next(), shape, lo, hi, dtype=jnp.int32)

    def uniform(self, shape, lo=0.0, hi=1.0):
        return jax.random.uniform(self._next(), shape, jnp.bfloat16, lo, hi)

    def permutation(self, n):
        return jax.random.permutation(self._next(), n)
kernel_name = 'adaLN_cond__compressed_kv_cla__mixer_s_mlp__prompt'

def setup_inputs():
    _rng = _Rng(jax.random.key(int.from_bytes(__import__("os").urandom(4), "little")))
    _w = lambda a: (lambda t: t.astype(jnp.bfloat16) if jnp.issubdtype(t.dtype, jnp.floating) else t)(jnp.asarray(a))

    def _A_setup():
        B, H, Sq, Sk, D, M = (1, 32, 2048, 2048, 128, 640)
        Dc = 4 * D
        return {'x': _w((lambda *s: _rng.normal(s) * 0.05)(B, Sq, M)), 'c_kv': _w((lambda *s: _rng.normal(s) * 0.05)(B, Sk, Dc)), 'w_q': _w((lambda *s: _rng.normal(s) * 0.05)(M, H, D) * M ** (-0.5)), 'w_uk': _w((lambda *s: _rng.normal(s) * 0.05)(Dc, H, D) * Dc ** (-0.5)), 'w_uv': _w((lambda *s: _rng.normal(s) * 0.05)(Dc, H, D) * Dc ** (-0.5)), 'w_o': _w((lambda *s: _rng.normal(s) * 0.05)(H, D, M) * (H * D) ** (-0.5))}
    _A_in = _A_setup()

    def _B_setup():
        B, S, D, F = (1, 2048, 640, 1728)
        return {'x': _w((lambda *s: _rng.normal(s) * 0.05)(B, S, D)), 'w1': _w((lambda *s: _rng.normal(s) * 0.05)(D, D) * D ** (-0.5)), 'w2': _w((lambda *s: _rng.normal(s) * 0.05)(D, D) * D ** (-0.5)), 'w3': _w((lambda *s: _rng.normal(s) * 0.05)(D, F) * D ** (-0.5)), 'w4': _w((lambda *s: _rng.normal(s) * 0.05)(F, D) * F ** (-0.5))}
    _B_in = _B_setup()
    return {'A_x': _A_in['x'], 'A_c_kv': _A_in['c_kv'], 'A_w_q': _A_in['w_q'], 'A_w_uk': _A_in['w_uk'], 'A_w_uv': _A_in['w_uv'], 'A_w_o': _A_in['w_o'], 'B_x': _B_in['x'], 'B_w1': _B_in['w1'], 'B_w2': _B_in['w2'], 'B_w3': _B_in['w3'], 'B_w4': _B_in['w4'], 'c': _w((lambda *s: _rng.normal(s) * 0.05)(1, 640)), 'w_mod': _w((lambda *s: _rng.normal(s) * 0.05)(640, 6 * 640) * 640 ** (-0.5))}

def reference(A_x, A_c_kv, A_w_q, A_w_uk, A_w_uv, A_w_o, B_x, B_w1, B_w2, B_w3, B_w4, c, w_mod):

    def _A_ref(x, c_kv, w_q, w_uk, w_uv, w_o):
        B, Sq, M = (x.shape[0], x.shape[1], x.shape[2])
        Sk = c_kv.shape[1]
        H, D = (w_q.shape[1], w_q.shape[2])
        q = jnp.einsum('bqm,mhd->bhqd', x, w_q)
        k = jnp.einsum('bkc,chd->bhkd', c_kv, w_uk)
        v = jnp.einsum('bkc,chd->bhkd', c_kv, w_uv)
        scores = jnp.einsum('bhqd,bhkd->bhqk', q, k) * D ** (-0.5)
        off = Sk - Sq
        qi = jnp.arange(Sq)[:, None]
        kj = jnp.arange(Sk)[None, :]
        cmask = kj <= qi + off
        scores = jnp.where(cmask[None, None], scores, -1000000000.0)
        p = _softmax(scores, axis=-1)
        ctx = jnp.einsum('bhqk,bhkd->bhqd', p, v)
        return jnp.einsum('bhqd,hdm->bqm', ctx, w_o)

    def _B_ref(x, w1, w2, w3, w4):
        B, S, D = x.shape
        h = _gelu(_layernorm(x, axis=-1) @ w1)
        c = D // 4
        g0 = jnp.pad(h[:, :, 0 * c:1 * c], ((0, 0), (1, 0), (0, 0)))[:, :S, :]
        g1 = jnp.pad(h[:, :, 1 * c:2 * c], ((0, 0), (0, 1), (0, 0)))[:, 1:, :]
        g2 = jnp.pad(h[:, :, 2 * c:3 * c], ((0, 0), (2, 0), (0, 0)))[:, :S, :]
        g3 = jnp.pad(h[:, :, 3 * c:], ((0, 0), (0, 2), (0, 0)))[:, 2:, :]
        hs = jnp.concatenate([g0, g1, g2, g3], axis=-1) @ w2
        x1 = x + hs
        h2 = _gelu(_layernorm(x1, axis=-1) @ w3) @ w4
        return x1 + h2
    x = A_x
    mod = (_silu(c) @ w_mod).reshape(c.shape[0], 6, 1, -1)
    sa, ca, ga, sb, cb, gb = (mod[:, 0].copy(), mod[:, 1].copy(), mod[:, 2].copy(), mod[:, 3].copy(), mod[:, 4].copy(), mod[:, 5].copy())
    h = _layernorm(x, axis=-1) * (1 + ca) + sa
    x = x + ga * _A_ref(h, A_c_kv, A_w_q, A_w_uk, A_w_uv, A_w_o)
    h = _layernorm(x, axis=-1) * (1 + cb) + sb
    x = x + gb * _B_ref(h, B_w1, B_w2, B_w3, B_w4)
    return x
```

```python
import math

import jax
import jax.numpy as jnp
import jax.experimental.pallas as pl
import jax.experimental.pallas.tpu as pltpu

BF16 = jnp.bfloat16
F32 = jnp.float32
U32 = jnp.uint32

LANES = 128
TQ = 128
TR = 256
HG = 16
PAD = 8
EPS = 1e-5
NEG = -1000000000.0
LOG2E = math.log2(math.e)

_NT = (((1,), (1,)), ((), ()))


def _ln(x):
    m = jnp.mean(x, axis=-1, keepdims=True)
    xc = x - m
    v = jnp.mean(xc * xc, axis=-1, keepdims=True)
    return xc * jax.lax.rsqrt(v + EPS)


def _gelu(x):
    return jax.nn.gelu(x, approximate=True)


def _dot(a, b):
    return jnp.dot(a, b, preferred_element_type=F32)


@jax.jit
def pallas_adaLN_cond__compressed_kv_cla__mixer_s_mlp__prompt_kernel(
    A_x: jax.Array,
    A_c_kv: jax.Array,
    A_w_q: jax.Array,
    A_w_uk: jax.Array,
    A_w_uv: jax.Array,
    A_w_o: jax.Array,
    B_x: jax.Array,
    B_w1: jax.Array,
    B_w2: jax.Array,
    B_w3: jax.Array,
    B_w4: jax.Array,
    c: jax.Array,
    w_mod: jax.Array,
):
    del B_x
    B, S, M = A_x.shape
    _, Sk, Dc = A_c_kv.shape
    _, H, D = A_w_q.shape
    Fh = B_w3.shape[1]
    assert B == 1 and Sk == S and D == LANES and H % HG == 0
    assert S % TQ == 0 and S % TR == 0 and M % LANES == 0 and M % 4 == 0
    NG = H // HG
    NQ = S // TQ
    NR = S // TR
    NC = M // LANES
    C4 = M // 4
    STQ = M + 1
    STK = Dc + 1
    qscale = float(D) ** -0.5 * LOG2E

    x2 = A_x.reshape(S, M)
    ckv2 = A_c_kv.reshape(S, Dc)
    wo2 = A_w_o.reshape(H * D, M)

    def kernel(x_hbm, ckv_hbm, wq_hbm, wuk_hbm, wuv_hbm, wo_hbm, w1_hbm, w2_hbm,
               w3_hbm, w4_hbm, c_ref, wmod_hbm, out_hbm,
               x_v, ckv_v, wq_r, wuk_r, wuv_r, wq_p, wuk_p, wuv_p, wo_v, w1_v,
               w2_v, w3_v, w4_v, wmod_v, mod_v, hn_v, q_v, k_v, v_v, ctx_v,
               x1_v, h2_v, hh_v, o_v, sems, osems):

        def cp(src, dst, i):
            return pltpu.make_async_copy(src, dst, sems.at[i])

        def grp(ref, g):
            return ref.at[:, pl.ds(g * HG, HG), :]

        c_ckv = cp(ckv_hbm, ckv_v, 0)
        c_x = cp(x_hbm, x_v, 1)
        c_mod = cp(wmod_hbm, wmod_v, 2)
        c_uk = [cp(grp(wuk_hbm, g), wuk_r.at[g], 3 + g) for g in range(NG)]
        c_uv = [cp(grp(wuv_hbm, g), wuv_r.at[g], 3 + NG + g) for g in range(NG)]
        c_q = [cp(grp(wq_hbm, g), wq_r.at[g], 3 + 2 * NG + g) for g in range(NG)]
        base = 3 + 3 * NG
        c_late = [cp(wo_hbm, wo_v, base), cp(w1_hbm, w1_v, base + 1),
                  cp(w2_hbm, w2_v, base + 2), cp(w3_hbm, w3_v, base + 3),
                  cp(w4_hbm, w4_v, base + 4)]

        c_x.start()
        c_mod.start()
        c_ckv.start()
        c_uk[0].start()
        c_uv[0].start()
        c_q[0].start()

        c_mod.wait()
        cc = c_ref[...].astype(F32)
        sc = (cc * jax.nn.sigmoid(cc)).astype(BF16)
        sc8 = jnp.broadcast_to(sc, (8, M))
        mod_v[...] = _dot(sc8, wmod_v[...])

        def mod(i):
            return mod_v[0:1, i * M:(i + 1) * M]

        c_x.wait()

        def ln1_body(r, carry):
            rows = pl.ds(pl.multiple_of(r * TR, TR), TR)
            xx = x_v[rows, :].astype(F32)
            hn_v[rows, :] = (_ln(xx) * (1.0 + mod(1)) + mod(0)).astype(BF16)
            return carry

        jax.lax.fori_loop(0, NR, ln1_body, 0)

        def relayout(raw, dst, g, rows, stride):
            def body(i, carry):
                for r in range(8):
                    m = i * 8 + r
                    val = pltpu.bitcast(raw[g, m], U32)
                    dst[pl.ds(g * (HG // 2) * stride + m, HG // 2, stride=stride), :] = val
                return carry
            for i in range(rows // 8):
                body(i, 0)

        def head_w(dst, h, rows, stride):
            u = dst[pl.ds((h // 2) * stride, rows), :]
            sh = (16 * (1 - h % 2)).astype(U32)
            return pltpu.bitcast((u << sh) & U32(0xFFFF0000), F32).astype(BF16)

        row_i = jax.lax.broadcasted_iota(jnp.int32, (TQ, TQ), 0)
        col_i = jax.lax.broadcasted_iota(jnp.int32, (TQ, TQ), 1)

        def head_body(h, carry):
            k_v[...] = _dot(ckv_v[...], head_w(wuk_p, h, Dc, STK)).astype(BF16)
            q_v[...] = (_dot(hn_v[...], head_w(wq_p, h, M, STQ)) * qscale).astype(BF16)
            v_v[...] = _dot(ckv_v[...], head_w(wuv_p, h, Dc, STK)).astype(BF16)
            causal = col_i <= row_i
            for i in range(NQ):
                n = (i + 1) * TQ
                qi = q_v[i * TQ:(i + 1) * TQ, :]
                s = jax.lax.dot_general(qi, k_v[0:n, :], _NT,
                                        preferred_element_type=F32)
                sd = jnp.where(causal, s[:, n - TQ:], NEG)
                if i > 0:
                    s = jnp.concatenate([s[:, :n - TQ], sd], axis=1)
                else:
                    s = sd
                m = jnp.max(s, axis=-1, keepdims=True)
                p = jnp.exp2(s - m)
                l = jnp.sum(p, axis=-1, keepdims=True)
                o = _dot(p.astype(BF16), v_v[0:n, :])
                ctx_v[h, i * TQ:(i + 1) * TQ, :] = (o / l).astype(BF16)
            return carry

        c_ckv.wait()
        for g in range(NG):
            c_uk[g].wait()
            relayout(wuk_r, wuk_p, g, Dc, STK)
            c_uv[g].wait()
            relayout(wuv_r, wuv_p, g, Dc, STK)
            c_q[g].wait()
            relayout(wq_r, wq_p, g, M, STQ)
            if g + 1 < NG:
                c_uk[g + 1].start()
                c_uv[g + 1].start()
                c_q[g + 1].start()
            if g == 0:
                for d in c_late:
                    d.start()

        jax.lax.fori_loop(0, H, head_body, 0)

        for d in c_late:
            d.wait()

        zpad = jnp.zeros((PAD, LANES), F32)
        for cidx in range(NC):
            hh_v[cidx, 0:PAD, :] = zpad
            hh_v[cidx, PAD + S:PAD + S + PAD, :] = zpad

        def stage1(r, carry):
            r0 = pl.multiple_of(r * TR, TR)
            rows = pl.ds(r0, TR)
            ctx = jnp.concatenate([ctx_v[h, rows, :] for h in range(H)], axis=1)
            att = _dot(ctx, wo_v[...])
            x1 = x_v[rows, :].astype(F32) + mod(2) * att
            x1_v[rows, :] = x1
            h2 = _ln(x1) * (1.0 + mod(4)) + mod(3)
            h2_v[rows, :] = h2
            u = _gelu(_dot(_ln(h2).astype(BF16), w1_v[...]))
            for cidx in range(NC):
                hh_v[cidx, pl.ds(r0 + PAD, TR), :] = u[:, cidx * LANES:(cidx + 1) * LANES]
            return carry

        jax.lax.fori_loop(0, NR, stage1, 0)

        shifts = (1, -1, 2, -2)
        lane_i = jax.lax.broadcasted_iota(jnp.int32, (TR, LANES), 1)

        def out_cp(r):
            rows = pl.ds(pl.multiple_of(r * TR, TR), TR)
            return pltpu.make_async_copy(o_v.at[rows, :], out_hbm.at[rows, :], osems.at[r])

        def stage2(r, carry):
            r0 = pl.multiple_of(r * TR, TR)
            rows = pl.ds(r0, TR)
            tiles = []
            for cidx in range(NC):
                lo, hi = cidx * LANES, (cidx + 1) * LANES
                g_lo, g_hi = lo // C4, (hi - 1) // C4
                t = hh_v[cidx, pl.ds(r0 + PAD - shifts[g_hi], TR), :]
                for g in range(g_hi - 1, g_lo - 1, -1):
                    tg = hh_v[cidx, pl.ds(r0 + PAD - shifts[g], TR), :]
                    t = jnp.where(lane_i < (g + 1) * C4 - lo, tg, t)
                tiles.append(t.astype(BF16))
            hs = _dot(jnp.concatenate(tiles, axis=1), w2_v[...])
            y1 = h2_v[rows, :] + hs
            gl = _gelu(_dot(_ln(y1).astype(BF16), w3_v[...])).astype(BF16)
            h3 = _dot(gl, w4_v[...])
            o_v[rows, :] = (x1_v[rows, :] + mod(5) * (y1 + h3)).astype(BF16)
            out_cp(r).start()
            return carry

        jax.lax.fori_loop(0, NR, stage2, 0)
        for r in range(NR):
            out_cp(r).wait()

    any_spec = pl.BlockSpec(memory_space=pl.ANY)
    vmem_spec = pl.BlockSpec(memory_space=pltpu.VMEM)
    V = pltpu.VMEM
    scratch = [
        V((S, M), BF16),
        V((S, Dc), BF16),
        V((NG, M, HG, D), BF16),
        V((NG, Dc, HG, D), BF16),
        V((NG, Dc, HG, D), BF16),
        V((H // 2 * STQ, D), U32),
        V((H // 2 * STK, D), U32),
        V((H // 2 * STK, D), U32),
        V((H * D, M), BF16),
        V((M, M), BF16),
        V((M, M), BF16),
        V((M, Fh), BF16),
        V((Fh, M), BF16),
        V((M, 6 * M), BF16),
        V((8, 6 * M), F32),
        V((S, M), BF16),
        V((S, D), BF16),
        V((S, D), BF16),
        V((S, D), BF16),
        V((H, S, D), BF16),
        V((S, M), F32),
        V((S, M), F32),
        V((NC, S + 2 * PAD, LANES), F32),
        V((S, M), BF16),
        pltpu.SemaphoreType.DMA((3 + 3 * NG + 5,)),
        pltpu.SemaphoreType.DMA((NR,)),
    ]
    out = pl.pallas_call(
        kernel,
        out_shape=jax.ShapeDtypeStruct((S, M), BF16),
        in_specs=[any_spec] * 10 + [vmem_spec, any_spec],
        out_specs=any_spec,
        scratch_shapes=scratch,
        compiler_params=pltpu.CompilerParams(vmem_limit_bytes=120 * 1024 * 1024),
        name="adaln_cla_mixer",
    )(x2, ckv2, A_w_q, A_w_uk, A_w_uv, wo2, B_w1, B_w2, B_w3, B_w4, c, w_mod)
    return out.reshape(B, S, M)
```

```python
import math

import jax
import jax.numpy as jnp
import jax.experimental.pallas as pl
import jax.experimental.pallas.tpu as pltpu

BF16 = jnp.bfloat16
F32 = jnp.float32
U32 = jnp.uint32

LANES = 128
TQ = 128
TR = 256
HG = 16
LOOK = 4
PC = 512
PIN = 4
PAD = 8
EPS = 1e-5
NEG = -1000000000.0
LOG2E = math.log2(math.e)

_NT = (((1,), (1,)), ((), ()))


def _ln(x):
    m = jnp.mean(x, axis=-1, keepdims=True)
    xc = x - m
    v = jnp.mean(xc * xc, axis=-1, keepdims=True)
    return xc * jax.lax.rsqrt(v + EPS)


def _gelu(x):
    return jax.nn.gelu(x, approximate=True)


def _dot(a, b):
    return jnp.dot(a, b, preferred_element_type=F32)


def _fold8(x, op):
    while x.shape[0] > 8:
        half = x.shape[0] // 2
        x = op(x[:half], x[half:])
    return x


def _tree(xs, op):
    xs = list(xs)
    while len(xs) > 1:
        xs = [op(xs[j], xs[j + 1]) if j + 1 < len(xs) else xs[j]
              for j in range(0, len(xs), 2)]
    return xs[0]


def _chain(xs):
    acc = xs[0]
    for x in xs[1:]:
        acc = acc + x
    return acc


def _pairsum8(x):
    return _chain([x[j:j + 8] + x[j + 8:j + 16] for j in range(0, x.shape[0], 16)])


@jax.jit
def pallas_adaLN_cond__compressed_kv_cla__mixer_s_mlp__prompt_kernel(
    A_x: jax.Array,
    A_c_kv: jax.Array,
    A_w_q: jax.Array,
    A_w_uk: jax.Array,
    A_w_uv: jax.Array,
    A_w_o: jax.Array,
    B_x: jax.Array,
    B_w1: jax.Array,
    B_w2: jax.Array,
    B_w3: jax.Array,
    B_w4: jax.Array,
    c: jax.Array,
    w_mod: jax.Array,
):
    del B_x
    B, S, M = A_x.shape
    _, Sk, Dc = A_c_kv.shape
    _, H, D = A_w_q.shape
    Fh = B_w3.shape[1]
    assert B == 1 and Sk == S and D == LANES and H % HG == 0
    assert S % TQ == 0 and S % TR == 0 and M % LANES == 0 and M % 4 == 0
    NG = H // HG
    NQ = S // TQ
    NR = S // TR
    NC = M // LANES
    C4 = M // 4
    STQ = M + 1
    STK = Dc + 1
    qscale = float(D) ** -0.5 * LOG2E

    x2 = A_x.reshape(S, M)
    ckv2 = A_c_kv.reshape(S, Dc)
    wo2 = A_w_o.reshape(H * D, M)

    def kernel(x_hbm, ckv_hbm, wq_hbm, wuk_hbm, wuv_hbm, wo_hbm, w1_hbm, w2_hbm,
               w3_hbm, w4_hbm, c_ref, wmod_hbm, out_hbm,
               x_v, ckv_v, wq_r, wuk_r, wuv_r, wq_p, wuk_p, wuv_p, wo_v, w1_v,
               w2_v, w3_v, w4_v, wmod_v, mod_v, hn_v, q_v, k_v, vt_v, ctx_v,
               x1_v, h2_v, hh_v, o_v, sems, osems):

        def cp(src, dst, i):
            return pltpu.make_async_copy(src, dst, sems.at[i])

        def grp(ref, g):
            return ref.at[:, pl.ds(g * HG, HG), :]

        c_ckv = cp(ckv_hbm, ckv_v, 0)
        c_x = cp(x_hbm, x_v, 1)
        c_mod = cp(wmod_hbm, wmod_v, 2)
        c_uk = [cp(grp(wuk_hbm, g), wuk_r.at[g], 3 + g) for g in range(NG)]
        c_uv = [cp(grp(wuv_hbm, g), wuv_r.at[g], 3 + NG + g) for g in range(NG)]
        c_q = [cp(grp(wq_hbm, g), wq_r.at[g], 3 + 2 * NG + g) for g in range(NG)]
        base = 3 + 3 * NG
        c_late = [cp(wo_hbm, wo_v, base), cp(w1_hbm, w1_v, base + 1),
                  cp(w2_hbm, w2_v, base + 2), cp(w3_hbm, w3_v, base + 3),
                  cp(w4_hbm, w4_v, base + 4)]

        c_x.start()
        c_mod.start()
        c_ckv.start()
        c_uk[0].start()
        c_uv[0].start()
        c_q[0].start()

        c_mod.wait()
        cc = c_ref[...].astype(F32)
        sc = (cc * jax.nn.sigmoid(cc)).astype(BF16)
        sc8 = jnp.broadcast_to(sc, (8, M))
        mod_v[...] = _dot(sc8, wmod_v[...])

        def mod(i):
            return mod_v[0:1, i * M:(i + 1) * M]

        c_x.wait()

        def ln1_body(r, carry):
            rows = pl.ds(pl.multiple_of(r * TR, TR), TR)
            xx = x_v[rows, :].astype(F32)
            hn_v[rows, :] = (_ln(xx) * (1.0 + mod(1)) + mod(0)).astype(BF16)
            return carry

        jax.lax.fori_loop(0, NR, ln1_body, 0)

        def relayout(raw, dst, g, rows, stride):
            def body(i, carry):
                for r in range(8):
                    m = i * 8 + r
                    val = pltpu.bitcast(raw[g, m], U32)
                    dst[pl.ds(g * (HG // 2) * stride + m, HG // 2, stride=stride), :] = val
                return carry
            for i in range(rows // 8):
                body(i, 0)

        def head_w(dst, h, rows, stride):
            u = dst[pl.ds((h // 2) * stride, rows), :]
            sh = (16 * (1 - h % 2)).astype(U32)
            return pltpu.bitcast((u << sh) & U32(0xFFFF0000), F32)

        key_i = jax.lax.broadcasted_iota(jnp.int32, (TQ, TQ), 0)
        qry_i = jax.lax.broadcasted_iota(jnp.int32, (TQ, TQ), 1)

        def head_body(h, carry):
            causal = key_i <= qry_i

            def qk(i):
                qi = q_v[i * TQ:(i + 1) * TQ, :]
                tiles = [jax.lax.dot_general(k_v[t * TQ:(t + 1) * TQ, :], qi, _NT,
                                             preferred_element_type=F32)
                         for t in range(i + 1)]
                tiles[i] = jnp.where(causal, tiles[i], NEG)
                m8 = _tree([_fold8(t, jnp.maximum) for t in tiles], jnp.maximum)
                m = jnp.max(m8, axis=0, keepdims=True)
                return tiles, m

            parts = []

            def pv(i, tiles, m):
                n = (i + 1) * TQ
                m8 = jnp.broadcast_to(m, (8, TQ))
                ps = []
                l8 = None
                for t in tiles:
                    mt = m8
                    if len(parts) >= PIN:
                        mt = m8 + 0.0 * parts[-PIN]
                    p = jnp.exp2(t.reshape(TQ // 8, 8, TQ) - mt[None]).reshape(TQ, TQ)
                    part = _pairsum8(p)
                    l8 = part if l8 is None else l8 + part
                    parts.append(l8)
                    ps.append(p)
                l = jnp.sum(l8, axis=0, keepdims=True)
                pb = jnp.concatenate(ps, axis=0) if i > 0 else ps[0]
                ot = _dot(vt_v[:, 0:n], pb.astype(BF16))
                ot = ot * (1.0 / l)
                ctx_v[h, i * TQ:(i + 1) * TQ, :] = ot.T.astype(BF16)

            wk = head_w(wuk_p, h, Dc, STK).astype(BF16)
            wq = head_w(wq_p, h, M, STQ).astype(BF16)
            for r in range(S // PC):
                rows = slice(r * PC, (r + 1) * PC)
                q_v[rows, :] = (_dot(hn_v[rows, :], wq) * qscale).astype(BF16)
                k_v[rows, :] = _dot(ckv_v[rows, :], wk).astype(BF16)
            pend = [qk(i) for i in range(LOOK)]
            wvt = head_w(wuv_p, h, Dc, STK).T.astype(BF16)
            vt_v[...] = jax.lax.dot_general(wvt, ckv_v[...], _NT,
                                            preferred_element_type=F32).astype(BF16)
            for i in range(NQ):
                if i >= LOOK - 1 and i + 1 < NQ:
                    pend.append(qk(i + 1))
                pv(i, *pend[i])
            return carry

        c_ckv.wait()
        for g in range(NG):
            c_uk[g].wait()
            relayout(wuk_r, wuk_p, g, Dc, STK)
            c_uv[g].wait()
            relayout(wuv_r, wuv_p, g, Dc, STK)
            c_q[g].wait()
            relayout(wq_r, wq_p, g, M, STQ)
            if g + 1 < NG:
                c_uk[g + 1].start()
                c_uv[g + 1].start()
                c_q[g + 1].start()
            if g == 0:
                for d in c_late:
                    d.start()

        jax.lax.fori_loop(0, H, head_body, 0)

        for d in c_late:
            d.wait()

        zpad = jnp.zeros((PAD, LANES), F32)
        for cidx in range(NC):
            hh_v[cidx, 0:PAD, :] = zpad
            hh_v[cidx, PAD + S:PAD + S + PAD, :] = zpad

        def stage1(r, carry):
            r0 = pl.multiple_of(r * TR, TR)
            rows = pl.ds(r0, TR)
            ctx = jnp.concatenate([ctx_v[h, rows, :] for h in range(H)], axis=1)
            att = _dot(ctx, wo_v[...])
            x1 = x_v[rows, :].astype(F32) + mod(2) * att
            x1_v[rows, :] = x1
            h2 = _ln(x1) * (1.0 + mod(4)) + mod(3)
            h2_v[rows, :] = h2
            u = _gelu(_dot(_ln(h2).astype(BF16), w1_v[...]))
            for cidx in range(NC):
                hh_v[cidx, pl.ds(r0 + PAD, TR), :] = u[:, cidx * LANES:(cidx + 1) * LANES]
            return carry

        jax.lax.fori_loop(0, NR, stage1, 0)

        shifts = (1, -1, 2, -2)
        lane_i = jax.lax.broadcasted_iota(jnp.int32, (TR, LANES), 1)

        def out_cp(r):
            rows = pl.ds(pl.multiple_of(r * TR, TR), TR)
            return pltpu.make_async_copy(o_v.at[rows, :], out_hbm.at[rows, :], osems.at[r])

        def stage2(r, carry):
            r0 = pl.multiple_of(r * TR, TR)
            rows = pl.ds(r0, TR)
            tiles = []
            for cidx in range(NC):
                lo, hi = cidx * LANES, (cidx + 1) * LANES
                g_lo, g_hi = lo // C4, (hi - 1) // C4
                t = hh_v[cidx, pl.ds(r0 + PAD - shifts[g_hi], TR), :]
                for g in range(g_hi - 1, g_lo - 1, -1):
                    tg = hh_v[cidx, pl.ds(r0 + PAD - shifts[g], TR), :]
                    t = jnp.where(lane_i < (g + 1) * C4 - lo, tg, t)
                tiles.append(t.astype(BF16))
            hs = _dot(jnp.concatenate(tiles, axis=1), w2_v[...])
            y1 = h2_v[rows, :] + hs
            gl = _gelu(jax.lax.dot_general(_ln(y1).astype(BF16), w3_v[...], _NT,
                                           preferred_element_type=F32)).astype(BF16)
            h3 = _dot(gl, w4_v[...])
            o_v[rows, :] = (x1_v[rows, :] + mod(5) * (y1 + h3)).astype(BF16)
            out_cp(r).start()
            return carry

        jax.lax.fori_loop(0, NR, stage2, 0)
        for r in range(NR):
            out_cp(r).wait()

    any_spec = pl.BlockSpec(memory_space=pltpu.HBM)
    vmem_spec = pl.BlockSpec(memory_space=pltpu.VMEM)
    V = pltpu.VMEM
    scratch = [
        V((S, M), BF16),
        V((S, Dc), BF16),
        V((NG, M, HG, D), BF16),
        V((NG, Dc, HG, D), BF16),
        V((NG, Dc, HG, D), BF16),
        V((H // 2 * STQ, D), U32),
        V((H // 2 * STK, D), U32),
        V((H // 2 * STK, D), U32),
        V((H * D, M), BF16),
        V((M, M), BF16),
        V((M, M), BF16),
        V((Fh, M), BF16),
        V((Fh, M), BF16),
        V((M, 6 * M), BF16),
        V((8, 6 * M), F32),
        V((S, M), BF16),
        V((S, D), BF16),
        V((S, D), BF16),
        V((D, S), BF16),
        V((H, S, D), BF16),
        V((S, M), F32),
        V((S, M), F32),
        V((NC, S + 2 * PAD, LANES), F32),
        V((S, M), BF16),
        pltpu.SemaphoreType.DMA((3 + 3 * NG + 5,)),
        pltpu.SemaphoreType.DMA((NR,)),
    ]
    out = pl.pallas_call(
        kernel,
        out_shape=jax.ShapeDtypeStruct((S, M), BF16),
        in_specs=[any_spec] * 10 + [vmem_spec, any_spec],
        out_specs=any_spec,
        scratch_shapes=scratch,
        compiler_params=pltpu.CompilerParams(vmem_limit_bytes=120 * 1024 * 1024),
        name="adaln_cla_mixer",
    )(x2, ckv2, A_w_q, A_w_uk, A_w_uv, wo2, B_w1, B_w2, B_w3.T, B_w4, c, w_mod)
    return out.reshape(B, S, M)
```

```python
import math

import jax
import jax.numpy as jnp
import jax.experimental.pallas as pl
import jax.experimental.pallas.tpu as pltpu

BF16 = jnp.bfloat16
F32 = jnp.float32
U32 = jnp.uint32

LANES = 128
TQ = 128
TR = 256
HG = 16
LOOK = 4
PC = 512
PIN = 4
PAD = 8
EPS = 1e-5
NEG = -1000000000.0
LOG2E = math.log2(math.e)

_NT = (((1,), (1,)), ((), ()))


def _ln(x):
    m = jnp.mean(x, axis=-1, keepdims=True)
    xc = x - m
    v = jnp.mean(xc * xc, axis=-1, keepdims=True)
    return xc * jax.lax.rsqrt(v + EPS)


def _gelu(x):
    return jax.nn.gelu(x, approximate=True)


def _dot(a, b):
    return jnp.dot(a, b, preferred_element_type=F32)


def _fold8(x, op):
    while x.shape[0] > 8:
        half = x.shape[0] // 2
        x = op(x[:half], x[half:])
    return x


def _tree(xs, op):
    xs = list(xs)
    while len(xs) > 1:
        xs = [op(xs[j], xs[j + 1]) if j + 1 < len(xs) else xs[j]
              for j in range(0, len(xs), 2)]
    return xs[0]


def _chain(xs):
    acc = xs[0]
    for x in xs[1:]:
        acc = acc + x
    return acc


def _pairsum8(x):
    return _chain([x[j:j + 8] + x[j + 8:j + 16] for j in range(0, x.shape[0], 16)])


@jax.jit
def pallas_adaLN_cond__compressed_kv_cla__mixer_s_mlp__prompt_kernel(
    A_x: jax.Array,
    A_c_kv: jax.Array,
    A_w_q: jax.Array,
    A_w_uk: jax.Array,
    A_w_uv: jax.Array,
    A_w_o: jax.Array,
    B_x: jax.Array,
    B_w1: jax.Array,
    B_w2: jax.Array,
    B_w3: jax.Array,
    B_w4: jax.Array,
    c: jax.Array,
    w_mod: jax.Array,
):
    del B_x
    B, S, M = A_x.shape
    _, Sk, Dc = A_c_kv.shape
    _, H, D = A_w_q.shape
    Fh = B_w3.shape[1]
    assert B == 1 and Sk == S and D == LANES and H % HG == 0
    assert S % TQ == 0 and S % TR == 0 and M % LANES == 0 and M % 4 == 0
    NG = H // HG
    NQ = S // TQ
    NR = S // TR
    NC = M // LANES
    C4 = M // 4
    STQ = M + 1
    STK = Dc + 1
    qscale = float(D) ** -0.5 * LOG2E

    x2 = A_x.reshape(S, M)
    ckv2 = A_c_kv.reshape(S, Dc)
    wo2 = A_w_o.reshape(H * D, M)

    def kernel(x_hbm, ckv_hbm, wq_hbm, wuk_hbm, wuv_hbm, wo_hbm, w1_hbm, w2_hbm,
               w3_hbm, w4_hbm, c_ref, wmod_hbm, out_hbm,
               x_v, ckv_v, wq_r, wuk_r, wuv_r, wq_p, wuk_p, wuv_p, wo_v, w1_v,
               w2_v, w3_v, w4_v, wmod_v, mod_v, hn_v, q_v, k_v, vt_v, s0, s1, s2, s3, z_s, ctx_v,
               x1_v, h2_v, hh_v, o_v, sems, osems):

        s_v = (s0, s1, s2, s3)
        NSB = 4
        z_s[0] = 0
        z_s[1] = 0

        def cp(src, dst, i):
            return pltpu.make_async_copy(src, dst, sems.at[i])

        def grp(ref, g):
            return ref.at[:, pl.ds(g * HG, HG), :]

        c_ckv = cp(ckv_hbm, ckv_v, 0)
        c_x = cp(x_hbm, x_v, 1)
        c_mod = cp(wmod_hbm, wmod_v, 2)
        c_uk = [cp(grp(wuk_hbm, g), wuk_r.at[g], 3 + g) for g in range(NG)]
        c_uv = [cp(grp(wuv_hbm, g), wuv_r.at[g], 3 + NG + g) for g in range(NG)]
        c_q = [cp(grp(wq_hbm, g), wq_r.at[g], 3 + 2 * NG + g) for g in range(NG)]
        base = 3 + 3 * NG
        c_late = [cp(wo_hbm, wo_v, base), cp(w1_hbm, w1_v, base + 1),
                  cp(w2_hbm, w2_v, base + 2), cp(w3_hbm, w3_v, base + 3),
                  cp(w4_hbm, w4_v, base + 4)]

        c_x.start()
        c_mod.start()
        c_ckv.start()
        c_uk[0].start()
        c_uv[0].start()
        c_q[0].start()

        c_mod.wait()
        cc = c_ref[...].astype(F32)
        sc = (cc * jax.nn.sigmoid(cc)).astype(BF16)
        sc8 = jnp.broadcast_to(sc, (8, M))
        mod_v[...] = _dot(sc8, wmod_v[...])

        def mod(i):
            return mod_v[0:1, i * M:(i + 1) * M]

        c_x.wait()

        def ln1_body(r, carry):
            rows = pl.ds(pl.multiple_of(r * TR, TR), TR)
            xx = x_v[rows, :].astype(F32)
            hn_v[rows, :] = (_ln(xx) * (1.0 + mod(1)) + mod(0)).astype(BF16)
            return carry

        jax.lax.fori_loop(0, NR, ln1_body, 0)

        def relayout(raw, dst, g, rows, stride):
            def body(i, carry):
                for r in range(8):
                    m = i * 8 + r
                    val = pltpu.bitcast(raw[g, m], U32)
                    dst[pl.ds(g * (HG // 2) * stride + m, HG // 2, stride=stride), :] = val
                return carry
            for i in range(rows // 8):
                body(i, 0)

        def head_w(dst, h, rows, stride):
            u = dst[pl.ds((h // 2) * stride, rows), :]
            sh = (16 * (1 - h % 2)).astype(U32)
            return pltpu.bitcast((u << sh) & U32(0xFFFF0000), F32)

        key_i = jax.lax.broadcasted_iota(jnp.int32, (TQ, TQ), 0)
        qry_i = jax.lax.broadcasted_iota(jnp.int32, (TQ, TQ), 1)

        def head_body(h, carry):
            causal = key_i <= qry_i
            z_st = z_s[0]
            z_ld = z_s[1]

            def qk(i):
                qi = q_v[i * TQ:(i + 1) * TQ, :]
                tiles = [jax.lax.dot_general(k_v[t * TQ:(t + 1) * TQ, :], qi, _NT,
                                             preferred_element_type=F32)
                         for t in range(i + 1)]
                tiles[i] = jnp.where(causal, tiles[i], NEG)
                m8 = _tree([_fold8(t, jnp.maximum) for t in tiles], jnp.maximum)
                m = jnp.max(m8, axis=0, keepdims=True)
                sb = s_v[i % NSB]
                for t in range(i + 1):
                    sb[z_st + t] = tiles[t]
                return sb, m

            parts = []

            def pv(i, sb, m):
                n = (i + 1) * TQ
                m8 = jnp.broadcast_to(m, (8, TQ))
                ps = []
                l8 = None
                for tt in range(i + 1):
                    t = sb[z_ld + tt]
                    mt = m8
                    if len(parts) >= PIN:
                        mt = m8 + 0.0 * parts[-PIN]
                    p = jnp.exp2(t.reshape(TQ // 8, 8, TQ) - mt[None]).reshape(TQ, TQ)
                    part = _pairsum8(p)
                    l8 = part if l8 is None else l8 + part
                    parts.append(l8)
                    ps.append(p)
                l = jnp.sum(l8, axis=0, keepdims=True)
                pb = jnp.concatenate(ps, axis=0) if i > 0 else ps[0]
                ot = _dot(vt_v[:, 0:n], pb.astype(BF16))
                ot = ot * (1.0 / l)
                ctx_v[h, i * TQ:(i + 1) * TQ, :] = ot.T.astype(BF16)

            wk = head_w(wuk_p, h, Dc, STK).astype(BF16)
            wq = head_w(wq_p, h, M, STQ).astype(BF16)
            for r in range(S // PC):
                rows = slice(r * PC, (r + 1) * PC)
                q_v[rows, :] = (_dot(hn_v[rows, :], wq) * qscale).astype(BF16)
                k_v[rows, :] = _dot(ckv_v[rows, :], wk).astype(BF16)
            pend = [qk(i) for i in range(LOOK)]
            wvt = head_w(wuv_p, h, Dc, STK).T.astype(BF16)
            vt_v[...] = jax.lax.dot_general(wvt, ckv_v[...], _NT,
                                            preferred_element_type=F32).astype(BF16)
            for i in range(NQ):
                if i >= LOOK - 1 and i + 1 < NQ:
                    pend.append(qk(i + 1))
                pv(i, *pend[i])
            return carry

        c_ckv.wait()
        for g in range(NG):
            c_uk[g].wait()
            relayout(wuk_r, wuk_p, g, Dc, STK)
            c_uv[g].wait()
            relayout(wuv_r, wuv_p, g, Dc, STK)
            c_q[g].wait()
            relayout(wq_r, wq_p, g, M, STQ)
            if g + 1 < NG:
                c_uk[g + 1].start()
                c_uv[g + 1].start()
                c_q[g + 1].start()
            if g == 0:
                for d in c_late:
                    d.start()

        jax.lax.fori_loop(0, H, head_body, 0)

        for d in c_late:
            d.wait()

        zpad = jnp.zeros((PAD, LANES), F32)
        for cidx in range(NC):
            hh_v[cidx, 0:PAD, :] = zpad
            hh_v[cidx, PAD + S:PAD + S + PAD, :] = zpad

        def stage1(r, carry):
            r0 = pl.multiple_of(r * TR, TR)
            rows = pl.ds(r0, TR)
            ctx = jnp.concatenate([ctx_v[h, rows, :] for h in range(H)], axis=1)
            att = _dot(ctx, wo_v[...])
            x1 = x_v[rows, :].astype(F32) + mod(2) * att
            x1_v[rows, :] = x1
            h2 = _ln(x1) * (1.0 + mod(4)) + mod(3)
            h2_v[rows, :] = h2
            u = _gelu(_dot(_ln(h2).astype(BF16), w1_v[...]))
            for cidx in range(NC):
                hh_v[cidx, pl.ds(r0 + PAD, TR), :] = u[:, cidx * LANES:(cidx + 1) * LANES]
            return carry

        jax.lax.fori_loop(0, NR, stage1, 0)

        shifts = (1, -1, 2, -2)
        lane_i = jax.lax.broadcasted_iota(jnp.int32, (TR, LANES), 1)

        def out_cp(r):
            rows = pl.ds(pl.multiple_of(r * TR, TR), TR)
            return pltpu.make_async_copy(o_v.at[rows, :], out_hbm.at[rows, :], osems.at[r])

        def stage2(r, carry):
            r0 = pl.multiple_of(r * TR, TR)
            rows = pl.ds(r0, TR)
            tiles = []
            for cidx in range(NC):
                lo, hi = cidx * LANES, (cidx + 1) * LANES
                g_lo, g_hi = lo // C4, (hi - 1) // C4
                t = hh_v[cidx, pl.ds(r0 + PAD - shifts[g_hi], TR), :]
                for g in range(g_hi - 1, g_lo - 1, -1):
                    tg = hh_v[cidx, pl.ds(r0 + PAD - shifts[g], TR), :]
                    t = jnp.where(lane_i < (g + 1) * C4 - lo, tg, t)
                tiles.append(t.astype(BF16))
            hs = _dot(jnp.concatenate(tiles, axis=1), w2_v[...])
            y1 = h2_v[rows, :] + hs
            gl = _gelu(jax.lax.dot_general(_ln(y1).astype(BF16), w3_v[...], _NT,
                                           preferred_element_type=F32)).astype(BF16)
            h3 = _dot(gl, w4_v[...])
            o_v[rows, :] = (x1_v[rows, :] + mod(5) * (y1 + h3)).astype(BF16)
            out_cp(r).start()
            return carry

        jax.lax.fori_loop(0, NR, stage2, 0)
        for r in range(NR):
            out_cp(r).wait()

    any_spec = pl.BlockSpec(memory_space=pltpu.HBM)
    vmem_spec = pl.BlockSpec(memory_space=pltpu.VMEM)
    V = pltpu.VMEM
    scratch = [
        V((S, M), BF16),
        V((S, Dc), BF16),
        V((NG, M, HG, D), BF16),
        V((NG, Dc, HG, D), BF16),
        V((NG, Dc, HG, D), BF16),
        V((H // 2 * STQ, D), U32),
        V((H // 2 * STK, D), U32),
        V((H // 2 * STK, D), U32),
        V((H * D, M), BF16),
        V((M, M), BF16),
        V((M, M), BF16),
        V((Fh, M), BF16),
        V((Fh, M), BF16),
        V((M, 6 * M), BF16),
        V((8, 6 * M), F32),
        V((S, M), BF16),
        V((S, D), BF16),
        V((S, D), BF16),
        V((D, S), BF16),
        V((NQ, TQ, TQ), F32), V((NQ, TQ, TQ), F32), V((NQ, TQ, TQ), F32), V((NQ, TQ, TQ), F32),
        pltpu.SMEM((2,), jnp.int32),
        V((H, S, D), BF16),
        V((S, M), F32),
        V((S, M), F32),
        V((NC, S + 2 * PAD, LANES), F32),
        V((S, M), BF16),
        pltpu.SemaphoreType.DMA((3 + 3 * NG + 5,)),
        pltpu.SemaphoreType.DMA((NR,)),
    ]
    out = pl.pallas_call(
        kernel,
        out_shape=jax.ShapeDtypeStruct((S, M), BF16),
        in_specs=[any_spec] * 10 + [vmem_spec, any_spec],
        out_specs=any_spec,
        scratch_shapes=scratch,
        compiler_params=pltpu.CompilerParams(vmem_limit_bytes=120 * 1024 * 1024),
        name="adaln_cla_mixer",
    )(x2, ckv2, A_w_q, A_w_uk, A_w_uv, wo2, B_w1, B_w2, B_w3.T, B_w4, c, w_mod)
    return out.reshape(B, S, M)
```

```python
import math

import jax
import jax.numpy as jnp
import jax.experimental.pallas as pl
import jax.experimental.pallas.tpu as pltpu

BF16 = jnp.bfloat16
F32 = jnp.float32
U32 = jnp.uint32

LANES = 128
TQ = 128
TR = 256
HB = 128
HG = 8
LOOK = 4
NSB = 4
PC = 512
PIN = 4
PAD = 8
EPS = 1e-5
LOG2E = math.log2(math.e)
NEG = -1000000000.0 * LOG2E

_NT = (((1,), (1,)), ((), ()))


def _ln(x):
    m = jnp.mean(x, axis=-1, keepdims=True)
    xc = x - m
    v = jnp.mean(xc * xc, axis=-1, keepdims=True)
    return xc * jax.lax.rsqrt(v + EPS)


def _gelu(x):
    return jax.nn.gelu(x, approximate=True)


def _dot(a, b):
    return jnp.dot(a, b, preferred_element_type=F32)


def _dot_nt(a, b):
    return jax.lax.dot_general(a, b, _NT, preferred_element_type=F32)


def _fold8(x, op):
    parts = [op(x[j:j + 8], x[j + 8:j + 16]) for j in range(0, x.shape[0], 16)]
    acc = parts[0]
    for p in parts[1:]:
        acc = op(acc, p)
    return acc


@jax.jit
def pallas_adaLN_cond__compressed_kv_cla__mixer_s_mlp__prompt_kernel(
    A_x: jax.Array,
    A_c_kv: jax.Array,
    A_w_q: jax.Array,
    A_w_uk: jax.Array,
    A_w_uv: jax.Array,
    A_w_o: jax.Array,
    B_x: jax.Array,
    B_w1: jax.Array,
    B_w2: jax.Array,
    B_w3: jax.Array,
    B_w4: jax.Array,
    c: jax.Array,
    w_mod: jax.Array,
):
    del B_x
    B, S, M = A_x.shape
    _, Sk, Dc = A_c_kv.shape
    _, H, D = A_w_q.shape
    Fh = B_w3.shape[1]
    assert B == 1 and Sk == S and D == LANES and H % HG == 0 and HG == 8
    assert S % TQ == 0 and S % TR == 0 and S % PC == 0 and TR % HB == 0
    assert M % LANES == 0 and M % 64 == 0 and Dc % 64 == 0
    NG = H // HG
    NQ = S // TQ
    NR = S // TR
    NC = M // LANES
    C4 = M // 4
    PLQ = M // 2 + 1
    PLK = Dc // 2 + 1
    RCH = 4
    qscale = float(D) ** -0.5 * LOG2E

    x2 = A_x.reshape(S, M)
    ckv2 = A_c_kv.reshape(S, Dc)
    wo2 = A_w_o.reshape(H * D, M)

    def kernel(x_hbm, ckv_hbm, wq_hbm, wuk_hbm, wuv_hbm, wo_hbm, w1_hbm, w2_hbm,
               w3_hbm, w4_hbm, c_ref, wmod_hbm, out_hbm,
               x_v, ckv_v, wq_r, wuk_r, wuv_r, wq_p, wuk_p, wuv_p, wo_v, w1_v,
               w2_v, w3_v, w4_v, wmoda_v, wmodb_v, moda_v, modb_v, hn_v, q_v, k_v,
               vt_v, s0, s1, s2, s3, z_s, ctx_v, x1_v, h2_v, hh_v, o_v,
               sems, gsems, xsems, osems):

        s_v = (s0, s1, s2, s3)
        z_s[0] = 0
        z_s[1] = 0

        def cp(src, dst, i):
            return pltpu.make_async_copy(src, dst, sems.at[i])

        def gcp(which, g):
            src, dst = ((wq_hbm, wq_r), (wuk_hbm, wuk_r), (wuv_hbm, wuv_r))[which]
            off = g * HG if isinstance(g, int) else pl.multiple_of(g * HG, HG)
            return pltpu.make_async_copy(src.at[:, pl.ds(off, HG), :], dst.at[g],
                                         gsems.at[which * NG + g])

        def xcp(r):
            rows = pl.ds(r * TR, TR)
            return pltpu.make_async_copy(x_hbm.at[rows, :], x_v.at[rows, :], xsems.at[r])

        c_ckv = cp(ckv_hbm, ckv_v, 0)
        c_moda = cp(wmod_hbm.at[:, pl.ds(0, 2 * M)], wmoda_v, 1)
        c_late = [cp(wmod_hbm.at[:, pl.ds(2 * M, 4 * M)], wmodb_v, 2),
                  cp(wo_hbm, wo_v, 3), cp(w1_hbm, w1_v, 4), cp(w2_hbm, w2_v, 5),
                  cp(w3_hbm, w3_v, 6), cp(w4_hbm, w4_v, 7)]

        c_moda.start()
        for r in range(NR):
            xcp(r).start()
        gcp(0, 0).start()
        c_ckv.start()
        gcp(1, 0).start()
        gcp(2, 0).start()

        def relayout(raw, dst, g, chunk, rows, plane):
            n = rows // RCH // 2
            base = g * (8 * plane) + chunk * n
            if not isinstance(base, int):
                base = pl.multiple_of(base, 8)
            view = dst.at[pl.ds(base, 7 * plane + n), :]
            for j in range(n):
                val = raw[g, pl.ds(chunk * (2 * n) + 2 * j, 2)].reshape(2 * HG, D)
                view[pl.ds(j, 8, stride=plane), :] = pltpu.bitcast(val, U32)

        def head_w(src, h, rows, plane):
            base = (h // HG) * (8 * plane) + ((h % HG) // 2) * plane
            ev = src[pl.ds(base, rows // 2), :]
            od = src[pl.ds(base + 4 * plane, rows // 2), :]
            par = jnp.asarray(h % 2).astype(U32)
            lo = (ev >> (16 * par)) & U32(0xFFFF)
            hi = (od << (16 * (1 - par))) & U32(0xFFFF0000)
            return pltpu.bitcast(lo | hi, BF16)

        def q_proj(h):
            wq = head_w(wq_p, h, M, PLQ)
            for r in range(S // PC):
                rows = slice(r * PC, (r + 1) * PC)
                q_v[rows, :] = (_dot(hn_v[rows, :], wq) * qscale).astype(BF16)

        def k_proj(h):
            wk = head_w(wuk_p, h, Dc, PLK)
            for r in range(S // PC):
                rows = slice(r * PC, (r + 1) * PC)
                k_v[rows, :] = _dot(ckv_v[rows, :], wk).astype(BF16)

        cc = c_ref[...].astype(F32)
        sc8 = jnp.broadcast_to((cc * jax.nn.sigmoid(cc)).astype(BF16), (8, M))
        c_moda.wait()
        moda_v[...] = _dot(sc8, wmoda_v[...])

        def mod(i):
            if i < 2:
                return moda_v[0:1, i * M:(i + 1) * M]
            return modb_v[0:1, (i - 2) * M:(i - 1) * M]

        def ln1_body(r, carry):
            xcp(r).wait()
            rows = pl.ds(pl.multiple_of(r * TR, TR), TR)
            xx = x_v[rows, :].astype(F32)
            hn_v[rows, :] = (_ln(xx) * (1.0 + mod(1)) + mod(0)).astype(BF16)
            return carry

        jax.lax.fori_loop(0, NR, ln1_body, 0)

        gcp(0, 0).wait()
        for ch in range(RCH):
            relayout(wq_r, wq_p, 0, ch, M, PLQ)
        q_proj(0)
        c_ckv.wait()
        gcp(1, 0).wait()
        for ch in range(RCH):
            relayout(wuk_r, wuk_p, 0, ch, Dc, PLK)
        k_proj(0)
        gcp(2, 0).wait()
        for g in range(1, NG):
            for which in range(3):
                gcp(which, g).start()
        for d in c_late:
            d.start()
        for ch in range(RCH):
            relayout(wuv_r, wuv_p, 0, ch, Dc, PLK)

        def attention(h):
            key_i = jax.lax.broadcasted_iota(jnp.int32, (TQ, TQ), 0)
            qry_i = jax.lax.broadcasted_iota(jnp.int32, (TQ, TQ), 1)
            causal = key_i <= qry_i
            z_st = z_s[0]
            z_ld = z_s[1]

            def qk(i):
                qi = q_v[i * TQ:(i + 1) * TQ, :]
                sb = s_v[i % NSB]
                m8 = None
                for t in range(i + 1):
                    tile = _dot_nt(k_v[t * TQ:(t + 1) * TQ, :], qi)
                    if t == i:
                        tile = jnp.where(causal, tile, NEG)
                    sb[z_st + t] = tile
                    tm = _fold8(tile, jnp.maximum)
                    m8 = tm if m8 is None else jnp.maximum(m8, tm)
                return sb, jnp.max(m8, axis=0, keepdims=True)

            parts = []

            def pv(i, sb, m):
                n = (i + 1) * TQ
                m8 = jnp.broadcast_to(m, (8, TQ))
                ps = []
                l8 = None
                for t in range(i + 1):
                    mt = m8
                    if len(parts) >= PIN:
                        mt = m8 + 0.0 * parts[-PIN]
                    tile = sb[z_ld + t].reshape(TQ // 8, 8, TQ)
                    p = jnp.exp2(tile - mt[None]).reshape(TQ, TQ)
                    part = _fold8(p, jnp.add)
                    l8 = part if l8 is None else l8 + part
                    parts.append(l8)
                    ps.append(p)
                l = jnp.sum(l8, axis=0, keepdims=True)
                pb = jnp.concatenate(ps, axis=0) if i > 0 else ps[0]
                ot = _dot(vt_v[:, 0:n], pb.astype(BF16))
                ot = ot * (1.0 / l)
                ctx_v[h, i * TQ:(i + 1) * TQ, :] = ot.T.astype(BF16)

            pend = [qk(i) for i in range(LOOK)]
            vt_v[...] = _dot_nt(head_w(wuv_p, h, Dc, PLK).T, ckv_v[...]).astype(BF16)
            for i in range(NQ):
                if i >= LOOK - 1 and i + 1 < NQ:
                    pend.append(qk(i + 1))
                pv(i, *pend[i])

        def head_body(h, carry):
            nxt = (h % HG) >= RCH
            gsrc = jnp.minimum(h // HG + nxt.astype(jnp.int32), NG - 1)

            @pl.when(jnp.logical_and(h % HG == RCH, h // HG < NG - 1))
            def _():
                for which in range(3):
                    gcp(which, h // HG + 1).wait()

            attention(h)
            ch = h % RCH
            relayout(wuv_r, wuv_p, gsrc, ch, Dc, PLK)
            relayout(wq_r, wq_p, gsrc, ch, M, PLQ)
            relayout(wuk_r, wuk_p, gsrc, ch, Dc, PLK)
            q_proj(h + 1)
            k_proj(h + 1)
            return carry

        jax.lax.fori_loop(0, H - 1, head_body, 0)

        def sub_rows(r):
            out = []
            for j in range(TR // HB):
                r0 = r * TR + j * HB
                if not isinstance(r0, int):
                    r0 = pl.multiple_of(r0, HB)
                out.append(r0)
            return out

        def stage1(r):
            lns = []
            for r0 in sub_rows(r):
                rows = pl.ds(r0, HB)
                ctx = jnp.concatenate([ctx_v[h, rows, :] for h in range(H)], axis=1)
                att = _dot(ctx, wo_v[...])
                x1 = x_v[rows, :].astype(F32) + mod(2) * att
                x1_v[rows, :] = x1
                h2 = _ln(x1) * (1.0 + mod(4)) + mod(3)
                h2_v[rows, :] = h2
                lns.append(_ln(h2).astype(BF16))
            for r0, ln in zip(sub_rows(r), lns):
                u = _gelu(_dot(ln, w1_v[...]))
                for cidx in range(NC):
                    hh_v[cidx, pl.ds(r0 + PAD, HB), :] = u[:, cidx * LANES:(cidx + 1) * LANES]

        shifts = (1, -1, 2, -2)

        def out_cp(r):
            r0 = r * TR if isinstance(r, int) else pl.multiple_of(r * TR, TR)
            rows = pl.ds(r0, TR)
            return pltpu.make_async_copy(o_v.at[rows, :], out_hbm.at[rows, :], osems.at[r])

        def stage2(r):
            lane_i = jax.lax.broadcasted_iota(jnp.int32, (HB, LANES), 1)
            y1s = []
            for r0 in sub_rows(r):
                tiles = []
                for cidx in range(NC):
                    lo, hi = cidx * LANES, (cidx + 1) * LANES
                    g_lo, g_hi = lo // C4, (hi - 1) // C4
                    t = hh_v[cidx, pl.ds(r0 + PAD - shifts[g_hi], HB), :]
                    for g in range(g_hi - 1, g_lo - 1, -1):
                        tg = hh_v[cidx, pl.ds(r0 + PAD - shifts[g], HB), :]
                        t = jnp.where(lane_i < (g + 1) * C4 - lo, tg, t)
                    tiles.append(t)
                hs = _dot(jnp.concatenate(tiles, axis=1).astype(BF16), w2_v[...])
                y1s.append(h2_v[pl.ds(r0, HB), :] + hs)
            gls = [_gelu(_dot_nt(_ln(y1).astype(BF16), w3_v[...])).astype(BF16)
                   for y1 in y1s]
            for r0, y1, gl in zip(sub_rows(r), y1s, gls):
                rows = pl.ds(r0, HB)
                h3 = _dot(gl, w4_v[...])
                o_v[rows, :] = (x1_v[rows, :] + mod(5) * (y1 + h3)).astype(BF16)
            out_cp(r).start()

        for d in c_late:
            d.wait()
        zpad = jnp.zeros((PAD, LANES), F32)
        for cidx in range(NC):
            hh_v[cidx, 0:PAD, :] = zpad
            hh_v[cidx, PAD + S:PAD + S + PAD, :] = zpad
        attention(H - 1)
        modb_v[...] = _dot(sc8, wmodb_v[...])
        stage1(0)

        def mlp_body(r, carry):
            stage1(r + 1)
            stage2(r)
            return carry

        jax.lax.fori_loop(0, NR - 1, mlp_body, 0)
        stage2(NR - 1)
        for r in range(NR):
            out_cp(r).wait()

    hbm_spec = pl.BlockSpec(memory_space=pltpu.HBM)
    vmem_spec = pl.BlockSpec(memory_space=pltpu.VMEM)
    V = pltpu.VMEM
    scratch = [
        V((S, M), BF16),
        V((S, Dc), BF16),
        V((NG, M, HG, D), BF16),
        V((NG, Dc, HG, D), BF16),
        V((NG, Dc, HG, D), BF16),
        V((NG * 8 * PLQ, D), U32),
        V((NG * 8 * PLK, D), U32),
        V((NG * 8 * PLK, D), U32),
        V((H * D, M), BF16),
        V((M, M), BF16),
        V((M, M), BF16),
        V((Fh, M), BF16),
        V((Fh, M), BF16),
        V((M, 2 * M), BF16),
        V((M, 4 * M), BF16),
        V((8, 2 * M), F32),
        V((8, 4 * M), F32),
        V((S, M), BF16),
        V((S, D), BF16),
        V((S, D), BF16),
        V((D, S), BF16),
        V((NQ, TQ, TQ), F32),
        V((NQ, TQ, TQ), F32),
        V((NQ, TQ, TQ), F32),
        V((NQ, TQ, TQ), F32),
        pltpu.SMEM((2,), jnp.int32),
        V((H, S, D), BF16),
        V((S, M), F32),
        V((S, M), F32),
        V((NC, S + 2 * PAD, LANES), F32),
        V((S, M), BF16),
        pltpu.SemaphoreType.DMA((8,)),
        pltpu.SemaphoreType.DMA((3 * NG,)),
        pltpu.SemaphoreType.DMA((NR,)),
        pltpu.SemaphoreType.DMA((NR,)),
    ]
    out = pl.pallas_call(
        kernel,
        out_shape=jax.ShapeDtypeStruct((S, M), BF16),
        in_specs=[hbm_spec] * 10 + [vmem_spec, hbm_spec],
        out_specs=hbm_spec,
        scratch_shapes=scratch,
        compiler_params=pltpu.CompilerParams(vmem_limit_bytes=120 * 1024 * 1024),
        name="adaln_cla_mixer",
    )(x2, ckv2, A_w_q, A_w_uk, A_w_uv, wo2, B_w1, B_w2, B_w3.T, B_w4, c, w_mod)
    return out.reshape(B, S, M)
```

```python
import math

import jax
import jax.numpy as jnp
import jax.experimental.pallas as pl
import jax.experimental.pallas.tpu as pltpu

BF16 = jnp.bfloat16
F32 = jnp.float32
U32 = jnp.uint32

LANES = 128
TQ = 128
TR = 256
HB = 128
HG = 8
LOOK = 4
NSB = 4
PC = 512
PIN = 4
PAD = 16
EPS = 1e-5
LOG2E = math.log2(math.e)
NEG = -1000000000.0 * LOG2E

_NT = (((1,), (1,)), ((), ()))


def _ln(x):
    m = jnp.mean(x, axis=-1, keepdims=True)
    xc = x - m
    v = jnp.mean(xc * xc, axis=-1, keepdims=True)
    return xc * jax.lax.rsqrt(v + EPS)


def _gelu(x):
    return jax.nn.gelu(x, approximate=True)


def _dot(a, b):
    return jnp.dot(a, b, preferred_element_type=F32)


def _dot_nt(a, b):
    return jax.lax.dot_general(a, b, _NT, preferred_element_type=F32)


def _fold8(x, op):
    parts = [op(x[j:j + 8], x[j + 8:j + 16]) for j in range(0, x.shape[0], 16)]
    acc = parts[0]
    for p in parts[1:]:
        acc = op(acc, p)
    return acc


@jax.jit
def pallas_adaLN_cond__compressed_kv_cla__mixer_s_mlp__prompt_kernel(
    A_x: jax.Array,
    A_c_kv: jax.Array,
    A_w_q: jax.Array,
    A_w_uk: jax.Array,
    A_w_uv: jax.Array,
    A_w_o: jax.Array,
    B_x: jax.Array,
    B_w1: jax.Array,
    B_w2: jax.Array,
    B_w3: jax.Array,
    B_w4: jax.Array,
    c: jax.Array,
    w_mod: jax.Array,
):
    del B_x
    B, S, M = A_x.shape
    _, Sk, Dc = A_c_kv.shape
    _, H, D = A_w_q.shape
    Fh = B_w3.shape[1]
    assert B == 1 and Sk == S and D == LANES and H % HG == 0 and HG == 8
    assert S % TQ == 0 and S % TR == 0 and S % PC == 0 and TR % HB == 0
    assert M % LANES == 0 and M % 64 == 0 and Dc % 64 == 0
    NG = H // HG
    NQ = S // TQ
    NR = S // TR
    NC = M // LANES
    C4 = M // 4
    PLQ = M // 2 + 1
    PLK = Dc // 2 + 1
    RCH = 4
    qscale = float(D) ** -0.5 * LOG2E

    x2 = A_x.reshape(S, M)
    ckv2 = A_c_kv.reshape(S, Dc)
    wo2 = A_w_o.reshape(H * D, M)

    def kernel(x_hbm, ckv_hbm, wq_hbm, wuk_hbm, wuv_hbm, wo_hbm, w1_hbm, w2_hbm,
               w3_hbm, w4_hbm, c_hbm, wmod_hbm, out_hbm,
               x_v, ckv_v, wq_r, wuk_r, wuv_r, wq_p, wuk_p, wuv_p, wo_v, w1_v,
               w2_v, w3_v, w4_v, wmoda_v, wmodb_v, moda_v, modb_v, hn_v, q_v, k_v,
               vt_v, s0, s1, s2, s3, z_s, ctx_v, x1_v, h2_v, hh_v, o_v, c_v,
               sems, gsems, xsems, osems):

        s_v = (s0, s1, s2, s3)
        z_s[0] = 0
        z_s[1] = 0

        def cp(src, dst, i):
            return pltpu.make_async_copy(src, dst, sems.at[i])

        def gcp(which, g):
            src, dst = ((wq_hbm, wq_r), (wuk_hbm, wuk_r), (wuv_hbm, wuv_r))[which]
            off = g * HG if isinstance(g, int) else pl.multiple_of(g * HG, HG)
            return pltpu.make_async_copy(src.at[:, pl.ds(off, HG), :], dst.at[g],
                                         gsems.at[which * NG + g])

        def xcp(r):
            rows = pl.ds(r * TR, TR)
            return pltpu.make_async_copy(x_hbm.at[rows, :], x_v.at[rows, :], xsems.at[r])

        c_ckv = cp(ckv_hbm, ckv_v, 0)
        c_moda = cp(wmod_hbm.at[:, pl.ds(0, 2 * M)], wmoda_v, 1)
        c_late = [cp(wmod_hbm.at[:, pl.ds(2 * M, 4 * M)], wmodb_v, 2),
                  cp(wo_hbm, wo_v, 3), cp(w1_hbm, w1_v, 4), cp(w2_hbm, w2_v, 5),
                  cp(w3_hbm, w3_v, 6), cp(w4_hbm, w4_v, 7)]

        c_c = cp(c_hbm, c_v, 8)
        c_c.start()
        c_moda.start()
        for r in range(NR):
            xcp(r).start()
        gcp(0, 0).start()
        c_ckv.start()
        gcp(1, 0).start()
        gcp(2, 0).start()

        def relayout(raw, dst, g, chunk, rows, plane):
            n = rows // RCH // 2
            base = g * (8 * plane) + chunk * n
            if not isinstance(base, int):
                base = pl.multiple_of(base, 8)
            view = dst.at[pl.ds(base, 7 * plane + n), :]
            for j in range(n):
                val = raw[g, pl.ds(chunk * (2 * n) + 2 * j, 2)].reshape(2 * HG, D)
                view[pl.ds(j, 8, stride=plane), :] = pltpu.bitcast(val, U32)

        def head_w(src, h, rows, plane):
            base = (h // HG) * (8 * plane) + ((h % HG) // 2) * plane
            ev = src[pl.ds(base, rows // 2), :]
            od = src[pl.ds(base + 4 * plane, rows // 2), :]
            par = jnp.asarray(h % 2).astype(U32)
            lo = (ev >> (16 * par)) & U32(0xFFFF)
            hi = (od << (16 * (1 - par))) & U32(0xFFFF0000)
            return pltpu.bitcast(lo | hi, BF16)

        def q_proj(h):
            wq = head_w(wq_p, h, M, PLQ)
            for r in range(S // PC):
                rows = slice(r * PC, (r + 1) * PC)
                q_v[rows, :] = (_dot(hn_v[rows, :], wq) * qscale).astype(BF16)

        def k_proj(h):
            wk = head_w(wuk_p, h, Dc, PLK)
            for r in range(S // PC):
                rows = slice(r * PC, (r + 1) * PC)
                k_v[rows, :] = _dot(ckv_v[rows, :], wk).astype(BF16)

        c_c.wait()
        cc = c_v[...].astype(F32)
        sc8 = jnp.broadcast_to((cc * jax.nn.sigmoid(cc)).astype(BF16), (8, M))
        c_moda.wait()
        moda_v[0:8, :] = _dot(sc8, wmoda_v[...])

        def mod(i):
            if i < 2:
                return moda_v[0:1, i * M:(i + 1) * M]
            return modb_v[0:1, (i - 2) * M:(i - 1) * M]

        def ln1_body(r, carry):
            xcp(r).wait()
            rows = pl.ds(pl.multiple_of(r * TR, TR), TR)
            xx = x_v[rows, :].astype(F32)
            hn_v[rows, :] = (_ln(xx) * (1.0 + mod(1)) + mod(0)).astype(BF16)
            return carry

        jax.lax.fori_loop(0, NR, ln1_body, 0)

        gcp(0, 0).wait()
        for ch in range(RCH):
            relayout(wq_r, wq_p, 0, ch, M, PLQ)
        q_proj(0)
        c_ckv.wait()
        gcp(1, 0).wait()
        for ch in range(RCH):
            relayout(wuk_r, wuk_p, 0, ch, Dc, PLK)
        k_proj(0)
        gcp(2, 0).wait()
        for g in range(1, NG):
            for which in range(3):
                gcp(which, g).start()
        for d in c_late:
            d.start()
        for ch in range(RCH):
            relayout(wuv_r, wuv_p, 0, ch, Dc, PLK)

        def attention(h):
            key_i = jax.lax.broadcasted_iota(jnp.int32, (TQ, TQ), 0)
            qry_i = jax.lax.broadcasted_iota(jnp.int32, (TQ, TQ), 1)
            causal = key_i <= qry_i
            z_st = z_s[0]
            z_ld = z_s[1]

            def qk(i):
                qi = q_v[i * TQ:(i + 1) * TQ, :]
                sb = s_v[i % NSB]
                m8 = None
                for t in range(i + 1):
                    tile = _dot_nt(k_v[t * TQ:(t + 1) * TQ, :], qi)
                    if t == i:
                        tile = jnp.where(causal, tile, NEG)
                    sb[z_st + t] = tile
                    tm = _fold8(tile, jnp.maximum)
                    m8 = tm if m8 is None else jnp.maximum(m8, tm)
                return sb, jnp.max(m8, axis=0, keepdims=True)

            parts = []

            def pv(i, sb, m):
                n = (i + 1) * TQ
                m8 = jnp.broadcast_to(m, (8, TQ))
                ps = []
                l8 = None
                for t in range(i + 1):
                    mt = m8
                    if len(parts) >= PIN:
                        mt = m8 + 0.0 * parts[-PIN]
                    tile = sb[z_ld + t].reshape(TQ // 8, 8, TQ)
                    p = jnp.exp2(tile - mt[None]).reshape(TQ, TQ)
                    part = _fold8(p, jnp.add)
                    l8 = part if l8 is None else l8 + part
                    parts.append(l8)
                    ps.append(p)
                l = jnp.sum(l8, axis=0, keepdims=True)
                pb = jnp.concatenate(ps, axis=0) if i > 0 else ps[0]
                ot = _dot(vt_v[:, 0:n], pb.astype(BF16))
                ot = ot * (1.0 / l)
                ctx_v[h, i * TQ:(i + 1) * TQ, :] = ot.T.astype(BF16)

            pend = [qk(i) for i in range(LOOK)]
            vt_v[...] = _dot_nt(head_w(wuv_p, h, Dc, PLK).T, ckv_v[...]).astype(BF16)
            for i in range(NQ):
                if i >= LOOK - 1 and i + 1 < NQ:
                    pend.append(qk(i + 1))
                pv(i, *pend[i])

        def head_body(h, carry):
            nxt = (h % HG) >= RCH
            gsrc = jnp.minimum(h // HG + nxt.astype(jnp.int32), NG - 1)

            @pl.when(jnp.logical_and(h % HG == RCH, h // HG < NG - 1))
            def _():
                for which in range(3):
                    gcp(which, h // HG + 1).wait()

            attention(h)
            ch = h % RCH
            relayout(wuv_r, wuv_p, gsrc, ch, Dc, PLK)
            relayout(wq_r, wq_p, gsrc, ch, M, PLQ)
            relayout(wuk_r, wuk_p, gsrc, ch, Dc, PLK)
            q_proj(h + 1)
            k_proj(h + 1)
            return carry

        jax.lax.fori_loop(0, H - 1, head_body, 0)

        def sub_rows(r):
            out = []
            for j in range(TR // HB):
                r0 = r * TR + j * HB
                if not isinstance(r0, int):
                    r0 = pl.multiple_of(r0, HB)
                out.append(r0)
            return out

        def stage1(r):
            lns = []
            for r0 in sub_rows(r):
                rows = pl.ds(r0, HB)
                ctx = jnp.concatenate([ctx_v[h, rows, :] for h in range(H)], axis=1)
                att = _dot(ctx, wo_v[...])
                x1 = x_v[rows, :].astype(F32) + mod(2) * att
                x1_v[rows, :] = x1
                h2 = _ln(x1) * (1.0 + mod(4)) + mod(3)
                h2_v[rows, :] = h2
                lns.append(_ln(h2).astype(BF16))
            for r0, ln in zip(sub_rows(r), lns):
                u = _gelu(_dot(ln, w1_v[...]))
                for cidx in range(NC):
                    hh_v[cidx, pl.ds(r0 + PAD, HB), :] = u[:, cidx * LANES:(cidx + 1) * LANES]

        shifts = (1, -1, 2, -2)

        def out_cp(r):
            r0 = r * TR if isinstance(r, int) else pl.multiple_of(r * TR, TR)
            rows = pl.ds(r0, TR)
            return pltpu.make_async_copy(o_v.at[rows, :], out_hbm.at[rows, :], osems.at[r])

        def stage2(r):
            lane_i = jax.lax.broadcasted_iota(jnp.int32, (HB, LANES), 1)
            y1s = []
            for r0 in sub_rows(r):
                tiles = []
                for cidx in range(NC):
                    lo, hi = cidx * LANES, (cidx + 1) * LANES
                    g_lo, g_hi = lo // C4, (hi - 1) // C4
                    t = hh_v[cidx, pl.ds(r0 + PAD - shifts[g_hi], HB), :]
                    for g in range(g_hi - 1, g_lo - 1, -1):
                        tg = hh_v[cidx, pl.ds(r0 + PAD - shifts[g], HB), :]
                        t = jnp.where(lane_i < (g + 1) * C4 - lo, tg, t)
                    tiles.append(t)
                hs = _dot(jnp.concatenate(tiles, axis=1).astype(BF16), w2_v[...])
                y1s.append(h2_v[pl.ds(r0, HB), :] + hs)
            gls = [_gelu(_dot_nt(_ln(y1).astype(BF16), w3_v[...])).astype(BF16)
                   for y1 in y1s]
            for r0, y1, gl in zip(sub_rows(r), y1s, gls):
                rows = pl.ds(r0, HB)
                h3 = _dot(gl, w4_v[...])
                o_v[rows, :] = (x1_v[rows, :] + mod(5) * (y1 + h3)).astype(BF16)
            out_cp(r).start()

        for d in c_late:
            d.wait()
        zpad = jnp.zeros((PAD, LANES), F32)
        for cidx in range(NC):
            hh_v[cidx, 0:PAD, :] = zpad
            hh_v[cidx, PAD + S:PAD + S + PAD, :] = zpad
        attention(H - 1)
        modb_v[...] = _dot(sc8, wmodb_v[...])
        stage1(0)

        def mlp_body(r, carry):
            stage1(r + 1)
            stage2(r)
            return carry

        jax.lax.fori_loop(0, NR - 1, mlp_body, 0)
        stage2(NR - 1)
        for r in range(NR):
            out_cp(r).wait()

    hbm_spec = pl.BlockSpec(memory_space=pltpu.HBM)
    V = pltpu.VMEM
    scratch = [
        V((S, M), BF16),
        V((S, Dc), BF16),
        V((NG, M, HG, D), BF16),
        V((NG, Dc, HG, D), BF16),
        V((NG, Dc, HG, D), BF16),
        V((NG * 8 * PLQ, D), U32),
        V((NG * 8 * PLK, D), U32),
        V((NG * 8 * PLK, D), U32),
        V((H * D, M), BF16),
        V((M, M), BF16),
        V((M, M), BF16),
        V((Fh, M), BF16),
        V((Fh, M), BF16),
        V((M, 2 * M), BF16),
        V((M, 4 * M), BF16),
        V((16, 2 * M), F32),
        V((8, 4 * M), F32),
        V((S, M), BF16),
        V((S, D), BF16),
        V((S, D), BF16),
        V((D, S), BF16),
        V((NQ, TQ, TQ), F32),
        V((NQ, TQ, TQ), F32),
        V((NQ, TQ, TQ), F32),
        V((NQ, TQ, TQ), F32),
        pltpu.SMEM((2,), jnp.int32),
        V((H, S, D), BF16),
        V((S, M), F32),
        V((S, M), F32),
        V((NC, S + 2 * PAD, LANES), F32),
        V((S, M), BF16),
        V((1, M), BF16),
        pltpu.SemaphoreType.DMA((9,)),
        pltpu.SemaphoreType.DMA((3 * NG,)),
        pltpu.SemaphoreType.DMA((NR,)),
        pltpu.SemaphoreType.DMA((NR,)),
    ]
    out = pl.pallas_call(
        kernel,
        out_shape=jax.ShapeDtypeStruct((S, M), BF16),
        in_specs=[hbm_spec] * 12,
        out_specs=hbm_spec,
        scratch_shapes=scratch,
        compiler_params=pltpu.CompilerParams(vmem_limit_bytes=120 * 1024 * 1024),
        name="adaln_cla_mixer",
    )(x2, ckv2, A_w_q, A_w_uk, A_w_uv, wo2, B_w1, B_w2, B_w3.T, B_w4, c, w_mod)
    return out.reshape(B, S, M)
```

```python
import functools
import math

import jax
import jax.numpy as jnp
import jax.experimental.pallas as pl
import jax.experimental.pallas.tpu as pltpu

BF16 = jnp.bfloat16
F32 = jnp.float32
U32 = jnp.uint32

LANES = 128
TQ = 128
TR = 256
HB = 128
HG = 8
LOOK = 4
NSB = 4
PC = 512
PIN = 4
PAD = 16
EPS = 1e-5
LOG2E = math.log2(math.e)
NEG = -1000000000.0 * LOG2E

_NT = (((1,), (1,)), ((), ()))


def _ln(x):
    m = jnp.mean(x, axis=-1, keepdims=True)
    xc = x - m
    v = jnp.mean(xc * xc, axis=-1, keepdims=True)
    return xc * jax.lax.rsqrt(v + EPS)


def _gelu(x):
    return jax.nn.gelu(x, approximate=True)


def _dot(a, b):
    return jnp.dot(a, b, preferred_element_type=F32)


def _dot_nt(a, b):
    return jax.lax.dot_general(a, b, _NT, preferred_element_type=F32)


def _fold8(x, op):
    parts = [op(x[j:j + 8], x[j + 8:j + 16]) for j in range(0, x.shape[0], 16)]
    acc = parts[0]
    for p in parts[1:]:
        acc = op(acc, p)
    return acc


@jax.jit
def pallas_adaLN_cond__compressed_kv_cla__mixer_s_mlp__prompt_kernel(
    A_x: jax.Array,
    A_c_kv: jax.Array,
    A_w_q: jax.Array,
    A_w_uk: jax.Array,
    A_w_uv: jax.Array,
    A_w_o: jax.Array,
    B_x: jax.Array,
    B_w1: jax.Array,
    B_w2: jax.Array,
    B_w3: jax.Array,
    B_w4: jax.Array,
    c: jax.Array,
    w_mod: jax.Array,
):
    del B_x
    B, S, M = A_x.shape
    _, Sk, Dc = A_c_kv.shape
    _, H, D = A_w_q.shape
    Fh = B_w3.shape[1]
    assert B == 1 and Sk == S and D == LANES and H % HG == 0 and HG == 8
    assert S % TQ == 0 and S % TR == 0 and S % PC == 0 and TR % HB == 0
    assert M % LANES == 0 and M % 64 == 0 and Dc % 64 == 0
    NG = H // HG
    NQ = S // TQ
    NR = S // TR
    NC = M // LANES
    C4 = M // 4
    PLQ = M // 2 + 1
    PLK = Dc // 2 + 1
    RCH = 4
    qscale = float(D) ** -0.5 * LOG2E

    x2 = A_x.reshape(S, M)
    ckv2 = A_c_kv.reshape(S, Dc)
    wo2 = A_w_o.reshape(H * D, M)

    def kernel(x_hbm, ckv_hbm, wq_hbm, wuk_hbm, wuv_hbm, wo_hbm, w1_hbm, w2_hbm,
               w3_hbm, w4_hbm, c_hbm, wmod_hbm, out_hbm,
               x_v, ckv_v, wq_r, wuk_r, wuv_r, wq_p, wuk_p, wuv_p, wo_v, w1_v,
               w2_v, w3_v, w4_v, wmoda_v, wmodb_v, moda_v, modb_v, hn_v, q_v, k_v,
               vt_v, s0, s1, s2, s3, z_s, ctx_v, x1_v, h2_v, hh_v, o_v, c_v,
               sems, gsems, xsems, osems):

        s_v = (s0, s1, s2, s3)
        z_s[0] = 0
        z_s[1] = 0

        def cp(src, dst, i):
            return pltpu.make_async_copy(src, dst, sems.at[i])

        def gcp(which, g):
            src, dst = ((wq_hbm, wq_r), (wuk_hbm, wuk_r), (wuv_hbm, wuv_r))[which]
            off = g * HG if isinstance(g, int) else pl.multiple_of(g * HG, HG)
            return pltpu.make_async_copy(src.at[:, pl.ds(off, HG), :], dst.at[g],
                                         gsems.at[which * NG + g])

        def xcp(r):
            rows = pl.ds(r * TR, TR)
            return pltpu.make_async_copy(x_hbm.at[rows, :], x_v.at[rows, :], xsems.at[r])

        c_ckv = cp(ckv_hbm, ckv_v, 0)
        c_moda = cp(wmod_hbm.at[:, pl.ds(0, 2 * M)], wmoda_v, 1)
        c_late = [cp(wmod_hbm.at[:, pl.ds(2 * M, 4 * M)], wmodb_v, 2),
                  cp(wo_hbm, wo_v, 3), cp(w1_hbm, w1_v, 4), cp(w2_hbm, w2_v, 5),
                  cp(w3_hbm, w3_v, 6), cp(w4_hbm, w4_v, 7)]

        c_c = cp(c_hbm, c_v, 8)
        c_c.start()
        c_moda.start()
        for r in range(NR):
            xcp(r).start()
        gcp(0, 0).start()
        c_ckv.start()
        gcp(1, 0).start()
        gcp(2, 0).start()

        def relayout_steps(raw, dst, g, chunk, rows, plane):
            n = rows // RCH // 2
            base = g * (8 * plane) + chunk * n
            if not isinstance(base, int):
                base = pl.multiple_of(base, 8)
            view = dst.at[pl.ds(base, 7 * plane + n), :]

            def step(j, tie):
                val = raw[g, pl.ds(chunk * (2 * n) + 2 * j, 2)].reshape(2 * HG, D)
                val = pltpu.bitcast(val, U32)
                if tie is not None:
                    val = val | tie
                view[pl.ds(j, 8, stride=plane), :] = val

            return [functools.partial(step, j) for j in range(n)]

        def relayout(raw, dst, g, rows, plane):
            for ch in range(RCH):
                for step in relayout_steps(raw, dst, g, ch, rows, plane):
                    step(None)

        def head_w(src, h, rows, plane):
            base = (h // HG) * (8 * plane) + ((h % HG) // 2) * plane
            ev = src[pl.ds(base, rows // 2), :]
            od = src[pl.ds(base + 4 * plane, rows // 2), :]
            par = jnp.asarray(h % 2).astype(U32)
            lo = (ev >> (16 * par)) & U32(0xFFFF)
            hi = (od << (16 * (1 - par))) & U32(0xFFFF0000)
            return pltpu.bitcast(lo | hi, BF16)

        def q_proj(h):
            wq = head_w(wq_p, h, M, PLQ)
            for r in range(S // PC):
                rows = slice(r * PC, (r + 1) * PC)
                q_v[rows, :] = (_dot(hn_v[rows, :], wq) * qscale).astype(BF16)

        def k_proj(h):
            wk = head_w(wuk_p, h, Dc, PLK)
            for r in range(S // PC):
                rows = slice(r * PC, (r + 1) * PC)
                k_v[rows, :] = _dot(ckv_v[rows, :], wk).astype(BF16)

        c_c.wait()
        cc = c_v[...].astype(F32)
        sc8 = jnp.broadcast_to((cc * jax.nn.sigmoid(cc)).astype(BF16), (8, M))
        c_moda.wait()
        moda_v[0:8, :] = _dot(sc8, wmoda_v[...])

        def mod(i):
            if i < 2:
                return moda_v[0:1, i * M:(i + 1) * M]
            return modb_v[0:1, (i - 2) * M:(i - 1) * M]

        def ln1_body(r, carry):
            xcp(r).wait()
            rows = pl.ds(pl.multiple_of(r * TR, TR), TR)
            xx = x_v[rows, :].astype(F32)
            hn_v[rows, :] = (_ln(xx) * (1.0 + mod(1)) + mod(0)).astype(BF16)
            return carry

        jax.lax.fori_loop(0, NR, ln1_body, 0)

        gcp(0, 0).wait()
        relayout(wq_r, wq_p, 0, M, PLQ)
        q_proj(0)
        c_ckv.wait()
        gcp(1, 0).wait()
        relayout(wuk_r, wuk_p, 0, Dc, PLK)
        k_proj(0)
        gcp(2, 0).wait()
        for g in range(1, NG):
            for which in range(3):
                gcp(which, g).start()
        for d in c_late:
            d.start()
        relayout(wuv_r, wuv_p, 0, Dc, PLK)

        def attention(h, side=()):
            key_i = jax.lax.broadcasted_iota(jnp.int32, (TQ, TQ), 0)
            qry_i = jax.lax.broadcasted_iota(jnp.int32, (TQ, TQ), 1)
            causal = key_i <= qry_i
            z_st = z_s[0]
            z_ld = z_s[1]
            zero8 = jnp.full((8, TQ), z_ld, jnp.int32).astype(U32)

            def qk(i):
                qi = q_v[i * TQ:(i + 1) * TQ, :]
                sb = s_v[i % NSB]
                m8 = None
                for t in range(i + 1):
                    tile = _dot_nt(k_v[t * TQ:(t + 1) * TQ, :], qi)
                    if t == i:
                        tile = jnp.where(causal, tile, NEG)
                    sb[z_st + t] = tile
                    tm = _fold8(tile, jnp.maximum)
                    m8 = tm if m8 is None else jnp.maximum(m8, tm)
                return sb, jnp.max(m8, axis=0, keepdims=True)

            parts = []

            def pv(i, sb, m):
                n = (i + 1) * TQ
                m8 = jnp.broadcast_to(m, (8, TQ))
                ps = []
                l8 = None
                for t in range(i + 1):
                    mt = m8
                    if len(parts) >= PIN:
                        tie = pltpu.bitcast(parts[-PIN], U32) & zero8
                        mt = pltpu.bitcast(pltpu.bitcast(m8, U32) | tie, F32)
                    tile = sb[z_ld + t].reshape(TQ // 8, 8, TQ)
                    p = jnp.exp2(tile - mt[None]).reshape(TQ, TQ)
                    part = _fold8(p, jnp.add)
                    l8 = part if l8 is None else l8 + part
                    parts.append(l8)
                    ps.append(p)
                l = jnp.sum(l8, axis=0, keepdims=True)
                pb = jnp.concatenate(ps, axis=0) if i > 0 else ps[0]
                ot = _dot(vt_v[:, 0:n], pb.astype(BF16))
                ot = ot * (1.0 / l)
                ctx_v[h, i * TQ:(i + 1) * TQ, :] = ot.T.astype(BF16)

            pend = [qk(i) for i in range(LOOK)]
            vt = _dot_nt(head_w(wuv_p, h, Dc, PLK).T, ckv_v[...])
            vt_v[...] = vt.astype(BF16)
            per = -(-len(side) // NQ)
            assert per <= D // 8
            for j, step in enumerate(side):
                ct, rg = j // per, j % per
                src = vt[rg * 8:(rg + 1) * 8, ct * TQ:(ct + 1) * TQ]
                step(pltpu.bitcast(src, U32) & zero8)
            for i in range(NQ):
                if i >= LOOK - 1 and i + 1 < NQ:
                    pend.append(qk(i + 1))
                pv(i, *pend[i])

        def head_body(h, carry):
            ahead = ((h % HG) >= RCH).astype(jnp.int32)
            gsrc = jnp.minimum(h // HG + ahead, NG - 1)

            @pl.when(jnp.logical_and(h % HG == RCH, h // HG < NG - 1))
            def _():
                for which in range(3):
                    gcp(which, h // HG + 1).wait()

            ch = h % RCH
            side = (relayout_steps(wq_r, wq_p, gsrc, ch, M, PLQ)
                    + relayout_steps(wuk_r, wuk_p, gsrc, ch, Dc, PLK)
                    + relayout_steps(wuv_r, wuv_p, gsrc, ch, Dc, PLK))
            attention(h, side)
            q_proj(h + 1)
            k_proj(h + 1)
            return carry

        jax.lax.fori_loop(0, H - 1, head_body, 0)

        def sub_rows(r):
            out = []
            for j in range(TR // HB):
                r0 = r * TR + j * HB
                if not isinstance(r0, int):
                    r0 = pl.multiple_of(r0, HB)
                out.append(r0)
            return out

        def stage1(r):
            lns = []
            for r0 in sub_rows(r):
                rows = pl.ds(r0, HB)
                ctx = jnp.concatenate([ctx_v[h, rows, :] for h in range(H)], axis=1)
                att = _dot(ctx, wo_v[...])
                x1 = x_v[rows, :].astype(F32) + mod(2) * att
                x1_v[rows, :] = x1
                h2 = _ln(x1) * (1.0 + mod(4)) + mod(3)
                h2_v[rows, :] = h2
                lns.append(_ln(h2).astype(BF16))
            for r0, ln in zip(sub_rows(r), lns):
                u = _gelu(_dot(ln, w1_v[...]))
                for cidx in range(NC):
                    hh_v[cidx, pl.ds(r0 + PAD, HB), :] = u[:, cidx * LANES:(cidx + 1) * LANES]

        shifts = (1, -1, 2, -2)

        def out_cp(r):
            r0 = r * TR if isinstance(r, int) else pl.multiple_of(r * TR, TR)
            rows = pl.ds(r0, TR)
            return pltpu.make_async_copy(o_v.at[rows, :], out_hbm.at[rows, :], osems.at[r])

        def stage2(r):
            lane_i = jax.lax.broadcasted_iota(jnp.int32, (HB, LANES), 1)
            y1s = []
            for r0 in sub_rows(r):
                tiles = []
                for cidx in range(NC):
                    lo, hi = cidx * LANES, (cidx + 1) * LANES
                    g_lo, g_hi = lo // C4, (hi - 1) // C4
                    t = hh_v[cidx, pl.ds(r0 + PAD - shifts[g_hi], HB), :]
                    for g in range(g_hi - 1, g_lo - 1, -1):
                        tg = hh_v[cidx, pl.ds(r0 + PAD - shifts[g], HB), :]
                        t = jnp.where(lane_i < (g + 1) * C4 - lo, tg, t)
                    tiles.append(t)
                hs = _dot(jnp.concatenate(tiles, axis=1).astype(BF16), w2_v[...])
                y1s.append(h2_v[pl.ds(r0, HB), :] + hs)
            gls = [_gelu(_dot_nt(_ln(y1).astype(BF16), w3_v[...])).astype(BF16)
                   for y1 in y1s]
            for r0, y1, gl in zip(sub_rows(r), y1s, gls):
                rows = pl.ds(r0, HB)
                h3 = _dot(gl, w4_v[...])
                o_v[rows, :] = (x1_v[rows, :] + mod(5) * (y1 + h3)).astype(BF16)
            out_cp(r).start()

        for d in c_late:
            d.wait()
        zpad = jnp.zeros((PAD, LANES), F32)
        for cidx in range(NC):
            hh_v[cidx, 0:PAD, :] = zpad
            hh_v[cidx, PAD + S:PAD + S + PAD, :] = zpad
        attention(H - 1)
        modb_v[...] = _dot(sc8, wmodb_v[...])
        stage1(0)

        def mlp_body(r, carry):
            stage1(r + 1)
            stage2(r)
            return carry

        jax.lax.fori_loop(0, NR - 1, mlp_body, 0)
        stage2(NR - 1)
        for r in range(NR):
            out_cp(r).wait()

    hbm_spec = pl.BlockSpec(memory_space=pltpu.HBM)
    V = pltpu.VMEM
    scratch = [
        V((S, M), BF16),
        V((S, Dc), BF16),
        V((NG, M, HG, D), BF16),
        V((NG, Dc, HG, D), BF16),
        V((NG, Dc, HG, D), BF16),
        V((NG * 8 * PLQ, D), U32),
        V((NG * 8 * PLK, D), U32),
        V((NG * 8 * PLK, D), U32),
        V((H * D, M), BF16),
        V((M, M), BF16),
        V((M, M), BF16),
        V((Fh, M), BF16),
        V((Fh, M), BF16),
        V((M, 2 * M), BF16),
        V((M, 4 * M), BF16),
        V((16, 2 * M), F32),
        V((8, 4 * M), F32),
        V((S, M), BF16),
        V((S, D), BF16),
        V((S, D), BF16),
        V((D, S), BF16),
        V((NQ, TQ, TQ), F32),
        V((NQ, TQ, TQ), F32),
        V((NQ, TQ, TQ), F32),
        V((NQ, TQ, TQ), F32),
        pltpu.SMEM((2,), jnp.int32),
        V((H, S, D), BF16),
        V((S, M), F32),
        V((S, M), F32),
        V((NC, S + 2 * PAD, LANES), F32),
        V((S, M), BF16),
        V((1, M), BF16),
        pltpu.SemaphoreType.DMA((9,)),
        pltpu.SemaphoreType.DMA((3 * NG,)),
        pltpu.SemaphoreType.DMA((NR,)),
        pltpu.SemaphoreType.DMA((NR,)),
    ]
    out = pl.pallas_call(
        kernel,
        out_shape=jax.ShapeDtypeStruct((S, M), BF16),
        in_specs=[hbm_spec] * 12,
        out_specs=hbm_spec,
        scratch_shapes=scratch,
        compiler_params=pltpu.CompilerParams(vmem_limit_bytes=120 * 1024 * 1024),
        name="adaln_cla_mixer",
    )(x2, ckv2, A_w_q, A_w_uk, A_w_uv, wo2, B_w1, B_w2, B_w3.T, B_w4, c, w_mod)
    return out.reshape(B, S, M)
```

```python
import functools
import math
import os

import jax
import jax.numpy as jnp
import jax.experimental.pallas as pl
import jax.experimental.pallas.tpu as pltpu

BF16 = jnp.bfloat16
F32 = jnp.float32
U32 = jnp.uint32

LANES = 128
TQ = 128
TR = 256
HB = 128
HG = 8
LOOK = 4
AHEAD = int(os.environ.get('AHEAD', 2))
NSB = 4
PC = 512
DIST = int(os.environ.get('DIST', 12))
PIN = int(os.environ.get('PIN', 0))
PAD = 16
EPS = 1e-5
LOG2E = math.log2(math.e)
NEG = -1000000000.0 * LOG2E

_NT = (((1,), (1,)), ((), ()))


def _ln(x):
    m = jnp.mean(x, axis=-1, keepdims=True)
    xc = x - m
    v = jnp.mean(xc * xc, axis=-1, keepdims=True)
    return xc * jax.lax.rsqrt(v + EPS)


def _gelu(x):
    return jax.nn.gelu(x, approximate=True)


def _dot(a, b):
    return jnp.dot(a, b, preferred_element_type=F32)


def _dot_nt(a, b):
    return jax.lax.dot_general(a, b, _NT, preferred_element_type=F32)


def _fold8(x, op):
    parts = [op(x[j:j + 8], x[j + 8:j + 16]) for j in range(0, x.shape[0], 16)]
    acc = parts[0]
    for p in parts[1:]:
        acc = op(acc, p)
    return acc


def _run(*gens):
    gens = list(gens)
    while gens:
        for g in list(gens):
            if next(g, gens) is gens:
                gens.remove(g)


@jax.jit
def pallas_adaLN_cond__compressed_kv_cla__mixer_s_mlp__prompt_kernel(
    A_x: jax.Array,
    A_c_kv: jax.Array,
    A_w_q: jax.Array,
    A_w_uk: jax.Array,
    A_w_uv: jax.Array,
    A_w_o: jax.Array,
    B_x: jax.Array,
    B_w1: jax.Array,
    B_w2: jax.Array,
    B_w3: jax.Array,
    B_w4: jax.Array,
    c: jax.Array,
    w_mod: jax.Array,
):
    del B_x
    B, S, M = A_x.shape
    _, Sk, Dc = A_c_kv.shape
    _, H, D = A_w_q.shape
    Fh = B_w3.shape[1]
    assert B == 1 and Sk == S and D == LANES and H % HG == 0 and HG == 8
    assert S % TQ == 0 and S % TR == 0 and S % PC == 0 and TR % HB == 0
    assert M % LANES == 0 and M % 64 == 0 and Dc % 64 == 0
    NG = H // HG
    NQ = S // TQ
    NR = S // TR
    NC = M // LANES
    C4 = M // 4
    PLQ = M // 2 + 1
    PLK = Dc // 2 + 1
    RCH = 4
    qscale = float(D) ** -0.5 * LOG2E

    x2 = A_x.reshape(S, M)
    ckv2 = A_c_kv.reshape(S, Dc)
    wo2 = A_w_o.reshape(H * D, M)

    def kernel(x_hbm, ckv_hbm, wq_hbm, wuk_hbm, wuv_hbm, wo_hbm, w1_hbm, w2_hbm,
               w3_hbm, w4_hbm, c_hbm, wmod_hbm, out_hbm,
               x_v, ckv_v, wq_r, wuk_r, wuv_r, wq_p, wuk_p, wuv_p, wo_v, w1_v,
               w2_v, w3_v, w4_v, wmoda_v, wmodb_v, moda_v, modb_v, hn_v, q_v, k_v,
               vt_v, s0, s1, s2, s3, z_s, ctx_v, x1_v, h2_v, hh_v, o_v, c_v,
               sems, gsems, xsems, osems):

        s_v = (s0, s1, s2, s3)
        z_s[0] = 0
        z_s[1] = 0

        def cp(src, dst, i):
            return pltpu.make_async_copy(src, dst, sems.at[i])

        def gcp(which, g):
            src, dst = ((wq_hbm, wq_r), (wuk_hbm, wuk_r), (wuv_hbm, wuv_r))[which]
            off = g * HG if isinstance(g, int) else pl.multiple_of(g * HG, HG)
            return pltpu.make_async_copy(src.at[:, pl.ds(off, HG), :], dst.at[g],
                                         gsems.at[which * NG + g])

        def xcp(r):
            rows = pl.ds(r * TR, TR)
            return pltpu.make_async_copy(x_hbm.at[rows, :], x_v.at[rows, :], xsems.at[r])

        c_ckv = cp(ckv_hbm, ckv_v, 0)
        c_moda = cp(wmod_hbm.at[:, pl.ds(0, 2 * M)], wmoda_v, 1)
        c_late = [cp(wmod_hbm.at[:, pl.ds(2 * M, 4 * M)], wmodb_v, 2),
                  cp(wo_hbm, wo_v, 3), cp(w1_hbm, w1_v, 4), cp(w2_hbm, w2_v, 5),
                  cp(w3_hbm, w3_v, 6), cp(w4_hbm, w4_v, 7)]

        c_c = cp(c_hbm, c_v, 8)
        c_c.start()
        c_moda.start()
        for r in range(NR):
            xcp(r).start()
        gcp(0, 0).start()
        c_ckv.start()
        gcp(1, 0).start()
        gcp(2, 0).start()

        def relayout_steps(raw, dst, g, chunk, rows, plane):
            n = rows // RCH // 2
            base = g * (8 * plane) + chunk * n
            if not isinstance(base, int):
                base = pl.multiple_of(base, 8)
            view = dst.at[pl.ds(base, 7 * plane + n), :]

            def step(j, tie):
                val = raw[g, pl.ds(chunk * (2 * n) + 2 * j, 2)].reshape(2 * HG, D)
                val = pltpu.bitcast(val, U32)
                if tie is not None:
                    val = val | tie
                view[pl.ds(j, 8, stride=plane), :] = val

            return [functools.partial(step, j) for j in range(n)]

        def relayout(raw, dst, g, rows, plane):
            for ch in range(RCH):
                for step in relayout_steps(raw, dst, g, ch, rows, plane):
                    step(None)

        def head_w(src, h, rows, plane):
            base = (h // HG) * (8 * plane) + ((h % HG) // 2) * plane
            ev = src[pl.ds(base, rows // 2), :]
            od = src[pl.ds(base + 4 * plane, rows // 2), :]
            par = jnp.asarray(h % 2).astype(U32)
            lo = (ev >> (16 * par)) & U32(0xFFFF)
            hi = (od << (16 * (1 - par))) & U32(0xFFFF0000)
            return pltpu.bitcast(lo | hi, BF16)

        def q_proj(h):
            wq = head_w(wq_p, h, M, PLQ)
            for r in range(S // PC):
                rows = slice(r * PC, (r + 1) * PC)
                q_v[rows, :] = (_dot(hn_v[rows, :], wq) * qscale).astype(BF16)

        def k_proj(h):
            wk = head_w(wuk_p, h, Dc, PLK)
            for r in range(S // PC):
                rows = slice(r * PC, (r + 1) * PC)
                k_v[rows, :] = _dot(ckv_v[rows, :], wk).astype(BF16)

        c_c.wait()
        cc = c_v[...].astype(F32)
        sc8 = jnp.broadcast_to((cc * jax.nn.sigmoid(cc)).astype(BF16), (8, M))
        c_moda.wait()
        moda_v[0:8, :] = _dot(sc8, wmoda_v[...])

        def mod(i):
            if i < 2:
                return moda_v[0:1, i * M:(i + 1) * M]
            return modb_v[0:1, (i - 2) * M:(i - 1) * M]

        def ln1_body(r, carry):
            xcp(r).wait()
            rows = pl.ds(pl.multiple_of(r * TR, TR), TR)
            xx = x_v[rows, :].astype(F32)
            hn_v[rows, :] = (_ln(xx) * (1.0 + mod(1)) + mod(0)).astype(BF16)
            return carry

        jax.lax.fori_loop(0, NR, ln1_body, 0)

        gcp(0, 0).wait()
        relayout(wq_r, wq_p, 0, M, PLQ)
        q_proj(0)
        c_ckv.wait()
        gcp(1, 0).wait()
        relayout(wuk_r, wuk_p, 0, Dc, PLK)
        k_proj(0)
        gcp(2, 0).wait()
        for g in range(1, NG):
            for which in range(3):
                gcp(which, g).start()
        for d in c_late:
            d.start()
        relayout(wuv_r, wuv_p, 0, Dc, PLK)

        def attention(h, side=()):
            key_i = jax.lax.broadcasted_iota(jnp.int32, (TQ, TQ), 0)
            qry_i = jax.lax.broadcasted_iota(jnp.int32, (TQ, TQ), 1)
            causal = key_i <= qry_i
            z_st = z_s[0]
            z_ld = z_s[1]
            zero8 = jnp.full((8, TQ), z_ld, jnp.int32).astype(U32)

            mx = {}
            seq = []

            def qk(i):
                qi = q_v[i * TQ:(i + 1) * TQ, :]
                sb = s_v[i % NSB]
                m8 = None
                for t in range(i + 1):
                    tile = _dot_nt(k_v[t * TQ:(t + 1) * TQ, :], qi)
                    seq.append(tile[0:8])
                    if t == i:
                        tile = jnp.where(causal, tile, NEG)
                    sb[z_st + t] = tile
                    tm = _fold8(tile, jnp.maximum)
                    m8 = tm if m8 is None else jnp.maximum(m8, tm)
                    if t == i:
                        mx[i] = jnp.max(m8, axis=0, keepdims=True)
                    yield

            parts = []

            def pv(i):
                sb = s_v[i % NSB]
                m8 = jnp.broadcast_to(mx[i], (8, TQ))
                l8 = None
                ot = None
                for t in range(i + 1):
                    tie = pltpu.bitcast(seq[-DIST], U32)
                    if PIN and len(parts) >= PIN:
                        tie = tie | pltpu.bitcast(parts[-PIN], U32)
                    mt = pltpu.bitcast(pltpu.bitcast(m8, U32) | (tie & zero8), F32)
                    tile = sb[z_ld + t].reshape(TQ // 8, 8, TQ)
                    p = jnp.exp2(tile - mt[None]).reshape(TQ, TQ)
                    part = _fold8(p, jnp.add)
                    l8 = part if l8 is None else l8 + part
                    parts.append(l8)
                    o = _dot(vt_v[:, t * TQ:(t + 1) * TQ], p.astype(BF16))
                    seq.append(o[0:8])
                    ot = o if ot is None else ot + o
                    if t == i:
                        l = jnp.sum(l8, axis=0, keepdims=True)
                        ot = ot * (1.0 / l)
                        ctx_v[h, i * TQ:(i + 1) * TQ, :] = ot.T.astype(BF16)
                    yield

            for i in range(LOOK):
                _run(qk(i))
            vt = _dot_nt(head_w(wuv_p, h, Dc, PLK).T, ckv_v[...])
            vt_v[...] = vt.astype(BF16)
            for ct in range(NQ):
                seq.extend([vt[0:8, ct * TQ:(ct + 1) * TQ]] * (Dc // LANES))
            per = -(-len(side) // NQ)
            assert per <= D // 8
            for j, step in enumerate(side):
                ct, rg = j // per, j % per
                src = vt[rg * 8:(rg + 1) * 8, ct * TQ:(ct + 1) * TQ]
                step(pltpu.bitcast(src, U32) & zero8)
            for i in range(NQ):
                j = i + AHEAD
                if LOOK <= j < NQ:
                    _run(qk(j), pv(i))
                else:
                    _run(pv(i))

        def head_body(h, carry):
            ahead = ((h % HG) >= RCH).astype(jnp.int32)
            gsrc = jnp.minimum(h // HG + ahead, NG - 1)

            @pl.when(jnp.logical_and(h % HG == RCH, h // HG < NG - 1))
            def _():
                for which in range(3):
                    gcp(which, h // HG + 1).wait()

            ch = h % RCH
            side = (relayout_steps(wq_r, wq_p, gsrc, ch, M, PLQ)
                    + relayout_steps(wuk_r, wuk_p, gsrc, ch, Dc, PLK)
                    + relayout_steps(wuv_r, wuv_p, gsrc, ch, Dc, PLK))
            attention(h, side)
            q_proj(h + 1)
            k_proj(h + 1)
            return carry

        jax.lax.fori_loop(0, H - 1, head_body, 0)

        def sub_rows(r):
            out = []
            for j in range(TR // HB):
                r0 = r * TR + j * HB
                if not isinstance(r0, int):
                    r0 = pl.multiple_of(r0, HB)
                out.append(r0)
            return out

        def stage1(r):
            lns = []
            for r0 in sub_rows(r):
                rows = pl.ds(r0, HB)
                ctx = jnp.concatenate([ctx_v[h, rows, :] for h in range(H)], axis=1)
                att = _dot(ctx, wo_v[...])
                x1 = x_v[rows, :].astype(F32) + mod(2) * att
                x1_v[rows, :] = x1
                h2 = _ln(x1) * (1.0 + mod(4)) + mod(3)
                h2_v[rows, :] = h2
                lns.append(_ln(h2).astype(BF16))
            for r0, ln in zip(sub_rows(r), lns):
                u = _gelu(_dot(ln, w1_v[...]))
                for cidx in range(NC):
                    hh_v[cidx, pl.ds(r0 + PAD, HB), :] = u[:, cidx * LANES:(cidx + 1) * LANES]

        shifts = (1, -1, 2, -2)

        def out_cp(r):
            r0 = r * TR if isinstance(r, int) else pl.multiple_of(r * TR, TR)
            rows = pl.ds(r0, TR)
            return pltpu.make_async_copy(o_v.at[rows, :], out_hbm.at[rows, :], osems.at[r])

        def stage2(r):
            lane_i = jax.lax.broadcasted_iota(jnp.int32, (HB, LANES), 1)
            y1s = []
            for r0 in sub_rows(r):
                tiles = []
                for cidx in range(NC):
                    lo, hi = cidx * LANES, (cidx + 1) * LANES
                    g_lo, g_hi = lo // C4, (hi - 1) // C4
                    t = hh_v[cidx, pl.ds(r0 + PAD - shifts[g_hi], HB), :]
                    for g in range(g_hi - 1, g_lo - 1, -1):
                        tg = hh_v[cidx, pl.ds(r0 + PAD - shifts[g], HB), :]
                        t = jnp.where(lane_i < (g + 1) * C4 - lo, tg, t)
                    tiles.append(t)
                hs = _dot(jnp.concatenate(tiles, axis=1).astype(BF16), w2_v[...])
                y1s.append(h2_v[pl.ds(r0, HB), :] + hs)
            gls = [_gelu(_dot_nt(_ln(y1).astype(BF16), w3_v[...])).astype(BF16)
                   for y1 in y1s]
            for r0, y1, gl in zip(sub_rows(r), y1s, gls):
                rows = pl.ds(r0, HB)
                h3 = _dot(gl, w4_v[...])
                o_v[rows, :] = (x1_v[rows, :] + mod(5) * (y1 + h3)).astype(BF16)
            out_cp(r).start()

        for d in c_late:
            d.wait()
        zpad = jnp.zeros((PAD, LANES), F32)
        for cidx in range(NC):
            hh_v[cidx, 0:PAD, :] = zpad
            hh_v[cidx, PAD + S:PAD + S + PAD, :] = zpad
        attention(H - 1)
        modb_v[...] = _dot(sc8, wmodb_v[...])
        stage1(0)

        def mlp_body(r, carry):
            stage1(r + 1)
            stage2(r)
            return carry

        jax.lax.fori_loop(0, NR - 1, mlp_body, 0)
        stage2(NR - 1)
        for r in range(NR):
            out_cp(r).wait()

    hbm_spec = pl.BlockSpec(memory_space=pltpu.HBM)
    V = pltpu.VMEM
    scratch = [
        V((S, M), BF16),
        V((S, Dc), BF16),
        V((NG, M, HG, D), BF16),
        V((NG, Dc, HG, D), BF16),
        V((NG, Dc, HG, D), BF16),
        V((NG * 8 * PLQ, D), U32),
        V((NG * 8 * PLK, D), U32),
        V((NG * 8 * PLK, D), U32),
        V((H * D, M), BF16),
        V((M, M), BF16),
        V((M, M), BF16),
        V((Fh, M), BF16),
        V((Fh, M), BF16),
        V((M, 2 * M), BF16),
        V((M, 4 * M), BF16),
        V((16, 2 * M), F32),
        V((8, 4 * M), F32),
        V((S, M), BF16),
        V((S, D), BF16),
        V((S, D), BF16),
        V((D, S), BF16),
        V((NQ, TQ, TQ), F32),
        V((NQ, TQ, TQ), F32),
        V((NQ, TQ, TQ), F32),
        V((NQ, TQ, TQ), F32),
        pltpu.SMEM((2,), jnp.int32),
        V((H, S, D), BF16),
        V((S, M), F32),
        V((S, M), F32),
        V((NC, S + 2 * PAD, LANES), F32),
        V((S, M), BF16),
        V((1, M), BF16),
        pltpu.SemaphoreType.DMA((9,)),
        pltpu.SemaphoreType.DMA((3 * NG,)),
        pltpu.SemaphoreType.DMA((NR,)),
        pltpu.SemaphoreType.DMA((NR,)),
    ]
    out = pl.pallas_call(
        kernel,
        out_shape=jax.ShapeDtypeStruct((S, M), BF16),
        in_specs=[hbm_spec] * 12,
        out_specs=hbm_spec,
        scratch_shapes=scratch,
        compiler_params=pltpu.CompilerParams(vmem_limit_bytes=120 * 1024 * 1024),
        name="adaln_cla_mixer",
    )(x2, ckv2, A_w_q, A_w_uk, A_w_uv, wo2, B_w1, B_w2, B_w3.T, B_w4, c, w_mod)
    return out.reshape(B, S, M)
```

```python
import functools
import math
import os

import jax
import jax.numpy as jnp
import jax.experimental.pallas as pl
import jax.experimental.pallas.tpu as pltpu

BF16 = jnp.bfloat16
F32 = jnp.float32
U32 = jnp.uint32

LANES = 128
TQ = 128
TR = 256
HB = 128
HG = 8
LOOK = 4
AHEAD = int(os.environ.get('AHEAD', 2))
NSB = 4
KC = 256
QC = int(os.environ.get('QC', 128))
PC = 512
DIST = int(os.environ.get('DIST', 12))
PIN = int(os.environ.get('PIN', 0))
PAD = 16
EPS = 1e-5
LOG2E = math.log2(math.e)
NEG = -1000000000.0 * LOG2E

_NT = (((1,), (1,)), ((), ()))


def _ln(x):
    m = jnp.mean(x, axis=-1, keepdims=True)
    xc = x - m
    v = jnp.mean(xc * xc, axis=-1, keepdims=True)
    return xc * jax.lax.rsqrt(v + EPS)


def _gelu(x):
    return jax.nn.gelu(x, approximate=True)


def _dot(a, b):
    return jnp.dot(a, b, preferred_element_type=F32)


def _dot_nt(a, b):
    return jax.lax.dot_general(a, b, _NT, preferred_element_type=F32)


def _fold8(x, op):
    parts = [op(x[j:j + 8], x[j + 8:j + 16]) for j in range(0, x.shape[0], 16)]
    acc = parts[0]
    for p in parts[1:]:
        acc = op(acc, p)
    return acc


def _run(*gens):
    gens = list(gens)
    while gens:
        for g in list(gens):
            if next(g, gens) is gens:
                gens.remove(g)


@jax.jit
def pallas_adaLN_cond__compressed_kv_cla__mixer_s_mlp__prompt_kernel(
    A_x: jax.Array,
    A_c_kv: jax.Array,
    A_w_q: jax.Array,
    A_w_uk: jax.Array,
    A_w_uv: jax.Array,
    A_w_o: jax.Array,
    B_x: jax.Array,
    B_w1: jax.Array,
    B_w2: jax.Array,
    B_w3: jax.Array,
    B_w4: jax.Array,
    c: jax.Array,
    w_mod: jax.Array,
):
    del B_x
    B, S, M = A_x.shape
    _, Sk, Dc = A_c_kv.shape
    _, H, D = A_w_q.shape
    Fh = B_w3.shape[1]
    assert B == 1 and Sk == S and D == LANES and H % HG == 0 and HG == 8
    assert S % TQ == 0 and S % TR == 0 and S % PC == 0 and TR % HB == 0
    assert M % LANES == 0 and M % 64 == 0 and Dc % 64 == 0
    NG = H // HG
    NQ = S // TQ
    NR = S // TR
    NC = M // LANES
    C4 = M // 4
    PLQ = M // 2 + 1
    PLK = Dc // 2 + 1
    RCH = 4
    NK = S // KC
    XC = S // RCH
    NSEM = NK + 2 * RCH + 3 * NG - 1 + 8
    assert NK > RCH + 1 and LOOK * TQ <= PC
    qscale = float(D) ** -0.5 * LOG2E

    x2 = A_x.reshape(S, M)
    ckv2 = A_c_kv.reshape(S, Dc)
    wo2 = A_w_o.reshape(H * D, M)

    def kernel(x_hbm, ckv_hbm, wq_hbm, wuk_hbm, wuv_hbm, wo_hbm, w1_hbm, w2_hbm,
               w3_hbm, w4_hbm, c_hbm, wmod_hbm, out_hbm,
               x_v, ckv_v, wq_r, wuk_r, wuv_r, wq_p, wuk_p, wuv_p, wo_v, w1_v,
               w2_v, w3_v, w4_v, wmoda_v, wmodb_v, moda_v, modb_v, hn_v, q_v, k_v,
               vt_v, s0, s1, s2, s3, z_s, ctx_v, x1_v, h2_v, hh_v, o_v, c_v,
               sems, osems):

        s_v = (s0, s1, s2, s3)
        z_s[0] = 0
        z_s[1] = 0

        def aligned(i, n):
            return i * n if isinstance(i, int) else pl.multiple_of(i * n, n)

        def cp(src, dst, i):
            return pltpu.make_async_copy(src, dst, sems.at[i])

        def c_ckv(r):
            rows = pl.ds(aligned(r, KC), KC)
            return cp(ckv_hbm.at[rows, :], ckv_v.at[rows, :], r)

        def c_x(j):
            rows = pl.ds(aligned(j, XC), XC)
            return cp(x_hbm.at[rows, :], x_v.at[rows, :], NK + j)

        def c_q0(j):
            rows = pl.ds(aligned(j, M // RCH), M // RCH)
            return cp(wq_hbm.at[rows, pl.ds(0, HG), :], wq_r.at[0, rows], NK + RCH + j)

        nsem = [NK + 2 * RCH]

        def cp_next(src, dst):
            nsem[0] += 1
            return cp(src, dst, nsem[0] - 1)

        def gcp(src, dst, g):
            return cp_next(src.at[:, pl.ds(g * HG, HG), :], dst.at[g])

        c_k0 = gcp(wuk_hbm, wuk_r, 0)
        c_v0 = gcp(wuv_hbm, wuv_r, 0)
        c_c = cp_next(c_hbm, c_v)
        c_moda = cp_next(wmod_hbm.at[:, pl.ds(0, 2 * M)], wmoda_v)
        c_grp = [[gcp(wq_hbm, wq_r, g), gcp(wuk_hbm, wuk_r, g), gcp(wuv_hbm, wuv_r, g)]
                 for g in range(1, NG)]
        c_late = [cp_next(wmod_hbm.at[:, pl.ds(2 * M, 4 * M)], wmodb_v),
                  cp_next(wo_hbm, wo_v), cp_next(w1_hbm, w1_v), cp_next(w2_hbm, w2_v),
                  cp_next(w3_hbm, w3_v), cp_next(w4_hbm, w4_v)]
        assert nsem[0] == NSEM
        order = [c_k0] + [c_ckv(r) for r in range(NK - RCH)] + [c_c, c_moda]
        for j in range(RCH):
            order += [c_ckv(NK - RCH + j), c_x(j), c_q0(j)]
        order += [c_v0] + [d for grp in c_grp for d in grp] + c_late
        for d in order:
            d.start()

        def relayout_steps(raw, dst, g, chunk, rows, plane):
            n = rows // RCH // 2
            base = g * (8 * plane) + chunk * n
            if not isinstance(base, int):
                base = pl.multiple_of(base, 8)
            view = dst.at[pl.ds(base, 7 * plane + n), :]

            def step(j, tie):
                val = raw[g, pl.ds(chunk * (2 * n) + 2 * j, 2)].reshape(2 * HG, D)
                val = pltpu.bitcast(val, U32)
                if tie is not None:
                    val = val | tie
                view[pl.ds(j, 8, stride=plane), :] = val

            return [functools.partial(step, j) for j in range(n)]

        def relayout(raw, dst, g, rows, plane):
            for ch in range(RCH):
                for step in relayout_steps(raw, dst, g, ch, rows, plane):
                    step(None)

        def head_w(src, h, rows, plane, tie=None):
            base = (h // HG) * (8 * plane) + ((h % HG) // 2) * plane
            ev = src[pl.ds(base, rows // 2), :]
            od = src[pl.ds(base + 4 * plane, rows // 2), :]
            if not isinstance(h, int):
                par = (h % 2).astype(U32)
                w = (((ev >> (16 * par)) & U32(0xFFFF))
                     | ((od << (16 * (1 - par))) & U32(0xFFFF0000)))
            elif h % 2 == 0:
                w = (ev & U32(0xFFFF)) | (od << 16)
            else:
                w = (ev >> 16) | (od & U32(0xFFFF0000))
            if tie is not None:
                w = jnp.concatenate([w[0:8] | tie, w[8:]], axis=0)
            return pltpu.bitcast(w, BF16)

        def q_proj(h, chunks):
            wq = head_w(wq_p, h, M, PLQ)
            for r in chunks:
                for r0 in range(r * PC, (r + 1) * PC, QC):
                    rows = slice(r0, r0 + QC)
                    q_v[rows, :] = (_dot(hn_v[rows, :], wq) * qscale).astype(BF16)

        def k_proj(h):
            wk = head_w(wuk_p, h, Dc, PLK)
            for r in range(S // PC):
                rows = slice(r * PC, (r + 1) * PC)
                k_v[HG - 1, rows, :] = _dot(ckv_v[rows, :], wk).astype(BF16)

        def silu_c():
            cc = c_v[...].astype(F32)
            return jnp.broadcast_to((cc * jax.nn.sigmoid(cc)).astype(BF16), (8, M))

        def mod(i):
            if i < 2:
                return moda_v[0:1, i * M:(i + 1) * M]
            return modb_v[0:1, (i - 2) * M:(i - 1) * M]

        def zeros8():
            return jnp.full((8, LANES), z_s[1], jnp.int32).astype(U32)

        def k_chunk(r, after_head=None, ties=None):
            rows = pl.ds(aligned(r, KC), KC)
            lhs = ckv_v[rows, :]
            for h in range(HG):
                tie = None if ties is None else ties(h)
                res = _dot(lhs, head_w(wuk_p, h, Dc, PLK, tie))
                k_v[h, rows, :] = res.astype(BF16)
                if after_head is not None:
                    after_head(h, res)

        c_k0.wait()
        relayout(wuk_r, wuk_p, 0, Dc, PLK)

        def ka_body(r, carry):
            c_ckv(r).wait()
            k_chunk(r)
            return carry

        jax.lax.fori_loop(0, NK - RCH - 1, ka_body, 0)

        c_ckv(NK - RCH - 1).wait()
        c_c.wait()
        c_moda.wait()
        sc8 = silu_c()

        def mod_tiles(h, res):
            for ct in range(h, 2 * NC, HG):
                cols = slice(ct * LANES, (ct + 1) * LANES)
                moda_v[0:8, cols] = _dot(sc8, wmoda_v[:, cols])

        k_chunk(NK - RCH - 1, after_head=mod_tiles)

        def kb_body(j, carry):
            c_ckv(NK - RCH + j).wait()
            c_x(j).wait()
            c_q0(j).wait()
            zero8 = zeros8()
            lr = XC // HG
            done = []
            for i in range(HG):
                rows = pl.ds(pl.multiple_of(j * XC + i * lr, lr), lr)
                hn = _ln(x_v[rows, :].astype(F32)) * (1.0 + mod(1)) + mod(0)
                hn_v[rows, :] = hn.astype(BF16)
                done.append(hn)
            steps = relayout_steps(wq_r, wq_p, 0, j, M, PLQ)
            per = len(steps) // HG

            def ties(h):
                if h < 2:
                    return None
                return pltpu.bitcast(_fold8(done[h - 2][:, 0:LANES], jnp.maximum), U32) & zero8

            def side(h, res):
                for i, step in enumerate(steps[h * per:(h + 1) * per]):
                    step(pltpu.bitcast(res[i * 8:(i + 1) * 8], U32) & zero8)

            k_chunk(NK - RCH + j, after_head=side, ties=ties)
            return carry

        jax.lax.fori_loop(0, RCH, kb_body, 0)

        c_v0.wait()
        q_proj(0, [0])
        relayout(wuv_r, wuv_p, 0, Dc, PLK)

        def attention(h, kh, side):
            key_i = jax.lax.broadcasted_iota(jnp.int32, (TQ, TQ), 0)
            qry_i = jax.lax.broadcasted_iota(jnp.int32, (TQ, TQ), 1)
            causal = key_i <= qry_i
            z_st = z_s[0]
            z_ld = z_s[1]
            zero8 = zeros8()

            mx = {}
            seq = []

            def qk(i):
                qi = q_v[i * TQ:(i + 1) * TQ, :]
                sb = s_v[i % NSB]
                m8 = None
                for t in range(i + 1):
                    tile = _dot_nt(kh[t * TQ:(t + 1) * TQ, :], qi)
                    seq.append(tile[0:8])
                    if t == i:
                        tile = jnp.where(causal, tile, NEG)
                    sb[z_st + t] = tile
                    tm = _fold8(tile, jnp.maximum)
                    m8 = tm if m8 is None else jnp.maximum(m8, tm)
                    if t == i:
                        mx[i] = jnp.max(m8, axis=0, keepdims=True)
                    yield

            parts = []

            def pv(i):
                sb = s_v[i % NSB]
                m8 = jnp.broadcast_to(mx[i], (8, TQ))
                l8 = None
                ot = None
                for t in range(i + 1):
                    tie = pltpu.bitcast(seq[-DIST], U32)
                    if PIN and len(parts) >= PIN:
                        tie = tie | pltpu.bitcast(parts[-PIN], U32)
                    mt = pltpu.bitcast(pltpu.bitcast(m8, U32) | (tie & zero8), F32)
                    tile = sb[z_ld + t].reshape(TQ // 8, 8, TQ)
                    p = jnp.exp2(tile - mt[None]).reshape(TQ, TQ)
                    part = _fold8(p, jnp.add)
                    l8 = part if l8 is None else l8 + part
                    parts.append(l8)
                    o = _dot(vt_v[:, t * TQ:(t + 1) * TQ], p.astype(BF16))
                    seq.append(o[0:8])
                    ot = o if ot is None else ot + o
                    if t == i:
                        l = jnp.sum(l8, axis=0, keepdims=True)
                        ot = ot * (1.0 / l)
                        ctx_v[h, i * TQ:(i + 1) * TQ, :] = ot.T.astype(BF16)
                    yield

            q_proj(h, range(1, S // PC))
            for i in range(LOOK):
                _run(qk(i))
            vt = _dot_nt(head_w(wuv_p, h, Dc, PLK).T, ckv_v[...])
            vt_v[...] = vt.astype(BF16)
            for ct in range(NQ):
                seq.extend([vt[0:8, ct * TQ:(ct + 1) * TQ]] * (Dc // LANES))
            per = -(-len(side) // NQ)
            assert per <= D // 8
            for j, step in enumerate(side):
                ct, rg = j // per, j % per
                src = vt[rg * 8:(rg + 1) * 8, ct * TQ:(ct + 1) * TQ]
                step(pltpu.bitcast(src, U32) & zero8)
            for i in range(NQ):
                j = i + AHEAD
                if LOOK <= j < NQ:
                    _run(qk(j), pv(i))
                else:
                    _run(pv(i))

        def side_work(h):
            ahead = ((h % HG) >= RCH).astype(jnp.int32)
            gsrc = jnp.minimum(h // HG + ahead, NG - 1)
            ch = h % RCH
            return (relayout_steps(wq_r, wq_p, gsrc, ch, M, PLQ)
                    + relayout_steps(wuk_r, wuk_p, gsrc, ch, Dc, PLK)
                    + relayout_steps(wuv_r, wuv_p, gsrc, ch, Dc, PLK))

        def first_body(h, carry):
            @pl.when(h == RCH)
            def _():
                for d in c_grp[0]:
                    d.wait()

            attention(h, k_v.at[jnp.minimum(h, HG - 1)], side_work(h))
            q_proj(jnp.minimum(h + 1, H - 1), [0])
            return carry

        def head_body(h, carry):
            attention(h, k_v.at[HG - 1], side_work(h))
            q_proj(h + 1, [0])
            k_proj(h + 1)
            return carry

        def pass_body(p, carry):
            jax.lax.fori_loop(p * (H - 1), HG - 1 + p * (H - HG + 1), first_body, 0)

            @pl.when(p == 0)
            def _():
                for grp in c_grp[1:]:
                    for d in grp:
                        d.wait()
                for d in c_late:
                    d.wait()
                modb_v[...] = _dot(silu_c(), wmodb_v[...])
                jax.lax.fori_loop(HG - 1, H - 1, head_body, 0)

            return carry

        jax.lax.fori_loop(0, 2, pass_body, 0)

        def sub_rows(r):
            out = []
            for j in range(TR // HB):
                r0 = r * TR + j * HB
                if not isinstance(r0, int):
                    r0 = pl.multiple_of(r0, HB)
                out.append(r0)
            return out

        def stage1(r):
            lns = []
            for r0 in sub_rows(r):
                rows = pl.ds(r0, HB)
                ctx = jnp.concatenate([ctx_v[h, rows, :] for h in range(H)], axis=1)
                att = _dot(ctx, wo_v[...])
                x1 = x_v[rows, :].astype(F32) + mod(2) * att
                x1_v[rows, :] = x1
                h2 = _ln(x1) * (1.0 + mod(4)) + mod(3)
                h2_v[rows, :] = h2
                lns.append(_ln(h2).astype(BF16))
            for r0, ln in zip(sub_rows(r), lns):
                u = _gelu(_dot(ln, w1_v[...]))
                for cidx in range(NC):
                    hh_v[cidx, pl.ds(r0 + PAD, HB), :] = u[:, cidx * LANES:(cidx + 1) * LANES]

        shifts = (1, -1, 2, -2)

        def out_cp(r):
            r0 = r * TR if isinstance(r, int) else pl.multiple_of(r * TR, TR)
            rows = pl.ds(r0, TR)
            return pltpu.make_async_copy(o_v.at[rows, :], out_hbm.at[rows, :], osems.at[r])

        def stage2(r):
            lane_i = jax.lax.broadcasted_iota(jnp.int32, (HB, LANES), 1)
            y1s = []
            for r0 in sub_rows(r):
                tiles = []
                for cidx in range(NC):
                    lo, hi = cidx * LANES, (cidx + 1) * LANES
                    g_lo, g_hi = lo // C4, (hi - 1) // C4
                    t = hh_v[cidx, pl.ds(r0 + PAD - shifts[g_hi], HB), :]
                    for g in range(g_hi - 1, g_lo - 1, -1):
                        tg = hh_v[cidx, pl.ds(r0 + PAD - shifts[g], HB), :]
                        t = jnp.where(lane_i < (g + 1) * C4 - lo, tg, t)
                    tiles.append(t)
                hs = _dot(jnp.concatenate(tiles, axis=1).astype(BF16), w2_v[...])
                y1s.append(h2_v[pl.ds(r0, HB), :] + hs)
            gls = [_gelu(_dot_nt(_ln(y1).astype(BF16), w3_v[...])).astype(BF16)
                   for y1 in y1s]
            for r0, y1, gl in zip(sub_rows(r), y1s, gls):
                rows = pl.ds(r0, HB)
                h3 = _dot(gl, w4_v[...])
                o_v[rows, :] = (x1_v[rows, :] + mod(5) * (y1 + h3)).astype(BF16)
            out_cp(r).start()

        zpad = jnp.zeros((PAD, LANES), F32)
        for cidx in range(NC):
            hh_v[cidx, 0:PAD, :] = zpad
            hh_v[cidx, PAD + S:PAD + S + PAD, :] = zpad

        def s1_body(r, carry):
            stage1(r)
            return carry

        def s2_body(r, carry):
            stage2(r)
            return carry

        jax.lax.fori_loop(0, NR, s1_body, 0)
        jax.lax.fori_loop(0, NR, s2_body, 0)
        for r in range(NR):
            out_cp(r).wait()

    hbm_spec = pl.BlockSpec(memory_space=pltpu.HBM)
    V = pltpu.VMEM
    scratch = [
        V((S, M), BF16),
        V((S, Dc), BF16),
        V((NG, M, HG, D), BF16),
        V((NG, Dc, HG, D), BF16),
        V((NG, Dc, HG, D), BF16),
        V((NG * 8 * PLQ, D), U32),
        V((NG * 8 * PLK, D), U32),
        V((NG * 8 * PLK, D), U32),
        V((H * D, M), BF16),
        V((M, M), BF16),
        V((M, M), BF16),
        V((Fh, M), BF16),
        V((Fh, M), BF16),
        V((M, 2 * M), BF16),
        V((M, 4 * M), BF16),
        V((16, 2 * M), F32),
        V((8, 4 * M), F32),
        V((S, M), BF16),
        V((S, D), BF16),
        V((HG, S, D), BF16),
        V((D, S), BF16),
        V((NQ, TQ, TQ), F32),
        V((NQ, TQ, TQ), F32),
        V((NQ, TQ, TQ), F32),
        V((NQ, TQ, TQ), F32),
        pltpu.SMEM((2,), jnp.int32),
        V((H, S, D), BF16),
        V((S, M), F32),
        V((S, M), F32),
        V((NC, S + 2 * PAD, LANES), F32),
        V((S, M), BF16),
        V((1, M), BF16),
        pltpu.SemaphoreType.DMA((NSEM,)),
        pltpu.SemaphoreType.DMA((NR,)),
    ]
    out = pl.pallas_call(
        kernel,
        out_shape=jax.ShapeDtypeStruct((S, M), BF16),
        in_specs=[hbm_spec] * 12,
        out_specs=hbm_spec,
        scratch_shapes=scratch,
        compiler_params=pltpu.CompilerParams(vmem_limit_bytes=120 * 1024 * 1024),
        name="adaln_cla_mixer",
    )(x2, ckv2, A_w_q, A_w_uk, A_w_uv, wo2, B_w1, B_w2, B_w3.T, B_w4, c, w_mod)
    return out.reshape(B, S, M)
```

```python
import functools
import math
import os

import jax
import jax.numpy as jnp
import jax.experimental.pallas as pl
import jax.experimental.pallas.tpu as pltpu

BF16 = jnp.bfloat16
F32 = jnp.float32
U32 = jnp.uint32

LANES = 128
TQ = 128
TR = 256
HB = 128
HG = 8
LOOK = 4
AHEAD = int(os.environ.get('AHEAD', 2))
NSB = 4
KC = 256
QC = int(os.environ.get('QC', 128))
PC = 512
DIST = int(os.environ.get('DIST', 12))
PIN = int(os.environ.get('PIN', 0))
PAD = 16
EPS = 1e-5
LOG2E = math.log2(math.e)
NEG = -1000000000.0 * LOG2E

_NT = (((1,), (1,)), ((), ()))


def _ln(x):
    m = jnp.mean(x, axis=-1, keepdims=True)
    xc = x - m
    v = jnp.mean(xc * xc, axis=-1, keepdims=True)
    return xc * jax.lax.rsqrt(v + EPS)


def _gelu(x):
    return jax.nn.gelu(x, approximate=True)


def _dot(a, b):
    return jnp.dot(a, b, preferred_element_type=F32)


def _dot_nt(a, b):
    return jax.lax.dot_general(a, b, _NT, preferred_element_type=F32)


def _fold8(x, op):
    parts = [op(x[j:j + 8], x[j + 8:j + 16]) for j in range(0, x.shape[0], 16)]
    acc = parts[0]
    for p in parts[1:]:
        acc = op(acc, p)
    return acc


def _gstride(plane):
    return -(-8 * plane // 32) * 32


def _run(*gens):
    gens = list(gens)
    while gens:
        for g in list(gens):
            if next(g, gens) is gens:
                gens.remove(g)


@jax.jit
def pallas_adaLN_cond__compressed_kv_cla__mixer_s_mlp__prompt_kernel(
    A_x: jax.Array,
    A_c_kv: jax.Array,
    A_w_q: jax.Array,
    A_w_uk: jax.Array,
    A_w_uv: jax.Array,
    A_w_o: jax.Array,
    B_x: jax.Array,
    B_w1: jax.Array,
    B_w2: jax.Array,
    B_w3: jax.Array,
    B_w4: jax.Array,
    c: jax.Array,
    w_mod: jax.Array,
):
    del B_x
    B, S, M = A_x.shape
    _, Sk, Dc = A_c_kv.shape
    _, H, D = A_w_q.shape
    Fh = B_w3.shape[1]
    assert B == 1 and Sk == S and D == LANES and H % HG == 0 and HG == 8
    assert S % TQ == 0 and S % TR == 0 and S % PC == 0 and TR % HB == 0
    assert M % LANES == 0 and M % 64 == 0 and Dc % 64 == 0
    NG = H // HG
    NQ = S // TQ
    NR = S // TR
    NC = M // LANES
    C4 = M // 4
    PLQ = M // 2 + 1
    PLK = Dc // 2 + 1
    RCH = 4
    NK = S // KC
    XC = S // RCH
    NSEM = NK + 2 * RCH + 3 * NG - 1 + 8
    assert NK > RCH + 1 and LOOK * TQ <= PC and PC // QC == RCH
    qscale = float(D) ** -0.5 * LOG2E

    x2 = A_x.reshape(S, M)
    ckv2 = A_c_kv.reshape(S, Dc)
    wo2 = A_w_o.reshape(H * D, M)

    def kernel(x_hbm, ckv_hbm, wq_hbm, wuk_hbm, wuv_hbm, wo_hbm, w1_hbm, w2_hbm,
               w3_hbm, w4_hbm, c_hbm, wmod_hbm, out_hbm,
               x_v, ckv_v, wq_r, wuk_r, wuv_r, wq_p, wuk_p, wuv_p, wo_v, w1_v,
               w2_v, w3_v, w4_v, wmoda_v, wmodb_v, moda_v, modb_v, hn_v, wqc_v, q_v, k_v,
               vt_v, s0, s1, s2, s3, z_s, ctx_v, x1_v, h2_v, hh_v, o_v, c_v,
               sems, osems):

        s_v = (s0, s1, s2, s3)
        z_s[0] = 0
        z_s[1] = 0

        def aligned(i, n):
            return i * n if isinstance(i, int) else pl.multiple_of(i * n, n)

        def cp(src, dst, i):
            return pltpu.make_async_copy(src, dst, sems.at[i])

        def c_ckv(r):
            rows = pl.ds(aligned(r, KC), KC)
            return cp(ckv_hbm.at[rows, :], ckv_v.at[rows, :], r)

        def c_x(j):
            rows = pl.ds(aligned(j, XC), XC)
            return cp(x_hbm.at[rows, :], x_v.at[rows, :], NK + j)

        def c_q0(j):
            rows = pl.ds(aligned(j, M // RCH), M // RCH)
            return cp(wq_hbm.at[rows, pl.ds(0, HG), :], wq_r.at[0, rows], NK + RCH + j)

        nsem = [NK + 2 * RCH]

        def cp_next(src, dst):
            nsem[0] += 1
            return cp(src, dst, nsem[0] - 1)

        def gcp(src, dst, g):
            return cp_next(src.at[:, pl.ds(g * HG, HG), :], dst.at[g])

        c_k0 = gcp(wuk_hbm, wuk_r, 0)
        c_v0 = gcp(wuv_hbm, wuv_r, 0)
        c_c = cp_next(c_hbm, c_v)
        c_moda = cp_next(wmod_hbm.at[:, pl.ds(0, 2 * M)], wmoda_v)
        c_grp = [[gcp(wq_hbm, wq_r, g), gcp(wuk_hbm, wuk_r, g), gcp(wuv_hbm, wuv_r, g)]
                 for g in range(1, NG)]
        c_late = [cp_next(wmod_hbm.at[:, pl.ds(2 * M, 4 * M)], wmodb_v),
                  cp_next(wo_hbm, wo_v), cp_next(w1_hbm, w1_v), cp_next(w2_hbm, w2_v),
                  cp_next(w3_hbm, w3_v), cp_next(w4_hbm, w4_v)]
        assert nsem[0] == NSEM
        order = [c_k0] + [c_ckv(r) for r in range(NK - RCH)] + [c_c, c_moda]
        for j in range(RCH):
            order += [c_ckv(NK - RCH + j), c_x(j), c_q0(j)]
        order += [c_v0] + [d for grp in c_grp for d in grp] + c_late
        for d in order:
            d.start()

        def relayout_steps(raw, dst, g, chunk, rows, plane):
            n = rows // RCH // 2
            base = g * _gstride(plane) + chunk * n
            if not isinstance(base, int):
                base = pl.multiple_of(base, 8)
            view = dst.at[pl.ds(base, 7 * plane + n), :]

            def step(j, tie):
                val = raw[g, pl.ds(chunk * (2 * n) + 2 * j, 2)].reshape(2 * HG, D)
                val = pltpu.bitcast(val, U32)
                if tie is not None:
                    val = val | tie
                view[pl.ds(j, 8, stride=plane), :] = val

            return [functools.partial(step, j) for j in range(n)]

        def relayout(raw, dst, g, rows, plane):
            for ch in range(RCH):
                for step in relayout_steps(raw, dst, g, ch, rows, plane):
                    step(None)

        def head_w(src, h, rows, plane, tie=None, keep=None):
            base = (h // HG) * _gstride(plane) + ((h % HG) // 2) * plane
            ev = src[pl.ds(base, rows // 2), :]
            od = src[pl.ds(base + 4 * plane, rows // 2), :]
            if not isinstance(h, int):
                par = (h % 2).astype(U32)
                w = (((ev >> (16 * par)) & U32(0xFFFF))
                     | ((od << (16 * (1 - par))) & U32(0xFFFF0000)))
            elif h % 2 == 0:
                w = (ev & U32(0xFFFF)) | (od << 16)
            else:
                w = (ev >> 16) | (od & U32(0xFFFF0000))
            if tie is not None:
                w = jnp.concatenate([w[0:8] | tie, w[8:]], axis=0)
            if keep is not None:
                keep[...] = w
            return pltpu.bitcast(w, BF16)

        def q_rows(wq, lo, hi):
            res = []
            for r0 in range(lo, hi, QC):
                rows = slice(r0, r0 + QC)
                res.append(_dot(hn_v[rows, :], wq))
                q_v[rows, :] = (res[-1] * qscale).astype(BF16)
            return res

        def q_head(h):
            return q_rows(head_w(wq_p, h, M, PLQ, keep=wqc_v), 0, PC)

        def q_tail():
            q_rows(pltpu.bitcast(wqc_v[...], BF16), PC, S)

        def k_proj(h):
            wk = head_w(wuk_p, h, Dc, PLK)
            for r in range(S // PC):
                rows = slice(r * PC, (r + 1) * PC)
                k_v[HG - 1, rows, :] = _dot(ckv_v[rows, :], wk).astype(BF16)

        def silu_c():
            cc = c_v[...].astype(F32)
            return jnp.broadcast_to((cc * jax.nn.sigmoid(cc)).astype(BF16), (8, M))

        def mod(i):
            if i < 2:
                return moda_v[0:1, i * M:(i + 1) * M]
            return modb_v[0:1, (i - 2) * M:(i - 1) * M]

        def zeros8():
            return jnp.full((8, LANES), z_s[1], jnp.int32).astype(U32)

        def k_chunk(r, after_head=None, ties=None):
            rows = pl.ds(aligned(r, KC), KC)
            lhs = ckv_v[rows, :]
            for h in range(HG):
                tie = None if ties is None else ties(h)
                res = _dot(lhs, head_w(wuk_p, h, Dc, PLK, tie))
                k_v[h, rows, :] = res.astype(BF16)
                if after_head is not None:
                    after_head(h, res)

        c_k0.wait()
        relayout(wuk_r, wuk_p, 0, Dc, PLK)

        def ka_body(r, carry):
            c_ckv(r).wait()
            k_chunk(r)
            return carry

        jax.lax.fori_loop(0, NK - RCH - 1, ka_body, 0)

        c_ckv(NK - RCH - 1).wait()
        c_c.wait()
        c_moda.wait()
        sc8 = silu_c()

        def mod_tiles(h, res):
            for ct in range(h, 2 * NC, HG):
                cols = slice(ct * LANES, (ct + 1) * LANES)
                moda_v[0:8, cols] = _dot(sc8, wmoda_v[:, cols])

        k_chunk(NK - RCH - 1, after_head=mod_tiles)

        def kb_body(j, carry):
            c_ckv(NK - RCH + j).wait()
            c_x(j).wait()
            c_q0(j).wait()
            zero8 = zeros8()
            lr = XC // HG
            done = []
            for i in range(HG):
                rows = pl.ds(pl.multiple_of(j * XC + i * lr, lr), lr)
                hn = _ln(x_v[rows, :].astype(F32)) * (1.0 + mod(1)) + mod(0)
                hn_v[rows, :] = hn.astype(BF16)
                done.append(hn)
            steps = relayout_steps(wq_r, wq_p, 0, j, M, PLQ)
            per = len(steps) // HG

            def ties(h):
                if h < 2:
                    return None
                return pltpu.bitcast(_fold8(done[h - 2][:, 0:LANES], jnp.maximum), U32) & zero8

            def side(h, res):
                for i, step in enumerate(steps[h * per:(h + 1) * per]):
                    step(pltpu.bitcast(res[i * 8:(i + 1) * 8], U32) & zero8)

            k_chunk(NK - RCH + j, after_head=side, ties=ties)
            return carry

        jax.lax.fori_loop(0, RCH, kb_body, 0)

        c_v0.wait()
        zero8 = zeros8()
        for ch, res in enumerate(q_head(0)):
            for i, step in enumerate(relayout_steps(wuv_r, wuv_p, 0, ch, Dc, PLK)):
                i = i % (QC // 8)
                step(pltpu.bitcast(res[i * 8:(i + 1) * 8], U32) & zero8)

        def attention(h, kh, side):
            key_i = jax.lax.broadcasted_iota(jnp.int32, (TQ, TQ), 0)
            qry_i = jax.lax.broadcasted_iota(jnp.int32, (TQ, TQ), 1)
            causal = key_i <= qry_i
            z_st = z_s[0]
            z_ld = z_s[1]
            zero8 = zeros8()

            mx = {}
            seq = []

            def qk(i):
                qi = q_v[i * TQ:(i + 1) * TQ, :]
                sb = s_v[i % NSB]
                m8 = None
                for t in range(i + 1):
                    tile = _dot_nt(kh[t * TQ:(t + 1) * TQ, :], qi)
                    seq.append(tile[0:8])
                    if t == i:
                        tile = jnp.where(causal, tile, NEG)
                    sb[z_st + t] = tile
                    tm = _fold8(tile, jnp.maximum)
                    m8 = tm if m8 is None else jnp.maximum(m8, tm)
                    if t == i:
                        mx[i] = jnp.max(m8, axis=0, keepdims=True)
                    yield

            parts = []

            def pv(i):
                sb = s_v[i % NSB]
                m8 = jnp.broadcast_to(mx[i], (8, TQ))
                l8 = None
                ot = None
                for t in range(i + 1):
                    tie = pltpu.bitcast(seq[-DIST], U32)
                    if PIN and len(parts) >= PIN:
                        tie = tie | pltpu.bitcast(parts[-PIN], U32)
                    mt = pltpu.bitcast(pltpu.bitcast(m8, U32) | (tie & zero8), F32)
                    tile = sb[z_ld + t].reshape(TQ // 8, 8, TQ)
                    p = jnp.exp2(tile - mt[None]).reshape(TQ, TQ)
                    part = _fold8(p, jnp.add)
                    l8 = part if l8 is None else l8 + part
                    parts.append(l8)
                    o = _dot(vt_v[:, t * TQ:(t + 1) * TQ], p.astype(BF16))
                    seq.append(o[0:8])
                    ot = o if ot is None else ot + o
                    if t == i:
                        l = jnp.sum(l8, axis=0, keepdims=True)
                        ot = ot * (1.0 / l)
                        ctx_v[h, i * TQ:(i + 1) * TQ, :] = ot.T.astype(BF16)
                    yield

            q_tail()
            for i in range(LOOK):
                _run(qk(i))
            vt = _dot_nt(head_w(wuv_p, h, Dc, PLK).T, ckv_v[...])
            vt_v[...] = vt.astype(BF16)
            for ct in range(NQ):
                seq.extend([vt[0:8, ct * TQ:(ct + 1) * TQ]] * (Dc // LANES))
            per = -(-len(side) // NQ)
            assert per <= D // 8
            for j, step in enumerate(side):
                ct, rg = j // per, j % per
                src = vt[rg * 8:(rg + 1) * 8, ct * TQ:(ct + 1) * TQ]
                step(pltpu.bitcast(src, U32) & zero8)
            for i in range(NQ):
                j = i + AHEAD
                if LOOK <= j < NQ:
                    _run(qk(j), pv(i))
                else:
                    _run(pv(i))

        def side_work(h):
            ahead = ((h % HG) >= RCH).astype(jnp.int32)
            gsrc = jnp.minimum(h // HG + ahead, NG - 1)
            ch = h % RCH
            return (relayout_steps(wq_r, wq_p, gsrc, ch, M, PLQ)
                    + relayout_steps(wuk_r, wuk_p, gsrc, ch, Dc, PLK)
                    + relayout_steps(wuv_r, wuv_p, gsrc, ch, Dc, PLK))

        def first_body(h, carry):
            @pl.when(h == RCH)
            def _():
                for d in c_grp[0]:
                    d.wait()

            attention(h, k_v.at[jnp.minimum(h, HG - 1)], side_work(h))
            q_head(jnp.minimum(h + 1, H - 1))
            return carry

        def head_body(h, carry):
            attention(h, k_v.at[HG - 1], side_work(h))
            q_head(h + 1)
            k_proj(h + 1)
            return carry

        def pass_body(p, carry):
            jax.lax.fori_loop(p * (H - 1), HG - 1 + p * (H - HG + 1), first_body, 0)

            @pl.when(p == 0)
            def _():
                for grp in c_grp[1:]:
                    for d in grp:
                        d.wait()
                for d in c_late:
                    d.wait()
                modb_v[...] = _dot(silu_c(), wmodb_v[...])
                jax.lax.fori_loop(HG - 1, H - 1, head_body, 0)

            return carry

        jax.lax.fori_loop(0, 2, pass_body, 0)

        def sub_rows(r):
            out = []
            for j in range(TR // HB):
                r0 = r * TR + j * HB
                if not isinstance(r0, int):
                    r0 = pl.multiple_of(r0, HB)
                out.append(r0)
            return out

        def stage1(r):
            lns = []
            for r0 in sub_rows(r):
                rows = pl.ds(r0, HB)
                ctx = jnp.concatenate([ctx_v[h, rows, :] for h in range(H)], axis=1)
                att = _dot(ctx, wo_v[...])
                x1 = x_v[rows, :].astype(F32) + mod(2) * att
                x1_v[rows, :] = x1
                h2 = _ln(x1) * (1.0 + mod(4)) + mod(3)
                h2_v[rows, :] = h2
                lns.append(_ln(h2).astype(BF16))
            for r0, ln in zip(sub_rows(r), lns):
                u = _gelu(_dot(ln, w1_v[...]))
                for cidx in range(NC):
                    hh_v[cidx, pl.ds(r0 + PAD, HB), :] = u[:, cidx * LANES:(cidx + 1) * LANES]

        shifts = (1, -1, 2, -2)

        def out_cp(r):
            r0 = r * TR if isinstance(r, int) else pl.multiple_of(r * TR, TR)
            rows = pl.ds(r0, TR)
            return pltpu.make_async_copy(o_v.at[rows, :], out_hbm.at[rows, :], osems.at[r])

        def stage2(r):
            lane_i = jax.lax.broadcasted_iota(jnp.int32, (HB, LANES), 1)
            y1s = []
            for r0 in sub_rows(r):
                tiles = []
                for cidx in range(NC):
                    lo, hi = cidx * LANES, (cidx + 1) * LANES
                    g_lo, g_hi = lo // C4, (hi - 1) // C4
                    t = hh_v[cidx, pl.ds(r0 + PAD - shifts[g_hi], HB), :]
                    for g in range(g_hi - 1, g_lo - 1, -1):
                        tg = hh_v[cidx, pl.ds(r0 + PAD - shifts[g], HB), :]
                        t = jnp.where(lane_i < (g + 1) * C4 - lo, tg, t)
                    tiles.append(t)
                hs = _dot(jnp.concatenate(tiles, axis=1).astype(BF16), w2_v[...])
                y1s.append(h2_v[pl.ds(r0, HB), :] + hs)
            gls = [_gelu(_dot_nt(_ln(y1).astype(BF16), w3_v[...])).astype(BF16)
                   for y1 in y1s]
            for r0, y1, gl in zip(sub_rows(r), y1s, gls):
                rows = pl.ds(r0, HB)
                h3 = _dot(gl, w4_v[...])
                o_v[rows, :] = (x1_v[rows, :] + mod(5) * (y1 + h3)).astype(BF16)
            out_cp(r).start()

        zpad = jnp.zeros((PAD, LANES), F32)
        for cidx in range(NC):
            hh_v[cidx, 0:PAD, :] = zpad
            hh_v[cidx, PAD + S:PAD + S + PAD, :] = zpad

        def s1_body(r, carry):
            stage1(r)
            return carry

        def s2_body(r, carry):
            stage2(r)
            return carry

        jax.lax.fori_loop(0, NR, s1_body, 0)
        jax.lax.fori_loop(0, NR, s2_body, 0)
        for r in range(NR):
            out_cp(r).wait()

    hbm_spec = pl.BlockSpec(memory_space=pltpu.HBM)
    V = pltpu.VMEM
    scratch = [
        V((S, M), BF16),
        V((S, Dc), BF16),
        V((NG, M, HG, D), BF16),
        V((NG, Dc, HG, D), BF16),
        V((NG, Dc, HG, D), BF16),
        V((NG * _gstride(PLQ), D), U32),
        V((NG * _gstride(PLK), D), U32),
        V((NG * _gstride(PLK), D), U32),
        V((H * D, M), BF16),
        V((M, M), BF16),
        V((M, M), BF16),
        V((Fh, M), BF16),
        V((Fh, M), BF16),
        V((M, 2 * M), BF16),
        V((M, 4 * M), BF16),
        V((16, 2 * M), F32),
        V((8, 4 * M), F32),
        V((S, M), BF16),
        V((M // 2, D), U32),
        V((S, D), BF16),
        V((HG, S, D), BF16),
        V((D, S), BF16),
        V((NQ, TQ, TQ), F32),
        V((NQ, TQ, TQ), F32),
        V((NQ, TQ, TQ), F32),
        V((NQ, TQ, TQ), F32),
        pltpu.SMEM((2,), jnp.int32),
        V((H, S, D), BF16),
        V((S, M), F32),
        V((S, M), F32),
        V((NC, S + 2 * PAD, LANES), F32),
        V((S, M), BF16),
        V((1, M), BF16),
        pltpu.SemaphoreType.DMA((NSEM,)),
        pltpu.SemaphoreType.DMA((NR,)),
    ]
    out = pl.pallas_call(
        kernel,
        out_shape=jax.ShapeDtypeStruct((S, M), BF16),
        in_specs=[hbm_spec] * 12,
        out_specs=hbm_spec,
        scratch_shapes=scratch,
        compiler_params=pltpu.CompilerParams(vmem_limit_bytes=120 * 1024 * 1024),
        name="adaln_cla_mixer",
    )(x2, ckv2, A_w_q, A_w_uk, A_w_uv, wo2, B_w1, B_w2, B_w3.T, B_w4, c, w_mod)
    return out.reshape(B, S, M)
```

```python
import functools
import math
import os

import jax
import jax.numpy as jnp
import jax.experimental.pallas as pl
import jax.experimental.pallas.tpu as pltpu

BF16 = jnp.bfloat16
F32 = jnp.float32
U32 = jnp.uint32

LANES = 128
TQ = 128
TR = 256
HB = 128
HG = 8
LOOK = 4
AHEAD = int(os.environ.get('AHEAD', 2))
NSB = 4
KC = 256
QC = int(os.environ.get('QC', 128))
MOD0 = int(os.environ.get('MOD0', 2))
LN0 = int(os.environ.get('LN0', 2))
KSUB = int(os.environ.get('KSUB', 1))
PC = 512
DIST = int(os.environ.get('DIST', 12))
PIN = int(os.environ.get('PIN', 0))
PAD = 16
EPS = 1e-5
LOG2E = math.log2(math.e)
NEG = -1000000000.0 * LOG2E

_NT = (((1,), (1,)), ((), ()))


def _ln(x):
    m = jnp.mean(x, axis=-1, keepdims=True)
    xc = x - m
    v = jnp.mean(xc * xc, axis=-1, keepdims=True)
    return xc * jax.lax.rsqrt(v + EPS)


def _gelu(x):
    return jax.nn.gelu(x, approximate=True)


def _dot(a, b):
    return jnp.dot(a, b, preferred_element_type=F32)


def _dot_nt(a, b):
    return jax.lax.dot_general(a, b, _NT, preferred_element_type=F32)


def _fold8(x, op):
    parts = [op(x[j:j + 8], x[j + 8:j + 16]) for j in range(0, x.shape[0], 16)]
    acc = parts[0]
    for p in parts[1:]:
        acc = op(acc, p)
    return acc


def _rows_op(op, x, v8):
    r, m = x.shape
    return op(x.reshape(r // 8, 8, m), v8[None]).reshape(r, m)


def _modulate(x, scale8, shift8):
    r, m = x.shape
    return (x.reshape(r // 8, 8, m) * scale8[None] + shift8[None]).reshape(r, m)


def _gstride(plane):
    return -(-8 * plane // 32) * 32


def _tied(w, tie):
    return jnp.concatenate([w[0:8] | tie, w[8:]], axis=0)


def _run(*gens):
    gens = list(gens)
    while gens:
        for g in list(gens):
            if next(g, gens) is gens:
                gens.remove(g)


@jax.jit
def pallas_adaLN_cond__compressed_kv_cla__mixer_s_mlp__prompt_kernel(
    A_x: jax.Array,
    A_c_kv: jax.Array,
    A_w_q: jax.Array,
    A_w_uk: jax.Array,
    A_w_uv: jax.Array,
    A_w_o: jax.Array,
    B_x: jax.Array,
    B_w1: jax.Array,
    B_w2: jax.Array,
    B_w3: jax.Array,
    B_w4: jax.Array,
    c: jax.Array,
    w_mod: jax.Array,
):
    del B_x
    B, S, M = A_x.shape
    _, Sk, Dc = A_c_kv.shape
    _, H, D = A_w_q.shape
    Fh = B_w3.shape[1]
    assert B == 1 and Sk == S and D == LANES and H % HG == 0 and HG == 8
    assert S % TQ == 0 and S % TR == 0 and S % PC == 0 and TR % HB == 0
    assert M % LANES == 0 and M % 64 == 0 and Dc % 64 == 0
    NG = H // HG
    NQ = S // TQ
    NR = S // TR
    NC = M // LANES
    C4 = M // 4
    PLQ = M // 2 + 1
    PLK = Dc // 2 + 1
    RCH = 4
    NK = S // KC
    XC = S // RCH
    NSEM = NK + 2 * RCH + 6
    assert NK > RCH + 1 and LOOK * TQ <= PC and PC // QC == RCH
    qscale = float(D) ** -0.5 * LOG2E

    x2 = A_x.reshape(S, M)
    ckv2 = A_c_kv.reshape(S, Dc)
    wo2 = A_w_o.reshape(H * D, M)

    def kernel(x_hbm, ckv_hbm, wq_hbm, wuk_hbm, wuv_hbm, wo_hbm, w1_hbm, w2_hbm,
               w3_hbm, w4_hbm, c_hbm, wmod_hbm, out_hbm,
               x_v, ckv_v, wq_r, wuk_r, wuv_r, wq_p, wuk_p, wuv_p, wo_v, w1_v,
               w2_v, w3_v, w4_v, wmoda_v, wmodb_v, moda_v, modb_v, scb_v, hn_v, wqc_v, wk0_v, q_v, k_v,
               vt_v, s0, s1, s2, s3, z_s, ctx_v, x1_v, h2_v, hh_v, o_v, c_v,
               sems, osems):

        s_v = (s0, s1, s2, s3)
        z_s[0] = 0
        z_s[1] = 0

        def aligned(i, n):
            return i * n if isinstance(i, int) else pl.multiple_of(i * n, n)

        def cp(src, dst, i):
            return pltpu.make_async_copy(src, dst, sems.at[i])

        def c_ckv(r):
            rows = pl.ds(aligned(r, KC), KC)
            return cp(ckv_hbm.at[rows, :], ckv_v.at[rows, :], r)

        def c_x(j):
            rows = pl.ds(aligned(j, XC), XC)
            return cp(x_hbm.at[rows, :], x_v.at[rows, :], NK + j)

        def c_q0(j):
            rows = pl.ds(aligned(j, M // RCH), M // RCH)
            return cp(wq_hbm.at[rows, pl.ds(0, HG), :], wq_r.at[0, rows], NK + RCH + j)

        nsem = [NK + 2 * RCH]

        def cp_next(src, dst):
            nsem[0] += 1
            return cp(src, dst, nsem[0] - 1)

        def gcp(src, dst, g):
            return cp_next(src.at[:, pl.ds(g * HG, HG), :], dst.at[g])

        c_k0 = gcp(wuk_hbm, wuk_r, 0)
        c_v0 = gcp(wuv_hbm, wuv_r, 0)
        c_k1 = gcp(wuk_hbm, wuk_r, 1)
        c_c = cp_next(c_hbm, c_v)
        c_moda = cp_next(wmod_hbm.at[:, pl.ds(0, 2 * M)], wmoda_v)
        assert nsem[0] == NSEM - 1
        c_late = []
        for g in range(1, NG):
            for src, dst, gg in ((wq_hbm, wq_r, g), (wuv_hbm, wuv_r, g), (wuk_hbm, wuk_r, g + 1)):
                if gg < NG:
                    c_late.append(cp(src.at[:, pl.ds(gg * HG, HG), :], dst.at[gg], NSEM - 1))
        for ct in range(4 * NC):
            c_late.append(cp(wmod_hbm.at[:, pl.ds(2 * M + ct * LANES, LANES)],
                             wmodb_v.at[ct], NSEM - 1))
        for src, dst in ((wo_hbm, wo_v), (w1_hbm, w1_v), (w2_hbm, w2_v),
                         (w3_hbm, w3_v), (w4_hbm, w4_v)):
            c_late.append(cp(src, dst, NSEM - 1))
        order = [c_c, c_k0] + [c_ckv(r) for r in range(NK - RCH)] + [c_moda]
        for j in range(RCH):
            order += [c_ckv(NK - RCH + j), c_x(j), c_q0(j)]
        order += [c_v0, c_k1] + c_late
        for d in order:
            d.start()

        def relayout_steps(raw, dst, g, chunk, rows, plane):
            n = rows // RCH // 2
            base = g * _gstride(plane) + chunk * n
            if not isinstance(base, int):
                base = pl.multiple_of(base, 8)
            view = dst.at[pl.ds(base, 7 * plane + n), :]

            def step(j, tie):
                val = raw[g, pl.ds(chunk * (2 * n) + 2 * j, 2)].reshape(2 * HG, D)
                val = pltpu.bitcast(val, U32)
                if tie is not None:
                    val = val | tie
                view[pl.ds(j, 8, stride=plane), :] = val

            return [functools.partial(step, j) for j in range(n)]

        def relayout(raw, dst, g, rows, plane):
            for ch in range(RCH):
                for step in relayout_steps(raw, dst, g, ch, rows, plane):
                    step(None)

        def head_w32(src, h, rows, plane):
            base = (h // HG) * _gstride(plane) + ((h % HG) // 2) * plane
            ev = src[pl.ds(base, rows // 2), :]
            od = src[pl.ds(base + 4 * plane, rows // 2), :]
            if not isinstance(h, int):
                par = (h % 2).astype(U32)
                w = (((ev >> (16 * par)) & U32(0xFFFF))
                     | ((od << (16 * (1 - par))) & U32(0xFFFF0000)))
            elif h % 2 == 0:
                w = (ev & U32(0xFFFF)) | (od << 16)
            else:
                w = (ev >> 16) | (od & U32(0xFFFF0000))
            return w

        def head_w(src, h, rows, plane):
            return pltpu.bitcast(head_w32(src, h, rows, plane), BF16)

        def q_rows(wq, lo, hi, ties=()):
            res = []
            for r0 in range(lo, hi, QC):
                rows = slice(r0, r0 + QC)
                w = _tied(wq, ties[len(res)]) if len(res) in ties else wq
                res.append(_dot(hn_v[rows, :], pltpu.bitcast(w, BF16)))
                q_v[rows, :] = (res[-1] * qscale).astype(BF16)
            return res

        def q_head(h):
            wq = head_w32(wq_p, h, M, PLQ)
            wqc_v[...] = wq
            return q_rows(wq, 0, PC)

        def q_tail(ties=()):
            q_rows(wqc_v[...], PC, S, ties)

        def k_proj(h, kh):
            wk = head_w(wuk_p, h, Dc, PLK)
            for r in range(S // PC):
                rows = slice(r * PC, (r + 1) * PC)
                kh[rows, :] = _dot(ckv_v[rows, :], wk).astype(BF16)

        def mod_tile(w):
            acc = _fold8(w.astype(F32) * scb_v[...], jnp.add)
            return jnp.broadcast_to(jnp.sum(acc, axis=0, keepdims=True), (8, LANES))

        def mod(i):
            if i < 2:
                return moda_v[0:8, i * M:(i + 1) * M]
            return jnp.concatenate(
                [modb_v[(i - 2) * NC + ct] for ct in range(NC)], axis=1)

        def zeros8():
            return jnp.full((8, LANES), z_s[1], jnp.int32).astype(U32)

        def k_chunk(r, nsub=1, ties=(), after=None, unpack=False):
            n = KC // nsub
            lhs = ckv_v[pl.ds(aligned(r, KC), KC), :]
            for h in range(HG):
                if unpack:
                    w32 = head_w32(wuk_p, h, Dc, PLK)
                    wk0_v[h] = w32
                else:
                    w32 = wk0_v[h]
                for j in range(nsub):
                    i = h * nsub + j
                    rows = pl.ds(aligned(r * nsub + j, n), n)
                    w = _tied(w32, ties[i]) if i in ties else w32
                    res = _dot(lhs[j * n:(j + 1) * n], pltpu.bitcast(w, BF16))
                    k_v[h, rows, :] = res.astype(BF16)
                    if after is not None:
                        after(i, res)

        c_c.wait()
        cc = c_v[...].astype(F32)
        sc = (cc * jax.nn.sigmoid(cc)).astype(BF16).astype(F32)
        scb_v[...] = jnp.broadcast_to(sc, (LANES, M)).T
        zpad = jnp.zeros((PAD, LANES), F32)
        for cidx in range(NC):
            hh_v[cidx, 0:PAD, :] = zpad
            hh_v[cidx, PAD + S:PAD + S + PAD, :] = zpad
        c_k0.wait()
        relayout(wuk_r, wuk_p, 0, Dc, PLK)

        def ka_body(r, carry):
            c_ckv(r).wait()
            k_chunk(r, unpack=True)
            return carry

        jax.lax.fori_loop(0, NK - RCH - 1, ka_body, 0)

        c_ckv(NK - RCH - 1).wait()
        c_moda.wait()
        zero8 = zeros8()
        ties = {}
        for ct in range(2 * NC):
            cols = slice(ct * LANES, (ct + 1) * LANES)
            tile = mod_tile(wmoda_v[:, cols])
            moda_v[0:8, cols] = tile
            ties[MOD0 + (ct * (2 * HG - MOD0)) // (2 * NC)] = pltpu.bitcast(tile, U32) & zero8
        k_chunk(NK - RCH - 1, 2, ties)

        def kb_body(j, carry):
            c_ckv(NK - RCH + j).wait()
            c_x(j).wait()
            c_q0(j).wait()
            zero8 = zeros8()
            nstep = KSUB * HG
            lr = XC // nstep
            ties = {}
            scale, shift = 1.0 + mod(1), mod(0)
            for i in range(nstep):
                rows = pl.ds(pl.multiple_of(j * XC + i * lr, lr), lr)
                hn = _modulate(_ln(x_v[rows, :].astype(F32)), scale, shift)
                hn_v[rows, :] = hn.astype(BF16)
                ties[i + LN0] = pltpu.bitcast(_fold8(hn[:, 0:LANES], jnp.maximum), U32) & zero8
            steps = relayout_steps(wq_r, wq_p, 0, j, M, PLQ)
            per = len(steps) // nstep

            def side(i, res):
                for k, step in enumerate(steps[i * per:(i + 1) * per]):
                    step(pltpu.bitcast(res[k * 8:(k + 1) * 8], U32) & zero8)

            k_chunk(NK - RCH + j, KSUB, ties, side)
            return carry

        jax.lax.fori_loop(0, RCH, kb_body, 0)

        c_v0.wait()
        c_k1.wait()
        zero8 = zeros8()
        for ch, res in enumerate(q_head(0)):
            for i, step in enumerate(relayout_steps(wuv_r, wuv_p, 0, ch, Dc, PLK)
                                     + relayout_steps(wuk_r, wuk_p, 1, ch, Dc, PLK)):
                i = i % (QC // 8)
                step(pltpu.bitcast(res[i * 8:(i + 1) * 8], U32) & zero8)

        def attention(h, kh, side):
            key_i = jax.lax.broadcasted_iota(jnp.int32, (TQ, TQ), 0)
            qry_i = jax.lax.broadcasted_iota(jnp.int32, (TQ, TQ), 1)
            causal = key_i <= qry_i
            z_st = z_s[0]
            z_ld = z_s[1]
            zero8 = zeros8()

            mx = {}
            seq = []

            def qk(i):
                qi = q_v[i * TQ:(i + 1) * TQ, :]
                sb = s_v[i % NSB]
                m8 = None
                for t in range(i + 1):
                    tile = _dot_nt(kh[t * TQ:(t + 1) * TQ, :], qi)
                    seq.append(tile[0:8])
                    if t == i:
                        tile = jnp.where(causal, tile, NEG)
                    sb[z_st + t] = tile
                    tm = _fold8(tile, jnp.maximum)
                    m8 = tm if m8 is None else jnp.maximum(m8, tm)
                    if t == i:
                        mx[i] = jnp.max(m8, axis=0, keepdims=True)
                    yield

            parts = []

            def pv(i):
                sb = s_v[i % NSB]
                m8 = jnp.broadcast_to(mx[i], (8, TQ))
                l8 = None
                ot = None
                for t in range(i + 1):
                    tie = pltpu.bitcast(seq[-DIST], U32)
                    if PIN and len(parts) >= PIN:
                        tie = tie | pltpu.bitcast(parts[-PIN], U32)
                    mt = pltpu.bitcast(pltpu.bitcast(m8, U32) | (tie & zero8), F32)
                    tile = sb[z_ld + t].reshape(TQ // 8, 8, TQ)
                    p = jnp.exp2(tile - mt[None]).reshape(TQ, TQ)
                    part = _fold8(p, jnp.add)
                    l8 = part if l8 is None else l8 + part
                    parts.append(l8)
                    o = _dot(vt_v[:, t * TQ:(t + 1) * TQ], p.astype(BF16))
                    seq.append(o[0:8])
                    ot = o if ot is None else ot + o
                    if t == i:
                        l = jnp.sum(l8, axis=0, keepdims=True)
                        ot = ot * (1.0 / l)
                        ctx_v[h, i * TQ:(i + 1) * TQ, :] = ot.T.astype(BF16)
                    yield

            for i in range(LOOK):
                _run(qk(i))
            vt = _dot_nt(head_w(wuv_p, h, Dc, PLK).T, ckv_v[...])
            vt_v[...] = vt.astype(BF16)
            for ct in range(NQ):
                seq.extend([vt[0:8, ct * TQ:(ct + 1) * TQ]] * (Dc // LANES))
            per = max(1, -(-len(side) // NQ))
            assert per <= D // 8
            for j, step in enumerate(side):
                ct, rg = j // per, j % per
                src = vt[rg * 8:(rg + 1) * 8, ct * TQ:(ct + 1) * TQ]
                step(pltpu.bitcast(src, U32) & zero8)
            for i in range(NQ):
                j = i + AHEAD
                if LOOK <= j < NQ:
                    _run(qk(j), pv(i))
                else:
                    _run(pv(i))

        def side_work(h):
            g = h // HG + ((h % HG) >= RCH).astype(jnp.int32)
            ch = h % RCH
            return (relayout_steps(wq_r, wq_p, g, ch, M, PLQ)
                    + relayout_steps(wuk_r, wuk_p, jnp.minimum(g + 1, NG - 1), ch, Dc, PLK)
                    + relayout_steps(wuv_r, wuv_p, g, ch, Dc, PLK))

        def head_body(h, carry):
            @pl.when(h == RCH)
            def _():
                for d in c_late:
                    d.wait()

            kh = k_v.at[h % HG]
            q_tail()
            attention(h, kh, side_work(h))
            q_head(h + 1)
            k_proj(h + HG, kh)
            return carry

        jax.lax.fori_loop(0, H - HG, head_body, 0)

        def last_body(h, carry):
            per = -(-4 * NC // HG)
            zero8 = zeros8()
            ties = {}
            for i in range(per):
                ct = jnp.minimum((h - (H - HG)) * per + i, 4 * NC - 1)
                tile = mod_tile(wmodb_v[ct])
                modb_v[ct] = tile
                ties[3 * i + 3] = pltpu.bitcast(tile, U32) & zero8
            q_tail(ties)
            attention(h, k_v.at[h % HG], ())
            q_head(jnp.minimum(h + 1, H - 1))
            return carry

        jax.lax.fori_loop(H - HG, H, last_body, 0)

        def sub_rows(r):
            out = []
            for j in range(TR // HB):
                r0 = r * TR + j * HB
                if not isinstance(r0, int):
                    r0 = pl.multiple_of(r0, HB)
                out.append(r0)
            return out

        def stage1(r):
            lns = []
            for r0 in sub_rows(r):
                rows = pl.ds(r0, HB)
                ctx = jnp.concatenate([ctx_v[h, rows, :] for h in range(H)], axis=1)
                att = _dot(ctx, wo_v[...])
                x1 = x_v[rows, :].astype(F32) + _rows_op(jnp.multiply, att, mod(2))
                x1_v[rows, :] = x1
                h2 = _modulate(_ln(x1), 1.0 + mod(4), mod(3))
                h2_v[rows, :] = h2
                lns.append(_ln(h2).astype(BF16))
            for r0, ln in zip(sub_rows(r), lns):
                u = _gelu(_dot(ln, w1_v[...]))
                for cidx in range(NC):
                    hh_v[cidx, pl.ds(r0 + PAD, HB), :] = u[:, cidx * LANES:(cidx + 1) * LANES]

        shifts = (1, -1, 2, -2)

        def out_cp(r):
            r0 = r * TR if isinstance(r, int) else pl.multiple_of(r * TR, TR)
            rows = pl.ds(r0, TR)
            return pltpu.make_async_copy(o_v.at[rows, :], out_hbm.at[rows, :], osems.at[r])

        def stage2(r):
            lane_i = jax.lax.broadcasted_iota(jnp.int32, (HB, LANES), 1)
            y1s = []
            for r0 in sub_rows(r):
                tiles = []
                for cidx in range(NC):
                    lo, hi = cidx * LANES, (cidx + 1) * LANES
                    g_lo, g_hi = lo // C4, (hi - 1) // C4
                    t = hh_v[cidx, pl.ds(r0 + PAD - shifts[g_hi], HB), :]
                    for g in range(g_hi - 1, g_lo - 1, -1):
                        tg = hh_v[cidx, pl.ds(r0 + PAD - shifts[g], HB), :]
                        t = jnp.where(lane_i < (g + 1) * C4 - lo, tg, t)
                    tiles.append(t)
                hs = _dot(jnp.concatenate(tiles, axis=1).astype(BF16), w2_v[...])
                y1s.append(h2_v[pl.ds(r0, HB), :] + hs)
            gls = [_gelu(_dot_nt(_ln(y1).astype(BF16), w3_v[...])).astype(BF16)
                   for y1 in y1s]
            for r0, y1, gl in zip(sub_rows(r), y1s, gls):
                rows = pl.ds(r0, HB)
                h3 = _dot(gl, w4_v[...])
                o_v[rows, :] = (x1_v[rows, :]
                                + _rows_op(jnp.multiply, y1 + h3, mod(5))).astype(BF16)
            out_cp(r).start()

        def s1_body(r, carry):
            stage1(r)
            return carry

        def s2_body(r, carry):
            stage2(r)
            return carry

        jax.lax.fori_loop(0, NR, s1_body, 0)
        jax.lax.fori_loop(0, NR, s2_body, 0)
        for r in range(NR):
            out_cp(r).wait()

    hbm_spec = pl.BlockSpec(memory_space=pltpu.HBM)
    V = pltpu.VMEM
    scratch = [
        V((S, M), BF16),
        V((S, Dc), BF16),
        V((NG, M, HG, D), BF16),
        V((NG, Dc, HG, D), BF16),
        V((NG, Dc, HG, D), BF16),
        V((NG * _gstride(PLQ), D), U32),
        V((NG * _gstride(PLK), D), U32),
        V((NG * _gstride(PLK), D), U32),
        V((H * D, M), BF16),
        V((M, M), BF16),
        V((M, M), BF16),
        V((Fh, M), BF16),
        V((Fh, M), BF16),
        V((M, 2 * M), BF16),
        V((4 * NC, M, LANES), BF16),
        V((16, 2 * M), F32),
        V((4 * NC, 8, LANES), F32),
        V((M, LANES), F32),
        V((S, M), BF16),
        V((M // 2, D), U32),
        V((HG, Dc // 2, D), U32),
        V((S, D), BF16),
        V((HG, S, D), BF16),
        V((D, S), BF16),
        V((NQ, TQ, TQ), F32),
        V((NQ, TQ, TQ), F32),
        V((NQ, TQ, TQ), F32),
        V((NQ, TQ, TQ), F32),
        pltpu.SMEM((2,), jnp.int32),
        V((H, S, D), BF16),
        V((S, M), F32),
        V((S, M), F32),
        V((NC, S + 2 * PAD, LANES), F32),
        V((S, M), BF16),
        V((1, M), BF16),
        pltpu.SemaphoreType.DMA((NSEM,)),
        pltpu.SemaphoreType.DMA((NR,)),
    ]
    out = pl.pallas_call(
        kernel,
        out_shape=jax.ShapeDtypeStruct((S, M), BF16),
        in_specs=[hbm_spec] * 12,
        out_specs=hbm_spec,
        scratch_shapes=scratch,
        compiler_params=pltpu.CompilerParams(vmem_limit_bytes=120 * 1024 * 1024),
        name="adaln_cla_mixer",
    )(x2, ckv2, A_w_q, A_w_uk, A_w_uv, wo2, B_w1, B_w2, B_w3.T, B_w4, c, w_mod)
    return out.reshape(B, S, M)
```

```python
import functools
import math
import os

import jax
import jax.numpy as jnp
import jax.experimental.pallas as pl
import jax.experimental.pallas.tpu as pltpu

BF16 = jnp.bfloat16
F32 = jnp.float32
U32 = jnp.uint32

LANES = 128
TQ = 128
TR = 256
HB = 128
HG = 8
LOOK = 4
AHEAD = int(os.environ.get('AHEAD', 2))
NSB = 4
KC = 256
QC = int(os.environ.get('QC', 128))
MOD0 = int(os.environ.get('MOD0', 2))
LN0 = int(os.environ.get('LN0', 2))
KSUB = int(os.environ.get('KSUB', 1))
PC = 512
DIST = int(os.environ.get('DIST', 12))
PIN = int(os.environ.get('PIN', 0))
PAD = 16
EPS = 1e-5
LOG2E = math.log2(math.e)
NEG = -1000000000.0 * LOG2E

_NT = (((1,), (1,)), ((), ()))


def _ln(x):
    m = jnp.mean(x, axis=-1, keepdims=True)
    xc = x - m
    v = jnp.mean(xc * xc, axis=-1, keepdims=True)
    return xc * jax.lax.rsqrt(v + EPS)


def _gelu(x):
    return jax.nn.gelu(x, approximate=True)


def _dot(a, b):
    return jnp.dot(a, b, preferred_element_type=F32)


def _dot_nt(a, b):
    return jax.lax.dot_general(a, b, _NT, preferred_element_type=F32)


def _fold8(x, op):
    parts = [op(x[j:j + 8], x[j + 8:j + 16]) for j in range(0, x.shape[0], 16)]
    acc = parts[0]
    for p in parts[1:]:
        acc = op(acc, p)
    return acc


def _rows_op(op, x, v8):
    r, m = x.shape
    return op(x.reshape(r // 8, 8, m), v8[None]).reshape(r, m)


def _modulate(x, scale8, shift8):
    r, m = x.shape
    return (x.reshape(r // 8, 8, m) * scale8[None] + shift8[None]).reshape(r, m)


def _pack(x):
    return pltpu.bitcast(x.astype(BF16), U32)


def _unpack(w):
    return pltpu.bitcast(w, BF16)


def _gstride(plane):
    return -(-8 * plane // 32) * 32


def _tied(w, tie):
    return jnp.concatenate([w[0:8] | tie, w[8:]], axis=0)


def _run(*gens):
    gens = list(gens)
    while gens:
        for g in list(gens):
            if next(g, gens) is gens:
                gens.remove(g)


@jax.jit
def pallas_adaLN_cond__compressed_kv_cla__mixer_s_mlp__prompt_kernel(
    A_x: jax.Array,
    A_c_kv: jax.Array,
    A_w_q: jax.Array,
    A_w_uk: jax.Array,
    A_w_uv: jax.Array,
    A_w_o: jax.Array,
    B_x: jax.Array,
    B_w1: jax.Array,
    B_w2: jax.Array,
    B_w3: jax.Array,
    B_w4: jax.Array,
    c: jax.Array,
    w_mod: jax.Array,
):
    del B_x
    B, S, M = A_x.shape
    _, Sk, Dc = A_c_kv.shape
    _, H, D = A_w_q.shape
    Fh = B_w3.shape[1]
    assert B == 1 and Sk == S and D == LANES and H % HG == 0 and HG == 8
    assert S % TQ == 0 and S % TR == 0 and S % PC == 0 and TR % HB == 0
    assert M % LANES == 0 and M % 64 == 0 and Dc % 64 == 0
    NG = H // HG
    NQ = S // TQ
    NR = S // TR
    NC = M // LANES
    C4 = M // 4
    PLQ = M // 2 + 1
    PLK = Dc // 2 + 1
    RCH = 4
    NK = S // KC
    XC = S // RCH
    NSEM = NK + 2 * RCH + 6
    assert NK > RCH + 1 and LOOK * TQ <= PC and PC // QC == RCH
    qscale = float(D) ** -0.5 * LOG2E

    x2 = A_x.reshape(S, M)
    ckv2 = A_c_kv.reshape(S, Dc)
    wo2 = A_w_o.reshape(H * D, M)

    def kernel(x_hbm, ckv_hbm, wq_hbm, wuk_hbm, wuv_hbm, wo_hbm, w1_hbm, w2_hbm,
               w3_hbm, w4_hbm, c_hbm, wmod_hbm, out_hbm,
               x_v, ckv_v, wq_r, wuk_r, wuv_r, wq_p, wuk_p, wuv_p, wo_v, w1_v,
               w2_v, w3_v, w4_v, wmoda_v, wmodb_v, moda_v, modb_v, scb_v, hn_v, wqc_v, wk0_v, q_v, k_v,
               vt_v, s0, s1, s2, s3, z_s, ctx_v, x1_v, h2_v, hh_v, o_v, c_v,
               sems, osems):

        s_v = (s0, s1, s2, s3)
        z_s[0] = 0
        z_s[1] = 0

        def aligned(i, n):
            return i * n if isinstance(i, int) else pl.multiple_of(i * n, n)

        def cp(src, dst, i):
            return pltpu.make_async_copy(src, dst, sems.at[i])

        def c_ckv(r):
            rows = pl.ds(aligned(r, KC), KC)
            return cp(ckv_hbm.at[rows, :], ckv_v.at[rows, :], r)

        def c_x(j):
            rows = pl.ds(aligned(j, XC), XC)
            return cp(x_hbm.at[rows, :], x_v.at[rows, :], NK + j)

        def c_q0(j):
            rows = pl.ds(aligned(j, M // RCH), M // RCH)
            return cp(wq_hbm.at[rows, pl.ds(0, HG), :], wq_r.at[0, rows], NK + RCH + j)

        nsem = [NK + 2 * RCH]

        def cp_next(src, dst):
            nsem[0] += 1
            return cp(src, dst, nsem[0] - 1)

        def gcp(src, dst, g):
            return cp_next(src.at[:, pl.ds(g * HG, HG), :], dst.at[g])

        c_k0 = gcp(wuk_hbm, wuk_r, 0)
        c_v0 = gcp(wuv_hbm, wuv_r, 0)
        c_k1 = gcp(wuk_hbm, wuk_r, 1)
        c_c = cp_next(c_hbm, c_v)
        c_moda = cp_next(wmod_hbm.at[:, pl.ds(0, 2 * M)], wmoda_v)
        assert nsem[0] == NSEM - 1
        c_late = []
        for g in range(1, NG):
            for src, dst, gg in ((wq_hbm, wq_r, g), (wuv_hbm, wuv_r, g), (wuk_hbm, wuk_r, g + 1)):
                if gg < NG:
                    c_late.append(cp(src.at[:, pl.ds(gg * HG, HG), :], dst.at[gg], NSEM - 1))
        for ct in range(4 * NC):
            c_late.append(cp(wmod_hbm.at[:, pl.ds(2 * M + ct * LANES, LANES)],
                             wmodb_v.at[ct], NSEM - 1))
        for src, dst in ((wo_hbm, wo_v), (w1_hbm, w1_v), (w2_hbm, w2_v),
                         (w3_hbm, w3_v), (w4_hbm, w4_v)):
            c_late.append(cp(src, dst, NSEM - 1))
        order = [c_c, c_k0] + [c_ckv(r) for r in range(NK - RCH)] + [c_moda]
        for j in range(RCH):
            order += [c_ckv(NK - RCH + j), c_x(j), c_q0(j)]
        order += [c_v0, c_k1] + c_late
        for d in order:
            d.start()

        def relayout_steps(raw, dst, g, chunk, rows, plane):
            n = rows // RCH // 2
            base = g * _gstride(plane) + chunk * n
            if not isinstance(base, int):
                base = pl.multiple_of(base, 8)
            view = dst.at[pl.ds(base, 7 * plane + n), :]

            def step(j, tie):
                val = raw[g, pl.ds(chunk * (2 * n) + 2 * j, 2)].reshape(2 * HG, D)
                val = pltpu.bitcast(val, U32)
                if tie is not None:
                    val = val | tie
                view[pl.ds(j, 8, stride=plane), :] = val

            return [functools.partial(step, j) for j in range(n)]

        def relayout(raw, dst, g, rows, plane):
            for ch in range(RCH):
                for step in relayout_steps(raw, dst, g, ch, rows, plane):
                    step(None)

        def head_w32(src, h, rows, plane):
            base = (h // HG) * _gstride(plane) + ((h % HG) // 2) * plane
            ev = src[pl.ds(base, rows // 2), :]
            od = src[pl.ds(base + 4 * plane, rows // 2), :]
            if not isinstance(h, int):
                par = (h % 2).astype(U32)
                w = (((ev >> (16 * par)) & U32(0xFFFF))
                     | ((od << (16 * (1 - par))) & U32(0xFFFF0000)))
            elif h % 2 == 0:
                w = (ev & U32(0xFFFF)) | (od << 16)
            else:
                w = (ev >> 16) | (od & U32(0xFFFF0000))
            return w

        def head_w(src, h, rows, plane):
            return pltpu.bitcast(head_w32(src, h, rows, plane), BF16)

        def q_rows(wq, lo, hi, ties=()):
            res = []
            for r0 in range(lo, hi, QC):
                rows = slice(r0, r0 + QC)
                w = _tied(wq, ties[len(res)]) if len(res) in ties else wq
                res.append(_dot(hn_v[rows, :], pltpu.bitcast(w, BF16)))
                q_v[rows, :] = (res[-1] * qscale).astype(BF16)
            return res

        def q_head(h):
            wq = head_w32(wq_p, h, M, PLQ)
            wqc_v[...] = wq
            return q_rows(wq, 0, PC)

        def q_mid(ties=()):
            q_rows(wqc_v[...], PC, S - PC, ties)

        def q_tail():
            return q_rows(wqc_v[...], S - PC, S)

        def k_proj(h, kh):
            wk = head_w(wuk_p, h, Dc, PLK)
            for r in range(S // PC):
                rows = slice(r * PC, (r + 1) * PC)
                kh[r * PC // 2:(r + 1) * PC // 2, :] = _pack(_dot(ckv_v[rows, :], wk))

        def mod_tile(w):
            acc = _fold8(w.astype(F32) * scb_v[...], jnp.add)
            return jnp.broadcast_to(jnp.sum(acc, axis=0, keepdims=True), (8, LANES))

        def mod(i):
            if i < 2:
                return moda_v[0:8, i * M:(i + 1) * M]
            return jnp.concatenate(
                [modb_v[(i - 2) * NC + ct] for ct in range(NC)], axis=1)

        def zeros8():
            return jnp.full((8, LANES), z_s[1], jnp.int32).astype(U32)

        def k_chunk(r, nsub=1, ties=(), after=None, unpack=False):
            n = KC // nsub
            lhs = ckv_v[pl.ds(aligned(r, KC), KC), :]
            for h in range(HG):
                if unpack:
                    w32 = head_w32(wuk_p, h, Dc, PLK)
                    wk0_v[h] = w32
                else:
                    w32 = wk0_v[h]
                for j in range(nsub):
                    i = h * nsub + j
                    rows = pl.ds(aligned(r * nsub + j, n // 2), n // 2)
                    w = _tied(w32, ties[i]) if i in ties else w32
                    res = _dot(lhs[j * n:(j + 1) * n], pltpu.bitcast(w, BF16))
                    k_v[h, rows, :] = _pack(res)
                    if after is not None:
                        after(i, res)

        c_c.wait()
        cc = c_v[...].astype(F32)
        sc = (cc * jax.nn.sigmoid(cc)).astype(BF16).astype(F32)
        scb_v[...] = jnp.broadcast_to(sc, (LANES, M)).T
        zpad = jnp.zeros((PAD, LANES), F32)
        for cidx in range(NC):
            hh_v[cidx, 0:PAD, :] = zpad
            hh_v[cidx, PAD + S:PAD + S + PAD, :] = zpad
        c_k0.wait()
        relayout(wuk_r, wuk_p, 0, Dc, PLK)

        def ka_body(r, carry):
            c_ckv(r).wait()
            k_chunk(r, unpack=True)
            return carry

        jax.lax.fori_loop(0, NK - RCH - 1, ka_body, 0)

        c_ckv(NK - RCH - 1).wait()
        c_moda.wait()
        zero8 = zeros8()
        ties = {}
        for ct in range(2 * NC):
            cols = slice(ct * LANES, (ct + 1) * LANES)
            tile = mod_tile(wmoda_v[:, cols])
            moda_v[0:8, cols] = tile
            ties[MOD0 + (ct * (2 * HG - MOD0)) // (2 * NC)] = pltpu.bitcast(tile, U32) & zero8
        k_chunk(NK - RCH - 1, 2, ties)

        def kb_body(j, carry):
            c_ckv(NK - RCH + j).wait()
            c_x(j).wait()
            c_q0(j).wait()
            zero8 = zeros8()
            nstep = KSUB * HG
            lr = XC // nstep
            ties = {}
            scale, shift = 1.0 + mod(1), mod(0)
            for i in range(nstep):
                rows = pl.ds(pl.multiple_of(j * XC + i * lr, lr), lr)
                hn = _modulate(_ln(x_v[rows, :].astype(F32)), scale, shift)
                hn_v[rows, :] = hn.astype(BF16)
                ties[i + LN0] = pltpu.bitcast(_fold8(hn[:, 0:LANES], jnp.maximum), U32) & zero8
            steps = relayout_steps(wq_r, wq_p, 0, j, M, PLQ)
            per = len(steps) // nstep

            def side(i, res):
                for k, step in enumerate(steps[i * per:(i + 1) * per]):
                    step(pltpu.bitcast(res[k * 8:(k + 1) * 8], U32) & zero8)

            k_chunk(NK - RCH + j, KSUB, ties, side)
            return carry

        jax.lax.fori_loop(0, RCH, kb_body, 0)

        c_v0.wait()
        c_k1.wait()
        zero8 = zeros8()
        for ch, res in enumerate(q_head(0)):
            for i, step in enumerate(relayout_steps(wuv_r, wuv_p, 0, ch, Dc, PLK)
                                     + relayout_steps(wuk_r, wuk_p, 1, ch, Dc, PLK)):
                i = i % (QC // 8)
                step(pltpu.bitcast(res[i * 8:(i + 1) * 8], U32) & zero8)

        def attention(h, kh, side):
            key_i = jax.lax.broadcasted_iota(jnp.int32, (TQ, TQ), 0)
            qry_i = jax.lax.broadcasted_iota(jnp.int32, (TQ, TQ), 1)
            causal = key_i <= qry_i
            z_st = z_s[0]
            z_ld = z_s[1]
            zero8 = zeros8()

            mx = {}
            seq = []

            def qk(i):
                qi = q_v[i * TQ:(i + 1) * TQ, :]
                sb = s_v[i % NSB]
                m8 = None
                for t in range(i + 1):
                    tile = _dot_nt(_unpack(kh[t * TQ // 2:(t + 1) * TQ // 2, :]), qi)
                    seq.append(tile[0:8])
                    if t == i:
                        tile = jnp.where(causal, tile, NEG)
                    sb[z_st + t] = tile
                    tm = _fold8(tile, jnp.maximum)
                    m8 = tm if m8 is None else jnp.maximum(m8, tm)
                    if t == i:
                        mx[i] = jnp.max(m8, axis=0, keepdims=True)
                    yield

            parts = []

            def pv(i):
                sb = s_v[i % NSB]
                m8 = jnp.broadcast_to(mx[i], (8, TQ))
                l8 = None
                ot = None
                for t in range(i + 1):
                    tie = pltpu.bitcast(seq[-DIST], U32)
                    if PIN and len(parts) >= PIN:
                        tie = tie | pltpu.bitcast(parts[-PIN], U32)
                    mt = pltpu.bitcast(pltpu.bitcast(m8, U32) | (tie & zero8), F32)
                    tile = sb[z_ld + t].reshape(TQ // 8, 8, TQ)
                    p = jnp.exp2(tile - mt[None]).reshape(TQ, TQ)
                    part = _fold8(p, jnp.add)
                    l8 = part if l8 is None else l8 + part
                    parts.append(l8)
                    o = _dot(_unpack(vt_v[z_ld, :, t * TQ:(t + 1) * TQ]), p.astype(BF16))
                    seq.append(o[0:8])
                    ot = o if ot is None else ot + o
                    if t == i:
                        l = jnp.sum(l8, axis=0, keepdims=True)
                        ot = ot * (1.0 / l)
                        ctx_v[h, i * TQ:(i + 1) * TQ, :] = ot.T.astype(BF16)
                    yield

            for i in range(LOOK):
                _run(qk(i))
            vt = _dot_nt(head_w(wuv_p, h, Dc, PLK).T, ckv_v[...])
            vt_v[z_st] = _pack(vt)
            prev = vt[0:8, S - TQ:S]
            for res in q_tail():
                seq.extend([prev] * NC)
                prev = res[0:8]
            per = max(1, -(-len(side) // NQ))
            assert per <= D // 8
            for j, step in enumerate(side):
                ct, rg = j // per, j % per
                src = vt[rg * 8:(rg + 1) * 8, ct * TQ:(ct + 1) * TQ]
                step(pltpu.bitcast(src, U32) & zero8)
            for i in range(NQ):
                j = i + AHEAD
                if LOOK <= j < NQ:
                    _run(qk(j), pv(i))
                else:
                    _run(pv(i))

        def side_work(h):
            g = h // HG + ((h % HG) >= RCH).astype(jnp.int32)
            ch = h % RCH
            return (relayout_steps(wq_r, wq_p, g, ch, M, PLQ)
                    + relayout_steps(wuk_r, wuk_p, jnp.minimum(g + 1, NG - 1), ch, Dc, PLK)
                    + relayout_steps(wuv_r, wuv_p, g, ch, Dc, PLK))

        def head_body(h, carry):
            @pl.when(h == RCH)
            def _():
                for d in c_late:
                    d.wait()

            kh = k_v.at[h % HG]
            q_mid()
            attention(h, kh, side_work(h))
            q_head(h + 1)
            k_proj(h + HG, kh)
            return carry

        jax.lax.fori_loop(0, H - HG, head_body, 0)

        def last_body(h, carry):
            per = -(-4 * NC // HG)
            zero8 = zeros8()
            ties = {}
            for i in range(per):
                ct = jnp.minimum((h - (H - HG)) * per + i, 4 * NC - 1)
                tile = mod_tile(wmodb_v[ct])
                modb_v[ct] = tile
                ties[2 * i + 3] = pltpu.bitcast(tile, U32) & zero8
            q_mid(ties)
            attention(h, k_v.at[h % HG], ())
            q_head(jnp.minimum(h + 1, H - 1))
            return carry

        jax.lax.fori_loop(H - HG, H, last_body, 0)

        def sub_rows(r):
            out = []
            for j in range(TR // HB):
                r0 = r * TR + j * HB
                if not isinstance(r0, int):
                    r0 = pl.multiple_of(r0, HB)
                out.append(r0)
            return out

        def stage1(r):
            lns = []
            for r0 in sub_rows(r):
                rows = pl.ds(r0, HB)
                ctx = jnp.concatenate([ctx_v[h, rows, :] for h in range(H)], axis=1)
                att = _dot(ctx, wo_v[...])
                x1 = x_v[rows, :].astype(F32) + _rows_op(jnp.multiply, att, mod(2))
                x1_v[rows, :] = x1
                h2 = _modulate(_ln(x1), 1.0 + mod(4), mod(3))
                h2_v[rows, :] = h2
                lns.append(_ln(h2).astype(BF16))
            for r0, ln in zip(sub_rows(r), lns):
                u = _gelu(_dot(ln, w1_v[...]))
                for cidx in range(NC):
                    hh_v[cidx, pl.ds(r0 + PAD, HB), :] = u[:, cidx * LANES:(cidx + 1) * LANES]

        shifts = (1, -1, 2, -2)

        def out_cp(r):
            r0 = r * TR if isinstance(r, int) else pl.multiple_of(r * TR, TR)
            rows = pl.ds(r0, TR)
            return pltpu.make_async_copy(o_v.at[rows, :], out_hbm.at[rows, :], osems.at[r])

        def stage2(r):
            lane_i = jax.lax.broadcasted_iota(jnp.int32, (HB, LANES), 1)
            y1s = []
            for r0 in sub_rows(r):
                tiles = []
                for cidx in range(NC):
                    lo, hi = cidx * LANES, (cidx + 1) * LANES
                    g_lo, g_hi = lo // C4, (hi - 1) // C4
                    t = hh_v[cidx, pl.ds(r0 + PAD - shifts[g_hi], HB), :]
                    for g in range(g_hi - 1, g_lo - 1, -1):
                        tg = hh_v[cidx, pl.ds(r0 + PAD - shifts[g], HB), :]
                        t = jnp.where(lane_i < (g + 1) * C4 - lo, tg, t)
                    tiles.append(t)
                hs = _dot(jnp.concatenate(tiles, axis=1).astype(BF16), w2_v[...])
                y1s.append(h2_v[pl.ds(r0, HB), :] + hs)
            gls = [_gelu(_dot_nt(_ln(y1).astype(BF16), w3_v[...])).astype(BF16)
                   for y1 in y1s]
            for r0, y1, gl in zip(sub_rows(r), y1s, gls):
                rows = pl.ds(r0, HB)
                h3 = _dot(gl, w4_v[...])
                o_v[rows, :] = (x1_v[rows, :]
                                + _rows_op(jnp.multiply, y1 + h3, mod(5))).astype(BF16)
            out_cp(r).start()

        def s1_body(r, carry):
            stage1(r)
            return carry

        def s2_body(r, carry):
            stage2(r)
            return carry

        jax.lax.fori_loop(0, NR, s1_body, 0)
        jax.lax.fori_loop(0, NR, s2_body, 0)
        for r in range(NR):
            out_cp(r).wait()

    hbm_spec = pl.BlockSpec(memory_space=pltpu.HBM)
    V = pltpu.VMEM
    scratch = [
        V((S, M), BF16),
        V((S, Dc), BF16),
        V((NG, M, HG, D), BF16),
        V((NG, Dc, HG, D), BF16),
        V((NG, Dc, HG, D), BF16),
        V((NG * _gstride(PLQ), D), U32),
        V((NG * _gstride(PLK), D), U32),
        V((NG * _gstride(PLK), D), U32),
        V((H * D, M), BF16),
        V((M, M), BF16),
        V((M, M), BF16),
        V((Fh, M), BF16),
        V((Fh, M), BF16),
        V((M, 2 * M), BF16),
        V((4 * NC, M, LANES), BF16),
        V((16, 2 * M), F32),
        V((4 * NC, 8, LANES), F32),
        V((M, LANES), F32),
        V((S, M), BF16),
        V((M // 2, D), U32),
        V((HG, Dc // 2, D), U32),
        V((S, D), BF16),
        V((HG, S // 2, D), U32),
        V((1, D // 2, S), U32),
        V((NQ, TQ, TQ), F32),
        V((NQ, TQ, TQ), F32),
        V((NQ, TQ, TQ), F32),
        V((NQ, TQ, TQ), F32),
        pltpu.SMEM((2,), jnp.int32),
        V((H, S, D), BF16),
        V((S, M), F32),
        V((S, M), F32),
        V((NC, S + 2 * PAD, LANES), F32),
        V((S, M), BF16),
        V((1, M), BF16),
        pltpu.SemaphoreType.DMA((NSEM,)),
        pltpu.SemaphoreType.DMA((NR,)),
    ]
    out = pl.pallas_call(
        kernel,
        out_shape=jax.ShapeDtypeStruct((S, M), BF16),
        in_specs=[hbm_spec] * 12,
        out_specs=hbm_spec,
        scratch_shapes=scratch,
        compiler_params=pltpu.CompilerParams(vmem_limit_bytes=120 * 1024 * 1024),
        name="adaln_cla_mixer",
    )(x2, ckv2, A_w_q, A_w_uk, A_w_uv, wo2, B_w1, B_w2, B_w3.T, B_w4, c, w_mod)
    return out.reshape(B, S, M)
```

```python
import functools
import math
import os

import jax
import jax.numpy as jnp
import jax.experimental.pallas as pl
import jax.experimental.pallas.tpu as pltpu

BF16 = jnp.bfloat16
F32 = jnp.float32
U32 = jnp.uint32

LANES = 128
TQ = 128
TR = 256
HB = 128
HG = 8
LOOK = 4
AHEAD = int(os.environ.get('AHEAD', 2))
NSB = 4
KC = 256
QC = int(os.environ.get('QC', 128))
MOD0 = int(os.environ.get('MOD0', 2))
LN0 = int(os.environ.get('LN0', 2))
KSUB = int(os.environ.get('KSUB', 1))
QH = int(os.environ.get('QH', 256))
FREE = int(os.environ.get('FREE', 200))
PC = 512
DIST = int(os.environ.get('DIST', 12))
PIN = int(os.environ.get('PIN', 0))
PAD = 16
EPS = 1e-5
LOG2E = math.log2(math.e)
NEG = -1000000000.0 * LOG2E

_NT = (((1,), (1,)), ((), ()))


def _ln(x):
    m = jnp.mean(x, axis=-1, keepdims=True)
    xc = x - m
    v = jnp.mean(xc * xc, axis=-1, keepdims=True)
    return xc * jax.lax.rsqrt(v + EPS)


def _gelu(x):
    return jax.nn.gelu(x, approximate=True)


def _dot(a, b):
    return jnp.dot(a, b, preferred_element_type=F32)


def _dot_nt(a, b):
    return jax.lax.dot_general(a, b, _NT, preferred_element_type=F32)


def _fold8(x, op):
    parts = [op(x[j:j + 8], x[j + 8:j + 16]) for j in range(0, x.shape[0], 16)]
    acc = parts[0]
    for p in parts[1:]:
        acc = op(acc, p)
    return acc


def _rows_op(op, x, v8):
    r, m = x.shape
    return op(x.reshape(r // 8, 8, m), v8[None]).reshape(r, m)


def _modulate(x, scale8, shift8):
    r, m = x.shape
    return (x.reshape(r // 8, 8, m) * scale8[None] + shift8[None]).reshape(r, m)


def _pack(x):
    return pltpu.bitcast(x.astype(BF16), U32)


def _unpack(w):
    return pltpu.bitcast(w, BF16)


def _gstride(plane):
    return -(-8 * plane // 32) * 32


def _tied(w, tie):
    return jnp.concatenate([w[0:8] | tie, w[8:]], axis=0)


def _run(*gens):
    gens = list(gens)
    while gens:
        for g in list(gens):
            if next(g, gens) is gens:
                gens.remove(g)


@jax.jit
def pallas_adaLN_cond__compressed_kv_cla__mixer_s_mlp__prompt_kernel(
    A_x: jax.Array,
    A_c_kv: jax.Array,
    A_w_q: jax.Array,
    A_w_uk: jax.Array,
    A_w_uv: jax.Array,
    A_w_o: jax.Array,
    B_x: jax.Array,
    B_w1: jax.Array,
    B_w2: jax.Array,
    B_w3: jax.Array,
    B_w4: jax.Array,
    c: jax.Array,
    w_mod: jax.Array,
):
    del B_x
    B, S, M = A_x.shape
    _, Sk, Dc = A_c_kv.shape
    _, H, D = A_w_q.shape
    Fh = B_w3.shape[1]
    assert B == 1 and Sk == S and D == LANES and H % HG == 0 and HG == 8
    assert S % TQ == 0 and S % TR == 0 and S % PC == 0 and TR % HB == 0
    assert M % LANES == 0 and M % 64 == 0 and Dc % 64 == 0
    NG = H // HG
    NQ = S // TQ
    NR = S // TR
    NC = M // LANES
    C4 = M // 4
    PLQ = M // 2 + 1
    PLK = Dc // 2 + 1
    RCH = 4
    NK = S // KC
    XC = S // RCH
    NSEM = NK + 4
    assert NK > RCH + 1
    qscale = float(D) ** -0.5 * LOG2E

    x2 = A_x.reshape(S, M)
    ckv2 = A_c_kv.reshape(S, Dc)
    wo2 = A_w_o.reshape(H * D, M)

    def kernel(x_hbm, ckv_hbm, wq_hbm, wuk_hbm, wuv_hbm, wo_hbm, w1_hbm, w2_hbm,
               w3_hbm, w4_hbm, c_hbm, wmod_hbm, out_hbm,
               x_v, ckv_v, wq_r, wuk_r, wuv_r, wq_p, wuk_p, wuv_p, wo_v, w1_v,
               w2_v, w3_v, w4_v, wmoda_v, wmodb_v, moda_v, modb_v, scb_v, hn_v, wqc_v, wk0_v, q_v, k_v,
               vt_v, s0, s1, s2, s3, z_s, ctx_v, x1_v, h2_v, hh_v, o_v, c_v,
               sems):

        s_v = (s0, s1, s2, s3)
        z_s[0] = 0
        z_s[1] = 0

        def aligned(i, n):
            return i * n if isinstance(i, int) else pl.multiple_of(i * n, n)

        def cp(src, dst, i):
            return pltpu.make_async_copy(src, dst, sems.at[i])

        def c_ckv(r):
            rows = pl.ds(aligned(r, KC), KC)
            return cp(ckv_hbm.at[rows, :], ckv_v.at[rows, :], r)

        def c_x(j):
            rows = pl.ds(aligned(j, XC), XC)
            return cp(x_hbm.at[rows, :], x_v.at[rows, :], NK - RCH + j)

        def c_q0(j):
            rows = pl.ds(aligned(j, M // RCH), M // RCH)
            return cp(wq_hbm.at[rows, pl.ds(0, HG), :], wq_r.at[0, rows], NK - RCH + j)

        def gcp(src, dst, g, i):
            return cp(src.at[:, pl.ds(g * HG, HG), :], dst.at[g], i)

        c_moda = cp(wmod_hbm.at[:, pl.ds(0, 2 * M)], wmoda_v, NK - RCH - 1)
        c_c = cp(c_hbm, c_v, NK)
        c_k0 = gcp(wuk_hbm, wuk_r, 0, NK + 1)
        c_v0 = gcp(wuv_hbm, wuv_r, 0, NK + 2)
        c_k1 = gcp(wuk_hbm, wuk_r, 1, NK + 2)
        c_late = []
        for g in range(1, NG):
            for src, dst, gg in ((wq_hbm, wq_r, g), (wuv_hbm, wuv_r, g), (wuk_hbm, wuk_r, g + 1)):
                if gg < NG:
                    c_late.append(gcp(src, dst, gg, NSEM - 1))
        for ct in range(4 * NC):
            c_late.append(cp(wmod_hbm.at[:, pl.ds(2 * M + ct * LANES, LANES)],
                             wmodb_v.at[ct], NSEM - 1))
        for src, dst in ((wo_hbm, wo_v), (w1_hbm, w1_v), (w2_hbm, w2_v),
                         (w3_hbm, w3_v), (w4_hbm, w4_v)):
            c_late.append(cp(src, dst, NSEM - 1))
        order = [c_c, c_k0] + [c_ckv(r) for r in range(NK - RCH)] + [c_moda]
        for j in range(RCH):
            order += [c_ckv(NK - RCH + j), c_x(j), c_q0(j)]
        order += [c_v0, c_k1] + c_late
        for d in order:
            d.start()

        def relayout_steps(raw, dst, g, chunk, rows, plane):
            n = rows // RCH // 2
            base = g * _gstride(plane) + chunk * n
            if not isinstance(base, int):
                base = pl.multiple_of(base, 8)
            view = dst.at[pl.ds(base, 7 * plane + n), :]

            def step(j, tie):
                val = raw[g, pl.ds(chunk * (2 * n) + 2 * j, 2)].reshape(2 * HG, D)
                val = pltpu.bitcast(val, U32)
                if tie is not None:
                    val = val | tie
                view[pl.ds(j, 8, stride=plane), :] = val

            return [functools.partial(step, j) for j in range(n)]

        def relayout(raw, dst, g, rows, plane):
            for ch in range(RCH):
                for step in relayout_steps(raw, dst, g, ch, rows, plane):
                    step(None)

        def head_w32(src, h, rows, plane):
            base = (h // HG) * _gstride(plane) + ((h % HG) // 2) * plane
            ev = src[pl.ds(base, rows // 2), :]
            od = src[pl.ds(base + 4 * plane, rows // 2), :]
            if not isinstance(h, int):
                par = (h % 2).astype(U32)
                w = (((ev >> (16 * par)) & U32(0xFFFF))
                     | ((od << (16 * (1 - par))) & U32(0xFFFF0000)))
            elif h % 2 == 0:
                w = (ev & U32(0xFFFF)) | (od << 16)
            else:
                w = (ev >> 16) | (od & U32(0xFFFF0000))
            return w

        def head_w(src, h, rows, plane):
            return pltpu.bitcast(head_w32(src, h, rows, plane), BF16)

        def q_rows(wq, lo, hi, ties=()):
            res = []
            for r0 in range(lo, hi, QC):
                rows = slice(r0, r0 + QC)
                w = _tied(wq, ties[len(res)]) if len(res) in ties else wq
                res.append(_dot(hn_v[rows, :], pltpu.bitcast(w, BF16)))
                q_v[rows, :] = (res[-1] * qscale).astype(BF16)
            return res

        def q_head(h):
            wq = head_w32(wq_p, h, M, PLQ)
            wqc_v[...] = wq
            return q_rows(wq, 0, QH)

        def q_mid(ties=()):
            q_rows(wqc_v[...], QH, S - PC, ties)

        def q_tail():
            return q_rows(wqc_v[...], S - PC, S)

        def k_proj(h, kh):
            wk = head_w(wuk_p, h, Dc, PLK)
            for r in range(S // PC):
                rows = slice(r * PC, (r + 1) * PC)
                kh[r * PC // 2:(r + 1) * PC // 2, :] = _pack(_dot(ckv_v[rows, :], wk))

        def mod_tile(w):
            acc = _fold8(w.astype(F32) * scb_v[...], jnp.add)
            return jnp.broadcast_to(jnp.sum(acc, axis=0, keepdims=True), (8, LANES))

        def mod(i):
            if i < 2:
                return moda_v[0:8, i * M:(i + 1) * M]
            return jnp.concatenate(
                [modb_v[(i - 2) * NC + ct] for ct in range(NC)], axis=1)

        def zeros8():
            return jnp.full((8, LANES), z_s[1], jnp.int32).astype(U32)

        def k_chunk(r, nsub=1, ties=(), after=None, unpack=False):
            n = KC // nsub
            lhs = ckv_v[pl.ds(aligned(r, KC), KC), :]
            for h in range(HG):
                if unpack:
                    w32 = head_w32(wuk_p, h, Dc, PLK)
                    wk0_v[h] = w32
                else:
                    w32 = wk0_v[h]
                for j in range(nsub):
                    i = h * nsub + j
                    rows = pl.ds(aligned(r * nsub + j, n // 2), n // 2)
                    w = _tied(w32, ties[i]) if i in ties else w32
                    res = _dot(lhs[j * n:(j + 1) * n], pltpu.bitcast(w, BF16))
                    k_v[h, rows, :] = _pack(res)
                    if after is not None:
                        after(i, res)

        c_c.wait()
        cc = c_v[...].astype(F32)
        sc = (cc * jax.nn.sigmoid(cc)).astype(BF16).astype(F32)
        scb_v[...] = jnp.broadcast_to(sc, (LANES, M)).T
        zpad = jnp.zeros((PAD, LANES), F32)
        for cidx in range(NC):
            hh_v[cidx, 0:PAD, :] = zpad
            hh_v[cidx, PAD + S:PAD + S + PAD, :] = zpad
        c_k0.wait()
        relayout(wuk_r, wuk_p, 0, Dc, PLK)

        def ka_body(r, carry):
            c_ckv(r).wait()
            k_chunk(r, unpack=True)
            return carry

        jax.lax.fori_loop(0, NK - RCH - 1, ka_body, 0)

        c_ckv(NK - RCH - 1).wait()
        c_moda.wait()
        zero8 = zeros8()
        ties = {}
        for ct in range(2 * NC):
            cols = slice(ct * LANES, (ct + 1) * LANES)
            tile = mod_tile(wmoda_v[:, cols])
            moda_v[0:8, cols] = tile
            ties[MOD0 + (ct * (2 * HG - MOD0)) // (2 * NC)] = pltpu.bitcast(tile, U32) & zero8
        k_chunk(NK - RCH - 1, 2, ties)

        def kb_body(j, carry):
            c_ckv(NK - RCH + j).wait()
            c_x(j).wait()
            c_q0(j).wait()
            zero8 = zeros8()
            nstep = KSUB * HG
            lr = XC // nstep
            ties = {}
            scale, shift = 1.0 + mod(1), mod(0)
            for i in range(nstep):
                rows = pl.ds(pl.multiple_of(j * XC + i * lr, lr), lr)
                hn = _modulate(_ln(x_v[rows, :].astype(F32)), scale, shift)
                hn_v[rows, :] = hn.astype(BF16)
                ties[i + LN0] = pltpu.bitcast(_fold8(hn[:, 0:LANES], jnp.maximum), U32) & zero8
            steps = relayout_steps(wq_r, wq_p, 0, j, M, PLQ)
            per = len(steps) // nstep

            def side(i, res):
                for k, step in enumerate(steps[i * per:(i + 1) * per]):
                    step(pltpu.bitcast(res[k * 8:(k + 1) * 8], U32) & zero8)

            k_chunk(NK - RCH + j, KSUB, ties, side)
            return carry

        jax.lax.fori_loop(0, RCH, kb_body, 0)

        c_v0.wait()
        c_k1.wait()
        zero8 = zeros8()
        res = jnp.concatenate(q_head(0), axis=0)
        steps = []
        for ch in range(RCH):
            steps += relayout_steps(wuv_r, wuv_p, 0, ch, Dc, PLK)
            steps += relayout_steps(wuk_r, wuk_p, 1, ch, Dc, PLK)
        for i, step in enumerate(steps):
            if i < FREE:
                step(None)
            else:
                k = (i - FREE) * (QH // 8) // (len(steps) - FREE)
                step(pltpu.bitcast(res[k * 8:(k + 1) * 8], U32) & zero8)

        def attention(h, kh, side):
            key_i = jax.lax.broadcasted_iota(jnp.int32, (TQ, TQ), 0)
            qry_i = jax.lax.broadcasted_iota(jnp.int32, (TQ, TQ), 1)
            causal = key_i <= qry_i
            z_st = z_s[0]
            z_ld = z_s[1]
            zero8 = zeros8()

            mx = {}
            seq = []

            def qk(i):
                qi = q_v[i * TQ:(i + 1) * TQ, :]
                sb = s_v[i % NSB]
                m8 = None
                for t in range(i + 1):
                    tile = _dot_nt(_unpack(kh[t * TQ // 2:(t + 1) * TQ // 2, :]), qi)
                    seq.append(tile[0:8])
                    if t == i:
                        tile = jnp.where(causal, tile, NEG)
                    sb[z_st + t] = tile
                    tm = _fold8(tile, jnp.maximum)
                    m8 = tm if m8 is None else jnp.maximum(m8, tm)
                    if t == i:
                        mx[i] = jnp.max(m8, axis=0, keepdims=True)
                    yield

            parts = []

            def pv(i):
                sb = s_v[i % NSB]
                m8 = jnp.broadcast_to(mx[i], (8, TQ))
                l8 = None
                ot = None
                for t in range(i + 1):
                    tie = pltpu.bitcast(seq[-DIST], U32)
                    if PIN and len(parts) >= PIN:
                        tie = tie | pltpu.bitcast(parts[-PIN], U32)
                    mt = pltpu.bitcast(pltpu.bitcast(m8, U32) | (tie & zero8), F32)
                    tile = sb[z_ld + t].reshape(TQ // 8, 8, TQ)
                    p = jnp.exp2(tile - mt[None]).reshape(TQ, TQ)
                    part = _fold8(p, jnp.add)
                    l8 = part if l8 is None else l8 + part
                    parts.append(l8)
                    o = _dot(_unpack(vt_v[z_ld, :, t * TQ:(t + 1) * TQ]), p.astype(BF16))
                    seq.append(o[0:8])
                    ot = o if ot is None else ot + o
                    if t == i:
                        l = jnp.sum(l8, axis=0, keepdims=True)
                        ot = ot * (1.0 / l)
                        ctx_v[h, i * TQ:(i + 1) * TQ, :] = ot.T.astype(BF16)
                    yield

            for i in range(LOOK):
                _run(qk(i))
            vt = _dot_nt(head_w(wuv_p, h, Dc, PLK).T, ckv_v[...])
            vt_v[z_st] = _pack(vt)
            prev = vt[0:8, S - TQ:S]
            for res in q_tail():
                seq.extend([prev] * NC)
                prev = res[0:8]
            per = max(1, -(-len(side) // NQ))
            assert per <= D // 8
            for j, step in enumerate(side):
                ct, rg = j // per, j % per
                src = vt[rg * 8:(rg + 1) * 8, ct * TQ:(ct + 1) * TQ]
                step(pltpu.bitcast(src, U32) & zero8)
            for i in range(NQ):
                j = i + AHEAD
                if LOOK <= j < NQ:
                    _run(qk(j), pv(i))
                else:
                    _run(pv(i))

        def side_work(h):
            g = h // HG + ((h % HG) >= RCH).astype(jnp.int32)
            ch = h % RCH
            return (relayout_steps(wq_r, wq_p, g, ch, M, PLQ)
                    + relayout_steps(wuk_r, wuk_p, jnp.minimum(g + 1, NG - 1), ch, Dc, PLK)
                    + relayout_steps(wuv_r, wuv_p, g, ch, Dc, PLK))

        def head_body(h, carry):
            @pl.when(h == RCH)
            def _():
                for d in c_late:
                    d.wait()

            kh = k_v.at[h % HG]
            q_mid()
            attention(h, kh, side_work(h))
            q_head(h + 1)
            k_proj(h + HG, kh)
            return carry

        jax.lax.fori_loop(0, H - HG, head_body, 0)

        def last_body(h, carry):
            per = -(-4 * NC // HG)
            zero8 = zeros8()
            ties = {}
            for i in range(per):
                ct = jnp.minimum((h - (H - HG)) * per + i, 4 * NC - 1)
                tile = mod_tile(wmodb_v[ct])
                modb_v[ct] = tile
                ties[2 * i + 3] = pltpu.bitcast(tile, U32) & zero8
            q_mid(ties)
            attention(h, k_v.at[h % HG], ())
            q_head(jnp.minimum(h + 1, H - 1))
            return carry

        jax.lax.fori_loop(H - HG, H, last_body, 0)

        def sub_rows(r):
            out = []
            for j in range(TR // HB):
                r0 = r * TR + j * HB
                if not isinstance(r0, int):
                    r0 = pl.multiple_of(r0, HB)
                out.append(r0)
            return out

        def stage1(r):
            lns = []
            for r0 in sub_rows(r):
                rows = pl.ds(r0, HB)
                ctx = jnp.concatenate([ctx_v[h, rows, :] for h in range(H)], axis=1)
                att = _dot(ctx, wo_v[...])
                x1 = x_v[rows, :].astype(F32) + _rows_op(jnp.multiply, att, mod(2))
                x1_v[rows, :] = x1
                h2 = _modulate(_ln(x1), 1.0 + mod(4), mod(3))
                h2_v[rows, :] = h2
                lns.append(_ln(h2).astype(BF16))
            for r0, ln in zip(sub_rows(r), lns):
                u = _gelu(_dot(ln, w1_v[...]))
                for cidx in range(NC):
                    hh_v[cidx, pl.ds(r0 + PAD, HB), :] = u[:, cidx * LANES:(cidx + 1) * LANES]

        shifts = (1, -1, 2, -2)

        def out_cp(r0):
            rows = pl.ds(r0, HB)
            return cp(o_v.at[rows, :], out_hbm.at[rows, :], 0)

        def stage2(r):
            lane_i = jax.lax.broadcasted_iota(jnp.int32, (HB, LANES), 1)
            y1s = []
            for r0 in sub_rows(r):
                tiles = []
                for cidx in range(NC):
                    lo, hi = cidx * LANES, (cidx + 1) * LANES
                    g_lo, g_hi = lo // C4, (hi - 1) // C4
                    t = hh_v[cidx, pl.ds(r0 + PAD - shifts[g_hi], HB), :]
                    for g in range(g_hi - 1, g_lo - 1, -1):
                        tg = hh_v[cidx, pl.ds(r0 + PAD - shifts[g], HB), :]
                        t = jnp.where(lane_i < (g + 1) * C4 - lo, tg, t)
                    tiles.append(t)
                hs = _dot(jnp.concatenate(tiles, axis=1).astype(BF16), w2_v[...])
                y1s.append(h2_v[pl.ds(r0, HB), :] + hs)
            gls = [_gelu(_dot_nt(_ln(y1).astype(BF16), w3_v[...])).astype(BF16)
                   for y1 in y1s]
            for r0, y1, gl in zip(sub_rows(r), y1s, gls):
                rows = pl.ds(r0, HB)
                h3 = _dot(gl, w4_v[...])
                o_v[rows, :] = (x1_v[rows, :]
                                + _rows_op(jnp.multiply, y1 + h3, mod(5))).astype(BF16)
                out_cp(r0).start()

        def s1_body(r, carry):
            stage1(r)
            return carry

        def s2_body(r, carry):
            stage2(r)
            return carry

        jax.lax.fori_loop(0, NR, s1_body, 0)
        jax.lax.fori_loop(0, NR, s2_body, 0)
        cp(o_v, out_hbm, 0).wait()

    hbm_spec = pl.BlockSpec(memory_space=pltpu.HBM)
    V = pltpu.VMEM
    scratch = [
        V((S, M), BF16),
        V((S, Dc), BF16),
        V((NG, M, HG, D), BF16),
        V((NG, Dc, HG, D), BF16),
        V((NG, Dc, HG, D), BF16),
        V((NG * _gstride(PLQ), D), U32),
        V((NG * _gstride(PLK), D), U32),
        V((NG * _gstride(PLK), D), U32),
        V((H * D, M), BF16),
        V((M, M), BF16),
        V((M, M), BF16),
        V((Fh, M), BF16),
        V((Fh, M), BF16),
        V((M, 2 * M), BF16),
        V((4 * NC, M, LANES), BF16),
        V((16, 2 * M), F32),
        V((4 * NC, 8, LANES), F32),
        V((M, LANES), F32),
        V((S, M), BF16),
        V((M // 2, D), U32),
        V((HG, Dc // 2, D), U32),
        V((S, D), BF16),
        V((HG, S // 2, D), U32),
        V((1, D // 2, S), U32),
        V((NQ, TQ, TQ), F32),
        V((NQ, TQ, TQ), F32),
        V((NQ, TQ, TQ), F32),
        V((NQ, TQ, TQ), F32),
        pltpu.SMEM((2,), jnp.int32),
        V((H, S, D), BF16),
        V((S, M), F32),
        V((S, M), F32),
        V((NC, S + 2 * PAD, LANES), F32),
        V((S, M), BF16),
        V((1, M), BF16),
        pltpu.SemaphoreType.DMA((NSEM,)),
    ]
    out = pl.pallas_call(
        kernel,
        out_shape=jax.ShapeDtypeStruct((S, M), BF16),
        in_specs=[hbm_spec] * 12,
        out_specs=hbm_spec,
        scratch_shapes=scratch,
        compiler_params=pltpu.CompilerParams(vmem_limit_bytes=120 * 1024 * 1024),
        name="adaln_cla_mixer",
    )(x2, ckv2, A_w_q, A_w_uk, A_w_uv, wo2, B_w1, B_w2, B_w3.T, B_w4, c, w_mod)
    return out.reshape(B, S, M)
```

```python
import functools
import math
import os

import jax
import jax.numpy as jnp
import jax.experimental.pallas as pl
import jax.experimental.pallas.tpu as pltpu

BF16 = jnp.bfloat16
F32 = jnp.float32
U32 = jnp.uint32

LANES = 128
TQ = 128
TR = 256
HB = 128
HG = 8
LOOK = 4
AHEAD = int(os.environ.get('AHEAD', 2))
NSB = 4
KC = 256
QC = int(os.environ.get('QC', 128))
MOD0 = int(os.environ.get('MOD0', 2))
LN0 = int(os.environ.get('LN0', 2))
KSUB = int(os.environ.get('KSUB', 1))
QH = int(os.environ.get('QH', 256))
FREE = int(os.environ.get('FREE', 0))
PC = 512
DIST = int(os.environ.get('DIST', 12))
PIN = int(os.environ.get('PIN', 0))
PAD = 16
EPS = 1e-5
LOG2E = math.log2(math.e)
NEG = -1000000000.0 * LOG2E

_NT = (((1,), (1,)), ((), ()))


def _ln(x):
    m = jnp.mean(x, axis=-1, keepdims=True)
    xc = x - m
    v = jnp.mean(xc * xc, axis=-1, keepdims=True)
    return xc * jax.lax.rsqrt(v + EPS)


def _gelu(x):
    return jax.nn.gelu(x, approximate=True)


def _dot(a, b):
    return jnp.dot(a, b, preferred_element_type=F32)


def _dot_nt(a, b):
    return jax.lax.dot_general(a, b, _NT, preferred_element_type=F32)


def _fold8(x, op):
    parts = [op(x[j:j + 8], x[j + 8:j + 16]) for j in range(0, x.shape[0], 16)]
    acc = parts[0]
    for p in parts[1:]:
        acc = op(acc, p)
    return acc


def _rows_op(op, x, v8):
    r, m = x.shape
    return op(x.reshape(r // 8, 8, m), v8[None]).reshape(r, m)


def _modulate(x, scale8, shift8):
    r, m = x.shape
    return (x.reshape(r // 8, 8, m) * scale8[None] + shift8[None]).reshape(r, m)


def _pack(x):
    return pltpu.bitcast(x.astype(BF16), U32)


def _unpack(w):
    return pltpu.bitcast(w, BF16)


def _gstride(plane):
    return -(-8 * plane // 32) * 32


def _tied(w, tie):
    return jnp.concatenate([w[0:8] | tie, w[8:]], axis=0)


def _run(*gens):
    gens = list(gens)
    while gens:
        for g in list(gens):
            if next(g, gens) is gens:
                gens.remove(g)


@jax.jit
def pallas_adaLN_cond__compressed_kv_cla__mixer_s_mlp__prompt_kernel(
    A_x: jax.Array,
    A_c_kv: jax.Array,
    A_w_q: jax.Array,
    A_w_uk: jax.Array,
    A_w_uv: jax.Array,
    A_w_o: jax.Array,
    B_x: jax.Array,
    B_w1: jax.Array,
    B_w2: jax.Array,
    B_w3: jax.Array,
    B_w4: jax.Array,
    c: jax.Array,
    w_mod: jax.Array,
):
    del B_x
    B, S, M = A_x.shape
    _, Sk, Dc = A_c_kv.shape
    _, H, D = A_w_q.shape
    Fh = B_w3.shape[1]
    assert B == 1 and Sk == S and D == LANES and H % HG == 0 and HG == 8
    assert S % TQ == 0 and S % TR == 0 and S % PC == 0 and TR % HB == 0
    assert M % LANES == 0 and M % 64 == 0 and Dc % 64 == 0
    NG = H // HG
    NQ = S // TQ
    NR = S // TR
    NC = M // LANES
    C4 = M // 4
    PLQ = M // 2 + 1
    PLK = Dc // 2 + 1
    RCH = 4
    NK = S // KC
    XC = S // RCH
    NSEM = NK + 5
    assert NK > RCH + 1
    qscale = float(D) ** -0.5 * LOG2E

    x2 = A_x.reshape(S, M)
    ckv2 = A_c_kv.reshape(S, Dc)
    wo2 = A_w_o.reshape(H * D, M)

    def kernel(x_hbm, ckv_hbm, wq_hbm, wuk_hbm, wuv_hbm, wo_hbm, w1_hbm, w2_hbm,
               w3_hbm, w4_hbm, c_hbm, wmod_hbm, out_hbm,
               x_v, ckv_v, wq_r, wuk_r, wuv_r, wq_p, wuk_p, wuv_p, wo_v, w1_v,
               w2_v, w3_v, w4_v, wmoda_v, wmodb_v, moda_v, modb_v, scb_v, hn_v, wqc_v, wk0_v, q_v, k_v,
               vt_v, s0, s1, s2, s3, z_s, ctx_v, x1_v, h2_v, hh_v, o_v, c_v,
               sems):

        s_v = (s0, s1, s2, s3)
        z_s[0] = 0
        z_s[1] = 0

        def aligned(i, n):
            return i * n if isinstance(i, int) else pl.multiple_of(i * n, n)

        def cp(src, dst, i):
            return pltpu.make_async_copy(src, dst, sems.at[i])

        def c_ckv(r):
            rows = pl.ds(aligned(r, KC), KC)
            return cp(ckv_hbm.at[rows, :], ckv_v.at[rows, :], r)

        def c_x(j):
            rows = pl.ds(aligned(j, XC), XC)
            return cp(x_hbm.at[rows, :], x_v.at[rows, :], NK - RCH + j)

        def c_q0(j):
            rows = pl.ds(aligned(j, M // RCH), M // RCH)
            return cp(wq_hbm.at[rows, pl.ds(0, HG), :], wq_r.at[0, rows], NK - RCH + j)

        def gcp(src, dst, g, i):
            return cp(src.at[:, pl.ds(g * HG, HG), :], dst.at[g], i)

        c_moda = cp(wmod_hbm.at[:, pl.ds(0, 2 * M)], wmoda_v, NK - RCH - 1)
        c_c = cp(c_hbm, c_v, NK)
        c_k0 = gcp(wuk_hbm, wuk_r, 0, NK + 1)
        c_v0 = gcp(wuv_hbm, wuv_r, 0, NK + 2)
        c_k1 = gcp(wuk_hbm, wuk_r, 1, NK + 3)
        c_late = []
        for g in range(1, NG):
            for src, dst, gg in ((wq_hbm, wq_r, g), (wuv_hbm, wuv_r, g), (wuk_hbm, wuk_r, g + 1)):
                if gg < NG:
                    c_late.append(gcp(src, dst, gg, NSEM - 1))
        for ct in range(4 * NC):
            c_late.append(cp(wmod_hbm.at[:, pl.ds(2 * M + ct * LANES, LANES)],
                             wmodb_v.at[ct], NSEM - 1))
        for src, dst in ((wo_hbm, wo_v), (w1_hbm, w1_v), (w2_hbm, w2_v),
                         (w3_hbm, w3_v), (w4_hbm, w4_v)):
            c_late.append(cp(src, dst, NSEM - 1))
        order = [c_c, c_k0] + [c_ckv(r) for r in range(NK - RCH)] + [c_moda]
        for j in range(RCH):
            order += [c_ckv(NK - RCH + j), c_x(j), c_q0(j)]
        order += [c_v0, c_k1] + c_late
        for d in order:
            d.start()

        def relayout_steps(raw, dst, g, chunk, rows, plane):
            n = rows // RCH // 2
            base = g * _gstride(plane) + chunk * n
            if not isinstance(base, int):
                base = pl.multiple_of(base, 8)
            view = dst.at[pl.ds(base, 7 * plane + n), :]

            def step(j, tie):
                val = raw[g, pl.ds(chunk * (2 * n) + 2 * j, 2)].reshape(2 * HG, D)
                val = pltpu.bitcast(val, U32)
                if tie is not None:
                    val = val | tie
                view[pl.ds(j, 8, stride=plane), :] = val

            return [functools.partial(step, j) for j in range(n)]

        def relayout(raw, dst, g, rows, plane):
            for ch in range(RCH):
                for step in relayout_steps(raw, dst, g, ch, rows, plane):
                    step(None)

        def head_w32(src, h, rows, plane):
            base = (h // HG) * _gstride(plane) + ((h % HG) // 2) * plane
            ev = src[pl.ds(base, rows // 2), :]
            od = src[pl.ds(base + 4 * plane, rows // 2), :]
            if not isinstance(h, int):
                par = (h % 2).astype(U32)
                w = (((ev >> (16 * par)) & U32(0xFFFF))
                     | ((od << (16 * (1 - par))) & U32(0xFFFF0000)))
            elif h % 2 == 0:
                w = (ev & U32(0xFFFF)) | (od << 16)
            else:
                w = (ev >> 16) | (od & U32(0xFFFF0000))
            return w

        def head_w(src, h, rows, plane):
            return pltpu.bitcast(head_w32(src, h, rows, plane), BF16)

        def q_rows(wq, lo, hi, ties=()):
            res = []
            for r0 in range(lo, hi, QC):
                rows = slice(r0, r0 + QC)
                w = _tied(wq, ties[len(res)]) if len(res) in ties else wq
                res.append(_dot(hn_v[rows, :], pltpu.bitcast(w, BF16)))
                q_v[rows, :] = (res[-1] * qscale).astype(BF16)
            return res

        def q_head(h):
            wq = head_w32(wq_p, h, M, PLQ)
            wqc_v[...] = wq
            return wq, q_rows(wq, 0, QH)

        def q_mid(ties=()):
            q_rows(wqc_v[...], QH, S - PC, ties)

        def q_tail():
            return q_rows(wqc_v[...], S - PC, S)

        def k_proj(h, kh):
            wk = head_w(wuk_p, h, Dc, PLK)
            for r in range(S // PC):
                rows = slice(r * PC, (r + 1) * PC)
                kh[r * PC // 2:(r + 1) * PC // 2, :] = _pack(_dot(ckv_v[rows, :], wk))

        def mod_tile(w):
            acc = _fold8(w.astype(F32) * scb_v[...], jnp.add)
            return jnp.broadcast_to(jnp.sum(acc, axis=0, keepdims=True), (8, LANES))

        def mod(i):
            if i < 2:
                return moda_v[0:8, i * M:(i + 1) * M]
            return jnp.concatenate(
                [modb_v[(i - 2) * NC + ct] for ct in range(NC)], axis=1)

        def zeros8():
            return jnp.full((8, LANES), z_s[1], jnp.int32).astype(U32)

        def k_chunk(r, nsub=1, ties=(), after=None, unpack=False):
            n = KC // nsub
            lhs = ckv_v[pl.ds(aligned(r, KC), KC), :]
            for h in range(HG):
                if unpack:
                    w32 = head_w32(wuk_p, h, Dc, PLK)
                    wk0_v[h] = w32
                else:
                    w32 = wk0_v[h]
                for j in range(nsub):
                    i = h * nsub + j
                    rows = pl.ds(aligned(r * nsub + j, n // 2), n // 2)
                    w = _tied(w32, ties[i]) if i in ties else w32
                    res = _dot(lhs[j * n:(j + 1) * n], pltpu.bitcast(w, BF16))
                    k_v[h, rows, :] = _pack(res)
                    if after is not None:
                        after(i, res)

        c_c.wait()
        cc = c_v[...].astype(F32)
        sc = (cc * jax.nn.sigmoid(cc)).astype(BF16).astype(F32)
        scb_v[...] = jnp.broadcast_to(sc, (LANES, M)).T
        zpad = jnp.zeros((PAD, LANES), F32)
        for cidx in range(NC):
            hh_v[cidx, 0:PAD, :] = zpad
            hh_v[cidx, PAD + S:PAD + S + PAD, :] = zpad
        c_k0.wait()
        relayout(wuk_r, wuk_p, 0, Dc, PLK)

        def ka_body(r, carry):
            c_ckv(r).wait()
            k_chunk(r, unpack=True)
            return carry

        jax.lax.fori_loop(0, NK - RCH - 1, ka_body, 0)

        c_ckv(NK - RCH - 1).wait()
        c_moda.wait()
        zero8 = zeros8()
        ties = {}
        for ct in range(2 * NC):
            cols = slice(ct * LANES, (ct + 1) * LANES)
            tile = mod_tile(wmoda_v[:, cols])
            moda_v[0:8, cols] = tile
            ties[MOD0 + (ct * (2 * HG - MOD0)) // (2 * NC)] = pltpu.bitcast(tile, U32) & zero8
        k_chunk(NK - RCH - 1, 2, ties)

        def kb_body(j, carry):
            c_ckv(NK - RCH + j).wait()
            c_x(j).wait()
            c_q0(j).wait()
            zero8 = zeros8()
            nstep = KSUB * HG
            lr = XC // nstep
            ties = {}
            scale, shift = 1.0 + mod(1), mod(0)
            for i in range(nstep):
                rows = pl.ds(pl.multiple_of(j * XC + i * lr, lr), lr)
                hn = _modulate(_ln(x_v[rows, :].astype(F32)), scale, shift)
                hn_v[rows, :] = hn.astype(BF16)
                ties[i + LN0] = pltpu.bitcast(_fold8(hn[:, 0:LANES], jnp.maximum), U32) & zero8
            steps = relayout_steps(wq_r, wq_p, 0, j, M, PLQ)
            per = len(steps) // nstep

            def side(i, res):
                for k, step in enumerate(steps[i * per:(i + 1) * per]):
                    step(pltpu.bitcast(res[k * 8:(k + 1) * 8], U32) & zero8)

            k_chunk(NK - RCH + j, KSUB, ties, side)
            return carry

        jax.lax.fori_loop(0, RCH, kb_body, 0)

        c_v0.wait()
        zero8 = zeros8()
        wq0, res = q_head(0)
        res = jnp.concatenate(res, axis=0)
        steps = []
        for ch in range(RCH):
            steps += relayout_steps(wuv_r, wuv_p, 0, ch, Dc, PLK)
        for i, step in enumerate(steps):
            if i < FREE:
                step(wq0[0:8] & zero8)
            else:
                k = (i - FREE) * (QH // 8) // (len(steps) - FREE)
                step(pltpu.bitcast(res[k * 8:(k + 1) * 8], U32) & zero8)

        def attention(h, kh, side):
            key_i = jax.lax.broadcasted_iota(jnp.int32, (TQ, TQ), 0)
            qry_i = jax.lax.broadcasted_iota(jnp.int32, (TQ, TQ), 1)
            causal = key_i <= qry_i
            z_st = z_s[0]
            z_ld = z_s[1]
            zero8 = zeros8()

            mx = {}
            seq = []

            def qk(i):
                qi = q_v[i * TQ:(i + 1) * TQ, :]
                sb = s_v[i % NSB]
                m8 = None
                for t in range(i + 1):
                    tile = _dot_nt(_unpack(kh[t * TQ // 2:(t + 1) * TQ // 2, :]), qi)
                    seq.append(tile[0:8])
                    if t == i:
                        tile = jnp.where(causal, tile, NEG)
                    sb[z_st + t] = tile
                    tm = _fold8(tile, jnp.maximum)
                    m8 = tm if m8 is None else jnp.maximum(m8, tm)
                    if t == i:
                        mx[i] = jnp.max(m8, axis=0, keepdims=True)
                    yield

            parts = []

            def pv(i):
                sb = s_v[i % NSB]
                m8 = jnp.broadcast_to(mx[i], (8, TQ))
                l8 = None
                ot = None
                for t in range(i + 1):
                    tie = pltpu.bitcast(seq[-DIST], U32)
                    if PIN and len(parts) >= PIN:
                        tie = tie | pltpu.bitcast(parts[-PIN], U32)
                    mt = pltpu.bitcast(pltpu.bitcast(m8, U32) | (tie & zero8), F32)
                    tile = sb[z_ld + t].reshape(TQ // 8, 8, TQ)
                    p = jnp.exp2(tile - mt[None]).reshape(TQ, TQ)
                    part = _fold8(p, jnp.add)
                    l8 = part if l8 is None else l8 + part
                    parts.append(l8)
                    o = _dot(_unpack(vt_v[z_ld, :, t * TQ:(t + 1) * TQ]), p.astype(BF16))
                    seq.append(o[0:8])
                    ot = o if ot is None else ot + o
                    if t == i:
                        l = jnp.sum(l8, axis=0, keepdims=True)
                        ot = ot * (1.0 / l)
                        ctx_v[h, i * TQ:(i + 1) * TQ, :] = ot.T.astype(BF16)
                    yield

            for i in range(LOOK):
                _run(qk(i))
            vt = _dot_nt(head_w(wuv_p, h, Dc, PLK).T, ckv_v[...])
            vt_v[z_st] = _pack(vt)
            prev = vt[0:8, S - TQ:S]
            for res in q_tail():
                seq.extend([prev] * NC)
                prev = res[0:8]
            per = max(1, -(-len(side) // NQ))
            for j, step in enumerate(side):
                ct, rg = j // per, (j % per) * (D // 8) // per
                src = vt[rg * 8:(rg + 1) * 8, ct * TQ:(ct + 1) * TQ]
                step(pltpu.bitcast(src, U32) & zero8)
            for i in range(NQ):
                j = i + AHEAD
                if LOOK <= j < NQ:
                    _run(qk(j), pv(i))
                else:
                    _run(pv(i))

        def side_work(h):
            g = h // HG + ((h % HG) >= RCH).astype(jnp.int32)
            ch = h % RCH
            steps = (relayout_steps(wq_r, wq_p, g, ch, M, PLQ)
                     + relayout_steps(wuv_r, wuv_p, g, ch, Dc, PLK))
            for c in range(RCH):
                steps += relayout_steps(wuk_r, wuk_p, h // HG + 1, c, Dc, PLK)
            return steps

        def head_body(h, carry):
            @pl.when(h == RCH)
            def _():
                for d in c_late:
                    d.wait()

            kh = k_v.at[h % HG]
            q_mid()
            attention(h, kh, side_work(h))
            q_head(h + 1)
            k_proj(h + HG, kh)
            return carry

        c_k1.wait()
        jax.lax.fori_loop(0, H - HG, head_body, 0)

        def last_body(h, carry):
            per = -(-4 * NC // HG)
            zero8 = zeros8()
            ties = {}
            for i in range(per):
                ct = jnp.minimum((h - (H - HG)) * per + i, 4 * NC - 1)
                tile = mod_tile(wmodb_v[ct])
                modb_v[ct] = tile
                ties[2 * i + 3] = pltpu.bitcast(tile, U32) & zero8
            q_mid(ties)
            attention(h, k_v.at[h % HG], ())
            q_head(jnp.minimum(h + 1, H - 1))
            return carry

        jax.lax.fori_loop(H - HG, H, last_body, 0)

        def sub_rows(r):
            out = []
            for j in range(TR // HB):
                r0 = r * TR + j * HB
                if not isinstance(r0, int):
                    r0 = pl.multiple_of(r0, HB)
                out.append(r0)
            return out

        def stage1(r):
            lns = []
            for r0 in sub_rows(r):
                rows = pl.ds(r0, HB)
                ctx = jnp.concatenate([ctx_v[h, rows, :] for h in range(H)], axis=1)
                att = _dot(ctx, wo_v[...])
                x1 = x_v[rows, :].astype(F32) + _rows_op(jnp.multiply, att, mod(2))
                x1_v[rows, :] = x1
                h2 = _modulate(_ln(x1), 1.0 + mod(4), mod(3))
                h2_v[rows, :] = h2
                lns.append(_ln(h2).astype(BF16))
            for r0, ln in zip(sub_rows(r), lns):
                u = _gelu(_dot(ln, w1_v[...]))
                for cidx in range(NC):
                    hh_v[cidx, pl.ds(r0 + PAD, HB), :] = u[:, cidx * LANES:(cidx + 1) * LANES]

        shifts = (1, -1, 2, -2)

        def out_cp(r0):
            rows = pl.ds(r0, HB)
            return cp(o_v.at[rows, :], out_hbm.at[rows, :], 0)

        def stage2(r):
            lane_i = jax.lax.broadcasted_iota(jnp.int32, (HB, LANES), 1)
            y1s = []
            for r0 in sub_rows(r):
                tiles = []
                for cidx in range(NC):
                    lo, hi = cidx * LANES, (cidx + 1) * LANES
                    g_lo, g_hi = lo // C4, (hi - 1) // C4
                    t = hh_v[cidx, pl.ds(r0 + PAD - shifts[g_hi], HB), :]
                    for g in range(g_hi - 1, g_lo - 1, -1):
                        tg = hh_v[cidx, pl.ds(r0 + PAD - shifts[g], HB), :]
                        t = jnp.where(lane_i < (g + 1) * C4 - lo, tg, t)
                    tiles.append(t)
                hs = _dot(jnp.concatenate(tiles, axis=1).astype(BF16), w2_v[...])
                y1s.append(h2_v[pl.ds(r0, HB), :] + hs)
            gls = [_gelu(_dot_nt(_ln(y1).astype(BF16), w3_v[...])).astype(BF16)
                   for y1 in y1s]
            for r0, y1, gl in zip(sub_rows(r), y1s, gls):
                rows = pl.ds(r0, HB)
                h3 = _dot(gl, w4_v[...])
                o_v[rows, :] = (x1_v[rows, :]
                                + _rows_op(jnp.multiply, y1 + h3, mod(5))).astype(BF16)
                out_cp(r0).start()

        def s1_body(r, carry):
            stage1(r)
            return carry

        def s2_body(r, carry):
            stage2(r)
            return carry

        jax.lax.fori_loop(0, NR, s1_body, 0)
        jax.lax.fori_loop(0, NR, s2_body, 0)
        cp(o_v, out_hbm, 0).wait()

    hbm_spec = pl.BlockSpec(memory_space=pltpu.HBM)
    V = pltpu.VMEM
    scratch = [
        V((S, M), BF16),
        V((S, Dc), BF16),
        V((NG, M, HG, D), BF16),
        V((NG, Dc, HG, D), BF16),
        V((NG, Dc, HG, D), BF16),
        V((NG * _gstride(PLQ), D), U32),
        V((NG * _gstride(PLK), D), U32),
        V((NG * _gstride(PLK), D), U32),
        V((H * D, M), BF16),
        V((M, M), BF16),
        V((M, M), BF16),
        V((Fh, M), BF16),
        V((Fh, M), BF16),
        V((M, 2 * M), BF16),
        V((4 * NC, M, LANES), BF16),
        V((16, 2 * M), F32),
        V((4 * NC, 8, LANES), F32),
        V((M, LANES), F32),
        V((S, M), BF16),
        V((M // 2, D), U32),
        V((HG, Dc // 2, D), U32),
        V((S, D), BF16),
        V((HG, S // 2, D), U32),
        V((1, D // 2, S), U32),
        V((NQ, TQ, TQ), F32),
        V((NQ, TQ, TQ), F32),
        V((NQ, TQ, TQ), F32),
        V((NQ, TQ, TQ), F32),
        pltpu.SMEM((2,), jnp.int32),
        V((H, S, D), BF16),
        V((S, M), F32),
        V((S, M), F32),
        V((NC, S + 2 * PAD, LANES), F32),
        V((S, M), BF16),
        V((1, M), BF16),
        pltpu.SemaphoreType.DMA((NSEM,)),
    ]
    out = pl.pallas_call(
        kernel,
        out_shape=jax.ShapeDtypeStruct((S, M), BF16),
        in_specs=[hbm_spec] * 12,
        out_specs=hbm_spec,
        scratch_shapes=scratch,
        compiler_params=pltpu.CompilerParams(vmem_limit_bytes=120 * 1024 * 1024),
        name="adaln_cla_mixer",
    )(x2, ckv2, A_w_q, A_w_uk, A_w_uv, wo2, B_w1, B_w2, B_w3.T, B_w4, c, w_mod)
    return out.reshape(B, S, M)
```

```python
import functools
import math
import os

import jax
import jax.numpy as jnp
import jax.experimental.pallas as pl
import jax.experimental.pallas.tpu as pltpu

BF16 = jnp.bfloat16
F32 = jnp.float32
U32 = jnp.uint32

LANES = 128
TQ = 128
TR = 256
HB = 128
HG = 8
LOOK = 4
AHEAD = int(os.environ.get('AHEAD', 2))
NSB = 4
KC = 256
QC = int(os.environ.get('QC', 128))
MOD0 = int(os.environ.get('MOD0', 2))
LN0 = int(os.environ.get('LN0', 2))
KSUB = int(os.environ.get('KSUB', 1))
QH = int(os.environ.get('QH', 256))
FREE = int(os.environ.get('FREE', 0))
U2 = int(os.environ.get('U2', 2))
PC = 512
DIST = int(os.environ.get('DIST', 12))
PIN = int(os.environ.get('PIN', 0))
PAD = 16
EPS = 1e-5
LOG2E = math.log2(math.e)
NEG = -1000000000.0 * LOG2E

_NT = (((1,), (1,)), ((), ()))


def _ln(x):
    m = jnp.mean(x, axis=-1, keepdims=True)
    xc = x - m
    v = jnp.mean(xc * xc, axis=-1, keepdims=True)
    return xc * jax.lax.rsqrt(v + EPS)


def _gelu(x):
    return jax.nn.gelu(x, approximate=True)


def _dot(a, b):
    return jnp.dot(a, b, preferred_element_type=F32)


def _dot_nt(a, b):
    return jax.lax.dot_general(a, b, _NT, preferred_element_type=F32)


def _fold8(x, op):
    parts = [op(x[j:j + 8], x[j + 8:j + 16]) for j in range(0, x.shape[0], 16)]
    acc = parts[0]
    for p in parts[1:]:
        acc = op(acc, p)
    return acc


def _rows_op(op, x, v8):
    r, m = x.shape
    return op(x.reshape(r // 8, 8, m), v8[None]).reshape(r, m)


def _modulate(x, scale8, shift8):
    r, m = x.shape
    return (x.reshape(r // 8, 8, m) * scale8[None] + shift8[None]).reshape(r, m)


def _pack(x):
    return pltpu.bitcast(x.astype(BF16), U32)


def _unpack(w):
    return pltpu.bitcast(w, BF16)


def _gstride(plane):
    return -(-8 * plane // 32) * 32


def _tied(w, tie):
    return jnp.concatenate([w[0:8] | tie, w[8:]], axis=0)


def _run(*gens):
    gens = list(gens)
    while gens:
        for g in list(gens):
            if next(g, gens) is gens:
                gens.remove(g)


@jax.jit
def pallas_adaLN_cond__compressed_kv_cla__mixer_s_mlp__prompt_kernel(
    A_x: jax.Array,
    A_c_kv: jax.Array,
    A_w_q: jax.Array,
    A_w_uk: jax.Array,
    A_w_uv: jax.Array,
    A_w_o: jax.Array,
    B_x: jax.Array,
    B_w1: jax.Array,
    B_w2: jax.Array,
    B_w3: jax.Array,
    B_w4: jax.Array,
    c: jax.Array,
    w_mod: jax.Array,
):
    del B_x
    B, S, M = A_x.shape
    _, Sk, Dc = A_c_kv.shape
    _, H, D = A_w_q.shape
    Fh = B_w3.shape[1]
    assert B == 1 and Sk == S and D == LANES and H % HG == 0 and HG == 8
    assert S % TQ == 0 and S % TR == 0 and S % PC == 0 and TR % HB == 0
    assert M % LANES == 0 and M % 64 == 0 and Dc % 64 == 0
    NG = H // HG
    NQ = S // TQ
    NR = S // TR
    NC = M // LANES
    C4 = M // 4
    PLQ = M // 2 + 1
    PLK = Dc // 2 + 1
    RCH = 4
    NK = S // KC
    XC = S // RCH
    NSEM = NK + 5
    assert NK > RCH + 1
    qscale = float(D) ** -0.5 * LOG2E

    x2 = A_x.reshape(S, M)
    ckv2 = A_c_kv.reshape(S, Dc)
    wo2 = A_w_o.reshape(H * D, M)

    def kernel(x_hbm, ckv_hbm, wq_hbm, wuk_hbm, wuv_hbm, wo_hbm, w1_hbm, w2_hbm,
               w3_hbm, w4_hbm, c_hbm, wmod_hbm, out_hbm,
               x_v, ckv_v, wq_r, wuk_r, wuv_r, wq_p, wuk_p, wuv_p, wo_v, w1_v,
               w2_v, w3_v, w4_v, wmoda_v, wmodb_v, moda_v, modb_v, scb_v, hn_v, wqc_v, wk0_v, q_v, k_v,
               vt_v, s0, s1, s2, s3, z_s, ctx_v, x1_v, h2_v, hh_v, o_v, c_v,
               sems):

        s_v = (s0, s1, s2, s3)
        z_s[0] = 0
        z_s[1] = 0

        def aligned(i, n):
            return i * n if isinstance(i, int) else pl.multiple_of(i * n, n)

        def cp(src, dst, i):
            return pltpu.make_async_copy(src, dst, sems.at[i])

        def c_ckv(r):
            rows = pl.ds(aligned(r, KC), KC)
            return cp(ckv_hbm.at[rows, :], ckv_v.at[rows, :], r)

        def c_x(j):
            rows = pl.ds(aligned(j, XC), XC)
            return cp(x_hbm.at[rows, :], x_v.at[rows, :], NK - RCH + j)

        def c_q0(j):
            rows = pl.ds(aligned(j, M // RCH), M // RCH)
            return cp(wq_hbm.at[rows, pl.ds(0, HG), :], wq_r.at[0, rows], NK - RCH + j)

        def gcp(src, dst, g, i):
            return cp(src.at[:, pl.ds(g * HG, HG), :], dst.at[g], i)

        c_moda = cp(wmod_hbm.at[:, pl.ds(0, 2 * M)], wmoda_v, NK - RCH - 1)
        c_c = cp(c_hbm, c_v, NK)
        c_k0 = gcp(wuk_hbm, wuk_r, 0, NK + 1)
        c_v0 = gcp(wuv_hbm, wuv_r, 0, NK + 2)
        c_k1 = gcp(wuk_hbm, wuk_r, 1, NK + 3)
        c_late = []
        for g in range(1, NG):
            for src, dst, gg in ((wq_hbm, wq_r, g), (wuv_hbm, wuv_r, g), (wuk_hbm, wuk_r, g + 1)):
                if gg < NG:
                    c_late.append(gcp(src, dst, gg, NSEM - 1))
        for ct in range(4 * NC):
            c_late.append(cp(wmod_hbm.at[:, pl.ds(2 * M + ct * LANES, LANES)],
                             wmodb_v.at[ct], NSEM - 1))
        for src, dst in ((wo_hbm, wo_v), (w1_hbm, w1_v), (w2_hbm, w2_v),
                         (w3_hbm, w3_v), (w4_hbm, w4_v)):
            c_late.append(cp(src, dst, NSEM - 1))
        order = [c_c, c_k0] + [c_ckv(r) for r in range(NK - RCH)] + [c_moda]
        for j in range(RCH):
            order += [c_ckv(NK - RCH + j), c_x(j), c_q0(j)]
        order += [c_v0, c_k1] + c_late
        for d in order:
            d.start()

        def relayout_steps(raw, dst, g, chunk, rows, plane):
            n = rows // RCH // 2
            base = g * _gstride(plane) + chunk * n
            if not isinstance(base, int):
                base = pl.multiple_of(base, 8)
            view = dst.at[pl.ds(base, 7 * plane + n), :]

            def step(j, tie):
                val = raw[g, pl.ds(chunk * (2 * n) + 2 * j, 2)].reshape(2 * HG, D)
                val = pltpu.bitcast(val, U32)
                if tie is not None:
                    val = val | tie
                view[pl.ds(j, 8, stride=plane), :] = val

            return [functools.partial(step, j) for j in range(n)]

        def relayout(raw, dst, g, rows, plane):
            for ch in range(RCH):
                for step in relayout_steps(raw, dst, g, ch, rows, plane):
                    step(None)

        def head_w32(src, h, rows, plane):
            base = (h // HG) * _gstride(plane) + ((h % HG) // 2) * plane
            ev = src[pl.ds(base, rows // 2), :]
            od = src[pl.ds(base + 4 * plane, rows // 2), :]
            if not isinstance(h, int):
                par = (h % 2).astype(U32)
                w = (((ev >> (16 * par)) & U32(0xFFFF))
                     | ((od << (16 * (1 - par))) & U32(0xFFFF0000)))
            elif h % 2 == 0:
                w = (ev & U32(0xFFFF)) | (od << 16)
            else:
                w = (ev >> 16) | (od & U32(0xFFFF0000))
            return w

        def head_w(src, h, rows, plane):
            return pltpu.bitcast(head_w32(src, h, rows, plane), BF16)

        def q_rows(wq, lo, hi, ties=()):
            res = []
            for r0 in range(lo, hi, QC):
                rows = slice(r0, r0 + QC)
                w = _tied(wq, ties[len(res)]) if len(res) in ties else wq
                res.append(_dot(hn_v[rows, :], pltpu.bitcast(w, BF16)))
                q_v[rows, :] = (res[-1] * qscale).astype(BF16)
            return res

        def q_head(h):
            wq = head_w32(wq_p, h, M, PLQ)
            wqc_v[...] = wq
            return wq, q_rows(wq, 0, QH)

        def q_mid(ties=()):
            q_rows(wqc_v[...], QH, S - PC, ties)

        def q_tail():
            return q_rows(wqc_v[...], S - PC, S)

        def k_proj(h, kh):
            wk = head_w(wuk_p, h, Dc, PLK)
            for r in range(S // PC):
                rows = slice(r * PC, (r + 1) * PC)
                kh[r * PC // 2:(r + 1) * PC // 2, :] = _pack(_dot(ckv_v[rows, :], wk))

        def mod_tile(w):
            acc = _fold8(w.astype(F32) * scb_v[...], jnp.add)
            return jnp.broadcast_to(jnp.sum(acc, axis=0, keepdims=True), (8, LANES))

        def mod(i):
            if i < 2:
                return moda_v[0:8, i * M:(i + 1) * M]
            return jnp.concatenate(
                [modb_v[(i - 2) * NC + ct] for ct in range(NC)], axis=1)

        def zeros8():
            return jnp.full((8, LANES), z_s[1], jnp.int32).astype(U32)

        def k_chunk(r, nsub=1, ties=(), after=None, unpack=False):
            n = KC // nsub
            lhs = ckv_v[pl.ds(aligned(r, KC), KC), :]
            for h in range(HG):
                if unpack:
                    w32 = head_w32(wuk_p, h, Dc, PLK)
                    wk0_v[h] = w32
                else:
                    w32 = wk0_v[h]
                for j in range(nsub):
                    i = h * nsub + j
                    rows = pl.ds(aligned(r * nsub + j, n // 2), n // 2)
                    w = _tied(w32, ties[i]) if i in ties else w32
                    res = _dot(lhs[j * n:(j + 1) * n], pltpu.bitcast(w, BF16))
                    k_v[h, rows, :] = _pack(res)
                    if after is not None:
                        after(i, res)

        c_c.wait()
        cc = c_v[...].astype(F32)
        sc = (cc * jax.nn.sigmoid(cc)).astype(BF16).astype(F32)
        scb_v[...] = jnp.broadcast_to(sc, (LANES, M)).T
        zpad = jnp.zeros((PAD, LANES), F32)
        for cidx in range(NC):
            hh_v[cidx, 0:PAD, :] = zpad
            hh_v[cidx, PAD + S:PAD + S + PAD, :] = zpad
        c_k0.wait()
        relayout(wuk_r, wuk_p, 0, Dc, PLK)

        def ka_body(r, carry):
            c_ckv(r).wait()
            k_chunk(r, unpack=True)
            return carry

        jax.lax.fori_loop(0, NK - RCH - 1, ka_body, 0)

        c_ckv(NK - RCH - 1).wait()
        c_moda.wait()
        zero8 = zeros8()
        ties = {}
        for ct in range(2 * NC):
            cols = slice(ct * LANES, (ct + 1) * LANES)
            tile = mod_tile(wmoda_v[:, cols])
            moda_v[0:8, cols] = tile
            ties[MOD0 + (ct * (2 * HG - MOD0)) // (2 * NC)] = pltpu.bitcast(tile, U32) & zero8
        k_chunk(NK - RCH - 1, 2, ties)

        def kb_body(j, carry):
            c_ckv(NK - RCH + j).wait()
            c_x(j).wait()
            c_q0(j).wait()
            zero8 = zeros8()
            nstep = KSUB * HG
            lr = XC // nstep
            ties = {}
            scale, shift = 1.0 + mod(1), mod(0)
            for i in range(nstep):
                rows = pl.ds(pl.multiple_of(j * XC + i * lr, lr), lr)
                hn = _modulate(_ln(x_v[rows, :].astype(F32)), scale, shift)
                hn_v[rows, :] = hn.astype(BF16)
                ties[i + LN0] = pltpu.bitcast(_fold8(hn[:, 0:LANES], jnp.maximum), U32) & zero8
            steps = relayout_steps(wq_r, wq_p, 0, j, M, PLQ)
            per = len(steps) // nstep

            def side(i, res):
                for k, step in enumerate(steps[i * per:(i + 1) * per]):
                    step(pltpu.bitcast(res[k * 8:(k + 1) * 8], U32) & zero8)

            k_chunk(NK - RCH + j, KSUB, ties, side)
            return carry

        jax.lax.fori_loop(0, RCH, kb_body, 0)

        c_v0.wait()
        zero8 = zeros8()
        wq0, res = q_head(0)
        res = jnp.concatenate(res, axis=0)
        steps = []
        for ch in range(RCH):
            steps += relayout_steps(wuv_r, wuv_p, 0, ch, Dc, PLK)
        for i, step in enumerate(steps):
            if i < FREE:
                step(wq0[0:8] & zero8)
            else:
                k = (i - FREE) * (QH // 8) // (len(steps) - FREE)
                step(pltpu.bitcast(res[k * 8:(k + 1) * 8], U32) & zero8)

        def attention(h, kh, side):
            key_i = jax.lax.broadcasted_iota(jnp.int32, (TQ, TQ), 0)
            qry_i = jax.lax.broadcasted_iota(jnp.int32, (TQ, TQ), 1)
            causal = key_i <= qry_i
            z_st = z_s[0]
            z_ld = z_s[1]
            zero8 = zeros8()

            mx = {}
            seq = []

            def qk(i):
                qi = q_v[i * TQ:(i + 1) * TQ, :]
                sb = s_v[i % NSB]
                m8 = None
                for t in range(i + 1):
                    tile = _dot_nt(_unpack(kh[t * TQ // 2:(t + 1) * TQ // 2, :]), qi)
                    seq.append(tile[0:8])
                    if t == i:
                        tile = jnp.where(causal, tile, NEG)
                    sb[z_st + t] = tile
                    tm = _fold8(tile, jnp.maximum)
                    m8 = tm if m8 is None else jnp.maximum(m8, tm)
                    if t == i:
                        mx[i] = jnp.max(m8, axis=0, keepdims=True)
                    yield

            parts = []

            def pv(i):
                sb = s_v[i % NSB]
                m8 = jnp.broadcast_to(mx[i], (8, TQ))
                l8 = None
                ot = None
                for t in range(i + 1):
                    tie = pltpu.bitcast(seq[-DIST], U32)
                    if PIN and len(parts) >= PIN:
                        tie = tie | pltpu.bitcast(parts[-PIN], U32)
                    mt = pltpu.bitcast(pltpu.bitcast(m8, U32) | (tie & zero8), F32)
                    tile = sb[z_ld + t].reshape(TQ // 8, 8, TQ)
                    p = jnp.exp2(tile - mt[None]).reshape(TQ, TQ)
                    part = _fold8(p, jnp.add)
                    l8 = part if l8 is None else l8 + part
                    parts.append(l8)
                    o = _dot(_unpack(vt_v[z_ld, :, t * TQ:(t + 1) * TQ]), p.astype(BF16))
                    seq.append(o[0:8])
                    ot = o if ot is None else ot + o
                    if t == i:
                        l = jnp.sum(l8, axis=0, keepdims=True)
                        ot = ot * (1.0 / l)
                        ctx_v[h, i * TQ:(i + 1) * TQ, :] = ot.T.astype(BF16)
                    yield

            for i in range(LOOK):
                _run(qk(i))
            vt = _dot_nt(head_w(wuv_p, h, Dc, PLK).T, ckv_v[...])
            vt_v[z_st] = _pack(vt)
            prev = vt[0:8, S - TQ:S]
            for res in q_tail():
                seq.extend([prev] * NC)
                prev = res[0:8]
            per = max(1, -(-len(side) // NQ))
            for j, step in enumerate(side):
                ct, rg = j // per, (j % per) * (D // 8) // per
                src = vt[rg * 8:(rg + 1) * 8, ct * TQ:(ct + 1) * TQ]
                step(pltpu.bitcast(src, U32) & zero8)
            for i in range(NQ):
                j = i + AHEAD
                if LOOK <= j < NQ:
                    _run(qk(j), pv(i))
                else:
                    _run(pv(i))

        def side_work(h):
            g = h // HG + ((h % HG) >= RCH).astype(jnp.int32)
            ch = h % RCH
            steps = (relayout_steps(wq_r, wq_p, g, ch, M, PLQ)
                     + relayout_steps(wuv_r, wuv_p, g, ch, Dc, PLK))
            for c in range(RCH):
                steps += relayout_steps(wuk_r, wuk_p, h // HG + 1, c, Dc, PLK)
            return steps

        def head_body(h, carry):
            @pl.when(h == RCH)
            def _():
                for d in c_late:
                    d.wait()

            kh = k_v.at[h % HG]
            q_mid()
            attention(h, kh, side_work(h))
            q_head(h + 1)
            k_proj(h + HG, kh)
            return carry

        c_k1.wait()
        jax.lax.fori_loop(0, H - HG, head_body, 0)

        def last_body(h, carry):
            per = -(-4 * NC // HG)
            zero8 = zeros8()
            ties = {}
            for i in range(per):
                ct = jnp.minimum((h - (H - HG)) * per + i, 4 * NC - 1)
                tile = mod_tile(wmodb_v[ct])
                modb_v[ct] = tile
                ties[2 * i + 3] = pltpu.bitcast(tile, U32) & zero8
            q_mid(ties)
            attention(h, k_v.at[h % HG], ())
            q_head(jnp.minimum(h + 1, H - 1))
            return carry

        jax.lax.fori_loop(H - HG, H, last_body, 0)

        def sub_rows(r):
            out = []
            for j in range(TR // HB):
                r0 = r * TR + j * HB
                if not isinstance(r0, int):
                    r0 = pl.multiple_of(r0, HB)
                out.append(r0)
            return out

        def stage1(r):
            lns = []
            for r0 in sub_rows(r):
                rows = pl.ds(r0, HB)
                ctx = jnp.concatenate([ctx_v[h, rows, :] for h in range(H)], axis=1)
                att = _dot(ctx, wo_v[...])
                x1 = x_v[rows, :].astype(F32) + _rows_op(jnp.multiply, att, mod(2))
                x1_v[rows, :] = x1
                h2 = _modulate(_ln(x1), 1.0 + mod(4), mod(3))
                h2_v[rows, :] = h2
                lns.append(_ln(h2).astype(BF16))
            for r0, ln in zip(sub_rows(r), lns):
                u = _gelu(_dot(ln, w1_v[...]))
                for cidx in range(NC):
                    hh_v[cidx, pl.ds(r0 + PAD, HB), :] = u[:, cidx * LANES:(cidx + 1) * LANES]

        shifts = (1, -1, 2, -2)

        def out_cp(r0):
            rows = pl.ds(r0, HB)
            return cp(o_v.at[rows, :], out_hbm.at[rows, :], 0)

        def stage2(r):
            lane_i = jax.lax.broadcasted_iota(jnp.int32, (HB, LANES), 1)
            y1s = []
            for r0 in sub_rows(r):
                tiles = []
                for cidx in range(NC):
                    lo, hi = cidx * LANES, (cidx + 1) * LANES
                    g_lo, g_hi = lo // C4, (hi - 1) // C4
                    t = hh_v[cidx, pl.ds(r0 + PAD - shifts[g_hi], HB), :]
                    for g in range(g_hi - 1, g_lo - 1, -1):
                        tg = hh_v[cidx, pl.ds(r0 + PAD - shifts[g], HB), :]
                        t = jnp.where(lane_i < (g + 1) * C4 - lo, tg, t)
                    tiles.append(t)
                hs = _dot(jnp.concatenate(tiles, axis=1).astype(BF16), w2_v[...])
                y1s.append(h2_v[pl.ds(r0, HB), :] + hs)
            gls = [_gelu(_dot_nt(_ln(y1).astype(BF16), w3_v[...])).astype(BF16)
                   for y1 in y1s]
            for r0, y1, gl in zip(sub_rows(r), y1s, gls):
                rows = pl.ds(r0, HB)
                h3 = _dot(gl, w4_v[...])
                o_v[rows, :] = (x1_v[rows, :]
                                + _rows_op(jnp.multiply, y1 + h3, mod(5))).astype(BF16)
                out_cp(r0).start()

        def s1_body(r, carry):
            stage1(r)
            return carry

        def s2_body(r, carry):
            for u in range(U2):
                stage2(r * U2 + u)
            return carry

        jax.lax.fori_loop(0, NR, s1_body, 0)
        jax.lax.fori_loop(0, NR // U2, s2_body, 0)
        cp(o_v, out_hbm, 0).wait()

    hbm_spec = pl.BlockSpec(memory_space=pltpu.HBM)
    V = pltpu.VMEM
    scratch = [
        V((S, M), BF16),
        V((S, Dc), BF16),
        V((NG, M, HG, D), BF16),
        V((NG, Dc, HG, D), BF16),
        V((NG, Dc, HG, D), BF16),
        V((NG * _gstride(PLQ), D), U32),
        V((NG * _gstride(PLK), D), U32),
        V((NG * _gstride(PLK), D), U32),
        V((H * D, M), BF16),
        V((M, M), BF16),
        V((M, M), BF16),
        V((Fh, M), BF16),
        V((Fh, M), BF16),
        V((M, 2 * M), BF16),
        V((4 * NC, M, LANES), BF16),
        V((16, 2 * M), F32),
        V((4 * NC, 8, LANES), F32),
        V((M, LANES), F32),
        V((S, M), BF16),
        V((M // 2, D), U32),
        V((HG, Dc // 2, D), U32),
        V((S, D), BF16),
        V((HG, S // 2, D), U32),
        V((1, D // 2, S), U32),
        V((NQ, TQ, TQ), F32),
        V((NQ, TQ, TQ), F32),
        V((NQ, TQ, TQ), F32),
        V((NQ, TQ, TQ), F32),
        pltpu.SMEM((2,), jnp.int32),
        V((H, S, D), BF16),
        V((S, M), F32),
        V((S, M), F32),
        V((NC, S + 2 * PAD, LANES), F32),
        V((S, M), BF16),
        V((1, M), BF16),
        pltpu.SemaphoreType.DMA((NSEM,)),
    ]
    out = pl.pallas_call(
        kernel,
        out_shape=jax.ShapeDtypeStruct((S, M), BF16),
        in_specs=[hbm_spec] * 12,
        out_specs=hbm_spec,
        scratch_shapes=scratch,
        compiler_params=pltpu.CompilerParams(vmem_limit_bytes=120 * 1024 * 1024),
        name="adaln_cla_mixer",
    )(x2, ckv2, A_w_q, A_w_uk, A_w_uv, wo2, B_w1, B_w2, B_w3.T, B_w4, c, w_mod)
    return out.reshape(B, S, M)
```

```python
import functools
import math
import os

import jax
import jax.numpy as jnp
import jax.experimental.pallas as pl
import jax.experimental.pallas.tpu as pltpu

BF16 = jnp.bfloat16
F32 = jnp.float32
U32 = jnp.uint32

LANES = 128
TQ = 128
TR = 256
HB = 128
HG = 8
LOOK = 4
AHEAD = int(os.environ.get('AHEAD', 2))
NSB = 4
KC = 256
QC = int(os.environ.get('QC', 128))
MOD0 = int(os.environ.get('MOD0', 2))
LN0 = int(os.environ.get('LN0', 2))
KSUB = int(os.environ.get('KSUB', 1))
QH = int(os.environ.get('QH', 256))
FREE = int(os.environ.get('FREE', 0))
U2 = int(os.environ.get('U2', 2))
PC = 512
DIST = int(os.environ.get('DIST', 12))
PIN = int(os.environ.get('PIN', 0))
PAD = 16
EPS = 1e-5
LOG2E = math.log2(math.e)
NEG = -1000000000.0 * LOG2E

_NT = (((1,), (1,)), ((), ()))


def _ln(x):
    m = jnp.mean(x, axis=-1, keepdims=True)
    xc = x - m
    v = jnp.mean(xc * xc, axis=-1, keepdims=True)
    return xc * jax.lax.rsqrt(v + EPS)


def _gelu(x):
    return jax.nn.gelu(x, approximate=True)


def _dot(a, b):
    return jnp.dot(a, b, preferred_element_type=F32)


def _dot_nt(a, b):
    return jax.lax.dot_general(a, b, _NT, preferred_element_type=F32)


def _fold8(x, op):
    parts = [op(x[j:j + 8], x[j + 8:j + 16]) for j in range(0, x.shape[0], 16)]
    acc = parts[0]
    for p in parts[1:]:
        acc = op(acc, p)
    return acc


def _rows_op(op, x, v8):
    r, m = x.shape
    return op(x.reshape(r // 8, 8, m), v8[None]).reshape(r, m)


def _modulate(x, scale8, shift8):
    r, m = x.shape
    return (x.reshape(r // 8, 8, m) * scale8[None] + shift8[None]).reshape(r, m)


def _pack(x):
    return pltpu.bitcast(x.astype(BF16), U32)


def _unpack(w):
    return pltpu.bitcast(w, BF16)


def _gstride(plane):
    return -(-8 * plane // 32) * 32


def _tied(w, tie):
    return jnp.concatenate([w[0:8] | tie, w[8:]], axis=0)


def _run(*gens):
    gens = list(gens)
    while gens:
        for g in list(gens):
            if next(g, gens) is gens:
                gens.remove(g)


@jax.jit
def pallas_adaLN_cond__compressed_kv_cla__mixer_s_mlp__prompt_kernel(
    A_x: jax.Array,
    A_c_kv: jax.Array,
    A_w_q: jax.Array,
    A_w_uk: jax.Array,
    A_w_uv: jax.Array,
    A_w_o: jax.Array,
    B_x: jax.Array,
    B_w1: jax.Array,
    B_w2: jax.Array,
    B_w3: jax.Array,
    B_w4: jax.Array,
    c: jax.Array,
    w_mod: jax.Array,
):
    del B_x
    B, S, M = A_x.shape
    _, Sk, Dc = A_c_kv.shape
    _, H, D = A_w_q.shape
    Fh = B_w3.shape[1]
    assert B == 1 and Sk == S and D == LANES and H % HG == 0 and HG == 8
    assert S % TQ == 0 and S % TR == 0 and S % PC == 0 and TR % HB == 0
    assert M % LANES == 0 and M % 64 == 0 and Dc % 64 == 0
    NG = H // HG
    NQ = S // TQ
    NR = S // TR
    NC = M // LANES
    C4 = M // 4
    PLQ = M // 2 + 1
    PLK = Dc // 2 + 1
    RCH = 4
    NK = S // KC
    XC = S // RCH
    NSEM = NK + 5
    assert NK > RCH + 1
    qscale = float(D) ** -0.5 * LOG2E

    x2 = A_x.reshape(S, M)
    ckv2 = A_c_kv.reshape(S, Dc)
    wo2 = A_w_o.reshape(H * D, M)

    def kernel(x_hbm, ckv_hbm, wq_hbm, wuk_hbm, wuv_hbm, wo_hbm, w1_hbm, w2_hbm,
               w3_hbm, w4_hbm, c_hbm, wmod_hbm, out_hbm,
               x_v, ckv_v, wq_r, wuk_r, wuv_r, wq_p, wuk_p, wuv_p, wo_v, w1_v,
               w2_v, w3_v, w4_v, wmoda_v, wmodb_v, moda_v, modb_v, scb_v, hn_v, wqc_v, wk0_v, q_v, k_v,
               vt_v, s0, s1, s2, s3, z_s, ctx_v, x1_v, h2_v, hh_v, o_v, c_v,
               sems):

        s_v = (s0, s1, s2, s3)
        z_s[0] = 0
        z_s[1] = 0

        def aligned(i, n):
            return i * n if isinstance(i, int) else pl.multiple_of(i * n, n)

        def cp(src, dst, i):
            return pltpu.make_async_copy(src, dst, sems.at[i])

        def c_ckv(r):
            rows = pl.ds(aligned(r, KC), KC)
            return cp(ckv_hbm.at[rows, :], ckv_v.at[rows, :], r)

        def c_x(j):
            rows = pl.ds(aligned(j, XC), XC)
            return cp(x_hbm.at[rows, :], x_v.at[rows, :], NK - RCH + j)

        def c_q0(j):
            rows = pl.ds(aligned(j, M // RCH), M // RCH)
            return cp(wq_hbm.at[rows, pl.ds(0, HG), :], wq_r.at[0, rows], NK - RCH + j)

        def gcp(src, dst, g, i):
            return cp(src.at[:, pl.ds(g * HG, HG), :], dst.at[g], i)

        c_moda = cp(wmod_hbm.at[:, pl.ds(0, 2 * M)], wmoda_v, NK - RCH - 1)
        c_c = cp(c_hbm, c_v, NK)
        c_k0 = gcp(wuk_hbm, wuk_r, 0, NK + 1)
        c_v0 = gcp(wuv_hbm, wuv_r, 0, NK + 2)
        c_k1 = gcp(wuk_hbm, wuk_r, 1, NK + 3)
        c_late = []
        for g in range(1, NG):
            for src, dst, gg in ((wq_hbm, wq_r, g), (wuv_hbm, wuv_r, g), (wuk_hbm, wuk_r, g + 1)):
                if gg < NG:
                    c_late.append(gcp(src, dst, gg, NSEM - 1))
        for ct in range(4 * NC):
            c_late.append(cp(wmod_hbm.at[:, pl.ds(2 * M + ct * LANES, LANES)],
                             wmodb_v.at[ct], NSEM - 1))
        for src, dst in ((wo_hbm, wo_v), (w1_hbm, w1_v), (w2_hbm, w2_v),
                         (w3_hbm, w3_v), (w4_hbm, w4_v)):
            c_late.append(cp(src, dst, NSEM - 1))
        order = [c_c, c_k0] + [c_ckv(r) for r in range(NK - RCH)] + [c_moda]
        for j in range(RCH):
            order += [c_ckv(NK - RCH + j), c_x(j), c_q0(j)]
        order += [c_v0, c_k1] + c_late
        for d in order:
            d.start()

        def relayout_steps(raw, dst, g, chunk, rows, plane):
            n = rows // RCH // 2
            base = g * _gstride(plane) + chunk * n
            if not isinstance(base, int):
                base = pl.multiple_of(base, 8)
            view = dst.at[pl.ds(base, 7 * plane + n), :]

            def step(j, tie):
                val = raw[g, pl.ds(chunk * (2 * n) + 2 * j, 2)].reshape(2 * HG, D)
                val = pltpu.bitcast(val, U32)
                if tie is not None:
                    val = val | tie
                view[pl.ds(j, 8, stride=plane), :] = val

            return [functools.partial(step, j) for j in range(n)]

        def relayout(raw, dst, g, rows, plane):
            for ch in range(RCH):
                for step in relayout_steps(raw, dst, g, ch, rows, plane):
                    step(None)

        def head_w32(src, h, rows, plane):
            base = (h // HG) * _gstride(plane) + ((h % HG) // 2) * plane
            ev = src[pl.ds(base, rows // 2), :]
            od = src[pl.ds(base + 4 * plane, rows // 2), :]
            if not isinstance(h, int):
                par = (h % 2).astype(U32)
                w = (((ev >> (16 * par)) & U32(0xFFFF))
                     | ((od << (16 * (1 - par))) & U32(0xFFFF0000)))
            elif h % 2 == 0:
                w = (ev & U32(0xFFFF)) | (od << 16)
            else:
                w = (ev >> 16) | (od & U32(0xFFFF0000))
            return w

        def head_w(src, h, rows, plane):
            return pltpu.bitcast(head_w32(src, h, rows, plane), BF16)

        def q_rows(wq, lo, hi, ties=()):
            res = []
            for r0 in range(lo, hi, QC):
                rows = slice(r0, r0 + QC)
                w = _tied(wq, ties[len(res)]) if len(res) in ties else wq
                res.append(_dot(hn_v[rows, :], pltpu.bitcast(w, BF16)))
                q_v[rows, :] = (res[-1] * qscale).astype(BF16)
            return res

        def q_head(h):
            wq = head_w32(wq_p, h, M, PLQ)
            wqc_v[...] = wq
            return wq, q_rows(wq, 0, QH)

        def q_mid(ties=()):
            q_rows(wqc_v[...], QH, S - PC, ties)

        def q_tail():
            return q_rows(wqc_v[...], S - PC, S)

        def k_proj(h, kh):
            wk = head_w(wuk_p, h, Dc, PLK)
            for r in range(S // PC):
                rows = slice(r * PC, (r + 1) * PC)
                kh[r * PC // 2:(r + 1) * PC // 2, :] = _pack(_dot(ckv_v[rows, :], wk))

        def mod_tile(w):
            acc = _fold8(w.astype(F32) * scb_v[...], jnp.add)
            return jnp.broadcast_to(jnp.sum(acc, axis=0, keepdims=True), (8, LANES))

        def mod(i):
            if i < 2:
                return moda_v[0:8, i * M:(i + 1) * M]
            return jnp.concatenate(
                [modb_v[(i - 2) * NC + ct] for ct in range(NC)], axis=1)

        def zeros8():
            return jnp.full((8, LANES), z_s[1], jnp.int32).astype(U32)

        def k_chunk(r, nsub=1, ties=(), after=None, unpack=False):
            n = KC // nsub
            lhs = ckv_v[pl.ds(aligned(r, KC), KC), :]
            for h in range(HG):
                if unpack:
                    w32 = head_w32(wuk_p, h, Dc, PLK)
                    wk0_v[h] = w32
                else:
                    w32 = wk0_v[h]
                for j in range(nsub):
                    i = h * nsub + j
                    rows = pl.ds(aligned(r * nsub + j, n // 2), n // 2)
                    w = _tied(w32, ties[i]) if i in ties else w32
                    res = _dot(lhs[j * n:(j + 1) * n], pltpu.bitcast(w, BF16))
                    k_v[h, rows, :] = _pack(res)
                    if after is not None:
                        after(i, res)

        c_c.wait()
        cc = c_v[...].astype(F32)
        sc = (cc * jax.nn.sigmoid(cc)).astype(BF16).astype(F32)
        scb_v[...] = jnp.broadcast_to(sc, (LANES, M)).T
        zpad = jnp.zeros((PAD, LANES), F32)
        for cidx in range(NC):
            hh_v[cidx, 0:PAD, :] = zpad
            hh_v[cidx, PAD + S:PAD + S + PAD, :] = zpad
        c_k0.wait()
        relayout(wuk_r, wuk_p, 0, Dc, PLK)

        def ka_body(r, carry):
            c_ckv(r).wait()
            k_chunk(r, unpack=True)
            return carry

        jax.lax.fori_loop(0, NK - RCH - 1, ka_body, 0)

        c_ckv(NK - RCH - 1).wait()
        c_moda.wait()
        zero8 = zeros8()
        ties = {}
        for ct in range(2 * NC):
            cols = slice(ct * LANES, (ct + 1) * LANES)
            tile = mod_tile(wmoda_v[:, cols])
            moda_v[0:8, cols] = tile
            ties[MOD0 + (ct * (2 * HG - MOD0)) // (2 * NC)] = pltpu.bitcast(tile, U32) & zero8
        k_chunk(NK - RCH - 1, 2, ties)

        def kb_body(j, carry):
            c_ckv(NK - RCH + j).wait()
            c_x(j).wait()
            c_q0(j).wait()
            zero8 = zeros8()
            nstep = KSUB * HG
            lr = XC // nstep
            ties = {}
            scale, shift = 1.0 + mod(1), mod(0)
            for i in range(nstep):
                rows = pl.ds(pl.multiple_of(j * XC + i * lr, lr), lr)
                hn = _modulate(_ln(x_v[rows, :].astype(F32)), scale, shift)
                hn_v[rows, :] = hn.astype(BF16)
                ties[i + LN0] = pltpu.bitcast(_fold8(hn[:, 0:LANES], jnp.maximum), U32) & zero8
            steps = relayout_steps(wq_r, wq_p, 0, j, M, PLQ)
            per = len(steps) // nstep

            def side(i, res):
                for k, step in enumerate(steps[i * per:(i + 1) * per]):
                    step(pltpu.bitcast(res[k * 8:(k + 1) * 8], U32) & zero8)

            k_chunk(NK - RCH + j, KSUB, ties, side)
            return carry

        jax.lax.fori_loop(0, RCH, kb_body, 0)

        c_v0.wait()
        zero8 = zeros8()
        wq0, res = q_head(0)
        res = jnp.concatenate(res, axis=0)
        steps = []
        for ch in range(RCH):
            steps += relayout_steps(wuv_r, wuv_p, 0, ch, Dc, PLK)
        for i, step in enumerate(steps):
            if i < FREE:
                step(wq0[0:8] & zero8)
            else:
                k = (i - FREE) * (QH // 8) // (len(steps) - FREE)
                step(pltpu.bitcast(res[k * 8:(k + 1) * 8], U32) & zero8)

        def attention(h, kh, side):
            key_i = jax.lax.broadcasted_iota(jnp.int32, (TQ, TQ), 0)
            qry_i = jax.lax.broadcasted_iota(jnp.int32, (TQ, TQ), 1)
            causal = key_i <= qry_i
            z_st = z_s[0]
            z_ld = z_s[1]
            zero8 = zeros8()

            mx = {}
            seq = []

            def qk(i):
                qi = q_v[i * TQ:(i + 1) * TQ, :]
                sb = s_v[i % NSB]
                m8 = None
                for t in range(i + 1):
                    tile = _dot_nt(_unpack(kh[t * TQ // 2:(t + 1) * TQ // 2, :]), qi)
                    seq.append(tile[0:8])
                    if t == i:
                        tile = jnp.where(causal, tile, NEG)
                    sb[z_st + t] = tile
                    tm = _fold8(tile, jnp.maximum)
                    m8 = tm if m8 is None else jnp.maximum(m8, tm)
                    if t == i:
                        mx[i] = jnp.max(m8, axis=0, keepdims=True)
                    yield

            parts = []

            def pv(i):
                sb = s_v[i % NSB]
                m8 = jnp.broadcast_to(mx[i], (8, TQ))
                l8 = None
                ot = None
                for t in range(i + 1):
                    tie = pltpu.bitcast(seq[-DIST], U32)
                    if PIN and len(parts) >= PIN:
                        tie = tie | pltpu.bitcast(parts[-PIN], U32)
                    mt = pltpu.bitcast(pltpu.bitcast(m8, U32) | (tie & zero8), F32)
                    tile = sb[z_ld + t].reshape(TQ // 8, 8, TQ)
                    p = jnp.exp2(tile - mt[None]).reshape(TQ, TQ)
                    part = _fold8(p, jnp.add)
                    l8 = part if l8 is None else l8 + part
                    parts.append(l8)
                    o = _dot(_unpack(vt_v[z_ld, :, t * TQ:(t + 1) * TQ]), p.astype(BF16))
                    seq.append(o[0:8])
                    ot = o if ot is None else ot + o
                    if t == i:
                        l = jnp.sum(l8, axis=0, keepdims=True)
                        ot = ot * (1.0 / l)
                        ctx_v[h, i * TQ:(i + 1) * TQ, :] = ot.T.astype(BF16)
                    yield

            for i in range(LOOK):
                _run(qk(i))
            vt = _dot_nt(head_w(wuv_p, h, Dc, PLK).T, ckv_v[...])
            vt_v[z_st] = _pack(vt)
            prev = vt[0:8, S - TQ:S]
            for res in q_tail():
                seq.extend([prev] * NC)
                prev = res[0:8]
            per = max(1, -(-len(side) // NQ))
            for j, step in enumerate(side):
                ct, rg = j // per, (j % per) * (D // 8) // per
                src = vt[rg * 8:(rg + 1) * 8, ct * TQ:(ct + 1) * TQ]
                step(pltpu.bitcast(src, U32) & zero8)
            for i in range(NQ):
                j = i + AHEAD
                if LOOK <= j < NQ:
                    _run(qk(j), pv(i))
                else:
                    _run(pv(i))

        def side_work(h):
            g = h // HG + ((h % HG) >= RCH).astype(jnp.int32)
            ch = h % RCH
            steps = (relayout_steps(wq_r, wq_p, g, ch, M, PLQ)
                     + relayout_steps(wuv_r, wuv_p, g, ch, Dc, PLK))
            for c in range(RCH):
                steps += relayout_steps(wuk_r, wuk_p, h // HG + 1, c, Dc, PLK)
            return steps

        def head_body(h, carry):
            @pl.when(h == RCH)
            def _():
                for d in c_late:
                    d.wait()

            kh = k_v.at[h % HG]
            q_mid()
            attention(h, kh, side_work(h))
            q_head(h + 1)
            k_proj(h + HG, kh)
            return carry

        c_k1.wait()
        jax.lax.fori_loop(0, H - HG, head_body, 0)

        def last_body(h, carry):
            per = -(-4 * NC // HG)
            zero8 = zeros8()
            ties = {}
            for i in range(per):
                ct = jnp.minimum((h - (H - HG)) * per + i, 4 * NC - 1)
                tile = mod_tile(wmodb_v[ct])
                modb_v[ct] = tile
                ties[2 * i + 3] = pltpu.bitcast(tile, U32) & zero8
            q_mid(ties)
            attention(h, k_v.at[h % HG], ())
            q_head(jnp.minimum(h + 1, H - 1))
            return carry

        jax.lax.fori_loop(H - HG, H, last_body, 0)

        def sub_rows(r):
            out = []
            for j in range(TR // HB):
                r0 = r * TR + j * HB
                if not isinstance(r0, int):
                    r0 = pl.multiple_of(r0, HB)
                out.append(r0)
            return out

        def stage1(r):
            lns = []
            for r0 in sub_rows(r):
                rows = pl.ds(r0, HB)
                ctx = jnp.concatenate([ctx_v[h, rows, :] for h in range(H)], axis=1)
                att = _dot(ctx, wo_v[...])
                x1 = x_v[rows, :].astype(F32) + _rows_op(jnp.multiply, att, mod(2))
                x1_v[rows, :] = x1
                h2 = _modulate(_ln(x1), 1.0 + mod(4), mod(3))
                h2_v[rows, :] = h2
                lns.append(_ln(h2).astype(BF16))
            for r0, ln in zip(sub_rows(r), lns):
                u = _gelu(_dot(ln, w1_v[...]))
                for cidx in range(NC):
                    hh_v[cidx, pl.ds(r0 + PAD, HB), :] = u[:, cidx * LANES:(cidx + 1) * LANES]

        shifts = (1, -1, 2, -2)

        def out_cp(r0):
            rows = pl.ds(r0, HB)
            return cp(o_v.at[rows, :], out_hbm.at[rows, :], 0)

        def stage2(r):
            lane_i = jax.lax.broadcasted_iota(jnp.int32, (HB, LANES), 1)
            y1s = []
            for r0 in sub_rows(r):
                tiles = []
                for cidx in range(NC):
                    lo, hi = cidx * LANES, (cidx + 1) * LANES
                    g_lo, g_hi = lo // C4, (hi - 1) // C4
                    t = hh_v[cidx, pl.ds(r0 + PAD - shifts[g_hi], HB), :]
                    for g in range(g_hi - 1, g_lo - 1, -1):
                        tg = hh_v[cidx, pl.ds(r0 + PAD - shifts[g], HB), :]
                        t = jnp.where(lane_i < (g + 1) * C4 - lo, tg, t)
                    tiles.append(t)
                hs = _dot(jnp.concatenate(tiles, axis=1).astype(BF16), w2_v[...])
                y1s.append(h2_v[pl.ds(r0, HB), :] + hs)
            gls = []
            f0 = Fh // LANES * LANES
            for y1 in y1s:
                ln = _ln(y1).astype(BF16)
                parts = [_gelu(_dot_nt(ln, w3_v[0:f0 // 2 // LANES * LANES, :]))]
                if f0 < Fh:
                    tail = _gelu(_dot_nt(w3_v[f0:Fh, :], ln)).T
                parts.append(_gelu(_dot_nt(ln, w3_v[f0 // 2 // LANES * LANES:f0, :])))
                if f0 < Fh:
                    parts.append(tail)
                gls.append(jnp.concatenate(parts, axis=1).astype(BF16))
            for r0, y1, gl in zip(sub_rows(r), y1s, gls):
                rows = pl.ds(r0, HB)
                h3 = _dot(gl, w4_v[...])
                o_v[rows, :] = (x1_v[rows, :]
                                + _rows_op(jnp.multiply, y1 + h3, mod(5))).astype(BF16)
                out_cp(r0).start()

        def s1_body(r, carry):
            stage1(r)
            return carry

        def s2_body(r, carry):
            for u in range(U2):
                stage2(r * U2 + u)
            return carry

        jax.lax.fori_loop(0, NR, s1_body, 0)
        jax.lax.fori_loop(0, NR // U2, s2_body, 0)
        cp(o_v, out_hbm, 0).wait()

    hbm_spec = pl.BlockSpec(memory_space=pltpu.HBM)
    V = pltpu.VMEM
    scratch = [
        V((S, M), BF16),
        V((S, Dc), BF16),
        V((NG, M, HG, D), BF16),
        V((NG, Dc, HG, D), BF16),
        V((NG, Dc, HG, D), BF16),
        V((NG * _gstride(PLQ), D), U32),
        V((NG * _gstride(PLK), D), U32),
        V((NG * _gstride(PLK), D), U32),
        V((H * D, M), BF16),
        V((M, M), BF16),
        V((M, M), BF16),
        V((Fh, M), BF16),
        V((Fh, M), BF16),
        V((M, 2 * M), BF16),
        V((4 * NC, M, LANES), BF16),
        V((16, 2 * M), F32),
        V((4 * NC, 8, LANES), F32),
        V((M, LANES), F32),
        V((S, M), BF16),
        V((M // 2, D), U32),
        V((HG, Dc // 2, D), U32),
        V((S, D), BF16),
        V((HG, S // 2, D), U32),
        V((1, D // 2, S), U32),
        V((NQ, TQ, TQ), F32),
        V((NQ, TQ, TQ), F32),
        V((NQ, TQ, TQ), F32),
        V((NQ, TQ, TQ), F32),
        pltpu.SMEM((2,), jnp.int32),
        V((H, S, D), BF16),
        V((S, M), F32),
        V((S, M), F32),
        V((NC, S + 2 * PAD, LANES), F32),
        V((S, M), BF16),
        V((1, M), BF16),
        pltpu.SemaphoreType.DMA((NSEM,)),
    ]
    out = pl.pallas_call(
        kernel,
        out_shape=jax.ShapeDtypeStruct((S, M), BF16),
        in_specs=[hbm_spec] * 12,
        out_specs=hbm_spec,
        scratch_shapes=scratch,
        compiler_params=pltpu.CompilerParams(vmem_limit_bytes=120 * 1024 * 1024),
        name="adaln_cla_mixer",
    )(x2, ckv2, A_w_q, A_w_uk, A_w_uv, wo2, B_w1, B_w2, B_w3.T, B_w4, c, w_mod)
    return out.reshape(B, S, M)
```

```python
import functools
import math

import jax
import jax.numpy as jnp
import jax.experimental.pallas as pl
import jax.experimental.pallas.tpu as pltpu

BF16 = jnp.bfloat16
F32 = jnp.float32
U32 = jnp.uint32

LANES = 128
TQ = 128
TR = 256
HB = 128
HG = 8
RCH = 4
LOOK = 4
AHEAD = 2
NSB = 4
DIST = 12
KC = 256
PC = 512
QC = 128
QH = 256
U2 = 2
PAD = 16
EPS = 1e-5
LOG2E = math.log2(math.e)
NEG = -1000000000.0 * LOG2E

_NT = (((1,), (1,)), ((), ()))


def _ln(x):
    m = jnp.mean(x, axis=-1, keepdims=True)
    xc = x - m
    v = jnp.mean(xc * xc, axis=-1, keepdims=True)
    return xc * jax.lax.rsqrt(v + EPS)


def _gelu(x):
    return jax.nn.gelu(x, approximate=True)


def _dot(a, b):
    return jnp.dot(a, b, preferred_element_type=F32)


def _dot_nt(a, b):
    return jax.lax.dot_general(a, b, _NT, preferred_element_type=F32)


def _fold8(x, op):
    parts = [op(x[j:j + 8], x[j + 8:j + 16]) for j in range(0, x.shape[0], 16)]
    acc = parts[0]
    for p in parts[1:]:
        acc = op(acc, p)
    return acc


def _rows_op(op, x, v8):
    r, m = x.shape
    return op(x.reshape(r // 8, 8, m), v8[None]).reshape(r, m)


def _modulate(x, scale8, shift8):
    r, m = x.shape
    return (x.reshape(r // 8, 8, m) * scale8[None] + shift8[None]).reshape(r, m)


def _pack(x):
    return pltpu.bitcast(x.astype(BF16), U32)


def _unpack(w):
    return pltpu.bitcast(w, BF16)


def _gstride(plane):
    return -(-8 * plane // 32) * 32


def _tied(w, tie):
    return jnp.concatenate([w[0:8] | tie, w[8:]], axis=0)


def _run(*gens):
    gens = list(gens)
    while gens:
        for g in list(gens):
            if next(g, gens) is gens:
                gens.remove(g)


@jax.jit
def pallas_adaLN_cond__compressed_kv_cla__mixer_s_mlp__prompt_kernel(
    A_x: jax.Array,
    A_c_kv: jax.Array,
    A_w_q: jax.Array,
    A_w_uk: jax.Array,
    A_w_uv: jax.Array,
    A_w_o: jax.Array,
    B_x: jax.Array,
    B_w1: jax.Array,
    B_w2: jax.Array,
    B_w3: jax.Array,
    B_w4: jax.Array,
    c: jax.Array,
    w_mod: jax.Array,
):
    del B_x
    B, S, M = A_x.shape
    _, Sk, Dc = A_c_kv.shape
    _, H, D = A_w_q.shape
    Fh = B_w3.shape[1]
    assert B == 1 and Sk == S and D == LANES and H % HG == 0 and HG == 8
    assert S % TQ == 0 and S % TR == 0 and S % PC == 0 and TR % HB == 0
    assert M % LANES == 0 and M % 64 == 0 and Dc % 64 == 0
    NG = H // HG
    NQ = S // TQ
    NR = S // TR
    NC = M // LANES
    C4 = M // 4
    PLQ = M // 2 + 1
    PLK = Dc // 2 + 1
    NK = S // KC
    XC = S // RCH
    NSEM = NK + 5
    assert NK > RCH + 1 and NQ % 2 == 0 and LOOK % 2 == 0
    qscale = float(D) ** -0.5 * LOG2E

    x2 = A_x.reshape(S, M)
    ckv2 = A_c_kv.reshape(S, Dc)
    wo2 = A_w_o.reshape(H * D, M)

    def kernel(x_hbm, ckv_hbm, wq_hbm, wuk_hbm, wuv_hbm, wo_hbm, w1_hbm, w2_hbm,
               w3_hbm, w4_hbm, c_hbm, wmod_hbm, out_hbm,
               x_v, ckv_v, wq_r, wuk_r, wuv_r, wq_p, wuk_p, wuv_p, wo_v, w1_v,
               w2_v, w3_v, w4_v, wmoda_v, wmodb_v, moda_v, modb_v, scb_v, hn_v, wqc_v, wk0_v, q_v, k_v,
               vt_v, s0, s1, s2, s3, z_s, ctx_v, x1_v, h2_v, hh_v, o_v, c_v,
               sems):

        s_v = (s0, s1, s2, s3)
        z_s[0] = 0
        z_s[1] = 0

        def aligned(i, n):
            return i * n if isinstance(i, int) else pl.multiple_of(i * n, n)

        def cp(src, dst, i):
            return pltpu.make_async_copy(src, dst, sems.at[i])

        def c_ckv(r):
            rows = pl.ds(aligned(r, KC), KC)
            return cp(ckv_hbm.at[rows, :], ckv_v.at[rows, :], r)

        def c_x(j):
            rows = pl.ds(aligned(j, XC), XC)
            return cp(x_hbm.at[rows, :], x_v.at[rows, :], NK - RCH + j)

        def c_q0(j):
            rows = pl.ds(aligned(j, M // RCH), M // RCH)
            return cp(wq_hbm.at[rows, pl.ds(0, HG), :], wq_r.at[0, rows], NK - RCH + j)

        def gcp(src, dst, g, i):
            return cp(src.at[:, pl.ds(g * HG, HG), :], dst.at[g], i)

        c_moda = cp(wmod_hbm.at[:, pl.ds(0, 2 * M)], wmoda_v, NK - RCH - 1)
        c_c = cp(c_hbm, c_v, NK)
        c_k0 = gcp(wuk_hbm, wuk_r, 0, NK + 1)
        c_v0 = gcp(wuv_hbm, wuv_r, 0, NK + 2)
        c_k1 = gcp(wuk_hbm, wuk_r, 1, NK + 3)
        c_late = []
        for g in range(1, NG):
            for src, dst, gg in ((wq_hbm, wq_r, g), (wuv_hbm, wuv_r, g), (wuk_hbm, wuk_r, g + 1)):
                if gg < NG:
                    c_late.append(gcp(src, dst, gg, NSEM - 1))
        for ct in range(4 * NC):
            c_late.append(cp(wmod_hbm.at[:, pl.ds(2 * M + ct * LANES, LANES)],
                             wmodb_v.at[ct], NSEM - 1))
        for src, dst in ((wo_hbm, wo_v), (w1_hbm, w1_v), (w2_hbm, w2_v),
                         (w3_hbm, w3_v), (w4_hbm, w4_v)):
            c_late.append(cp(src, dst, NSEM - 1))
        order = [c_c, c_k0] + [c_ckv(r) for r in range(NK - RCH)] + [c_moda]
        for j in range(RCH):
            order += [c_ckv(NK - RCH + j), c_x(j), c_q0(j)]
        order += [c_v0, c_k1] + c_late
        for d in order:
            d.start()

        def relayout_steps(raw, dst, g, chunk, rows, plane):
            n = rows // RCH // 2
            base = g * _gstride(plane) + chunk * n
            if not isinstance(base, int):
                base = pl.multiple_of(base, 8)
            view = dst.at[pl.ds(base, 7 * plane + n), :]

            def step(j, tie):
                val = raw[g, pl.ds(chunk * (2 * n) + 2 * j, 2)].reshape(2 * HG, D)
                val = pltpu.bitcast(val, U32)
                if tie is not None:
                    val = val | tie
                view[pl.ds(j, 8, stride=plane), :] = val

            return [functools.partial(step, j) for j in range(n)]

        def relayout(raw, dst, g, rows, plane):
            for ch in range(RCH):
                for step in relayout_steps(raw, dst, g, ch, rows, plane):
                    step(None)

        def head_w32(src, h, rows, plane):
            base = (h // HG) * _gstride(plane) + ((h % HG) // 2) * plane
            ev = src[pl.ds(base, rows // 2), :]
            od = src[pl.ds(base + 4 * plane, rows // 2), :]
            if not isinstance(h, int):
                par = (h % 2).astype(U32)
                w = (((ev >> (16 * par)) & U32(0xFFFF))
                     | ((od << (16 * (1 - par))) & U32(0xFFFF0000)))
            elif h % 2 == 0:
                w = (ev & U32(0xFFFF)) | (od << 16)
            else:
                w = (ev >> 16) | (od & U32(0xFFFF0000))
            return w

        def head_w(src, h, rows, plane):
            return pltpu.bitcast(head_w32(src, h, rows, plane), BF16)

        def q_rows(wq, lo, hi, ties=()):
            res = []
            for r0 in range(lo, hi, QC):
                rows = slice(r0, r0 + QC)
                w = _tied(wq, ties[len(res)]) if len(res) in ties else wq
                res.append(_dot(hn_v[rows, :], pltpu.bitcast(w, BF16)))
                q_v[rows, :] = (res[-1] * qscale).astype(BF16)
            return res

        def q_head(h):
            wq = head_w32(wq_p, h, M, PLQ)
            wqc_v[...] = wq
            return q_rows(wq, 0, QH)

        def q_mid(ties=()):
            q_rows(wqc_v[...], QH, S - PC, ties)

        def q_tail():
            return q_rows(wqc_v[...], S - PC, S)

        def k_proj(h, kh):
            wk = head_w(wuk_p, h, Dc, PLK)
            for r in range(S // PC):
                rows = slice(r * PC, (r + 1) * PC)
                kh[r * PC // 2:(r + 1) * PC // 2, :] = _pack(_dot(ckv_v[rows, :], wk))

        def mod_tile(w):
            acc = _fold8(w.astype(F32) * scb_v[...], jnp.add)
            return jnp.broadcast_to(jnp.sum(acc, axis=0, keepdims=True), (8, LANES))

        def mod(i):
            if i < 2:
                return moda_v[0:8, i * M:(i + 1) * M]
            return jnp.concatenate(
                [modb_v[(i - 2) * NC + ct] for ct in range(NC)], axis=1)

        def zeros8():
            return jnp.full((8, LANES), z_s[1], jnp.int32).astype(U32)

        def k_chunk(r, nsub=1, ties=(), after=None, unpack=False):
            n = KC // nsub
            lhs = ckv_v[pl.ds(aligned(r, KC), KC), :]
            for h in range(HG):
                if unpack:
                    w32 = head_w32(wuk_p, h, Dc, PLK)
                    wk0_v[h] = w32
                else:
                    w32 = wk0_v[h]
                for j in range(nsub):
                    i = h * nsub + j
                    rows = pl.ds(aligned(r * nsub + j, n // 2), n // 2)
                    w = _tied(w32, ties[i]) if i in ties else w32
                    res = _dot(lhs[j * n:(j + 1) * n], pltpu.bitcast(w, BF16))
                    k_v[h, rows, :] = _pack(res)
                    if after is not None:
                        after(i, res)

        c_c.wait()
        cc = c_v[...].astype(F32)
        sc = (cc * jax.nn.sigmoid(cc)).astype(BF16).astype(F32)
        scb_v[...] = jnp.broadcast_to(sc, (LANES, M)).T
        zpad = jnp.zeros((PAD, LANES), F32)
        for cidx in range(NC):
            hh_v[cidx, 0:PAD, :] = zpad
            hh_v[cidx, PAD + S:PAD + S + PAD, :] = zpad
        c_k0.wait()
        relayout(wuk_r, wuk_p, 0, Dc, PLK)

        def ka_body(r, carry):
            c_ckv(r).wait()
            k_chunk(r, unpack=True)
            return carry

        jax.lax.fori_loop(0, NK - RCH - 1, ka_body, 0)

        c_ckv(NK - RCH - 1).wait()
        c_moda.wait()
        zero8 = zeros8()
        ties = {}
        for ct in range(2 * NC):
            cols = slice(ct * LANES, (ct + 1) * LANES)
            tile = mod_tile(wmoda_v[:, cols])
            moda_v[0:8, cols] = tile
            ties[2 + (ct * (2 * HG - 2)) // (2 * NC)] = pltpu.bitcast(tile, U32) & zero8
        k_chunk(NK - RCH - 1, 2, ties)

        def kb_body(j, carry):
            c_ckv(NK - RCH + j).wait()
            c_x(j).wait()
            c_q0(j).wait()
            zero8 = zeros8()
            lr = XC // HG
            ties = {}
            scale, shift = 1.0 + mod(1), mod(0)
            for i in range(HG):
                rows = pl.ds(pl.multiple_of(j * XC + i * lr, lr), lr)
                hn = _modulate(_ln(x_v[rows, :].astype(F32)), scale, shift)
                hn_v[rows, :] = hn.astype(BF16)
                ties[i + 2] = pltpu.bitcast(_fold8(hn[:, 0:LANES], jnp.maximum), U32) & zero8
            steps = relayout_steps(wq_r, wq_p, 0, j, M, PLQ)
            per = len(steps) // HG

            def side(i, res):
                for k, step in enumerate(steps[i * per:(i + 1) * per]):
                    step(pltpu.bitcast(res[k * 8:(k + 1) * 8], U32) & zero8)

            k_chunk(NK - RCH + j, 1, ties, side)
            return carry

        jax.lax.fori_loop(0, RCH, kb_body, 0)

        c_v0.wait()
        zero8 = zeros8()
        res = jnp.concatenate(q_head(0), axis=0)
        steps = []
        for ch in range(RCH):
            steps += relayout_steps(wuv_r, wuv_p, 0, ch, Dc, PLK)
        for i, step in enumerate(steps):
            k = i * (QH // 8) // len(steps)
            step(pltpu.bitcast(res[k * 8:(k + 1) * 8], U32) & zero8)

        def attention(h, kh, side):
            HT = TQ // 2
            key_i = jax.lax.broadcasted_iota(jnp.int32, (HT, TQ), 0)
            qry_i = jax.lax.broadcasted_iota(jnp.int32, (HT, TQ), 1)
            causal_lo = key_i <= qry_i
            causal_hi = key_i + HT <= qry_i
            z_st = z_s[0]
            z_ld = z_s[1]
            zero8 = zeros8()

            m8 = {}
            seq = []

            def keys(*halves):
                ks = [kh[a * HT // 2:b * HT // 2, :] for a, b in halves]
                return _unpack(ks[0] if len(ks) == 1 else jnp.concatenate(ks, axis=0))

            def put(i, half, val):
                for k in range(val.shape[0] // HT):
                    t, off = (half + k) // 2, (half + k) % 2 * HT
                    s_v[i % NSB][z_st + t, off:off + HT, :] = val[k * HT:(k + 1) * HT]
                tm = _fold8(val, jnp.maximum)
                m8[i] = jnp.maximum(m8[i], tm) if i in m8 else tm

            def mm(a, b):
                res = _dot_nt(a, b)
                seq.append(res[0:8])
                return res

            def qk(i):
                qi = q_v[i * TQ:(i + 1) * TQ, :]
                if i % 2 == 0:
                    j = i + 1
                    strip = mm(q_v[j * TQ + HT:(j + 1) * TQ, :],
                               keys((2 * i + 1, 2 * i + 2), (2 * j + 1, 2 * j + 2)))
                    yield
                    qmix = jnp.concatenate(
                        [q_v[j * TQ:j * TQ + HT, :], q_v[i * TQ + HT:(i + 1) * TQ, :]], axis=0)
                    mix = mm(keys((2 * i + 1, 2 * i + 2)), qmix)
                    put(i, 2 * i + 1, jnp.where(causal_hi, mix, NEG))
                    st = jnp.concatenate([strip, strip], axis=0).T
                    put(j, 2 * i + 1, jnp.where(qry_i < HT, mix, st[0:HT]))
                    put(j, 2 * j + 1, jnp.where(causal_hi, st[HT:TQ], NEG))
                    yield
                for t in range(i - 1):
                    put(i, 2 * t, mm(keys((2 * t, 2 * t + 2)), qi))
                    yield
                if i % 2 == 0:
                    lo = max(2 * i - 2, 0)
                    res = mm(keys((lo, 2 * i + 1)), qi)
                    if i > 0:
                        put(i, lo, res[0:TQ])
                else:
                    res = mm(keys((2 * i - 2, 2 * i - 1), (2 * i, 2 * i + 1)), qi)
                    put(i, 2 * i - 2, res[0:HT])
                put(i, 2 * i, jnp.where(causal_lo, res[res.shape[0] - HT:], NEG))
                yield

            def pv(i):
                sb = s_v[i % NSB]
                mb = jnp.broadcast_to(jnp.max(m8[i], axis=0, keepdims=True), (8, TQ))
                l8 = None
                ot = None
                for t in range(i + 1):
                    tie = pltpu.bitcast(seq[-DIST], U32) & zero8
                    mt = pltpu.bitcast(pltpu.bitcast(mb, U32) | tie, F32)
                    tile = sb[z_ld + t].reshape(TQ // 8, 8, TQ)
                    p = jnp.exp2(tile - mt[None]).reshape(TQ, TQ)
                    part = _fold8(p, jnp.add)
                    l8 = part if l8 is None else l8 + part
                    o = _dot(_unpack(vt_v[z_ld, :, t * TQ:(t + 1) * TQ]), p.astype(BF16))
                    seq.append(o[0:8])
                    ot = o if ot is None else ot + o
                    if t == i:
                        l = jnp.sum(l8, axis=0, keepdims=True)
                        ot = ot * (1.0 / l)
                        ctx_v[h, i * TQ:(i + 1) * TQ, :] = ot.T.astype(BF16)
                    yield

            for i in range(LOOK):
                _run(qk(i))
            vt = _dot_nt(head_w(wuv_p, h, Dc, PLK).T, ckv_v[...])
            vt_v[z_st] = _pack(vt)
            prev = vt[0:8, S - TQ:S]
            for res in q_tail():
                seq.extend([prev] * NC)
                prev = res[0:8]
            per = max(1, -(-len(side) // NQ))
            for j, step in enumerate(side):
                ct, rg = j // per, (j % per) * (D // 8) // per
                src = vt[rg * 8:(rg + 1) * 8, ct * TQ:(ct + 1) * TQ]
                step(pltpu.bitcast(src, U32) & zero8)
            for i in range(NQ):
                j = i + AHEAD
                if LOOK <= j < NQ:
                    _run(qk(j), pv(i))
                else:
                    _run(pv(i))

        def side_work(h):
            g = h // HG + ((h % HG) >= RCH).astype(jnp.int32)
            ch = h % RCH
            steps = (relayout_steps(wq_r, wq_p, g, ch, M, PLQ)
                     + relayout_steps(wuv_r, wuv_p, g, ch, Dc, PLK))
            for c in range(RCH):
                steps += relayout_steps(wuk_r, wuk_p, h // HG + 1, c, Dc, PLK)
            return steps

        def head_body(h, carry):
            @pl.when(h == RCH)
            def _():
                for d in c_late:
                    d.wait()

            kh = k_v.at[h % HG]
            q_mid()
            attention(h, kh, side_work(h))
            q_head(h + 1)
            k_proj(h + HG, kh)
            return carry

        c_k1.wait()
        jax.lax.fori_loop(0, H - HG, head_body, 0)

        def last_body(h, carry):
            per = -(-4 * NC // HG)
            zero8 = zeros8()
            ties = {}
            for i in range(per):
                ct = jnp.minimum((h - (H - HG)) * per + i, 4 * NC - 1)
                tile = mod_tile(wmodb_v[ct])
                modb_v[ct] = tile
                ties[2 * i + 3] = pltpu.bitcast(tile, U32) & zero8
            q_mid(ties)
            attention(h, k_v.at[h % HG], ())
            q_head(jnp.minimum(h + 1, H - 1))
            return carry

        jax.lax.fori_loop(H - HG, H, last_body, 0)

        def sub_rows(r):
            out = []
            for j in range(TR // HB):
                r0 = r * TR + j * HB
                if not isinstance(r0, int):
                    r0 = pl.multiple_of(r0, HB)
                out.append(r0)
            return out

        def stage1(r):
            atts = []
            for r0 in sub_rows(r):
                ctx = jnp.concatenate(
                    [ctx_v[h, pl.ds(r0, HB), :] for h in range(H)], axis=1)
                atts.append(_dot(ctx, wo_v[...]))
            lns = []
            for r0, att in zip(sub_rows(r), atts):
                rows = pl.ds(r0, HB)
                x1 = x_v[rows, :].astype(F32) + _rows_op(jnp.multiply, att, mod(2))
                x1_v[rows, :] = x1
                h2 = _modulate(_ln(x1), 1.0 + mod(4), mod(3))
                h2_v[rows, :] = h2
                lns.append(_ln(h2).astype(BF16))
            for r0, ln in zip(sub_rows(r), lns):
                u = _gelu(_dot(ln, w1_v[...]))
                for cidx in range(NC):
                    hh_v[cidx, pl.ds(r0 + PAD, HB), :] = u[:, cidx * LANES:(cidx + 1) * LANES]

        shifts = (1, -1, 2, -2)

        def out_cp(r0):
            rows = pl.ds(r0, HB)
            return cp(o_v.at[rows, :], out_hbm.at[rows, :], 0)

        def stage2(r):
            lane_i = jax.lax.broadcasted_iota(jnp.int32, (HB, LANES), 1)
            y1s = []
            for r0 in sub_rows(r):
                tiles = []
                for cidx in range(NC):
                    lo, hi = cidx * LANES, (cidx + 1) * LANES
                    g_lo, g_hi = lo // C4, (hi - 1) // C4
                    t = hh_v[cidx, pl.ds(r0 + PAD - shifts[g_hi], HB), :]
                    for g in range(g_hi - 1, g_lo - 1, -1):
                        tg = hh_v[cidx, pl.ds(r0 + PAD - shifts[g], HB), :]
                        t = jnp.where(lane_i < (g + 1) * C4 - lo, tg, t)
                    tiles.append(t)
                hs = _dot(jnp.concatenate(tiles, axis=1).astype(BF16), w2_v[...])
                y1s.append(h2_v[pl.ds(r0, HB), :] + hs)
            gls = []
            f0 = Fh // LANES * LANES
            for y1 in y1s:
                ln = _ln(y1).astype(BF16)
                parts = [_gelu(_dot_nt(ln, w3_v[0:f0 // 2 // LANES * LANES, :]))]
                if f0 < Fh:
                    tail = _gelu(_dot_nt(w3_v[f0:Fh, :], ln)).T
                parts.append(_gelu(_dot_nt(ln, w3_v[f0 // 2 // LANES * LANES:f0, :])))
                if f0 < Fh:
                    parts.append(tail)
                gls.append(jnp.concatenate(parts, axis=1).astype(BF16))
            for r0, y1, gl in zip(sub_rows(r), y1s, gls):
                rows = pl.ds(r0, HB)
                h3 = _dot(gl, w4_v[...])
                o_v[rows, :] = (x1_v[rows, :]
                                + _rows_op(jnp.multiply, y1 + h3, mod(5))).astype(BF16)
                out_cp(r0).start()

        def s1_body(r, carry):
            stage1(r)
            return carry

        def s2_body(r, carry):
            for u in range(U2):
                stage2(r * U2 + u)
            return carry

        jax.lax.fori_loop(0, NR, s1_body, 0)
        jax.lax.fori_loop(0, NR // U2, s2_body, 0)
        cp(o_v, out_hbm, 0).wait()

    hbm_spec = pl.BlockSpec(memory_space=pltpu.HBM)
    V = pltpu.VMEM
    scratch = [
        V((S, M), BF16),
        V((S, Dc), BF16),
        V((NG, M, HG, D), BF16),
        V((NG, Dc, HG, D), BF16),
        V((NG, Dc, HG, D), BF16),
        V((NG * _gstride(PLQ), D), U32),
        V((NG * _gstride(PLK), D), U32),
        V((NG * _gstride(PLK), D), U32),
        V((H * D, M), BF16),
        V((M, M), BF16),
        V((M, M), BF16),
        V((Fh, M), BF16),
        V((Fh, M), BF16),
        V((M, 2 * M), BF16),
        V((4 * NC, M, LANES), BF16),
        V((16, 2 * M), F32),
        V((4 * NC, 8, LANES), F32),
        V((M, LANES), F32),
        V((S, M), BF16),
        V((M // 2, D), U32),
        V((HG, Dc // 2, D), U32),
        V((S, D), BF16),
        V((HG, S // 2, D), U32),
        V((1, D // 2, S), U32),
        V((NQ, TQ, TQ), F32),
        V((NQ, TQ, TQ), F32),
        V((NQ, TQ, TQ), F32),
        V((NQ, TQ, TQ), F32),
        pltpu.SMEM((2,), jnp.int32),
        V((H, S, D), BF16),
        V((S, M), F32),
        V((S, M), F32),
        V((NC, S + 2 * PAD, LANES), F32),
        V((S, M), BF16),
        V((1, M), BF16),
        pltpu.SemaphoreType.DMA((NSEM,)),
    ]
    out = pl.pallas_call(
        kernel,
        out_shape=jax.ShapeDtypeStruct((S, M), BF16),
        in_specs=[hbm_spec] * 12,
        out_specs=hbm_spec,
        scratch_shapes=scratch,
        compiler_params=pltpu.CompilerParams(vmem_limit_bytes=120 * 1024 * 1024),
        name="adaln_cla_mixer",
    )(x2, ckv2, A_w_q, A_w_uk, A_w_uv, wo2, B_w1, B_w2, B_w3.T, B_w4, c, w_mod)
    return out.reshape(B, S, M)
```

```python
import functools
import math

import jax
import jax.numpy as jnp
import jax.experimental.pallas as pl
import jax.experimental.pallas.tpu as pltpu

BF16 = jnp.bfloat16
F32 = jnp.float32
U32 = jnp.uint32

LANES = 128
TQ = 128
TR = 256
HB = 128
HG = 8
RCH = 4
LOOK = 4
AHEAD = 2
NSB = 4
DIST = 12
KC = 256
PC = 512
QC = 128
QH = 256
U2 = 2
PAD = 16
EPS = 1e-5
LOG2E = math.log2(math.e)
NEG = -1000000000.0 * LOG2E

_NT = (((1,), (1,)), ((), ()))


def _ln(x):
    m = jnp.mean(x, axis=-1, keepdims=True)
    xc = x - m
    v = jnp.mean(xc * xc, axis=-1, keepdims=True)
    return xc * jax.lax.rsqrt(v + EPS)


def _gelu(x):
    return jax.nn.gelu(x, approximate=True)


def _dot(a, b):
    return jnp.dot(a, b, preferred_element_type=F32)


def _dot_nt(a, b):
    return jax.lax.dot_general(a, b, _NT, preferred_element_type=F32)


def _fold8(x, op):
    parts = [op(x[j:j + 8], x[j + 8:j + 16]) for j in range(0, x.shape[0], 16)]
    acc = parts[0]
    for p in parts[1:]:
        acc = op(acc, p)
    return acc


def _rows_op(op, x, v8):
    r, m = x.shape
    return op(x.reshape(r // 8, 8, m), v8[None]).reshape(r, m)


def _modulate(x, scale8, shift8):
    r, m = x.shape
    return (x.reshape(r // 8, 8, m) * scale8[None] + shift8[None]).reshape(r, m)


def _pack(x):
    return pltpu.bitcast(x.astype(BF16), U32)


def _unpack(w):
    return pltpu.bitcast(w, BF16)


def _gstride(plane):
    return -(-8 * plane // 32) * 32


def _tied(w, tie):
    return jnp.concatenate([w[0:8] | tie, w[8:]], axis=0)


def _run(*gens):
    gens = list(gens)
    while gens:
        for g in list(gens):
            if next(g, gens) is gens:
                gens.remove(g)


@jax.jit
def pallas_adaLN_cond__compressed_kv_cla__mixer_s_mlp__prompt_kernel(
    A_x: jax.Array,
    A_c_kv: jax.Array,
    A_w_q: jax.Array,
    A_w_uk: jax.Array,
    A_w_uv: jax.Array,
    A_w_o: jax.Array,
    B_x: jax.Array,
    B_w1: jax.Array,
    B_w2: jax.Array,
    B_w3: jax.Array,
    B_w4: jax.Array,
    c: jax.Array,
    w_mod: jax.Array,
):
    del B_x
    B, S, M = A_x.shape
    _, Sk, Dc = A_c_kv.shape
    _, H, D = A_w_q.shape
    Fh = B_w3.shape[1]
    assert B == 1 and Sk == S and D == LANES and H % HG == 0 and HG == 8
    assert S % TQ == 0 and S % TR == 0 and S % PC == 0 and TR % HB == 0
    assert M % LANES == 0 and M % 64 == 0 and Dc % 64 == 0
    NG = H // HG
    NQ = S // TQ
    NR = S // TR
    NC = M // LANES
    C4 = M // 4
    PLQ = M // 2 + 1
    PLK = Dc // 2 + 1
    NK = S // KC
    XC = S // RCH
    NSEM = NK + 5
    assert NK > RCH + 1 and NQ % 2 == 0 and LOOK % 2 == 0
    HS = Dc // D
    NSL = -(-HG // NC)
    assert H % 2 == 0 and RCH % 2 == 0 and RCH + 4 * NC <= H and NSL * HS + 2 < H - HG
    qscale = float(D) ** -0.5 * LOG2E

    x2 = A_x.reshape(S, M)
    ckv2 = A_c_kv.reshape(S, Dc)
    wo2 = A_w_o.reshape(H * D, M)

    def kernel(x_hbm, ckv_hbm, wq_hbm, wuk_hbm, wuv_hbm, wo_hbm, w1_hbm, w2_hbm,
               w3_hbm, w4_hbm, c_hbm, wmod_hbm, out_hbm, slab_hbm,
               x_v, lhs_v, wq_r, wuk_r, wuv_r, wq_p, wuk_p, wuv_p, wo_v, wou_v, w1_v,
               w2_v, w3_v, w4_v, wmoda_v, wmodb_v, moda_v, modb_v, scb_v, hn_v, wqc_v, wk0_v, q_v, k_v,
               vt_v, s0, s1, s2, s3, z_s, ctx_v, part_v, x1_v, h2_v, hh_v, o_v, c_v,
               sems):

        s_v = (s0, s1, s2, s3)
        ckv_v = lhs_v.at[0]
        z_s[0] = 0
        z_s[1] = 0

        def aligned(i, n):
            return i * n if isinstance(i, int) else pl.multiple_of(i * n, n)

        def cp(src, dst, i):
            return pltpu.make_async_copy(src, dst, sems.at[i])

        def c_ckv(r):
            rows = pl.ds(aligned(r, KC), KC)
            return cp(ckv_hbm.at[rows, :], ckv_v.at[rows, :], r)

        def c_x(j):
            rows = pl.ds(aligned(j, XC), XC)
            return cp(x_hbm.at[rows, :], x_v.at[rows, :], NK - RCH + j)

        def c_q0(j):
            rows = pl.ds(aligned(j, M // RCH), M // RCH)
            return cp(wq_hbm.at[rows, pl.ds(0, HG), :], wq_r.at[0, rows], NK - RCH + j)

        def gcp(src, dst, g, i):
            return cp(src.at[:, pl.ds(g * HG, HG), :], dst.at[g], i)

        c_moda = cp(wmod_hbm.at[:, pl.ds(0, 2 * M)], wmoda_v, NK - RCH - 1)
        c_c = cp(c_hbm, c_v, NK)
        c_k0 = gcp(wuk_hbm, wuk_r, 0, NK + 1)
        c_v0 = gcp(wuv_hbm, wuv_r, 0, NK + 2)
        c_k1 = gcp(wuk_hbm, wuk_r, 1, NK + 3)
        c_late = []
        for g in range(1, NG):
            for src, dst, gg in ((wq_hbm, wq_r, g), (wuv_hbm, wuv_r, g), (wuk_hbm, wuk_r, g + 1)):
                if gg < NG:
                    c_late.append(gcp(src, dst, gg, NSEM - 1))
        for ct in range(4 * NC):
            c_late.append(cp(wmod_hbm.at[:, pl.ds(2 * M + ct * LANES, LANES)],
                             wmodb_v.at[ct], NSEM - 1))
        for u in range(HG):
            c_late.append(cp(wo_hbm.at[pl.ds(u // NC * Dc, Dc), pl.ds(u % NC * D, D)],
                             wou_v.at[u], NSEM - 1))
        for src, dst in ((wo_hbm, wo_v), (w1_hbm, w1_v), (w2_hbm, w2_v),
                         (w3_hbm, w3_v), (w4_hbm, w4_v)):
            c_late.append(cp(src, dst, NSEM - 1))
        order = [c_c, c_k0] + [c_ckv(r) for r in range(NK - RCH)] + [c_moda]
        for j in range(RCH):
            order += [c_ckv(NK - RCH + j), c_x(j), c_q0(j)]
        order += [c_v0, c_k1] + c_late
        for d in order:
            d.start()

        def relayout_steps(raw, dst, g, chunk, rows, plane):
            n = rows // RCH // 2
            base = g * _gstride(plane) + chunk * n
            if not isinstance(base, int):
                base = pl.multiple_of(base, 8)
            view = dst.at[pl.ds(base, 7 * plane + n), :]

            def step(j, tie):
                val = raw[g, pl.ds(chunk * (2 * n) + 2 * j, 2)].reshape(2 * HG, D)
                val = pltpu.bitcast(val, U32)
                if tie is not None:
                    val = val | tie
                view[pl.ds(j, 8, stride=plane), :] = val

            return [functools.partial(step, j) for j in range(n)]

        def relayout(raw, dst, g, rows, plane):
            for ch in range(RCH):
                for step in relayout_steps(raw, dst, g, ch, rows, plane):
                    step(None)

        def head_w32(src, h, rows, plane, par=None):
            base = (h // HG) * _gstride(plane) + ((h % HG) // 2) * plane
            ev = src[pl.ds(base, rows // 2), :]
            od = src[pl.ds(base + 4 * plane, rows // 2), :]
            par = h % 2 if par is None else par
            if par == 0:
                return (ev & U32(0xFFFF)) | (od << 16)
            return (ev >> 16) | (od & U32(0xFFFF0000))

        def q_rows(wq, lo, hi, ties=()):
            res = []
            for r0 in range(lo, hi, QC):
                rows = slice(r0, r0 + QC)
                w = _tied(wq, ties[len(res)]) if len(res) in ties else wq
                res.append(_dot(hn_v[rows, :], pltpu.bitcast(w, BF16)))
                q_v[rows, :] = (res[-1] * qscale).astype(BF16)
            return res

        def q_head(h, par=None):
            wq = head_w32(wq_p, h, M, PLQ, par)
            wqc_v[...] = wq
            return q_rows(wq, 0, QH)

        def q_mid(ties=()):
            q_rows(wqc_v[...], QH, S - PC, ties)

        def q_tail():
            return q_rows(wqc_v[...], S - PC, S)

        def k_slot(h, par, kh):
            late = h >= H - HG
            u = jnp.maximum(h - (H - HG), 0)
            wk = head_w32(wuk_p, jnp.where(late, h, h + HG), Dc, PLK, par)
            wu = pltpu.bitcast(wou_v[jnp.where(late, u, HG)], U32)
            w = _unpack(jnp.where(late, wu, wk))
            lhs = lhs_v.at[jnp.where(late, 1 + u // NC, 0)]
            for r in range(S // PC):
                rows = slice(r * PC, (r + 1) * PC)
                res = _dot(lhs[rows, :], w)
                kh[r * PC // 2:(r + 1) * PC // 2, :] = _pack(res)
                part_v[u, rows, :] = res

        def mod_tile(w):
            acc = _fold8(w.astype(F32) * scb_v[...], jnp.add)
            return jnp.broadcast_to(jnp.sum(acc, axis=0, keepdims=True), (8, LANES))

        def mod(i):
            if i < 2:
                return moda_v[0:8, i * M:(i + 1) * M]
            return jnp.concatenate(
                [modb_v[(i - 2) * NC + ct] for ct in range(NC)], axis=1)

        def zeros8():
            return jnp.full((8, LANES), z_s[1], jnp.int32).astype(U32)

        def k_chunk(r, nsub=1, ties=(), after=None, unpack=False):
            n = KC // nsub
            lhs = ckv_v[pl.ds(aligned(r, KC), KC), :]
            for h in range(HG):
                if unpack:
                    w32 = head_w32(wuk_p, h, Dc, PLK)
                    wk0_v[h] = w32
                else:
                    w32 = wk0_v[h]
                for j in range(nsub):
                    i = h * nsub + j
                    rows = pl.ds(aligned(r * nsub + j, n // 2), n // 2)
                    w = _tied(w32, ties[i]) if i in ties else w32
                    res = _dot(lhs[j * n:(j + 1) * n], pltpu.bitcast(w, BF16))
                    k_v[h, rows, :] = _pack(res)
                    if after is not None:
                        after(i, res)

        c_c.wait()
        cc = c_v[...].astype(F32)
        sc = (cc * jax.nn.sigmoid(cc)).astype(BF16).astype(F32)
        scb_v[...] = jnp.broadcast_to(sc, (LANES, M)).T
        zpad = jnp.zeros((PAD, LANES), F32)
        for cidx in range(NC):
            hh_v[cidx, 0:PAD, :] = zpad
            hh_v[cidx, PAD + S:PAD + S + PAD, :] = zpad
        wou_v[HG] = jnp.zeros((Dc, D), BF16)
        wmodb_v[4 * NC] = jnp.zeros((M, LANES), BF16)
        c_k0.wait()
        relayout(wuk_r, wuk_p, 0, Dc, PLK)

        def ka_body(r, carry):
            c_ckv(r).wait()
            k_chunk(r, unpack=True)
            return carry

        jax.lax.fori_loop(0, NK - RCH - 1, ka_body, 0)

        c_ckv(NK - RCH - 1).wait()
        c_moda.wait()
        zero8 = zeros8()
        ties = {}
        for ct in range(2 * NC):
            cols = slice(ct * LANES, (ct + 1) * LANES)
            tile = mod_tile(wmoda_v[:, cols])
            moda_v[0:8, cols] = tile
            ties[2 + (ct * (2 * HG - 2)) // (2 * NC)] = pltpu.bitcast(tile, U32) & zero8
        k_chunk(NK - RCH - 1, 2, ties)

        def kb_body(j, carry):
            c_ckv(NK - RCH + j).wait()
            c_x(j).wait()
            c_q0(j).wait()
            zero8 = zeros8()
            lr = XC // HG
            ties = {}
            scale, shift = 1.0 + mod(1), mod(0)
            for i in range(HG):
                rows = pl.ds(pl.multiple_of(j * XC + i * lr, lr), lr)
                hn = _modulate(_ln(x_v[rows, :].astype(F32)), scale, shift)
                hn_v[rows, :] = hn.astype(BF16)
                ties[i + 2] = pltpu.bitcast(_fold8(hn[:, 0:LANES], jnp.maximum), U32) & zero8
            steps = relayout_steps(wq_r, wq_p, 0, j, M, PLQ)
            per = len(steps) // HG

            def side(i, res):
                for k, step in enumerate(steps[i * per:(i + 1) * per]):
                    step(pltpu.bitcast(res[k * 8:(k + 1) * 8], U32) & zero8)

            k_chunk(NK - RCH + j, 1, ties, side)
            return carry

        jax.lax.fori_loop(0, RCH, kb_body, 0)

        c_v0.wait()
        zero8 = zeros8()
        res = jnp.concatenate(q_head(0), axis=0)
        steps = []
        for ch in range(RCH):
            steps += relayout_steps(wuv_r, wuv_p, 0, ch, Dc, PLK)
        for i, step in enumerate(steps):
            k = i * (QH // 8) // len(steps)
            step(pltpu.bitcast(res[k * 8:(k + 1) * 8], U32) & zero8)

        def attention(h, par, kh, side):
            HT = TQ // 2
            key_i = jax.lax.broadcasted_iota(jnp.int32, (HT, TQ), 0)
            qry_i = jax.lax.broadcasted_iota(jnp.int32, (HT, TQ), 1)
            causal_lo = key_i <= qry_i
            causal_hi = key_i + HT <= qry_i
            z_st = z_s[0]
            z_ld = z_s[1]
            zero8 = zeros8()

            m8 = {}
            seq = []

            def keys(*halves):
                ks = [kh[a * HT // 2:b * HT // 2, :] for a, b in halves]
                return _unpack(ks[0] if len(ks) == 1 else jnp.concatenate(ks, axis=0))

            def put(i, half, val):
                for k in range(val.shape[0] // HT):
                    t, off = (half + k) // 2, (half + k) % 2 * HT
                    s_v[i % NSB][z_st + t, off:off + HT, :] = val[k * HT:(k + 1) * HT]
                tm = _fold8(val, jnp.maximum)
                m8[i] = jnp.maximum(m8[i], tm) if i in m8 else tm

            def mm(a, b):
                res = _dot_nt(a, b)
                seq.append(res[0:8])
                return res

            def qk(i):
                qi = q_v[i * TQ:(i + 1) * TQ, :]
                if i % 2 == 0:
                    j = i + 1
                    strip = mm(q_v[j * TQ + HT:(j + 1) * TQ, :],
                               keys((2 * i + 1, 2 * i + 2), (2 * j + 1, 2 * j + 2)))
                    yield
                    qmix = jnp.concatenate(
                        [q_v[j * TQ:j * TQ + HT, :], q_v[i * TQ + HT:(i + 1) * TQ, :]], axis=0)
                    mix = mm(keys((2 * i + 1, 2 * i + 2)), qmix)
                    put(i, 2 * i + 1, jnp.where(causal_hi, mix, NEG))
                    st = jnp.concatenate([strip, strip], axis=0).T
                    put(j, 2 * i + 1, jnp.where(qry_i < HT, mix, st[0:HT]))
                    put(j, 2 * j + 1, jnp.where(causal_hi, st[HT:TQ], NEG))
                    yield
                for t in range(i - 1):
                    put(i, 2 * t, mm(keys((2 * t, 2 * t + 2)), qi))
                    yield
                if i % 2 == 0:
                    lo = max(2 * i - 2, 0)
                    res = mm(keys((lo, 2 * i + 1)), qi)
                    if i > 0:
                        put(i, lo, res[0:TQ])
                else:
                    res = mm(keys((2 * i - 2, 2 * i - 1), (2 * i, 2 * i + 1)), qi)
                    put(i, 2 * i - 2, res[0:HT])
                put(i, 2 * i, jnp.where(causal_lo, res[res.shape[0] - HT:], NEG))
                yield

            def pv(i):
                sb = s_v[i % NSB]
                mb = jnp.broadcast_to(jnp.max(m8[i], axis=0, keepdims=True), (8, TQ))
                l8 = None
                ot = None
                for t in range(i + 1):
                    tie = pltpu.bitcast(seq[-DIST], U32) & zero8
                    mt = pltpu.bitcast(pltpu.bitcast(mb, U32) | tie, F32)
                    tile = sb[z_ld + t].reshape(TQ // 8, 8, TQ)
                    p = jnp.exp2(tile - mt[None]).reshape(TQ, TQ)
                    part = _fold8(p, jnp.add)
                    l8 = part if l8 is None else l8 + part
                    o = _dot(_unpack(vt_v[z_ld, :, t * TQ:(t + 1) * TQ]), p.astype(BF16))
                    seq.append(o[0:8])
                    ot = o if ot is None else ot + o
                    if t == i:
                        l = jnp.sum(l8, axis=0, keepdims=True)
                        ot = ot * (1.0 / l)
                        ctx_v[h, i * TQ:(i + 1) * TQ, :] = ot.T.astype(BF16)
                    yield

            for i in range(LOOK):
                _run(qk(i))
            vt = _dot_nt(_unpack(head_w32(wuv_p, h, Dc, PLK, par)).T, ckv_v[...])
            vt_v[z_st] = _pack(vt)
            prev = vt[0:8, S - TQ:S]
            for res in q_tail():
                seq.extend([prev] * NC)
                prev = res[0:8]
            per = max(1, -(-len(side) // NQ))
            for j, step in enumerate(side):
                ct, rg = j // per, (j % per) * (D // 8) // per
                src = vt[rg * 8:(rg + 1) * 8, ct * TQ:(ct + 1) * TQ]
                step(pltpu.bitcast(src, U32) & zero8)
            for i in range(NQ):
                j = i + AHEAD
                if LOOK <= j < NQ:
                    _run(qk(j), pv(i))
                else:
                    _run(pv(i))

        def side_work(h):
            g = jnp.minimum(h // HG + ((h % HG) >= RCH).astype(jnp.int32), NG - 1)
            ch = h % RCH
            steps = (relayout_steps(wq_r, wq_p, g, ch, M, PLQ)
                     + relayout_steps(wuv_r, wuv_p, g, ch, Dc, PLK))
            gk = jnp.minimum(h // HG + 1, NG - 1)
            for c in range(RCH):
                steps += relayout_steps(wuk_r, wuk_p, gk, c, Dc, PLK)
            return steps

        c_up = [cp(ctx_v.at[h], slab_hbm.at[h // HS, :, pl.ds(h % HS * D, D)], 1)
                for h in range(NSL * HS)]
        c_down = cp(slab_hbm, lhs_v.at[pl.ds(1, NSL)], 2)

        def head(h, par):
            ct = jnp.where(jnp.logical_and(h >= RCH, h < RCH + 4 * NC), h - RCH, 4 * NC)
            tile = mod_tile(wmodb_v[ct])
            modb_v[ct] = tile
            kh = k_v.at[h % HG]
            q_mid({4: pltpu.bitcast(tile, U32) & zeros8()})
            attention(h, par, kh, side_work(h))
            q_head(jnp.minimum(h + 1, H - 2 + (1 - par)), 1 - par)
            k_slot(h, par, kh)

        def pair_body(j, carry):
            h = 2 * j

            @pl.when(h == RCH)
            def _():
                for d in c_late:
                    d.wait()

            @pl.when(h == NSL * HS)
            def _():
                for d in c_up:
                    d.start()

            @pl.when(h == NSL * HS + 2)
            def _():
                for d in c_up:
                    d.wait()
                c_down.start()

            @pl.when(h == H - HG)
            def _():
                c_down.wait()

            head(h, 0)
            head(h + 1, 1)
            return carry

        c_k1.wait()
        jax.lax.fori_loop(0, H // 2, pair_body, 0)

        def sub_rows(r):
            out = []
            for j in range(TR // HB):
                r0 = r * TR + j * HB
                if not isinstance(r0, int):
                    r0 = pl.multiple_of(r0, HB)
                out.append(r0)
            return out

        def stage1(r):
            atts = []
            for r0 in sub_rows(r):
                rows = pl.ds(r0, HB)
                ctx = [ctx_v[h, rows, :] for h in range(H)]
                cols = []
                for ct in range(NC):
                    units = list(range(ct, HG, NC))
                    h0 = len(units) * HS
                    col = _dot(jnp.concatenate(ctx[h0:], axis=1),
                               wo_v[h0 * D:H * D, ct * LANES:(ct + 1) * LANES])
                    for u in units:
                        col = col + part_v[u, rows, :]
                    cols.append(col)
                atts.append(jnp.concatenate(cols, axis=1))
            lns = []
            for r0, att in zip(sub_rows(r), atts):
                rows = pl.ds(r0, HB)
                x1 = x_v[rows, :].astype(F32) + _rows_op(jnp.multiply, att, mod(2))
                x1_v[rows, :] = x1
                h2 = _modulate(_ln(x1), 1.0 + mod(4), mod(3))
                h2_v[rows, :] = h2
                lns.append(_ln(h2).astype(BF16))
            for r0, ln in zip(sub_rows(r), lns):
                u = _gelu(_dot(ln, w1_v[...]))
                for cidx in range(NC):
                    hh_v[cidx, pl.ds(r0 + PAD, HB), :] = u[:, cidx * LANES:(cidx + 1) * LANES]

        shifts = (1, -1, 2, -2)

        def out_cp(r0):
            rows = pl.ds(r0, HB)
            return cp(o_v.at[rows, :], out_hbm.at[rows, :], 0)

        def stage2(r):
            lane_i = jax.lax.broadcasted_iota(jnp.int32, (HB, LANES), 1)
            y1s = []
            for r0 in sub_rows(r):
                tiles = []
                for cidx in range(NC):
                    lo, hi = cidx * LANES, (cidx + 1) * LANES
                    g_lo, g_hi = lo // C4, (hi - 1) // C4
                    t = hh_v[cidx, pl.ds(r0 + PAD - shifts[g_hi], HB), :]
                    for g in range(g_hi - 1, g_lo - 1, -1):
                        tg = hh_v[cidx, pl.ds(r0 + PAD - shifts[g], HB), :]
                        t = jnp.where(lane_i < (g + 1) * C4 - lo, tg, t)
                    tiles.append(t)
                hs = _dot(jnp.concatenate(tiles, axis=1).astype(BF16), w2_v[...])
                y1s.append(h2_v[pl.ds(r0, HB), :] + hs)
            gls = []
            f0 = Fh // LANES * LANES
            for y1 in y1s:
                ln = _ln(y1).astype(BF16)
                parts = [_gelu(_dot_nt(ln, w3_v[0:f0 // 2 // LANES * LANES, :]))]
                if f0 < Fh:
                    tail = _gelu(_dot_nt(w3_v[f0:Fh, :], ln)).T
                parts.append(_gelu(_dot_nt(ln, w3_v[f0 // 2 // LANES * LANES:f0, :])))
                if f0 < Fh:
                    parts.append(tail)
                gls.append(jnp.concatenate(parts, axis=1).astype(BF16))
            for r0, y1, gl in zip(sub_rows(r), y1s, gls):
                rows = pl.ds(r0, HB)
                h3 = _dot(gl, w4_v[...])
                o_v[rows, :] = (x1_v[rows, :]
                                + _rows_op(jnp.multiply, y1 + h3, mod(5))).astype(BF16)
                out_cp(r0).start()

        def s1_body(r, carry):
            stage1(r)
            return carry

        def s2_body(r, carry):
            for u in range(U2):
                stage2(r * U2 + u)
            return carry

        jax.lax.fori_loop(0, NR, s1_body, 0)
        jax.lax.fori_loop(0, NR // U2, s2_body, 0)
        cp(o_v, out_hbm, 0).wait()

    hbm_spec = pl.BlockSpec(memory_space=pltpu.HBM)
    V = pltpu.VMEM
    scratch = [
        V((S, M), BF16),
        V((1 + NSL, S, Dc), BF16),
        V((NG, M, HG, D), BF16),
        V((NG, Dc, HG, D), BF16),
        V((NG, Dc, HG, D), BF16),
        V((NG * _gstride(PLQ), D), U32),
        V((NG * _gstride(PLK), D), U32),
        V((NG * _gstride(PLK), D), U32),
        V((H * D, M), BF16),
        V((HG + 1, Dc, D), BF16),
        V((M, M), BF16),
        V((M, M), BF16),
        V((Fh, M), BF16),
        V((Fh, M), BF16),
        V((M, 2 * M), BF16),
        V((4 * NC + 1, M, LANES), BF16),
        V((16, 2 * M), F32),
        V((4 * NC + 4, 8, LANES), F32),
        V((M, LANES), F32),
        V((S, M), BF16),
        V((M // 2, D), U32),
        V((HG, Dc // 2, D), U32),
        V((S, D), BF16),
        V((HG, S // 2, D), U32),
        V((1, D // 2, S), U32),
        V((NQ, TQ, TQ), F32),
        V((NQ, TQ, TQ), F32),
        V((NQ, TQ, TQ), F32),
        V((NQ, TQ, TQ), F32),
        pltpu.SMEM((2,), jnp.int32),
        V((H, S, D), BF16),
        V((HG, S, D), F32),
        V((S, M), F32),
        V((S, M), F32),
        V((NC, S + 2 * PAD, LANES), F32),
        V((S, M), BF16),
        V((1, M), BF16),
        pltpu.SemaphoreType.DMA((NSEM,)),
    ]
    out, _ = pl.pallas_call(
        kernel,
        out_shape=(jax.ShapeDtypeStruct((S, M), BF16),
                   jax.ShapeDtypeStruct((NSL, S, Dc), BF16)),
        in_specs=[hbm_spec] * 12,
        out_specs=(hbm_spec, hbm_spec),
        scratch_shapes=scratch,
        compiler_params=pltpu.CompilerParams(vmem_limit_bytes=120 * 1024 * 1024),
        name="adaln_cla_mixer",
    )(x2, ckv2, A_w_q, A_w_uk, A_w_uv, wo2, B_w1, B_w2, B_w3.T, B_w4, c, w_mod)
    return out.reshape(B, S, M)
```

```python
import functools
import math

import jax
import jax.numpy as jnp
import jax.experimental.pallas as pl
import jax.experimental.pallas.tpu as pltpu

BF16 = jnp.bfloat16
F32 = jnp.float32
U32 = jnp.uint32

LANES = 128
TQ = 128
TR = 256
HB = 128
HG = 8
RCH = 4
LOOK = 4
AHEAD = 2
NSB = 4
DIST = 12
KC = 256
PC = 512
QC = 128
QH = 256
U2 = 2
PAD = 16
EPS = 1e-5
LOG2E = math.log2(math.e)
NEG = -1000000000.0 * LOG2E

_NT = (((1,), (1,)), ((), ()))


def _ln(x):
    m = jnp.mean(x, axis=-1, keepdims=True)
    xc = x - m
    v = jnp.mean(xc * xc, axis=-1, keepdims=True)
    return xc * jax.lax.rsqrt(v + EPS)


def _gelu(x):
    return jax.nn.gelu(x, approximate=True)


def _dot(a, b):
    return jnp.dot(a, b, preferred_element_type=F32)


def _dot_nt(a, b):
    return jax.lax.dot_general(a, b, _NT, preferred_element_type=F32)


def _fold8(x, op):
    parts = [op(x[j:j + 8], x[j + 8:j + 16]) for j in range(0, x.shape[0], 16)]
    acc = parts[0]
    for p in parts[1:]:
        acc = op(acc, p)
    return acc


def _rows_op(op, x, v8):
    r, m = x.shape
    return op(x.reshape(r // 8, 8, m), v8[None]).reshape(r, m)


def _modulate(x, scale8, shift8):
    r, m = x.shape
    return (x.reshape(r // 8, 8, m) * scale8[None] + shift8[None]).reshape(r, m)


def _pack(x):
    return pltpu.bitcast(x.astype(BF16), U32)


def _unpack(w):
    return pltpu.bitcast(w, BF16)


def _gstride(plane):
    return -(-8 * plane // 32) * 32


def _tied(w, tie):
    return jnp.concatenate([w[0:8] | tie, w[8:]], axis=0)


def _run(*gens):
    gens = list(gens)
    while gens:
        for g in list(gens):
            if next(g, gens) is gens:
                gens.remove(g)


@jax.jit
def pallas_adaLN_cond__compressed_kv_cla__mixer_s_mlp__prompt_kernel(
    A_x: jax.Array,
    A_c_kv: jax.Array,
    A_w_q: jax.Array,
    A_w_uk: jax.Array,
    A_w_uv: jax.Array,
    A_w_o: jax.Array,
    B_x: jax.Array,
    B_w1: jax.Array,
    B_w2: jax.Array,
    B_w3: jax.Array,
    B_w4: jax.Array,
    c: jax.Array,
    w_mod: jax.Array,
):
    del B_x
    B, S, M = A_x.shape
    _, Sk, Dc = A_c_kv.shape
    _, H, D = A_w_q.shape
    Fh = B_w3.shape[1]
    assert B == 1 and Sk == S and D == LANES and H % HG == 0 and HG == 8
    assert S % TQ == 0 and S % TR == 0 and S % PC == 0 and TR % HB == 0
    assert M % LANES == 0 and M % 64 == 0 and Dc % 64 == 0
    NG = H // HG
    NQ = S // TQ
    NR = S // TR
    NC = M // LANES
    C4 = M // 4
    PLQ = M // 2 + 1
    PLK = Dc // 2 + 1
    NK = S // KC
    XC = S // RCH
    NSEM = NK + 5
    assert NK > RCH + 1 and NQ % 2 == 0 and LOOK % 2 == 0
    HS = Dc // D
    NSL = -(-HG // NC)
    assert H % 2 == 0 and RCH % 2 == 0 and RCH + 4 * NC <= H and NSL * HS + 2 < H - HG
    qscale = float(D) ** -0.5 * LOG2E

    x2 = A_x.reshape(S, M)
    ckv2 = A_c_kv.reshape(S, Dc)
    wo2 = A_w_o.reshape(H * D, M)

    def kernel(x_hbm, ckv_hbm, wq_hbm, wuk_hbm, wuv_hbm, wo_hbm, w1_hbm, w2_hbm,
               w3_hbm, w4_hbm, c_hbm, wmod_hbm, out_hbm, slab_hbm,
               x_v, lhs_v, wq_r, wuk_r, wuv_r, wq_p, wuk_p, wuv_p, wo_v, wou_v, w1_v,
               w2_v, w3_v, w4_v, wmoda_v, wmodb_v, moda_v, modb_v, scb_v, hn_v, wqc_v, wk0_v, q_v, k_v,
               vt_v, s0, s1, s2, s3, z_s, ctx_v, part_v, x1_v, h2_v, hh_v, o_v, c_v,
               sems):

        s_v = (s0, s1, s2, s3)
        ckv_v = lhs_v.at[0]
        z_s[0] = 0
        z_s[1] = 0

        def aligned(i, n):
            return i * n if isinstance(i, int) else pl.multiple_of(i * n, n)

        def cp(src, dst, i):
            return pltpu.make_async_copy(src, dst, sems.at[i])

        def c_ckv(r):
            rows = pl.ds(aligned(r, KC), KC)
            return cp(ckv_hbm.at[rows, :], ckv_v.at[rows, :], r)

        def c_x(j):
            rows = pl.ds(aligned(j, XC), XC)
            return cp(x_hbm.at[rows, :], x_v.at[rows, :], NK - RCH + j)

        def c_q0(j):
            rows = pl.ds(aligned(j, M // RCH), M // RCH)
            return cp(wq_hbm.at[rows, pl.ds(0, HG), :], wq_r.at[0, rows], NK - RCH + j)

        def gcp(src, dst, g, i):
            return cp(src.at[:, pl.ds(g * HG, HG), :], dst.at[g], i)

        c_moda = cp(wmod_hbm.at[:, pl.ds(0, 2 * M)], wmoda_v, NK - RCH - 1)
        c_c = cp(c_hbm, c_v, NK)
        c_k0 = gcp(wuk_hbm, wuk_r, 0, NK + 1)
        c_v0 = gcp(wuv_hbm, wuv_r, 0, NK + 2)
        c_k1 = gcp(wuk_hbm, wuk_r, 1, NK + 3)
        c_late = []
        for g in range(1, NG):
            for src, dst, gg in ((wq_hbm, wq_r, g), (wuv_hbm, wuv_r, g), (wuk_hbm, wuk_r, g + 1)):
                if gg < NG:
                    c_late.append(gcp(src, dst, gg, NSEM - 1))
        for ct in range(4 * NC):
            c_late.append(cp(wmod_hbm.at[:, pl.ds(2 * M + ct * LANES, LANES)],
                             wmodb_v.at[ct], NSEM - 1))
        for u in range(HG):
            c_late.append(cp(wo_hbm.at[pl.ds(u // NC * Dc, Dc), pl.ds(u % NC * D, D)],
                             wou_v.at[u], NSEM - 1))
        for src, dst in ((wo_hbm, wo_v), (w1_hbm, w1_v), (w2_hbm, w2_v),
                         (w3_hbm, w3_v), (w4_hbm, w4_v)):
            c_late.append(cp(src, dst, NSEM - 1))
        order = [c_c, c_k0] + [c_ckv(r) for r in range(NK - RCH)] + [c_moda]
        for j in range(RCH):
            order += [c_ckv(NK - RCH + j), c_x(j), c_q0(j)]
        order += [c_v0, c_k1] + c_late
        for d in order:
            d.start()

        def relayout_steps(raw, dst, g, chunk, rows, plane):
            n = rows // RCH // 2
            base = g * _gstride(plane) + chunk * n
            if not isinstance(base, int):
                base = pl.multiple_of(base, 8)
            view = dst.at[pl.ds(base, 7 * plane + n), :]

            def step(j, tie):
                val = raw[g, pl.ds(chunk * (2 * n) + 2 * j, 2)].reshape(2 * HG, D)
                val = pltpu.bitcast(val, U32)
                if tie is not None:
                    val = val | tie
                view[pl.ds(j, 8, stride=plane), :] = val

            return [functools.partial(step, j) for j in range(n)]

        def relayout(raw, dst, g, rows, plane):
            for ch in range(RCH):
                for step in relayout_steps(raw, dst, g, ch, rows, plane):
                    step(None)

        def head_w32(src, h, rows, plane, par=None):
            base = (h // HG) * _gstride(plane) + ((h % HG) // 2) * plane
            ev = src[pl.ds(base, rows // 2), :]
            od = src[pl.ds(base + 4 * plane, rows // 2), :]
            par = h % 2 if par is None else par
            if par == 0:
                return (ev & U32(0xFFFF)) | (od << 16)
            return (ev >> 16) | (od & U32(0xFFFF0000))

        def q_rows(wq, lo, hi, ties=()):
            res = []
            for r0 in range(lo, hi, QC):
                rows = slice(r0, r0 + QC)
                w = _tied(wq, ties[len(res)]) if len(res) in ties else wq
                res.append(_dot(hn_v[rows, :], pltpu.bitcast(w, BF16)))
                q_v[rows, :] = (res[-1] * qscale).astype(BF16)
            return res

        def q_head(h, par=None, tie=None):
            wq = head_w32(wq_p, h, M, PLQ, par)
            if tie is not None:
                wq = _rows_op(jnp.bitwise_or, wq, tie)
            wqc_v[...] = wq
            return q_rows(wq, 0, QH)

        def q_mid(ties=()):
            q_rows(wqc_v[...], QH, S - PC, ties)

        def q_tail():
            return q_rows(wqc_v[...], S - PC, S)

        def k_slot(h, par, kh):
            late = h >= H - HG
            u = jnp.maximum(h - (H - HG), 0)
            wk = head_w32(wuk_p, jnp.where(late, h, h + HG), Dc, PLK, par)
            wu = pltpu.bitcast(wou_v[jnp.where(late, u, HG)], U32)
            w = _unpack(jnp.where(late, wu, wk))
            lhs = lhs_v.at[jnp.where(late, 1 + u // NC, 0)]
            for r in range(S // PC):
                rows = slice(r * PC, (r + 1) * PC)
                res = _dot(lhs[rows, :], w)
                kh[r * PC // 2:(r + 1) * PC // 2, :] = _pack(res)
                part_v[u, rows, :] = res

        def mod_tile(w):
            acc = _fold8(w.astype(F32) * scb_v[...], jnp.add)
            return jnp.broadcast_to(jnp.sum(acc, axis=0, keepdims=True), (8, LANES))

        def mod(i):
            if i < 2:
                return moda_v[0:8, i * M:(i + 1) * M]
            return jnp.concatenate(
                [modb_v[(i - 2) * NC + ct] for ct in range(NC)], axis=1)

        def zeros8():
            return jnp.full((8, LANES), z_s[1], jnp.int32).astype(U32)

        def k_chunk(r, nsub=1, ties=(), after=None, unpack=False):
            n = KC // nsub
            lhs = ckv_v[pl.ds(aligned(r, KC), KC), :]
            for h in range(HG):
                if unpack:
                    w32 = head_w32(wuk_p, h, Dc, PLK)
                    wk0_v[h] = w32
                else:
                    w32 = wk0_v[h]
                for j in range(nsub):
                    i = h * nsub + j
                    rows = pl.ds(aligned(r * nsub + j, n // 2), n // 2)
                    w = _tied(w32, ties[i]) if i in ties else w32
                    res = _dot(lhs[j * n:(j + 1) * n], pltpu.bitcast(w, BF16))
                    k_v[h, rows, :] = _pack(res)
                    if after is not None:
                        after(i, res)

        c_c.wait()
        cc = c_v[...].astype(F32)
        sc = (cc * jax.nn.sigmoid(cc)).astype(BF16).astype(F32)
        scb_v[...] = jnp.broadcast_to(sc, (LANES, M)).T
        zpad = jnp.zeros((PAD, LANES), F32)
        for cidx in range(NC):
            hh_v[cidx, 0:PAD, :] = zpad
            hh_v[cidx, PAD + S:PAD + S + PAD, :] = zpad
        wou_v[HG] = jnp.zeros((Dc, D), BF16)
        wmodb_v[4 * NC] = jnp.zeros((M, LANES), BF16)
        c_k0.wait()
        relayout(wuk_r, wuk_p, 0, Dc, PLK)

        def ka_body(r, carry):
            c_ckv(r).wait()
            k_chunk(r, unpack=True)
            return carry

        jax.lax.fori_loop(0, NK - RCH - 1, ka_body, 0)

        c_ckv(NK - RCH - 1).wait()
        c_moda.wait()
        zero8 = zeros8()
        ties = {}
        for ct in range(2 * NC):
            cols = slice(ct * LANES, (ct + 1) * LANES)
            tile = mod_tile(wmoda_v[:, cols])
            moda_v[0:8, cols] = tile
            ties[2 + (ct * (2 * HG - 2)) // (2 * NC)] = pltpu.bitcast(tile, U32) & zero8
        k_chunk(NK - RCH - 1, 2, ties)

        def kb_body(j, carry):
            c_ckv(NK - RCH + j).wait()
            c_x(j).wait()
            c_q0(j).wait()
            zero8 = zeros8()
            lr = XC // HG
            ties = {}
            scale, shift = 1.0 + mod(1), mod(0)
            for i in range(HG):
                rows = pl.ds(pl.multiple_of(j * XC + i * lr, lr), lr)
                hn = _modulate(_ln(x_v[rows, :].astype(F32)), scale, shift)
                hn_v[rows, :] = hn.astype(BF16)
                ties[i + 2] = pltpu.bitcast(_fold8(hn[:, 0:LANES], jnp.maximum), U32) & zero8
            steps = relayout_steps(wq_r, wq_p, 0, j, M, PLQ)
            per = len(steps) // HG

            def side(i, res):
                for k, step in enumerate(steps[i * per:(i + 1) * per]):
                    step(pltpu.bitcast(res[k * 8:(k + 1) * 8], U32) & zero8)

            k_chunk(NK - RCH + j, 1, ties, side)
            return carry

        jax.lax.fori_loop(0, RCH, kb_body, 0)

        c_v0.wait()
        zero8 = zeros8()
        res = jnp.concatenate(q_head(0), axis=0)
        steps = []
        for ch in range(RCH):
            steps += relayout_steps(wuv_r, wuv_p, 0, ch, Dc, PLK)
        for i, step in enumerate(steps):
            k = i * (QH // 8) // len(steps)
            step(pltpu.bitcast(res[k * 8:(k + 1) * 8], U32) & zero8)

        def attention(h, par, kh, side):
            HT = TQ // 2
            key_i = jax.lax.broadcasted_iota(jnp.int32, (HT, TQ), 0)
            qry_i = jax.lax.broadcasted_iota(jnp.int32, (HT, TQ), 1)
            causal_lo = key_i <= qry_i
            causal_hi = key_i + HT <= qry_i
            z_st = z_s[0]
            z_ld = z_s[1]
            zero8 = zeros8()

            m8 = {}
            seq = []

            def keys(*halves):
                ks = [kh[a * HT // 2:b * HT // 2, :] for a, b in halves]
                return _unpack(ks[0] if len(ks) == 1 else jnp.concatenate(ks, axis=0))

            def put(i, half, val):
                for k in range(val.shape[0] // HT):
                    t, off = (half + k) // 2, (half + k) % 2 * HT
                    s_v[i % NSB][z_st + t, off:off + HT, :] = val[k * HT:(k + 1) * HT]
                tm = _fold8(val, jnp.maximum)
                m8[i] = jnp.maximum(m8[i], tm) if i in m8 else tm

            def mm(a, b):
                res = _dot_nt(a, b)
                seq.append(res[0:8])
                return res

            def qk(i):
                qi = q_v[i * TQ:(i + 1) * TQ, :]
                if i % 2 == 0:
                    j = i + 1
                    strip = mm(q_v[j * TQ + HT:(j + 1) * TQ, :],
                               keys((2 * i + 1, 2 * i + 2), (2 * j + 1, 2 * j + 2)))
                    yield
                    qmix = jnp.concatenate(
                        [q_v[j * TQ:j * TQ + HT, :], q_v[i * TQ + HT:(i + 1) * TQ, :]], axis=0)
                    mix = mm(keys((2 * i + 1, 2 * i + 2)), qmix)
                    put(i, 2 * i + 1, jnp.where(causal_hi, mix, NEG))
                    st = jnp.concatenate([strip, strip], axis=0).T
                    put(j, 2 * i + 1, jnp.where(qry_i < HT, mix, st[0:HT]))
                    put(j, 2 * j + 1, jnp.where(causal_hi, st[HT:TQ], NEG))
                    yield
                for t in range(i - 1):
                    put(i, 2 * t, mm(keys((2 * t, 2 * t + 2)), qi))
                    yield
                if i % 2 == 0:
                    lo = max(2 * i - 2, 0)
                    res = mm(keys((lo, 2 * i + 1)), qi)
                    if i > 0:
                        put(i, lo, res[0:TQ])
                else:
                    res = mm(keys((2 * i - 2, 2 * i - 1), (2 * i, 2 * i + 1)), qi)
                    put(i, 2 * i - 2, res[0:HT])
                put(i, 2 * i, jnp.where(causal_lo, res[res.shape[0] - HT:], NEG))
                yield

            def pv(i):
                sb = s_v[i % NSB]
                mb = jnp.broadcast_to(jnp.max(m8[i], axis=0, keepdims=True), (8, TQ))
                l8 = None
                ot = None
                for t in range(i + 1):
                    tie = pltpu.bitcast(seq[-DIST], U32) & zero8
                    mt = pltpu.bitcast(pltpu.bitcast(mb, U32) | tie, F32)
                    tile = sb[z_ld + t].reshape(TQ // 8, 8, TQ)
                    p = jnp.exp2(tile - mt[None]).reshape(TQ, TQ)
                    part = _fold8(p, jnp.add)
                    l8 = part if l8 is None else l8 + part
                    o = _dot(_unpack(vt_v[z_ld, :, t * TQ:(t + 1) * TQ]), p.astype(BF16))
                    seq.append(o[0:8])
                    ot = o if ot is None else ot + o
                    if t == i:
                        l = jnp.sum(l8, axis=0, keepdims=True)
                        ot = ot * (1.0 / l)
                        ctx_v[h, i * TQ:(i + 1) * TQ, :] = ot.T.astype(BF16)
                    yield

            for i in range(LOOK):
                _run(qk(i))
            vt = _dot_nt(_unpack(head_w32(wuv_p, h, Dc, PLK, par)).T, ckv_v[...])
            vt_v[z_st] = _pack(vt)
            prev = vt[0:8, S - TQ:S]
            for res in q_tail():
                seq.extend([prev] * NC)
                prev = res[0:8]
            per = max(1, -(-len(side) // NQ))
            for j, step in enumerate(side):
                ct, rg = j // per, (j % per) * (D // 8) // per
                src = vt[rg * 8:(rg + 1) * 8, ct * TQ:(ct + 1) * TQ]
                step(pltpu.bitcast(src, U32) & zero8)
            for i in range(NQ):
                j = i + AHEAD
                if LOOK <= j < NQ:
                    _run(qk(j), pv(i))
                else:
                    _run(pv(i))
            return pltpu.bitcast(seq[-DIST], U32) & zero8

        def side_work(h):
            g = jnp.minimum(h // HG + ((h % HG) >= RCH).astype(jnp.int32), NG - 1)
            ch = h % RCH
            steps = (relayout_steps(wq_r, wq_p, g, ch, M, PLQ)
                     + relayout_steps(wuv_r, wuv_p, g, ch, Dc, PLK))
            gk = jnp.minimum(h // HG + 1, NG - 1)
            for c in range(RCH):
                steps += relayout_steps(wuk_r, wuk_p, gk, c, Dc, PLK)
            return steps

        c_up = [cp(ctx_v.at[h], slab_hbm.at[h // HS, :, pl.ds(h % HS * D, D)], 1)
                for h in range(NSL * HS)]
        c_down = cp(slab_hbm, lhs_v.at[pl.ds(1, NSL)], 2)

        def head(h, par):
            ct = jnp.where(jnp.logical_and(h >= RCH, h < RCH + 4 * NC), h - RCH, 4 * NC)
            tile = mod_tile(wmodb_v[ct])
            modb_v[ct] = tile
            kh = k_v.at[h % HG]
            q_mid({4: pltpu.bitcast(tile, U32) & zeros8()})
            tie = attention(h, par, kh, side_work(h))
            q_head(jnp.minimum(h + 1, H - 2 + (1 - par)), 1 - par, tie)
            k_slot(h, par, kh)

        def pair_body(j, carry):
            h = 2 * j

            @pl.when(h == RCH)
            def _():
                for d in c_late:
                    d.wait()

            @pl.when(h == NSL * HS + 2)
            def _():
                for d in c_up:
                    d.wait()

            @pl.when(h == H - HG)
            def _():
                c_down.wait()

            @pl.when(h == NSL * HS)
            def _():
                for d in c_up:
                    d.start()

            @pl.when(h == NSL * HS + 2)
            def _():
                c_down.start()

            head(h, 0)
            head(h + 1, 1)
            return carry

        c_k1.wait()
        jax.lax.fori_loop(0, H // 2, pair_body, 0)

        def sub_rows(r):
            out = []
            for j in range(TR // HB):
                r0 = r * TR + j * HB
                if not isinstance(r0, int):
                    r0 = pl.multiple_of(r0, HB)
                out.append(r0)
            return out

        def stage1(r):
            atts = []
            for r0 in sub_rows(r):
                rows = pl.ds(r0, HB)
                ctx = [ctx_v[h, rows, :] for h in range(H)]
                cols = []
                for ct in range(NC):
                    units = list(range(ct, HG, NC))
                    h0 = len(units) * HS
                    col = _dot(jnp.concatenate(ctx[h0:], axis=1),
                               wo_v[h0 * D:H * D, ct * LANES:(ct + 1) * LANES])
                    for u in units:
                        col = col + part_v[u, rows, :]
                    cols.append(col)
                atts.append(jnp.concatenate(cols, axis=1))
            lns = []
            for r0, att in zip(sub_rows(r), atts):
                rows = pl.ds(r0, HB)
                x1 = x_v[rows, :].astype(F32) + _rows_op(jnp.multiply, att, mod(2))
                x1_v[rows, :] = x1
                h2 = _modulate(_ln(x1), 1.0 + mod(4), mod(3))
                h2_v[rows, :] = h2
                lns.append(_ln(h2).astype(BF16))
            for r0, ln in zip(sub_rows(r), lns):
                u = _gelu(_dot(ln, w1_v[...]))
                for cidx in range(NC):
                    hh_v[cidx, pl.ds(r0 + PAD, HB), :] = u[:, cidx * LANES:(cidx + 1) * LANES]

        shifts = (1, -1, 2, -2)

        def out_cp(r0):
            rows = pl.ds(r0, HB)
            return cp(o_v.at[rows, :], out_hbm.at[rows, :], 0)

        def stage2(r):
            lane_i = jax.lax.broadcasted_iota(jnp.int32, (HB, LANES), 1)
            y1s = []
            for r0 in sub_rows(r):
                tiles = []
                for cidx in range(NC):
                    lo, hi = cidx * LANES, (cidx + 1) * LANES
                    g_lo, g_hi = lo // C4, (hi - 1) // C4
                    t = hh_v[cidx, pl.ds(r0 + PAD - shifts[g_hi], HB), :]
                    for g in range(g_hi - 1, g_lo - 1, -1):
                        tg = hh_v[cidx, pl.ds(r0 + PAD - shifts[g], HB), :]
                        t = jnp.where(lane_i < (g + 1) * C4 - lo, tg, t)
                    tiles.append(t)
                hs = _dot(jnp.concatenate(tiles, axis=1).astype(BF16), w2_v[...])
                y1s.append(h2_v[pl.ds(r0, HB), :] + hs)
            gls = []
            f0 = Fh // LANES * LANES
            for y1 in y1s:
                ln = _ln(y1).astype(BF16)
                parts = [_gelu(_dot_nt(ln, w3_v[0:f0 // 2 // LANES * LANES, :]))]
                if f0 < Fh:
                    tail = _gelu(_dot_nt(w3_v[f0:Fh, :], ln)).T
                parts.append(_gelu(_dot_nt(ln, w3_v[f0 // 2 // LANES * LANES:f0, :])))
                if f0 < Fh:
                    parts.append(tail)
                gls.append(jnp.concatenate(parts, axis=1).astype(BF16))
            for r0, y1, gl in zip(sub_rows(r), y1s, gls):
                rows = pl.ds(r0, HB)
                h3 = _dot(gl, w4_v[...])
                o_v[rows, :] = (x1_v[rows, :]
                                + _rows_op(jnp.multiply, y1 + h3, mod(5))).astype(BF16)
                out_cp(r0).start()

        def s1_body(r, carry):
            stage1(r)
            return carry

        def s2_body(r, carry):
            for u in range(U2):
                stage2(r * U2 + u)
            return carry

        jax.lax.fori_loop(0, NR, s1_body, 0)
        jax.lax.fori_loop(0, NR // U2, s2_body, 0)
        cp(o_v, out_hbm, 0).wait()

    hbm_spec = pl.BlockSpec(memory_space=pltpu.HBM)
    V = pltpu.VMEM
    scratch = [
        V((S, M), BF16),
        V((1 + NSL, S, Dc), BF16),
        V((NG, M, HG, D), BF16),
        V((NG, Dc, HG, D), BF16),
        V((NG, Dc, HG, D), BF16),
        V((NG * _gstride(PLQ), D), U32),
        V((NG * _gstride(PLK), D), U32),
        V((NG * _gstride(PLK), D), U32),
        V((H * D, M), BF16),
        V((HG + 1, Dc, D), BF16),
        V((M, M), BF16),
        V((M, M), BF16),
        V((Fh, M), BF16),
        V((Fh, M), BF16),
        V((M, 2 * M), BF16),
        V((4 * NC + 1, M, LANES), BF16),
        V((16, 2 * M), F32),
        V((4 * NC + 4, 8, LANES), F32),
        V((M, LANES), F32),
        V((S, M), BF16),
        V((M // 2, D), U32),
        V((HG, Dc // 2, D), U32),
        V((S, D), BF16),
        V((HG, S // 2, D), U32),
        V((1, D // 2, S), U32),
        V((NQ, TQ, TQ), F32),
        V((NQ, TQ, TQ), F32),
        V((NQ, TQ, TQ), F32),
        V((NQ, TQ, TQ), F32),
        pltpu.SMEM((2,), jnp.int32),
        V((H, S, D), BF16),
        V((HG, S, D), F32),
        V((S, M), F32),
        V((S, M), F32),
        V((NC, S + 2 * PAD, LANES), F32),
        V((S, M), BF16),
        V((1, M), BF16),
        pltpu.SemaphoreType.DMA((NSEM,)),
    ]
    out, _ = pl.pallas_call(
        kernel,
        out_shape=(jax.ShapeDtypeStruct((S, M), BF16),
                   jax.ShapeDtypeStruct((NSL, S, Dc), BF16)),
        in_specs=[hbm_spec] * 12,
        out_specs=(hbm_spec, hbm_spec),
        scratch_shapes=scratch,
        compiler_params=pltpu.CompilerParams(vmem_limit_bytes=120 * 1024 * 1024),
        name="adaln_cla_mixer",
    )(x2, ckv2, A_w_q, A_w_uk, A_w_uv, wo2, B_w1, B_w2, B_w3.T, B_w4, c, w_mod)
    return out.reshape(B, S, M)
```

```python
import functools
import math
import os

import jax
import jax.numpy as jnp
import jax.experimental.pallas as pl
import jax.experimental.pallas.tpu as pltpu

BF16 = jnp.bfloat16
F32 = jnp.float32
U32 = jnp.uint32

LANES = 128
TQ = 128
TR = 256
HB = 128
HG = 8
RCH = 4
LOOK = int(os.environ.get('LOOK', 6))
AHEAD = int(os.environ.get('AHEAD', 2))
NSB = int(os.environ.get('NSB', 6))
DIST = int(os.environ.get('DIST', 11))
KC = 256
PC = int(os.environ.get('PC', 384))
QC = 128
U2 = 2
KS = int(os.environ.get('KS', 512))
TCH = int(os.environ.get('TCH', 0))
MT = int(os.environ.get('MT', 4))
PAD = 16
EPS = 1e-5
LOG2E = math.log2(math.e)
NEG = -1000000000.0 * LOG2E

_NT = (((1,), (1,)), ((), ()))


def _ln(x):
    m = jnp.mean(x, axis=-1, keepdims=True)
    xc = x - m
    v = jnp.mean(xc * xc, axis=-1, keepdims=True)
    return xc * jax.lax.rsqrt(v + EPS)


def _gelu(x):
    return jax.nn.gelu(x, approximate=True)


def _dot(a, b):
    return jnp.dot(a, b, preferred_element_type=F32)


def _dot_nt(a, b):
    return jax.lax.dot_general(a, b, _NT, preferred_element_type=F32)


def _fold8(x, op):
    parts = [op(x[j:j + 8], x[j + 8:j + 16]) for j in range(0, x.shape[0], 16)]
    acc = parts[0]
    for p in parts[1:]:
        acc = op(acc, p)
    return acc


def _rows_op(op, x, v8):
    r, m = x.shape
    return op(x.reshape(r // 8, 8, m), v8[None]).reshape(r, m)


def _modulate(x, scale8, shift8):
    r, m = x.shape
    return (x.reshape(r // 8, 8, m) * scale8[None] + shift8[None]).reshape(r, m)


def _pack(x):
    return pltpu.bitcast(x.astype(BF16), U32)


def _unpack(w):
    return pltpu.bitcast(w, BF16)


def _gstride(plane):
    return -(-8 * plane // 32) * 32


def _tied(w, tie):
    return jnp.concatenate([w[0:8] | tie, w[8:]], axis=0)


def _run(*gens):
    gens = list(gens)
    while gens:
        for g in list(gens):
            if next(g, gens) is gens:
                gens.remove(g)


@jax.jit
def pallas_adaLN_cond__compressed_kv_cla__mixer_s_mlp__prompt_kernel(
    A_x: jax.Array,
    A_c_kv: jax.Array,
    A_w_q: jax.Array,
    A_w_uk: jax.Array,
    A_w_uv: jax.Array,
    A_w_o: jax.Array,
    B_x: jax.Array,
    B_w1: jax.Array,
    B_w2: jax.Array,
    B_w3: jax.Array,
    B_w4: jax.Array,
    c: jax.Array,
    w_mod: jax.Array,
):
    del B_x
    B, S, M = A_x.shape
    _, Sk, Dc = A_c_kv.shape
    _, H, D = A_w_q.shape
    Fh = B_w3.shape[1]
    assert B == 1 and Sk == S and D == LANES and H % HG == 0 and HG == 8
    assert S % TQ == 0 and S % TR == 0 and TR % HB == 0
    assert M % LANES == 0 and M % 64 == 0 and Dc % 64 == 0
    NG = H // HG
    NQ = S // TQ
    NR = S // TR
    NC = M // LANES
    C4 = M // 4
    PLQ = M // 2 + 1
    PLK = Dc // 2 + 1
    NK = S // KC
    XC = S // RCH
    NSEM = NK + 5
    assert NK > RCH + 1 and NQ % 2 == 0 and LOOK % 2 == 0 and NSB >= max(LOOK, AHEAD + 2)
    HS = Dc // D
    NSL = -(-HG // NC)
    assert H % 2 == 0 and RCH % 2 == 0 and RCH + 4 * NC <= H and NSL * HS + 2 < H - HG
    qscale = float(D) ** -0.5 * LOG2E

    x2 = A_x.reshape(S, M)
    ckv2 = A_c_kv.reshape(S, Dc)
    wo2 = A_w_o.reshape(H * D, M)

    def kernel(x_hbm, ckv_hbm, wq_hbm, wuk_hbm, wuv_hbm, wo_hbm, w1_hbm, w2_hbm,
               w3_hbm, w4_hbm, c_hbm, wmod_hbm, out_hbm, slab_hbm,
               x_v, lhs_v, wq_r, wuk_r, wuv_r, wq_p, wuk_p, wuv_p, wo_v, wou_v, w1_v,
               w2_v, w3_v, w4_v, wmoda_v, wmodb_v, moda_v, modb_v, scb_v, hn_v, wqc_v, wk0_v, q_v, k_v,
               vt_v, s_v, z_s, ctx_v, part_v, x1_v, h2_v, hh_v, o_v, c_v,
               sems):

        ckv_v = lhs_v.at[0]
        z_s[0] = 0
        z_s[1] = 0

        def aligned(i, n):
            return i * n if isinstance(i, int) else pl.multiple_of(i * n, n)

        def cp(src, dst, i):
            return pltpu.make_async_copy(src, dst, sems.at[i])

        def c_ckv(r):
            rows = pl.ds(aligned(r, KC), KC)
            return cp(ckv_hbm.at[rows, :], ckv_v.at[rows, :], r)

        def c_x(j):
            rows = pl.ds(aligned(j, XC), XC)
            return cp(x_hbm.at[rows, :], x_v.at[rows, :], NK - RCH + j)

        def c_q0(j):
            rows = pl.ds(aligned(j, M // RCH), M // RCH)
            return cp(wq_hbm.at[rows, pl.ds(0, HG), :], wq_r.at[0, rows], NK - RCH + j)

        def gcp(src, dst, g, i):
            return cp(src.at[:, pl.ds(g * HG, HG), :], dst.at[g], i)

        c_moda = cp(wmod_hbm.at[:, pl.ds(0, 2 * M)], wmoda_v, NK - RCH - 1)
        c_c = cp(c_hbm, c_v, NK)
        c_k0 = gcp(wuk_hbm, wuk_r, 0, NK + 1)
        c_v0 = gcp(wuv_hbm, wuv_r, 0, NK + 2)
        c_k1 = gcp(wuk_hbm, wuk_r, 1, NK + 3)
        c_late = []
        for g in range(1, NG):
            for src, dst, gg in ((wq_hbm, wq_r, g), (wuv_hbm, wuv_r, g), (wuk_hbm, wuk_r, g + 1)):
                if gg < NG:
                    c_late.append(gcp(src, dst, gg, NSEM - 1))
        for ct in range(4 * NC):
            c_late.append(cp(wmod_hbm.at[:, pl.ds(2 * M + ct * LANES, LANES)],
                             wmodb_v.at[ct], NSEM - 1))
        for u in range(HG):
            c_late.append(cp(wo_hbm.at[pl.ds(u // NC * Dc, Dc), pl.ds(u % NC * D, D)],
                             wou_v.at[u], NSEM - 1))
        for src, dst in ((wo_hbm, wo_v), (w1_hbm, w1_v), (w2_hbm, w2_v),
                         (w3_hbm, w3_v), (w4_hbm, w4_v)):
            c_late.append(cp(src, dst, NSEM - 1))
        order = [c_c, c_k0] + [c_ckv(r) for r in range(NK - RCH)] + [c_moda]
        for j in range(RCH):
            order += [c_ckv(NK - RCH + j), c_x(j), c_q0(j)]
        order += [c_v0, c_k1] + c_late
        for d in order:
            d.start()

        def relayout_steps(raw, dst, g, chunk, rows, plane):
            n = rows // RCH // 2
            base = g * _gstride(plane) + chunk * n
            if not isinstance(base, int):
                base = pl.multiple_of(base, 8)
            view = dst.at[pl.ds(base, 7 * plane + n), :]

            def step(j, tie):
                val = raw[g, pl.ds(chunk * (2 * n) + 2 * j, 2)].reshape(2 * HG, D)
                val = pltpu.bitcast(val, U32)
                if tie is not None:
                    val = val | tie
                view[pl.ds(j, 8, stride=plane), :] = val

            return [functools.partial(step, j) for j in range(n)]

        def relayout(raw, dst, g, rows, plane):
            for ch in range(RCH):
                for step in relayout_steps(raw, dst, g, ch, rows, plane):
                    step(None)

        def head_w32(src, h, rows, plane, par=None):
            base = (h // HG) * _gstride(plane) + ((h % HG) // 2) * plane
            ev = src[pl.ds(base, rows // 2), :]
            od = src[pl.ds(base + 4 * plane, rows // 2), :]
            par = h % 2 if par is None else par
            if par == 0:
                return (ev & U32(0xFFFF)) | (od << 16)
            return (ev >> 16) | (od & U32(0xFFFF0000))

        def q_weight(h, par=None, tie=None):
            wq = head_w32(wq_p, h, M, PLQ, par)
            if tie is not None:
                wq = wq | _rows_op(jnp.bitwise_and, pltpu.bitcast(tie[0:M // 2], U32), zeros8())
            wqc_v[...] = wq

        def q_rows(lo, hi, ties=()):
            wq = wqc_v[...]
            res = []
            for r0 in range(lo, hi, QC):
                rows = slice(r0, r0 + QC)
                w = _tied(wq, ties[len(res)]) if len(res) in ties else wq
                res.append(_dot(hn_v[rows, :], _unpack(w)))
                q_v[rows, :] = (res[-1] * qscale).astype(BF16)
            return res

        def slot_weight(h, par):
            late = h >= H - HG
            wk = head_w32(wuk_p, jnp.where(late, h, h + HG), Dc, PLK, par)
            wu = pltpu.bitcast(wou_v[jnp.where(late, h - (H - HG), HG)], U32)
            return jnp.where(late, wu, wk)

        def k_slot(h, w, kh):
            u = jnp.maximum(h - (H - HG), 0)
            lhs = lhs_v.at[jnp.where(h >= H - HG, 1 + u // NC, 0)]
            first = None
            for r in range(S // KS):
                rows = slice(r * KS, (r + 1) * KS)
                res = _dot(lhs[rows, :], _unpack(w))
                kh[r * KS // 2:(r + 1) * KS // 2, :] = _pack(res)
                part_v[u, rows, :] = res
                first = res if r == TCH else first
            return first

        def mod_tile(w):
            acc = _fold8(w.astype(F32) * scb_v[...], jnp.add)
            return jnp.broadcast_to(jnp.sum(acc, axis=0, keepdims=True), (8, LANES))

        def mod(i):
            if i < 2:
                return moda_v[0:8, i * M:(i + 1) * M]
            return jnp.concatenate(
                [modb_v[(i - 2) * NC + ct] for ct in range(NC)], axis=1)

        def zeros8():
            return jnp.full((8, LANES), z_s[1], jnp.int32).astype(U32)

        def k_chunk(r, nsub=1, ties=(), after=None, unpack=False):
            n = KC // nsub
            lhs = ckv_v[pl.ds(aligned(r, KC), KC), :]
            for h in range(HG):
                if unpack:
                    w32 = head_w32(wuk_p, h, Dc, PLK)
                    wk0_v[h] = w32
                else:
                    w32 = wk0_v[h]
                for j in range(nsub):
                    i = h * nsub + j
                    rows = pl.ds(aligned(r * nsub + j, n // 2), n // 2)
                    w = _tied(w32, ties[i]) if i in ties else w32
                    res = _dot(lhs[j * n:(j + 1) * n], pltpu.bitcast(w, BF16))
                    k_v[h, rows, :] = _pack(res)
                    if after is not None:
                        after(i, res)

        c_c.wait()
        cc = c_v[...].astype(F32)
        sc = (cc * jax.nn.sigmoid(cc)).astype(BF16).astype(F32)
        scb_v[...] = jnp.broadcast_to(sc, (LANES, M)).T
        zpad = jnp.zeros((PAD, LANES), F32)
        for cidx in range(NC):
            hh_v[cidx, 0:PAD, :] = zpad
            hh_v[cidx, PAD + S:PAD + S + PAD, :] = zpad
        wou_v[HG] = jnp.zeros((Dc, D), BF16)
        wmodb_v[4 * NC] = jnp.zeros((M, LANES), BF16)
        c_k0.wait()
        relayout(wuk_r, wuk_p, 0, Dc, PLK)

        def ka_body(r, carry):
            c_ckv(r).wait()
            k_chunk(r, unpack=True)
            return carry

        jax.lax.fori_loop(0, NK - RCH - 1, ka_body, 0)

        c_ckv(NK - RCH - 1).wait()
        c_moda.wait()
        zero8 = zeros8()
        ties = {}
        for ct in range(2 * NC):
            cols = slice(ct * LANES, (ct + 1) * LANES)
            tile = mod_tile(wmoda_v[:, cols])
            moda_v[0:8, cols] = tile
            ties[2 + (ct * (2 * HG - 2)) // (2 * NC)] = pltpu.bitcast(tile, U32) & zero8
        k_chunk(NK - RCH - 1, 2, ties)

        def kb_body(j, carry):
            c_ckv(NK - RCH + j).wait()
            c_x(j).wait()
            c_q0(j).wait()
            zero8 = zeros8()
            lr = XC // HG
            ties = {}
            scale, shift = 1.0 + mod(1), mod(0)
            for i in range(HG):
                rows = pl.ds(pl.multiple_of(j * XC + i * lr, lr), lr)
                hn = _modulate(_ln(x_v[rows, :].astype(F32)), scale, shift)
                hn_v[rows, :] = hn.astype(BF16)
                ties[i + 2] = pltpu.bitcast(_fold8(hn[:, 0:LANES], jnp.maximum), U32) & zero8
            steps = relayout_steps(wq_r, wq_p, 0, j, M, PLQ)
            per = len(steps) // HG

            def side(i, res):
                for k, step in enumerate(steps[i * per:(i + 1) * per]):
                    step(pltpu.bitcast(res[k * 8:(k + 1) * 8], U32) & zero8)

            k_chunk(NK - RCH + j, 1, ties, side)
            return carry

        jax.lax.fori_loop(0, RCH, kb_body, 0)

        q_weight(0)
        c_v0.wait()
        relayout(wuv_r, wuv_p, 0, Dc, PLK)

        def attention(h, par, kh, side):
            HT = TQ // 2
            key_i = jax.lax.broadcasted_iota(jnp.int32, (HT, TQ), 0)
            qry_i = jax.lax.broadcasted_iota(jnp.int32, (HT, TQ), 1)
            causal_lo = key_i <= qry_i
            causal_hi = key_i + HT <= qry_i
            z_st = z_s[0]
            z_ld = z_s[1]
            zero8 = zeros8()

            m8 = {}
            seq = []

            def keys(*halves):
                ks = [kh[a * HT // 2:b * HT // 2, :] for a, b in halves]
                return _unpack(ks[0] if len(ks) == 1 else jnp.concatenate(ks, axis=0))

            def put(i, half, val):
                for k in range(val.shape[0] // HT):
                    t, off = (half + k) // 2, (half + k) % 2 * HT
                    s_v[i % NSB][z_st + t, off:off + HT, :] = val[k * HT:(k + 1) * HT]
                tm = _fold8(val, jnp.maximum)
                m8[i] = jnp.maximum(m8[i], tm) if i in m8 else tm

            def mm(a, b):
                res = _dot_nt(a, b)
                seq.append(res[0:8])
                return res

            def qk(i):
                qi = q_v[i * TQ:(i + 1) * TQ, :]
                if i % 2 == 0:
                    j = i + 1
                    strip = mm(q_v[j * TQ + HT:(j + 1) * TQ, :],
                               keys((2 * i + 1, 2 * i + 2), (2 * j + 1, 2 * j + 2)))
                    yield
                    qmix = jnp.concatenate(
                        [q_v[j * TQ:j * TQ + HT, :], q_v[i * TQ + HT:(i + 1) * TQ, :]], axis=0)
                    mix = mm(keys((2 * i + 1, 2 * i + 2)), qmix)
                    put(i, 2 * i + 1, jnp.where(causal_hi, mix, NEG))
                    st = jnp.concatenate([strip, strip], axis=0).T
                    put(j, 2 * i + 1, jnp.where(qry_i < HT, mix, st[0:HT]))
                    put(j, 2 * j + 1, jnp.where(causal_hi, st[HT:TQ], NEG))
                    yield
                for t in range(i - 1):
                    put(i, 2 * t, mm(keys((2 * t, 2 * t + 2)), qi))
                    yield
                if i % 2 == 0:
                    lo = max(2 * i - 2, 0)
                    res = mm(keys((lo, 2 * i + 1)), qi)
                    if i > 0:
                        put(i, lo, res[0:TQ])
                else:
                    res = mm(keys((2 * i - 2, 2 * i - 1), (2 * i, 2 * i + 1)), qi)
                    put(i, 2 * i - 2, res[0:HT])
                put(i, 2 * i, jnp.where(causal_lo, res[res.shape[0] - HT:], NEG))
                yield

            def pv(i):
                sb = s_v[i % NSB]
                mb = jnp.broadcast_to(jnp.max(m8[i], axis=0, keepdims=True), (8, TQ))
                l8 = None
                ot = None
                for t in range(i + 1):
                    tie = pltpu.bitcast(seq[-DIST], U32) & zero8
                    mt = pltpu.bitcast(pltpu.bitcast(mb, U32) | tie, F32)
                    tile = sb[z_ld + t].reshape(TQ // 8, 8, TQ)
                    p = jnp.exp2(tile - mt[None]).reshape(TQ, TQ)
                    part = _fold8(p, jnp.add)
                    l8 = part if l8 is None else l8 + part
                    o = _dot(_unpack(vt_v[z_ld, :, t * TQ:(t + 1) * TQ]), p.astype(BF16))
                    seq.append(o[0:8])
                    ot = o if ot is None else ot + o
                    if t == i:
                        l = jnp.sum(l8, axis=0, keepdims=True)
                        ot = ot * (1.0 / l)
                        ctx_v[h, i * TQ:(i + 1) * TQ, :] = ot.T.astype(BF16)
                    yield

            for i in range(LOOK):
                _run(qk(i))
            vt = _dot_nt(_unpack(head_w32(wuv_p, h, Dc, PLK, par)).T, ckv_v[...])
            vt_v[z_st] = _pack(vt)
            prev = vt[0:8, S - TQ:S]
            for res in q_rows(S - PC, S):
                seq.extend([prev] * NC)
                prev = res[0:8]
            per = max(1, -(-len(side) // NQ))
            for j, step in enumerate(side):
                ct, rg = j // per, (j % per) * (D // 8) // per
                src = vt[rg * 8:(rg + 1) * 8, ct * TQ:(ct + 1) * TQ]
                step(pltpu.bitcast(src, U32) & zero8)
            for i in range(NQ):
                j = i + AHEAD
                if LOOK <= j < NQ:
                    _run(qk(j), pv(i))
                else:
                    _run(pv(i))

        def side_work(h):
            g = jnp.minimum(h // HG + ((h % HG) >= RCH).astype(jnp.int32), NG - 1)
            ch = h % RCH
            steps = (relayout_steps(wq_r, wq_p, g, ch, M, PLQ)
                     + relayout_steps(wuv_r, wuv_p, g, ch, Dc, PLK))
            gk = jnp.minimum(h // HG + 1, NG - 1)
            for c in range(RCH):
                steps += relayout_steps(wuk_r, wuk_p, gk, c, Dc, PLK)
            return steps

        c_up = [cp(ctx_v.at[h], slab_hbm.at[h // HS, :, pl.ds(h % HS * D, D)], 1)
                for h in range(NSL * HS)]
        c_down = cp(slab_hbm, lhs_v.at[pl.ds(1, NSL)], 2)

        def head(h, par):
            ct = jnp.where(jnp.logical_and(h >= RCH, h < RCH + 4 * NC), h - RCH, 4 * NC)
            tile = mod_tile(wmodb_v[ct])
            modb_v[ct] = tile
            kh = k_v.at[h % HG]
            q_rows(0, S - PC, {MT: pltpu.bitcast(tile, U32) & zeros8()})
            attention(h, par, kh, side_work(h))
            tie = k_slot(h, slot_weight(h, par), kh)
            q_weight(jnp.minimum(h + 1, H - 2 + (1 - par)), 1 - par, tie)

        def pair_body(j, carry):
            h = 2 * j

            @pl.when(h == RCH)
            def _():
                for d in c_late:
                    d.wait()

            @pl.when(h == NSL * HS + 2)
            def _():
                for d in c_up:
                    d.wait()

            @pl.when(h == H - HG)
            def _():
                c_down.wait()

            @pl.when(h == NSL * HS)
            def _():
                for d in c_up:
                    d.start()

            @pl.when(h == NSL * HS + 2)
            def _():
                c_down.start()

            head(h, 0)
            head(h + 1, 1)
            return carry

        c_k1.wait()
        jax.lax.fori_loop(0, H // 2, pair_body, 0)

        def sub_rows(r):
            out = []
            for j in range(TR // HB):
                r0 = r * TR + j * HB
                if not isinstance(r0, int):
                    r0 = pl.multiple_of(r0, HB)
                out.append(r0)
            return out

        def stage1(r):
            atts = []
            for r0 in sub_rows(r):
                rows = pl.ds(r0, HB)
                ctx = [ctx_v[h, rows, :] for h in range(H)]
                cols = []
                for ct in range(NC):
                    units = list(range(ct, HG, NC))
                    h0 = len(units) * HS
                    col = _dot(jnp.concatenate(ctx[h0:], axis=1),
                               wo_v[h0 * D:H * D, ct * LANES:(ct + 1) * LANES])
                    for u in units:
                        col = col + part_v[u, rows, :]
                    cols.append(col)
                atts.append(jnp.concatenate(cols, axis=1))
            lns = []
            for r0, att in zip(sub_rows(r), atts):
                rows = pl.ds(r0, HB)
                x1 = x_v[rows, :].astype(F32) + _rows_op(jnp.multiply, att, mod(2))
                x1_v[rows, :] = x1
                h2 = _modulate(_ln(x1), 1.0 + mod(4), mod(3))
                h2_v[rows, :] = h2
                lns.append(_ln(h2).astype(BF16))
            for r0, ln in zip(sub_rows(r), lns):
                u = _gelu(_dot(ln, w1_v[...]))
                for cidx in range(NC):
                    hh_v[cidx, pl.ds(r0 + PAD, HB), :] = u[:, cidx * LANES:(cidx + 1) * LANES]

        shifts = (1, -1, 2, -2)

        def out_cp(r0):
            rows = pl.ds(r0, HB)
            return cp(o_v.at[rows, :], out_hbm.at[rows, :], 0)

        def stage2(r):
            lane_i = jax.lax.broadcasted_iota(jnp.int32, (HB, LANES), 1)
            y1s = []
            for r0 in sub_rows(r):
                tiles = []
                for cidx in range(NC):
                    lo, hi = cidx * LANES, (cidx + 1) * LANES
                    g_lo, g_hi = lo // C4, (hi - 1) // C4
                    t = hh_v[cidx, pl.ds(r0 + PAD - shifts[g_hi], HB), :]
                    for g in range(g_hi - 1, g_lo - 1, -1):
                        tg = hh_v[cidx, pl.ds(r0 + PAD - shifts[g], HB), :]
                        t = jnp.where(lane_i < (g + 1) * C4 - lo, tg, t)
                    tiles.append(t)
                hs = _dot(jnp.concatenate(tiles, axis=1).astype(BF16), w2_v[...])
                y1s.append(h2_v[pl.ds(r0, HB), :] + hs)
            gls = []
            f0 = Fh // LANES * LANES
            for y1 in y1s:
                ln = _ln(y1).astype(BF16)
                parts = [_gelu(_dot_nt(ln, w3_v[0:f0 // 2 // LANES * LANES, :]))]
                if f0 < Fh:
                    tail = _gelu(_dot_nt(w3_v[f0:Fh, :], ln)).T
                parts.append(_gelu(_dot_nt(ln, w3_v[f0 // 2 // LANES * LANES:f0, :])))
                if f0 < Fh:
                    parts.append(tail)
                gls.append(jnp.concatenate(parts, axis=1).astype(BF16))
            for r0, y1, gl in zip(sub_rows(r), y1s, gls):
                rows = pl.ds(r0, HB)
                h3 = _dot(gl, w4_v[...])
                o_v[rows, :] = (x1_v[rows, :]
                                + _rows_op(jnp.multiply, y1 + h3, mod(5))).astype(BF16)
                out_cp(r0).start()

        def s1_body(r, carry):
            stage1(r)
            return carry

        def s2_body(r, carry):
            for u in range(U2):
                stage2(r * U2 + u)
            return carry

        jax.lax.fori_loop(0, NR, s1_body, 0)
        jax.lax.fori_loop(0, NR // U2, s2_body, 0)
        cp(o_v, out_hbm, 0).wait()

    hbm_spec = pl.BlockSpec(memory_space=pltpu.HBM)
    V = pltpu.VMEM
    scratch = [
        V((S, M), BF16),
        V((1 + NSL, S, Dc), BF16),
        V((NG, M, HG, D), BF16),
        V((NG, Dc, HG, D), BF16),
        V((NG, Dc, HG, D), BF16),
        V((NG * _gstride(PLQ), D), U32),
        V((NG * _gstride(PLK), D), U32),
        V((NG * _gstride(PLK), D), U32),
        V((H * D, M), BF16),
        V((HG + 1, Dc, D), BF16),
        V((M, M), BF16),
        V((M, M), BF16),
        V((Fh, M), BF16),
        V((Fh, M), BF16),
        V((M, 2 * M), BF16),
        V((4 * NC + 1, M, LANES), BF16),
        V((16, 2 * M), F32),
        V((4 * NC + 4, 8, LANES), F32),
        V((M, LANES), F32),
        V((S, M), BF16),
        V((M // 2, D), U32),
        V((HG, Dc // 2, D), U32),
        V((S, D), BF16),
        V((HG, S // 2, D), U32),
        V((1, D // 2, S), U32),
        [V((NQ, TQ, TQ), F32)] * NSB,
        pltpu.SMEM((2,), jnp.int32),
        V((H, S, D), BF16),
        V((HG, S, D), F32),
        V((S, M), F32),
        V((S, M), F32),
        V((NC, S + 2 * PAD, LANES), F32),
        V((S, M), BF16),
        V((1, M), BF16),
        pltpu.SemaphoreType.DMA((NSEM,)),
    ]
    out, _ = pl.pallas_call(
        kernel,
        out_shape=(jax.ShapeDtypeStruct((S, M), BF16),
                   jax.ShapeDtypeStruct((NSL, S, Dc), BF16)),
        in_specs=[hbm_spec] * 12,
        out_specs=(hbm_spec, hbm_spec),
        scratch_shapes=scratch,
        compiler_params=pltpu.CompilerParams(vmem_limit_bytes=120 * 1024 * 1024),
        name="adaln_cla_mixer",
    )(x2, ckv2, A_w_q, A_w_uk, A_w_uv, wo2, B_w1, B_w2, B_w3.T, B_w4, c, w_mod)
    return out.reshape(B, S, M)
```

```python
import functools
import math
import os

import jax
import jax.numpy as jnp
import jax.experimental.pallas as pl
import jax.experimental.pallas.tpu as pltpu

BF16 = jnp.bfloat16
F32 = jnp.float32
U32 = jnp.uint32

LANES = 128
TQ = 128
TR = 256
HB = 128
HG = 8
RCH = 4
LOOK = int(os.environ.get('LOOK', 6))
AHEAD = int(os.environ.get('AHEAD', 2))
NSB = int(os.environ.get('NSB', 6))
DIST = int(os.environ.get('DIST', 11))
KC = 256
PC = int(os.environ.get('PC', 384))
QC = 128
U2 = 2
KS = int(os.environ.get('KS', 512))
TCH = int(os.environ.get('TCH', 0))
MT = int(os.environ.get('MT', 4))
PAD = 16
EPS = 1e-5
LOG2E = math.log2(math.e)
NEG = -1000000000.0 * LOG2E

_NT = (((1,), (1,)), ((), ()))


def _ln(x):
    m = jnp.mean(x, axis=-1, keepdims=True)
    xc = x - m
    v = jnp.mean(xc * xc, axis=-1, keepdims=True)
    return xc * jax.lax.rsqrt(v + EPS)


def _gelu(x):
    return jax.nn.gelu(x, approximate=True)


def _dot(a, b):
    return jnp.dot(a, b, preferred_element_type=F32)


def _dot_nt(a, b):
    return jax.lax.dot_general(a, b, _NT, preferred_element_type=F32)


def _fold8(x, op):
    parts = [op(x[j:j + 8], x[j + 8:j + 16]) for j in range(0, x.shape[0], 16)]
    acc = parts[0]
    for p in parts[1:]:
        acc = op(acc, p)
    return acc


def _rows_op(op, x, v8):
    r, m = x.shape
    return op(x.reshape(r // 8, 8, m), v8[None]).reshape(r, m)


def _modulate(x, scale8, shift8):
    r, m = x.shape
    return (x.reshape(r // 8, 8, m) * scale8[None] + shift8[None]).reshape(r, m)


def _pack(x):
    return pltpu.bitcast(x.astype(BF16), U32)


def _unpack(w):
    return pltpu.bitcast(w, BF16)


def _gstride(plane):
    return -(-8 * plane // 32) * 32


def _tied(w, tie):
    return jnp.concatenate([w[0:8] | tie, w[8:]], axis=0)


def _run(*gens):
    gens = list(gens)
    while gens:
        for g in list(gens):
            if next(g, gens) is gens:
                gens.remove(g)


@jax.jit
def pallas_adaLN_cond__compressed_kv_cla__mixer_s_mlp__prompt_kernel(
    A_x: jax.Array,
    A_c_kv: jax.Array,
    A_w_q: jax.Array,
    A_w_uk: jax.Array,
    A_w_uv: jax.Array,
    A_w_o: jax.Array,
    B_x: jax.Array,
    B_w1: jax.Array,
    B_w2: jax.Array,
    B_w3: jax.Array,
    B_w4: jax.Array,
    c: jax.Array,
    w_mod: jax.Array,
):
    del B_x
    B, S, M = A_x.shape
    _, Sk, Dc = A_c_kv.shape
    _, H, D = A_w_q.shape
    Fh = B_w3.shape[1]
    assert B == 1 and Sk == S and D == LANES and H % HG == 0 and HG == 8
    assert S % TQ == 0 and S % TR == 0 and TR % HB == 0
    assert M % LANES == 0 and M % 64 == 0 and Dc % 64 == 0
    NG = H // HG
    NQ = S // TQ
    NR = S // TR
    NC = M // LANES
    C4 = M // 4
    PLQ = M // 2 + 1
    PLK = Dc // 2 + 1
    NK = S // KC
    XC = S // RCH
    NSEM = NK + 5
    assert NK > RCH + 1 and NQ % 2 == 0 and LOOK % 2 == 0 and NSB >= max(LOOK, AHEAD + 2)
    HS = Dc // D
    NSL = -(-HG // NC)
    assert H % 2 == 0 and RCH % 2 == 0 and RCH + 4 * NC <= H and NSL * HS + 2 < H - HG
    qscale = float(D) ** -0.5 * LOG2E

    x2 = A_x.reshape(S, M)
    ckv2 = A_c_kv.reshape(S, Dc)
    wo2 = A_w_o.reshape(H * D, M)

    def kernel(x_hbm, ckv_hbm, wq_hbm, wuk_hbm, wuv_hbm, wo_hbm, w1_hbm, w2_hbm,
               w3_hbm, w4_hbm, c_hbm, wmod_hbm, out_hbm, slab_hbm,
               x_v, lhs_v, wq_r, wuk_r, wuv_r, wq_p, wuk_p, wuv_p, wo_v, wou_v, w1_v,
               w2_v, w3_v, w4_v, wmoda_v, wmodb_v, moda_v, modb_v, scb_v, hn_v, wqc_v, wk0_v, q_v, k_v,
               vt_v, s_v, z_s, ctx_v, part_v, x1_v, h2_v, hh_v, o_v, c_v,
               sems):

        ckv_v = lhs_v.at[0]
        z_s[0] = 0
        z_s[1] = 0

        def aligned(i, n):
            return i * n if isinstance(i, int) else pl.multiple_of(i * n, n)

        def cp(src, dst, i):
            return pltpu.make_async_copy(src, dst, sems.at[i])

        def c_ckv(r):
            rows = pl.ds(aligned(r, KC), KC)
            return cp(ckv_hbm.at[rows, :], ckv_v.at[rows, :], r)

        def c_x(j):
            rows = pl.ds(aligned(j, XC), XC)
            return cp(x_hbm.at[rows, :], x_v.at[rows, :], NK - RCH + j)

        def c_q0(j):
            rows = pl.ds(aligned(j, M // RCH), M // RCH)
            return cp(wq_hbm.at[rows, pl.ds(0, HG), :], wq_r.at[0, rows], NK - RCH + j)

        def gcp(src, dst, g, i):
            return cp(src.at[:, pl.ds(g * HG, HG), :], dst.at[g], i)

        c_moda = cp(wmod_hbm.at[:, pl.ds(0, 2 * M)], wmoda_v, NK - RCH - 1)
        c_c = cp(c_hbm, c_v, NK)
        c_k0 = gcp(wuk_hbm, wuk_r, 0, NK + 1)
        c_v0 = gcp(wuv_hbm, wuv_r, 0, NK + 2)
        c_k1 = gcp(wuk_hbm, wuk_r, 1, NK + 3)
        c_late = []
        for g in range(1, NG):
            for src, dst, gg in ((wq_hbm, wq_r, g), (wuv_hbm, wuv_r, g), (wuk_hbm, wuk_r, g + 1)):
                if gg < NG:
                    c_late.append(gcp(src, dst, gg, NSEM - 1))
        for ct in range(4 * NC):
            c_late.append(cp(wmod_hbm.at[:, pl.ds(2 * M + ct * LANES, LANES)],
                             wmodb_v.at[ct], NSEM - 1))
        for u in range(HG):
            c_late.append(cp(wo_hbm.at[pl.ds(u // NC * Dc, Dc), pl.ds(u % NC * D, D)],
                             wou_v.at[u], NSEM - 1))
        for src, dst in ((wo_hbm, wo_v), (w1_hbm, w1_v), (w2_hbm, w2_v),
                         (w3_hbm, w3_v), (w4_hbm, w4_v)):
            c_late.append(cp(src, dst, NSEM - 1))
        order = [c_c, c_k0] + [c_ckv(r) for r in range(NK - RCH)] + [c_moda]
        for j in range(RCH):
            order += [c_ckv(NK - RCH + j), c_x(j), c_q0(j)]
        order += [c_v0, c_k1] + c_late
        for d in order:
            d.start()

        def relayout_steps(raw, dst, g, chunk, rows, plane):
            n = rows // RCH // 2
            base = g * _gstride(plane) + chunk * n
            if not isinstance(base, int):
                base = pl.multiple_of(base, 8)
            view = dst.at[pl.ds(base, 7 * plane + n), :]

            def step(j, tie):
                val = raw[g, pl.ds(chunk * (2 * n) + 2 * j, 2)].reshape(2 * HG, D)
                val = pltpu.bitcast(val, U32)
                if tie is not None:
                    val = val | tie
                view[pl.ds(j, 8, stride=plane), :] = val

            return [functools.partial(step, j) for j in range(n)]

        def relayout(raw, dst, g, rows, plane):
            for ch in range(RCH):
                for step in relayout_steps(raw, dst, g, ch, rows, plane):
                    step(None)

        def head_w32(src, h, rows, plane, par=None):
            base = (h // HG) * _gstride(plane) + ((h % HG) // 2) * plane
            ev = src[pl.ds(base, rows // 2), :]
            od = src[pl.ds(base + 4 * plane, rows // 2), :]
            par = h % 2 if par is None else par
            if par == 0:
                return (ev & U32(0xFFFF)) | (od << 16)
            return (ev >> 16) | (od & U32(0xFFFF0000))

        def q_weight(h, par=None, tie=None):
            wq = head_w32(wq_p, h, M, PLQ, par)
            if tie is not None:
                wq = wq | _rows_op(jnp.bitwise_and, pltpu.bitcast(tie[0:M // 2], U32), zeros8())
            wqc_v[...] = wq

        def q_rows(lo, hi, ties=()):
            wq = wqc_v[...]
            res = []
            for r0 in range(lo, hi, QC):
                rows = slice(r0, r0 + QC)
                w = _tied(wq, ties[len(res)]) if len(res) in ties else wq
                res.append(_dot(hn_v[rows, :], _unpack(w)))
                q_v[rows, :] = (res[-1] * qscale).astype(BF16)
            return res

        def slot_weight(h, par):
            late = h >= H - HG
            wk = head_w32(wuk_p, jnp.where(late, h, h + HG), Dc, PLK, par)
            wu = pltpu.bitcast(wou_v[jnp.where(late, h - (H - HG), HG)], U32)
            return jnp.where(late, wu, wk)

        def k_slot(h, w, kh):
            u = jnp.maximum(h - (H - HG), 0)
            lhs = lhs_v.at[jnp.where(h >= H - HG, 1 + u // NC, 0)]
            first = None
            for r in range(S // KS):
                rows = slice(r * KS, (r + 1) * KS)
                res = _dot(lhs[rows, :], _unpack(w))
                kh[r * KS // 2:(r + 1) * KS // 2, :] = _pack(res)
                part_v[u, rows, :] = res
                first = res if r == TCH else first
            return first

        def mod_tile(w):
            acc = _fold8(w.astype(F32) * scb_v[...], jnp.add)
            return jnp.broadcast_to(jnp.sum(acc, axis=0, keepdims=True), (8, LANES))

        def mod(i):
            if i < 2:
                return moda_v[0:8, i * M:(i + 1) * M]
            return jnp.concatenate(
                [modb_v[(i - 2) * NC + ct] for ct in range(NC)], axis=1)

        def zeros8():
            return jnp.full((8, LANES), z_s[1], jnp.int32).astype(U32)

        def k_chunk(r, nsub=1, ties=(), after=None, unpack=False):
            n = KC // nsub
            lhs = ckv_v[pl.ds(aligned(r, KC), KC), :]
            for h in range(HG):
                if unpack:
                    w32 = head_w32(wuk_p, h, Dc, PLK)
                    wk0_v[h] = w32
                else:
                    w32 = wk0_v[h]
                for j in range(nsub):
                    i = h * nsub + j
                    rows = pl.ds(aligned(r * nsub + j, n // 2), n // 2)
                    w = _tied(w32, ties[i]) if i in ties else w32
                    res = _dot(lhs[j * n:(j + 1) * n], pltpu.bitcast(w, BF16))
                    k_v[h, rows, :] = _pack(res)
                    if after is not None:
                        after(i, res)

        c_c.wait()
        cc = c_v[...].astype(F32)
        sc = (cc * jax.nn.sigmoid(cc)).astype(BF16).astype(F32)
        scb_v[...] = jnp.broadcast_to(sc, (LANES, M)).T
        zpad = jnp.zeros((PAD, LANES), F32)
        for cidx in range(NC):
            hh_v[cidx, 0:PAD, :] = zpad
            hh_v[cidx, PAD + S:PAD + S + PAD, :] = zpad
        wou_v[HG] = jnp.zeros((Dc, D), BF16)
        wmodb_v[4 * NC] = jnp.zeros((M, LANES), BF16)
        c_k0.wait()
        relayout(wuk_r, wuk_p, 0, Dc, PLK)

        def ka_body(r, carry):
            c_ckv(r).wait()
            k_chunk(r, unpack=True)
            return carry

        jax.lax.fori_loop(0, NK - RCH - 1, ka_body, 0)

        c_ckv(NK - RCH - 1).wait()
        c_moda.wait()
        zero8 = zeros8()
        ties = {}
        for ct in range(2 * NC):
            cols = slice(ct * LANES, (ct + 1) * LANES)
            tile = mod_tile(wmoda_v[:, cols])
            moda_v[0:8, cols] = tile
            ties[2 + (ct * (2 * HG - 2)) // (2 * NC)] = pltpu.bitcast(tile, U32) & zero8
        k_chunk(NK - RCH - 1, 2, ties)

        def kb_body(j, carry):
            c_ckv(NK - RCH + j).wait()
            c_x(j).wait()
            c_q0(j).wait()
            zero8 = zeros8()
            lr = XC // HG
            ties = {}
            scale, shift = 1.0 + mod(1), mod(0)
            for i in range(HG):
                rows = pl.ds(pl.multiple_of(j * XC + i * lr, lr), lr)
                hn = _modulate(_ln(x_v[rows, :].astype(F32)), scale, shift)
                hn_v[rows, :] = hn.astype(BF16)
                ties[i + 2] = pltpu.bitcast(_fold8(hn[:, 0:LANES], jnp.maximum), U32) & zero8
            steps = relayout_steps(wq_r, wq_p, 0, j, M, PLQ)
            per = len(steps) // HG

            def side(i, res):
                for k, step in enumerate(steps[i * per:(i + 1) * per]):
                    step(pltpu.bitcast(res[k * 8:(k + 1) * 8], U32) & zero8)

            k_chunk(NK - RCH + j, 1, ties, side)
            return carry

        jax.lax.fori_loop(0, RCH, kb_body, 0)

        q_weight(0)
        c_v0.wait()
        relayout(wuv_r, wuv_p, 0, Dc, PLK)

        def attention(h, par, kh, side):
            HT = TQ // 2
            key_i = jax.lax.broadcasted_iota(jnp.int32, (HT, TQ), 0)
            qry_i = jax.lax.broadcasted_iota(jnp.int32, (HT, TQ), 1)
            causal_lo = key_i <= qry_i
            causal_hi = key_i + HT <= qry_i
            z_st = z_s[0]
            z_ld = z_s[1]
            zero8 = zeros8()

            m8 = {}
            seq = []

            def keys(*halves):
                ks = [kh[a * HT // 2:b * HT // 2, :] for a, b in halves]
                return _unpack(ks[0] if len(ks) == 1 else jnp.concatenate(ks, axis=0))

            def put(i, half, val):
                for k in range(val.shape[0] // HT):
                    t, off = (half + k) // 2, (half + k) % 2 * HT
                    s_v[i % NSB][z_st + t, off:off + HT, :] = val[k * HT:(k + 1) * HT]
                tm = _fold8(val, jnp.maximum)
                m8[i] = jnp.maximum(m8[i], tm) if i in m8 else tm

            def mm(a, b):
                res = _dot_nt(a, b)
                seq.append(res[0:8])
                return res

            def qk(i):
                qi = q_v[i * TQ:(i + 1) * TQ, :]
                if i % 2 == 0:
                    j = i + 1
                    strip = mm(q_v[j * TQ + HT:(j + 1) * TQ, :],
                               keys((2 * i + 1, 2 * i + 2), (2 * j + 1, 2 * j + 2)))
                    yield
                    qmix = jnp.concatenate(
                        [q_v[j * TQ:j * TQ + HT, :], q_v[i * TQ + HT:(i + 1) * TQ, :]], axis=0)
                    mix = mm(keys((2 * i + 1, 2 * i + 2)), qmix)
                    put(i, 2 * i + 1, jnp.where(causal_hi, mix, NEG))
                    st = jnp.concatenate([strip, strip], axis=0).T
                    put(j, 2 * i + 1, jnp.where(qry_i < HT, mix, st[0:HT]))
                    put(j, 2 * j + 1, jnp.where(causal_hi, st[HT:TQ], NEG))
                    yield
                for t in range(i - 1):
                    put(i, 2 * t, mm(keys((2 * t, 2 * t + 2)), qi))
                    yield
                if i % 2 == 0:
                    lo = max(2 * i - 2, 0)
                    res = mm(keys((lo, 2 * i + 1)), qi)
                    if i > 0:
                        put(i, lo, res[0:TQ])
                else:
                    res = mm(keys((2 * i - 2, 2 * i - 1), (2 * i, 2 * i + 1)), qi)
                    put(i, 2 * i - 2, res[0:HT])
                put(i, 2 * i, jnp.where(causal_lo, res[res.shape[0] - HT:], NEG))
                yield

            def pv(i):
                sb = s_v[i % NSB]
                mb = jnp.broadcast_to(jnp.max(m8[i], axis=0, keepdims=True), (8, TQ))
                l8 = None
                ot = None
                for t in range(i + 1):
                    tie = pltpu.bitcast(seq[-DIST], U32) & zero8
                    mt = pltpu.bitcast(pltpu.bitcast(mb, U32) | tie, F32)
                    tile = sb[z_ld + t].reshape(TQ // 8, 8, TQ)
                    p = jnp.exp2(tile - mt[None]).reshape(TQ, TQ)
                    part = _fold8(p, jnp.add)
                    l8 = part if l8 is None else l8 + part
                    o = _dot(_unpack(vt_v[z_ld, :, t * TQ:(t + 1) * TQ]), p.astype(BF16))
                    seq.append(o[0:8])
                    ot = o if ot is None else ot + o
                    if t == i:
                        l = jnp.sum(l8, axis=0, keepdims=True)
                        ot = ot * (1.0 / l)
                        ctx_v[h, i * TQ:(i + 1) * TQ, :] = ot.T.astype(BF16)
                    yield

            for i in range(LOOK):
                _run(qk(i))
            vt = _dot_nt(_unpack(head_w32(wuv_p, h, Dc, PLK, par)).T, ckv_v[...])
            vt_v[z_st] = _pack(vt)
            prev = vt[0:8, S - TQ:S]
            for res in q_rows(S - PC, S):
                seq.extend([prev] * NC)
                prev = res[0:8]
            per = max(1, -(-len(side) // NQ))
            for j, step in enumerate(side):
                ct, rg = j // per, (j % per) * (D // 8) // per
                src = vt[rg * 8:(rg + 1) * 8, ct * TQ:(ct + 1) * TQ]
                step(pltpu.bitcast(src, U32) & zero8)
            for i in range(NQ):
                j = i + AHEAD
                if LOOK <= j < NQ:
                    _run(qk(j), pv(i))
                else:
                    _run(pv(i))

        def side_work(h):
            g = jnp.minimum(h // HG + ((h % HG) >= RCH).astype(jnp.int32), NG - 1)
            ch = h % RCH
            steps = (relayout_steps(wq_r, wq_p, g, ch, M, PLQ)
                     + relayout_steps(wuv_r, wuv_p, g, ch, Dc, PLK))
            gk = jnp.minimum(h // HG + 1, NG - 1)
            for c in range(RCH):
                steps += relayout_steps(wuk_r, wuk_p, gk, c, Dc, PLK)
            return steps

        c_up = [cp(ctx_v.at[h], slab_hbm.at[h // HS, :, pl.ds(h % HS * D, D)], 1)
                for h in range(NSL * HS)]
        c_down = cp(slab_hbm, lhs_v.at[pl.ds(1, NSL)], 2)

        def head(h, par):
            ct = jnp.where(jnp.logical_and(h >= RCH, h < RCH + 4 * NC), h - RCH, 4 * NC)
            tile = mod_tile(wmodb_v[ct])
            modb_v[ct] = tile
            kh = k_v.at[h % HG]
            q_rows(0, S - PC, {MT: pltpu.bitcast(tile, U32) & zeros8()})
            attention(h, par, kh, side_work(h))
            tie = k_slot(h, slot_weight(h, par), kh)
            q_weight(jnp.minimum(h + 1, H - 2 + (1 - par)), 1 - par, tie)

        def pair_body(j, carry):
            h = 2 * j

            @pl.when(h == RCH)
            def _():
                for d in c_late:
                    d.wait()

            @pl.when(h == NSL * HS + 2)
            def _():
                for d in c_up:
                    d.wait()

            @pl.when(h == H - HG)
            def _():
                c_down.wait()

            @pl.when(h == NSL * HS)
            def _():
                for d in c_up:
                    d.start()

            @pl.when(h == NSL * HS + 2)
            def _():
                c_down.start()

            head(h, 0)
            head(h + 1, 1)
            return carry

        c_k1.wait()
        jax.lax.fori_loop(0, H // 2, pair_body, 0)

        def sub_rows(r):
            out = []
            for j in range(TR // HB):
                r0 = r * TR + j * HB
                if not isinstance(r0, int):
                    r0 = pl.multiple_of(r0, HB)
                out.append(r0)
            return out

        def stage1(r):
            atts = []
            for r0 in sub_rows(r):
                rows = pl.ds(r0, HB)
                ctx = [ctx_v[h, rows, :] for h in range(H)]
                cols = []
                for ct in range(NC):
                    units = list(range(ct, HG, NC))
                    h0 = len(units) * HS
                    col = _dot(jnp.concatenate(ctx[h0:], axis=1),
                               wo_v[h0 * D:H * D, ct * LANES:(ct + 1) * LANES])
                    for u in units:
                        col = col + part_v[u, rows, :]
                    cols.append(col)
                atts.append(jnp.concatenate(cols, axis=1))
            lns = []
            for r0, att in zip(sub_rows(r), atts):
                rows = pl.ds(r0, HB)
                x1 = x_v[rows, :].astype(F32) + _rows_op(jnp.multiply, att, mod(2))
                x1_v[rows, :] = x1
                h2 = _modulate(_ln(x1), 1.0 + mod(4), mod(3))
                h2_v[rows, :] = h2
                lns.append(_ln(h2).astype(BF16))
            for r0, ln in zip(sub_rows(r), lns):
                u = _gelu(_dot(ln, w1_v[...]))
                for cidx in range(NC):
                    hh_v[cidx, pl.ds(r0 + PAD, HB), :] = u[:, cidx * LANES:(cidx + 1) * LANES]

        shifts = (1, -1, 2, -2)

        def stage2(r, last):
            lane_i = jax.lax.broadcasted_iota(jnp.int32, (HB, LANES), 1)
            y1s = []
            for r0 in sub_rows(r):
                tiles = []
                for cidx in range(NC):
                    lo, hi = cidx * LANES, (cidx + 1) * LANES
                    g_lo, g_hi = lo // C4, (hi - 1) // C4
                    t = hh_v[cidx, pl.ds(r0 + PAD - shifts[g_hi], HB), :]
                    for g in range(g_hi - 1, g_lo - 1, -1):
                        tg = hh_v[cidx, pl.ds(r0 + PAD - shifts[g], HB), :]
                        t = jnp.where(lane_i < (g + 1) * C4 - lo, tg, t)
                    tiles.append(t)
                hs = _dot(jnp.concatenate(tiles, axis=1).astype(BF16), w2_v[...])
                y1s.append(h2_v[pl.ds(r0, HB), :] + hs)
            gls = []
            f0 = Fh // LANES * LANES
            for y1 in y1s:
                ln = _ln(y1).astype(BF16)
                parts = [_gelu(_dot_nt(ln, w3_v[0:f0 // 2 // LANES * LANES, :]))]
                if f0 < Fh:
                    tail = _gelu(_dot_nt(w3_v[f0:Fh, :], ln)).T
                parts.append(_gelu(_dot_nt(ln, w3_v[f0 // 2 // LANES * LANES:f0, :])))
                if f0 < Fh:
                    parts.append(tail)
                gls.append(jnp.concatenate(parts, axis=1).astype(BF16))
            for k, (r0, y1, gl) in enumerate(zip(sub_rows(r), y1s, gls)):
                rows = pl.ds(r0, HB)
                h3 = _dot(gl, w4_v[...])
                out = x1_v[rows, :] + _rows_op(jnp.multiply, y1 + h3, mod(5))
                split = last and k == len(gls) - 1
                for lo, hi in ((0, M - LANES), (M - LANES, M)) if split else ((0, M),):
                    cols = pl.ds(lo, hi - lo)
                    o_v[rows, cols] = out[:, lo:hi].astype(BF16)
                    cp(o_v.at[rows, cols], out_hbm.at[rows, cols], 0).start()

        def s1_body(r, carry):
            stage1(r)
            return carry

        def s2_body(r, carry):
            for u in range(U2):
                stage2(r * U2 + u, u == U2 - 1)
            return carry

        jax.lax.fori_loop(0, NR, s1_body, 0)
        jax.lax.fori_loop(0, NR // U2, s2_body, 0)
        cp(o_v, out_hbm, 0).wait()

    hbm_spec = pl.BlockSpec(memory_space=pltpu.HBM)
    V = pltpu.VMEM
    scratch = [
        V((S, M), BF16),
        V((1 + NSL, S, Dc), BF16),
        V((NG, M, HG, D), BF16),
        V((NG, Dc, HG, D), BF16),
        V((NG, Dc, HG, D), BF16),
        V((NG * _gstride(PLQ), D), U32),
        V((NG * _gstride(PLK), D), U32),
        V((NG * _gstride(PLK), D), U32),
        V((H * D, M), BF16),
        V((HG + 1, Dc, D), BF16),
        V((M, M), BF16),
        V((M, M), BF16),
        V((Fh, M), BF16),
        V((Fh, M), BF16),
        V((M, 2 * M), BF16),
        V((4 * NC + 1, M, LANES), BF16),
        V((16, 2 * M), F32),
        V((4 * NC + 4, 8, LANES), F32),
        V((M, LANES), F32),
        V((S, M), BF16),
        V((M // 2, D), U32),
        V((HG, Dc // 2, D), U32),
        V((S, D), BF16),
        V((HG, S // 2, D), U32),
        V((1, D // 2, S), U32),
        [V((NQ, TQ, TQ), F32)] * NSB,
        pltpu.SMEM((2,), jnp.int32),
        V((H, S, D), BF16),
        V((HG, S, D), F32),
        V((S, M), F32),
        V((S, M), F32),
        V((NC, S + 2 * PAD, LANES), F32),
        V((S, M), BF16),
        V((1, M), BF16),
        pltpu.SemaphoreType.DMA((NSEM,)),
    ]
    out, _ = pl.pallas_call(
        kernel,
        out_shape=(jax.ShapeDtypeStruct((S, M), BF16),
                   jax.ShapeDtypeStruct((NSL, S, Dc), BF16)),
        in_specs=[hbm_spec] * 12,
        out_specs=(hbm_spec, hbm_spec),
        scratch_shapes=scratch,
        compiler_params=pltpu.CompilerParams(vmem_limit_bytes=120 * 1024 * 1024),
        name="adaln_cla_mixer",
    )(x2, ckv2, A_w_q, A_w_uk, A_w_uv, wo2, B_w1, B_w2, B_w3.T, B_w4, c, w_mod)
    return out.reshape(B, S, M)
```

```python
import functools
import math
import os

import jax
import jax.numpy as jnp
import jax.experimental.pallas as pl
import jax.experimental.pallas.tpu as pltpu

BF16 = jnp.bfloat16
F32 = jnp.float32
U32 = jnp.uint32

LANES = 128
TQ = 128
TR = 256
HB = 128
HG = 8
RCH = 4
LOOK = int(os.environ.get('LOOK', 6))
AHEAD = int(os.environ.get('AHEAD', 2))
NSB = int(os.environ.get('NSB', 6))
DIST = int(os.environ.get('DIST', 11))
KC = 256
PC = int(os.environ.get('PC', 384))
QC = 128
U2 = 2
KS = int(os.environ.get('KS', 512))
TCH = int(os.environ.get('TCH', 0))
MT = int(os.environ.get('MT', 4))
PAD = 16
EPS = 1e-5
LOG2E = math.log2(math.e)
NEG = -1000000000.0 * LOG2E

_NT = (((1,), (1,)), ((), ()))


def _ln(x):
    m = jnp.mean(x, axis=-1, keepdims=True)
    xc = x - m
    v = jnp.mean(xc * xc, axis=-1, keepdims=True)
    return xc * jax.lax.rsqrt(v + EPS)


def _gelu(x):
    return jax.nn.gelu(x, approximate=True)


def _dot(a, b):
    return jnp.dot(a, b, preferred_element_type=F32)


def _dot_nt(a, b):
    return jax.lax.dot_general(a, b, _NT, preferred_element_type=F32)


def _fold8(x, op):
    parts = [op(x[j:j + 8], x[j + 8:j + 16]) for j in range(0, x.shape[0], 16)]
    acc = parts[0]
    for p in parts[1:]:
        acc = op(acc, p)
    return acc


def _rows_op(op, x, v8):
    r, m = x.shape
    return op(x.reshape(r // 8, 8, m), v8[None]).reshape(r, m)


def _modulate(x, scale8, shift8):
    r, m = x.shape
    return (x.reshape(r // 8, 8, m) * scale8[None] + shift8[None]).reshape(r, m)


def _pack(x):
    return pltpu.bitcast(x.astype(BF16), U32)


def _unpack(w):
    return pltpu.bitcast(w, BF16)


def _gstride(plane):
    return -(-8 * plane // 32) * 32


def _tied(w, tie):
    return jnp.concatenate([w[0:8] | tie, w[8:]], axis=0)


def _run(*gens):
    gens = list(gens)
    while gens:
        for g in list(gens):
            if next(g, gens) is gens:
                gens.remove(g)


@jax.jit
def pallas_adaLN_cond__compressed_kv_cla__mixer_s_mlp__prompt_kernel(
    A_x: jax.Array,
    A_c_kv: jax.Array,
    A_w_q: jax.Array,
    A_w_uk: jax.Array,
    A_w_uv: jax.Array,
    A_w_o: jax.Array,
    B_x: jax.Array,
    B_w1: jax.Array,
    B_w2: jax.Array,
    B_w3: jax.Array,
    B_w4: jax.Array,
    c: jax.Array,
    w_mod: jax.Array,
):
    del B_x
    B, S, M = A_x.shape
    _, Sk, Dc = A_c_kv.shape
    _, H, D = A_w_q.shape
    Fh = B_w3.shape[1]
    assert B == 1 and Sk == S and D == LANES and H % HG == 0 and HG == 8
    assert S % TQ == 0 and S % TR == 0 and TR % HB == 0
    assert M % LANES == 0 and M % 64 == 0 and Dc % 64 == 0
    NG = H // HG
    NQ = S // TQ
    NR = S // TR
    NC = M // LANES
    C4 = M // 4
    PLQ = M // 2 + 1
    PLK = Dc // 2 + 1
    NK = S // KC
    XC = S // RCH
    NSEM = NK + 5
    assert NK > RCH + 1 and NQ % 2 == 0 and LOOK % 2 == 0 and NSB >= max(LOOK, AHEAD + 2)
    HS = Dc // D
    NSL = -(-HG // NC)
    assert H % 2 == 0 and RCH % 2 == 0 and RCH + 4 * NC <= H and NSL * HS + 2 < H - HG
    qscale = float(D) ** -0.5 * LOG2E

    x2 = A_x.reshape(S, M)
    ckv2 = A_c_kv.reshape(S, Dc)
    wo2 = A_w_o.reshape(H * D, M)

    def kernel(x_hbm, ckv_hbm, wq_hbm, wuk_hbm, wuv_hbm, wo_hbm, w1_hbm, w2_hbm,
               w3_hbm, w4_hbm, c_hbm, wmod_hbm, out_hbm, slab_hbm,
               x_v, lhs_v, wq_r, wuk_r, wuv_r, wq_p, wuk_p, wuv_p, wo_v, wou_v, w1_v,
               w2_v, w3_v, w4_v, wmoda_v, wmodb_v, moda_v, modb_v, scb_v, hn_v, wqc_v, wk0_v, q_v, k_v,
               vt_v, s_v, z_s, ctx_v, part_v, x1_v, h2_v, hh_v, o_v, c_v,
               sems):

        ckv_v = lhs_v.at[0]
        z_s[0] = 0
        z_s[1] = 0

        def aligned(i, n):
            return i * n if isinstance(i, int) else pl.multiple_of(i * n, n)

        def cp(src, dst, i):
            return pltpu.make_async_copy(src, dst, sems.at[i])

        def c_ckv(r):
            rows = pl.ds(aligned(r, KC), KC)
            return cp(ckv_hbm.at[rows, :], ckv_v.at[rows, :], r)

        def c_x(j):
            rows = pl.ds(aligned(j, XC), XC)
            return cp(x_hbm.at[rows, :], x_v.at[rows, :], NK - RCH + j)

        def c_q0(j):
            rows = pl.ds(aligned(j, M // RCH), M // RCH)
            return cp(wq_hbm.at[rows, pl.ds(0, HG), :], wq_r.at[0, rows], NK - RCH + j)

        def gcp(src, dst, g, i):
            return cp(src.at[:, pl.ds(g * HG, HG), :], dst.at[g], i)

        c_moda = cp(wmod_hbm.at[:, pl.ds(0, 2 * M)], wmoda_v, NK - RCH - 1)
        c_c = cp(c_hbm, c_v, NK)
        c_k0 = gcp(wuk_hbm, wuk_r, 0, NK + 1)
        c_v0 = gcp(wuv_hbm, wuv_r, 0, NK + 2)
        c_k1 = gcp(wuk_hbm, wuk_r, 1, NK + 3)
        c_late = []
        for g in range(1, NG):
            for src, dst, gg in ((wq_hbm, wq_r, g), (wuv_hbm, wuv_r, g), (wuk_hbm, wuk_r, g + 1)):
                if gg < NG:
                    c_late.append(gcp(src, dst, gg, NSEM - 1))
        for ct in range(4 * NC):
            c_late.append(cp(wmod_hbm.at[:, pl.ds(2 * M + ct * LANES, LANES)],
                             wmodb_v.at[ct], NSEM - 1))
        for u in range(HG):
            c_late.append(cp(wo_hbm.at[pl.ds(u // NC * Dc, Dc), pl.ds(u % NC * D, D)],
                             wou_v.at[u], NSEM - 1))
        for src, dst in ((wo_hbm, wo_v), (w1_hbm, w1_v), (w2_hbm, w2_v),
                         (w3_hbm, w3_v), (w4_hbm, w4_v)):
            c_late.append(cp(src, dst, NSEM - 1))
        order = [c_c, c_k0] + [c_ckv(r) for r in range(NK - RCH)] + [c_moda]
        for j in range(RCH):
            order += [c_ckv(NK - RCH + j), c_x(j), c_q0(j)]
        order += [c_v0, c_k1] + c_late
        for d in order:
            d.start()

        def relayout_steps(raw, dst, g, chunk, rows, plane):
            n = rows // RCH // 2
            base = g * _gstride(plane) + chunk * n
            if not isinstance(base, int):
                base = pl.multiple_of(base, 8)
            view = dst.at[pl.ds(base, 7 * plane + n), :]

            def step(j, tie):
                val = raw[g, pl.ds(chunk * (2 * n) + 2 * j, 2)].reshape(2 * HG, D)
                val = pltpu.bitcast(val, U32)
                if tie is not None:
                    val = val | tie
                view[pl.ds(j, 8, stride=plane), :] = val

            return [functools.partial(step, j) for j in range(n)]

        def relayout(raw, dst, g, rows, plane):
            for ch in range(RCH):
                for step in relayout_steps(raw, dst, g, ch, rows, plane):
                    step(None)

        def head_w32(src, h, rows, plane, par=None):
            base = (h // HG) * _gstride(plane) + ((h % HG) // 2) * plane
            ev = src[pl.ds(base, rows // 2), :]
            od = src[pl.ds(base + 4 * plane, rows // 2), :]
            par = h % 2 if par is None else par
            if par == 0:
                return (ev & U32(0xFFFF)) | (od << 16)
            return (ev >> 16) | (od & U32(0xFFFF0000))

        def q_weight(h, par=None, tie=None):
            wq = head_w32(wq_p, h, M, PLQ, par)
            if tie is not None:
                wq = wq | _rows_op(jnp.bitwise_and, pltpu.bitcast(tie[0:M // 2], U32), zeros8())
            wqc_v[...] = wq

        def q_rows(lo, hi, ties=()):
            wq = wqc_v[...]
            res = []
            for r0 in range(lo, hi, QC):
                rows = slice(r0, r0 + QC)
                w = _tied(wq, ties[len(res)]) if len(res) in ties else wq
                res.append(_dot(hn_v[rows, :], _unpack(w)))
                q_v[rows, :] = (res[-1] * qscale).astype(BF16)
            return res

        def slot_weight(h, par):
            late = h >= H - HG
            wk = head_w32(wuk_p, jnp.where(late, h, h + HG), Dc, PLK, par)
            wu = pltpu.bitcast(wou_v[jnp.where(late, h - (H - HG), HG)], U32)
            return jnp.where(late, wu, wk)

        def k_slot(h, w, kh):
            u = jnp.maximum(h - (H - HG), 0)
            lhs = lhs_v.at[jnp.where(h >= H - HG, 1 + u // NC, 0)]
            first = None
            for r in range(S // KS):
                rows = slice(r * KS, (r + 1) * KS)
                res = _dot(lhs[rows, :], _unpack(w))
                kh[r * KS // 2:(r + 1) * KS // 2, :] = _pack(res)
                part_v[u, rows, :] = res
                first = res if r == TCH else first
            return first

        def mod_tile(w):
            acc = _fold8(w.astype(F32) * scb_v[...], jnp.add)
            return jnp.broadcast_to(jnp.sum(acc, axis=0, keepdims=True), (8, LANES))

        def mod(i):
            if i < 2:
                return moda_v[0:8, i * M:(i + 1) * M]
            return jnp.concatenate(
                [modb_v[(i - 2) * NC + ct] for ct in range(NC)], axis=1)

        def zeros8():
            return jnp.full((8, LANES), z_s[1], jnp.int32).astype(U32)

        def k_chunk(r, nsub=1, ties=(), after=None, unpack=False):
            n = KC // nsub
            lhs = ckv_v[pl.ds(aligned(r, KC), KC), :]
            for h in range(HG):
                if unpack:
                    w32 = head_w32(wuk_p, h, Dc, PLK)
                    wk0_v[h] = w32
                else:
                    w32 = wk0_v[h]
                for j in range(nsub):
                    i = h * nsub + j
                    rows = pl.ds(aligned(r * nsub + j, n // 2), n // 2)
                    w = _tied(w32, ties[i]) if i in ties else w32
                    res = _dot(lhs[j * n:(j + 1) * n], pltpu.bitcast(w, BF16))
                    k_v[h, rows, :] = _pack(res)
                    if after is not None:
                        after(i, res)

        c_c.wait()
        cc = c_v[...].astype(F32)
        sc = (cc * jax.nn.sigmoid(cc)).astype(BF16).astype(F32)
        scb_v[...] = jnp.broadcast_to(sc, (LANES, M)).T
        zpad = jnp.zeros((PAD, LANES), F32)
        for cidx in range(NC):
            hh_v[cidx, 0:PAD, :] = zpad
            hh_v[cidx, PAD + S:PAD + S + PAD, :] = zpad
        wou_v[HG] = jnp.zeros((Dc, D), BF16)
        wmodb_v[4 * NC] = jnp.zeros((M, LANES), BF16)
        c_k0.wait()
        relayout(wuk_r, wuk_p, 0, Dc, PLK)

        def ka_body(r, carry):
            c_ckv(r).wait()
            k_chunk(r, unpack=True)
            return carry

        jax.lax.fori_loop(0, NK - RCH - 1, ka_body, 0)

        c_ckv(NK - RCH - 1).wait()
        c_moda.wait()
        zero8 = zeros8()
        ties = {}
        for ct in range(2 * NC):
            cols = slice(ct * LANES, (ct + 1) * LANES)
            tile = mod_tile(wmoda_v[:, cols])
            moda_v[0:8, cols] = tile
            ties[2 + (ct * (2 * HG - 2)) // (2 * NC)] = pltpu.bitcast(tile, U32) & zero8
        k_chunk(NK - RCH - 1, 2, ties)

        def kb_body(j, carry):
            c_ckv(NK - RCH + j).wait()
            c_x(j).wait()
            c_q0(j).wait()
            zero8 = zeros8()
            lr = XC // HG
            ties = {}
            scale, shift = 1.0 + mod(1), mod(0)
            for i in range(HG):
                rows = pl.ds(pl.multiple_of(j * XC + i * lr, lr), lr)
                hn = _modulate(_ln(x_v[rows, :].astype(F32)), scale, shift)
                hn_v[rows, :] = hn.astype(BF16)
                ties[i + 2] = pltpu.bitcast(_fold8(hn[:, 0:LANES], jnp.maximum), U32) & zero8
            steps = relayout_steps(wq_r, wq_p, 0, j, M, PLQ)
            per = len(steps) // HG

            def side(i, res):
                for k, step in enumerate(steps[i * per:(i + 1) * per]):
                    step(pltpu.bitcast(res[k * 8:(k + 1) * 8], U32) & zero8)

            k_chunk(NK - RCH + j, 1, ties, side)
            return carry

        jax.lax.fori_loop(0, RCH, kb_body, 0)

        q_weight(0)
        c_v0.wait()
        relayout(wuv_r, wuv_p, 0, Dc, PLK)

        def attention(h, par, kh, side):
            HT = TQ // 2
            key_i = jax.lax.broadcasted_iota(jnp.int32, (HT, TQ), 0)
            qry_i = jax.lax.broadcasted_iota(jnp.int32, (HT, TQ), 1)
            causal_lo = key_i <= qry_i
            causal_hi = key_i + HT <= qry_i
            z_st = z_s[0]
            z_ld = z_s[1]
            zero8 = zeros8()

            m8 = {}
            seq = []

            def keys(*halves):
                ks = [kh[a * HT // 2:b * HT // 2, :] for a, b in halves]
                return _unpack(ks[0] if len(ks) == 1 else jnp.concatenate(ks, axis=0))

            def put(i, half, val):
                for k in range(val.shape[0] // HT):
                    t, off = (half + k) // 2, (half + k) % 2 * HT
                    s_v[i % NSB][z_st + t, off:off + HT, :] = val[k * HT:(k + 1) * HT]
                tm = _fold8(val, jnp.maximum)
                m8[i] = jnp.maximum(m8[i], tm) if i in m8 else tm

            def mm(a, b):
                res = _dot_nt(a, b)
                seq.append(res[0:8])
                return res

            def qk(i):
                qi = q_v[i * TQ:(i + 1) * TQ, :]
                if i % 2 == 0:
                    j = i + 1
                    strip = mm(q_v[j * TQ + HT:(j + 1) * TQ, :],
                               keys((2 * i + 1, 2 * i + 2), (2 * j + 1, 2 * j + 2)))
                    yield
                    qmix = jnp.concatenate(
                        [q_v[j * TQ:j * TQ + HT, :], q_v[i * TQ + HT:(i + 1) * TQ, :]], axis=0)
                    mix = mm(keys((2 * i + 1, 2 * i + 2)), qmix)
                    put(i, 2 * i + 1, jnp.where(causal_hi, mix, NEG))
                    st = jnp.concatenate([strip, strip], axis=0).T
                    put(j, 2 * i + 1, jnp.where(qry_i < HT, mix, st[0:HT]))
                    put(j, 2 * j + 1, jnp.where(causal_hi, st[HT:TQ], NEG))
                    yield
                for t in range(i - 1):
                    put(i, 2 * t, mm(keys((2 * t, 2 * t + 2)), qi))
                    yield
                if i % 2 == 0:
                    lo = max(2 * i - 2, 0)
                    res = mm(keys((lo, 2 * i + 1)), qi)
                    if i > 0:
                        put(i, lo, res[0:TQ])
                else:
                    res = mm(keys((2 * i - 2, 2 * i - 1), (2 * i, 2 * i + 1)), qi)
                    put(i, 2 * i - 2, res[0:HT])
                put(i, 2 * i, jnp.where(causal_lo, res[res.shape[0] - HT:], NEG))
                yield

            def pv(i):
                sb = s_v[i % NSB]
                mb = jnp.broadcast_to(jnp.max(m8[i], axis=0, keepdims=True), (8, TQ))
                l8 = None
                ot = None
                for t in range(i + 1):
                    tie = pltpu.bitcast(seq[-DIST], U32) & zero8
                    mt = pltpu.bitcast(pltpu.bitcast(mb, U32) | tie, F32)
                    tile = sb[z_ld + t].reshape(TQ // 8, 8, TQ)
                    p = jnp.exp2(tile - mt[None]).reshape(TQ, TQ)
                    part = _fold8(p, jnp.add)
                    l8 = part if l8 is None else l8 + part
                    o = _dot(_unpack(vt_v[z_ld, :, t * TQ:(t + 1) * TQ]), p.astype(BF16))
                    seq.append(o[0:8])
                    ot = o if ot is None else ot + o
                    if t == i:
                        l = jnp.sum(l8, axis=0, keepdims=True)
                        ot = ot * (1.0 / l)
                        ctx_v[h, i * TQ:(i + 1) * TQ, :] = ot.T.astype(BF16)
                    yield

            for i in range(LOOK):
                _run(qk(i))
            vt = _dot_nt(_unpack(head_w32(wuv_p, h, Dc, PLK, par)).T, ckv_v[...])
            vt_v[z_st] = _pack(vt)
            prev = vt[0:8, S - TQ:S]
            for res in q_rows(S - PC, S):
                seq.extend([prev] * NC)
                prev = res[0:8]
            per = max(1, -(-len(side) // NQ))
            for j, step in enumerate(side):
                ct, rg = j // per, (j % per) * (D // 8) // per
                src = vt[rg * 8:(rg + 1) * 8, ct * TQ:(ct + 1) * TQ]
                step(pltpu.bitcast(src, U32) & zero8)
            for i in range(NQ):
                j = i + AHEAD
                if LOOK <= j < NQ:
                    _run(qk(j), pv(i))
                else:
                    _run(pv(i))

        def side_work(h):
            g = jnp.minimum(h // HG + ((h % HG) >= RCH).astype(jnp.int32), NG - 1)
            ch = h % RCH
            steps = (relayout_steps(wq_r, wq_p, g, ch, M, PLQ)
                     + relayout_steps(wuv_r, wuv_p, g, ch, Dc, PLK))
            gk = jnp.minimum(h // HG + 1, NG - 1)
            for c in range(RCH):
                steps += relayout_steps(wuk_r, wuk_p, gk, c, Dc, PLK)
            return steps

        c_up = [cp(ctx_v.at[h], slab_hbm.at[h // HS, :, pl.ds(h % HS * D, D)], 1)
                for h in range(NSL * HS)]
        c_down = cp(slab_hbm, lhs_v.at[pl.ds(1, NSL)], 2)

        def head(h, par):
            ct = jnp.where(jnp.logical_and(h >= RCH, h < RCH + 4 * NC), h - RCH, 4 * NC)
            tile = mod_tile(wmodb_v[ct])
            modb_v[ct] = tile
            kh = k_v.at[h % HG]
            q_rows(0, S - PC, {MT: pltpu.bitcast(tile, U32) & zeros8()})
            attention(h, par, kh, side_work(h))
            tie = k_slot(h, slot_weight(h, par), kh)
            q_weight(jnp.minimum(h + 1, H - 2 + (1 - par)), 1 - par, tie)

        def pair_body(j, carry):
            h = 2 * j

            @pl.when(h == RCH)
            def _():
                for d in c_late:
                    d.wait()

            @pl.when(h == NSL * HS + 2)
            def _():
                for d in c_up:
                    d.wait()

            @pl.when(h == H - HG)
            def _():
                c_down.wait()

            @pl.when(h == NSL * HS)
            def _():
                for d in c_up:
                    d.start()

            @pl.when(h == NSL * HS + 2)
            def _():
                c_down.start()

            head(h, 0)
            head(h + 1, 1)
            return carry

        c_k1.wait()
        jax.lax.fori_loop(0, H // 2, pair_body, 0)

        def sub_rows(r):
            out = []
            for j in range(TR // HB):
                r0 = r * TR + j * HB
                if not isinstance(r0, int):
                    r0 = pl.multiple_of(r0, HB)
                out.append(r0)
            return out

        def stage1(r):
            atts = []
            for r0 in sub_rows(r):
                rows = pl.ds(r0, HB)
                ctx = [ctx_v[h, rows, :] for h in range(H)]
                cols = []
                for ct in range(NC):
                    units = list(range(ct, HG, NC))
                    h0 = len(units) * HS
                    col = _dot(jnp.concatenate(ctx[h0:], axis=1),
                               wo_v[h0 * D:H * D, ct * LANES:(ct + 1) * LANES])
                    for u in units:
                        col = col + part_v[u, rows, :]
                    cols.append(col)
                atts.append(jnp.concatenate(cols, axis=1))
            lns = []
            for r0, att in zip(sub_rows(r), atts):
                rows = pl.ds(r0, HB)
                x1 = x_v[rows, :].astype(F32) + _rows_op(jnp.multiply, att, mod(2))
                x1_v[rows, :] = x1
                h2 = _modulate(_ln(x1), 1.0 + mod(4), mod(3))
                h2_v[rows, :] = h2
                lns.append(_ln(h2).astype(BF16))
            for r0, ln in zip(sub_rows(r), lns):
                u = _gelu(_dot(ln, w1_v[...]))
                for cidx in range(NC):
                    hh_v[cidx, pl.ds(r0 + PAD, HB), :] = u[:, cidx * LANES:(cidx + 1) * LANES]

        shifts = (1, -1, 2, -2)

        def stage2(r, last):
            lane_i = jax.lax.broadcasted_iota(jnp.int32, (HB, LANES), 1)
            y1s = []
            for r0 in sub_rows(r):
                tiles = []
                for cidx in range(NC):
                    lo, hi = cidx * LANES, (cidx + 1) * LANES
                    g_lo, g_hi = lo // C4, (hi - 1) // C4
                    t = hh_v[cidx, pl.ds(r0 + PAD - shifts[g_hi], HB), :]
                    for g in range(g_hi - 1, g_lo - 1, -1):
                        tg = hh_v[cidx, pl.ds(r0 + PAD - shifts[g], HB), :]
                        t = jnp.where(lane_i < (g + 1) * C4 - lo, tg, t)
                    tiles.append(t)
                hs = _dot(jnp.concatenate(tiles, axis=1).astype(BF16), w2_v[...])
                y1s.append(h2_v[pl.ds(r0, HB), :] + hs)
            gls = []
            f0 = Fh // LANES * LANES
            for y1 in y1s:
                ln = _ln(y1).astype(BF16)
                parts = [_gelu(_dot_nt(ln, w3_v[0:f0 // 2 // LANES * LANES, :]))]
                if f0 < Fh:
                    tail = _gelu(_dot_nt(w3_v[f0:Fh, :], ln)).T
                parts.append(_gelu(_dot_nt(ln, w3_v[f0 // 2 // LANES * LANES:f0, :])))
                if f0 < Fh:
                    parts.append(tail)
                gls.append(jnp.concatenate(parts, axis=1).astype(BF16))
            for k, (r0, y1, gl) in enumerate(zip(sub_rows(r), y1s, gls)):
                rows = pl.ds(r0, HB)
                h3 = _dot(gl, w4_v[...])
                out = x1_v[rows, :] + _rows_op(jnp.multiply, y1 + h3, mod(5))
                split = last and k == len(gls) - 1
                for lo, hi in ((0, M - LANES), (M - LANES, M)) if split else ((0, M),):
                    cols = pl.ds(lo, hi - lo)
                    o_v[rows, cols] = out[:, lo:hi].astype(BF16)
                    cp(o_v.at[rows, cols], out_hbm.at[rows, cols], 0).start()

        def s1_body(r, carry):
            stage1(r)
            return carry

        def s2_body(r, carry):
            for u in range(U2):
                stage2(r * U2 + u, u == U2 - 1)
            return carry

        jax.lax.fori_loop(0, NR, s1_body, 0)
        jax.lax.fori_loop(0, NR // U2, s2_body, 0)
        cp(o_v, out_hbm, 0).wait()

    hbm_spec = pl.BlockSpec(memory_space=pltpu.HBM)
    V = pltpu.VMEM
    scratch = [
        V((S, M), BF16),
        V((1 + NSL, S, Dc), BF16),
        V((NG, M, HG, D), BF16),
        V((NG, Dc, HG, D), BF16),
        V((NG, Dc, HG, D), BF16),
        V((NG * _gstride(PLQ), D), U32),
        V((NG * _gstride(PLK), D), U32),
        V((NG * _gstride(PLK), D), U32),
        V((H * D, M), BF16),
        V((HG + 1, Dc, D), BF16),
        V((M, M), BF16),
        V((M, M), BF16),
        V((Fh, M), BF16),
        V((Fh, M), BF16),
        V((M, 2 * M), BF16),
        V((4 * NC + 1, M, LANES), BF16),
        V((16, 2 * M), F32),
        V((4 * NC + 4, 8, LANES), F32),
        V((M, LANES), F32),
        V((S, M), BF16),
        V((M // 2, D), U32),
        V((HG, Dc // 2, D), U32),
        V((S, D), BF16),
        V((HG, S // 2, D), U32),
        V((1, D // 2, S), U32),
        [V((NQ, TQ, TQ), F32)] * NSB,
        pltpu.SMEM((2,), jnp.int32),
        V((H, S, D), BF16),
        V((HG, S, D), F32),
        V((S, M), F32),
        V((S, M), F32),
        V((NC, S + 2 * PAD, LANES), F32),
        V((S, M), BF16),
        V((1, M), BF16),
        pltpu.SemaphoreType.DMA((NSEM,)),
    ]
    out, _ = pl.pallas_call(
        kernel,
        out_shape=(jax.ShapeDtypeStruct((S, M), BF16),
                   jax.ShapeDtypeStruct((NSL, S, Dc), BF16)),
        in_specs=[hbm_spec] * 12,
        out_specs=(hbm_spec, hbm_spec),
        scratch_shapes=scratch,
        compiler_params=pltpu.CompilerParams(
            vmem_limit_bytes=120 * 1024 * 1024,
            disable_bounds_checks=True,
            disable_semaphore_checks=True,
        ),
        name="adaln_cla_mixer",
    )(x2, ckv2, A_w_q, A_w_uk, A_w_uv, wo2, B_w1, B_w2, B_w3.T, B_w4, c, w_mod)
    return out.reshape(B, S, M)
```

```python
import functools
import math

import jax
import jax.numpy as jnp
import jax.experimental.pallas as pl
import jax.experimental.pallas.tpu as pltpu

BF16 = jnp.bfloat16
F32 = jnp.float32
U32 = jnp.uint32

LANES = 128
TQ = 128
TR = 256
HB = 128
HG = 8
RCH = 4
LOOK = 6
AHEAD = 2
NSB = 6
DIST = 11
KC = 256
KS = 512
QC = 128
QT = 384
U2 = 2
PAD = 16
EPS = 1e-5
LOG2E = math.log2(math.e)
NEG = -1000000000.0 * LOG2E

_NT = (((1,), (1,)), ((), ()))


def _ln(x):
    m = jnp.mean(x, axis=-1, keepdims=True)
    xc = x - m
    v = jnp.mean(xc * xc, axis=-1, keepdims=True)
    return xc * jax.lax.rsqrt(v + EPS)


def _gelu(x):
    return jax.nn.gelu(x, approximate=True)


def _dot(a, b):
    return jnp.dot(a, b, preferred_element_type=F32)


def _dot_nt(a, b):
    return jax.lax.dot_general(a, b, _NT, preferred_element_type=F32)


def _fold8(x, op):
    parts = [op(x[j:j + 8], x[j + 8:j + 16]) for j in range(0, x.shape[0], 16)]
    acc = parts[0]
    for p in parts[1:]:
        acc = op(acc, p)
    return acc


def _rows_op(op, x, v8):
    r, m = x.shape
    return op(x.reshape(r // 8, 8, m), v8[None]).reshape(r, m)


def _modulate(x, scale8, shift8):
    r, m = x.shape
    return (x.reshape(r // 8, 8, m) * scale8[None] + shift8[None]).reshape(r, m)


def _pack(x):
    return pltpu.bitcast(x.astype(BF16), U32)


def _unpack(w):
    return pltpu.bitcast(w, BF16)


def _gstride(plane):
    return -(-8 * plane // 32) * 32


def _tied(w, tie):
    return jnp.concatenate([w[0:8] | tie, w[8:]], axis=0)


def _run(*gens):
    gens = list(gens)
    while gens:
        for g in list(gens):
            if next(g, gens) is gens:
                gens.remove(g)


@jax.jit
def pallas_adaLN_cond__compressed_kv_cla__mixer_s_mlp__prompt_kernel(
    A_x: jax.Array,
    A_c_kv: jax.Array,
    A_w_q: jax.Array,
    A_w_uk: jax.Array,
    A_w_uv: jax.Array,
    A_w_o: jax.Array,
    B_x: jax.Array,
    B_w1: jax.Array,
    B_w2: jax.Array,
    B_w3: jax.Array,
    B_w4: jax.Array,
    c: jax.Array,
    w_mod: jax.Array,
):
    del B_x
    B, S, M = A_x.shape
    _, Sk, Dc = A_c_kv.shape
    _, H, D = A_w_q.shape
    Fh = B_w3.shape[1]
    assert B == 1 and Sk == S and D == LANES and H % HG == 0 and HG == 8
    assert S % TQ == 0 and S % (TR * U2) == 0 and TR % HB == 0 and S % KS == 0
    assert QT % QC == 0 and LOOK * TQ <= S - QT and KS >= M // 2
    assert M % LANES == 0 and M % 64 == 0 and Dc % 64 == 0
    NG = H // HG
    NQ = S // TQ
    NR = S // TR
    NC = M // LANES
    C4 = M // 4
    PLQ = M // 2 + 1
    PLK = Dc // 2 + 1
    NK = S // KC
    XC = S // RCH
    NSEM = NK + 5
    assert NK > RCH + 1 and NQ % 2 == 0 and LOOK % 2 == 0 and NSB >= max(LOOK, AHEAD + 2)
    HS = Dc // D
    NSL = -(-HG // NC)
    assert H % 2 == 0 and RCH % 2 == 0 and RCH + 4 * NC <= H and NSL * HS + 2 < H - HG
    qscale = float(D) ** -0.5 * LOG2E

    x2 = A_x.reshape(S, M)
    ckv2 = A_c_kv.reshape(S, Dc)
    wo2 = A_w_o.reshape(H * D, M)

    def kernel(x_hbm, ckv_hbm, wq_hbm, wuk_hbm, wuv_hbm, wo_hbm, w1_hbm, w2_hbm,
               w3_hbm, w4_hbm, c_hbm, wmod_hbm, out_hbm, slab_hbm,
               x_v, lhs_v, wq_r, wuk_r, wuv_r, wq_p, wuk_p, wuv_p, wo_v, wou_v, w1_v,
               w2_v, w3_v, w4_v, wmoda_v, wmodb_v, moda_v, modb_v, scb_v, hn_v, wqc_v, wk0_v, q_v, k_v,
               vt_v, s_v, z_s, ctx_v, part_v, x1_v, h2_v, hh_v, o_v, c_v,
               sems):

        ckv_v = lhs_v.at[0]
        z_s[0] = 0
        z_s[1] = 0

        def aligned(i, n):
            return i * n if isinstance(i, int) else pl.multiple_of(i * n, n)

        def cp(src, dst, i):
            return pltpu.make_async_copy(src, dst, sems.at[i])

        def c_ckv(r):
            rows = pl.ds(aligned(r, KC), KC)
            return cp(ckv_hbm.at[rows, :], ckv_v.at[rows, :], r)

        def c_x(j):
            rows = pl.ds(aligned(j, XC), XC)
            return cp(x_hbm.at[rows, :], x_v.at[rows, :], NK - RCH + j)

        def c_q0(j):
            rows = pl.ds(aligned(j, M // RCH), M // RCH)
            return cp(wq_hbm.at[rows, pl.ds(0, HG), :], wq_r.at[0, rows], NK - RCH + j)

        def gcp(src, dst, g, i):
            return cp(src.at[:, pl.ds(g * HG, HG), :], dst.at[g], i)

        c_moda = cp(wmod_hbm.at[:, pl.ds(0, 2 * M)], wmoda_v, NK - RCH - 1)
        c_c = cp(c_hbm, c_v, NK)
        c_k0 = gcp(wuk_hbm, wuk_r, 0, NK + 1)
        c_v0 = gcp(wuv_hbm, wuv_r, 0, NK + 2)
        c_k1 = gcp(wuk_hbm, wuk_r, 1, NK + 3)
        c_late = []
        for g in range(1, NG):
            for src, dst, gg in ((wq_hbm, wq_r, g), (wuv_hbm, wuv_r, g), (wuk_hbm, wuk_r, g + 1)):
                if gg < NG:
                    c_late.append(gcp(src, dst, gg, NSEM - 1))
        for ct in range(4 * NC):
            c_late.append(cp(wmod_hbm.at[:, pl.ds(2 * M + ct * LANES, LANES)],
                             wmodb_v.at[ct], NSEM - 1))
        for u in range(HG):
            c_late.append(cp(wo_hbm.at[pl.ds(u // NC * Dc, Dc), pl.ds(u % NC * D, D)],
                             wou_v.at[u], NSEM - 1))
        for src, dst in ((wo_hbm, wo_v), (w1_hbm, w1_v), (w2_hbm, w2_v),
                         (w3_hbm, w3_v), (w4_hbm, w4_v)):
            c_late.append(cp(src, dst, NSEM - 1))
        order = [c_c, c_k0] + [c_ckv(r) for r in range(NK - RCH)] + [c_moda]
        for j in range(RCH):
            order += [c_ckv(NK - RCH + j), c_x(j), c_q0(j)]
        order += [c_v0, c_k1] + c_late
        for d in order:
            d.start()

        def relayout_steps(raw, dst, g, chunk, rows, plane):
            n = rows // RCH // 2
            base = g * _gstride(plane) + chunk * n
            if not isinstance(base, int):
                base = pl.multiple_of(base, 8)
            view = dst.at[pl.ds(base, 7 * plane + n), :]

            def step(j, tie):
                val = raw[g, pl.ds(chunk * (2 * n) + 2 * j, 2)].reshape(2 * HG, D)
                val = pltpu.bitcast(val, U32)
                if tie is not None:
                    val = val | tie
                view[pl.ds(j, 8, stride=plane), :] = val

            return [functools.partial(step, j) for j in range(n)]

        def relayout(raw, dst, g, rows, plane):
            for ch in range(RCH):
                for step in relayout_steps(raw, dst, g, ch, rows, plane):
                    step(None)

        def head_w32(src, h, rows, plane, par=None):
            base = (h // HG) * _gstride(plane) + ((h % HG) // 2) * plane
            ev = src[pl.ds(base, rows // 2), :]
            od = src[pl.ds(base + 4 * plane, rows // 2), :]
            par = h % 2 if par is None else par
            if par == 0:
                return (ev & U32(0xFFFF)) | (od << 16)
            return (ev >> 16) | (od & U32(0xFFFF0000))

        def q_weight(h, par=None, tie=None):
            wq = head_w32(wq_p, h, M, PLQ, par)
            if tie is not None:
                wq = wq | _rows_op(jnp.bitwise_and, pltpu.bitcast(tie[0:M // 2], U32), zeros8())
            wqc_v[...] = wq

        def q_rows(lo, hi, ties=()):
            wq = wqc_v[...]
            res = []
            for r0 in range(lo, hi, QC):
                rows = slice(r0, r0 + QC)
                w = _tied(wq, ties[len(res)]) if len(res) in ties else wq
                res.append(_dot(hn_v[rows, :], _unpack(w)))
                q_v[rows, :] = (res[-1] * qscale).astype(BF16)
            return res

        def slot_weight(h, par):
            late = h >= H - HG
            wk = head_w32(wuk_p, jnp.where(late, h, h + HG), Dc, PLK, par)
            wu = pltpu.bitcast(wou_v[jnp.where(late, h - (H - HG), HG)], U32)
            return jnp.where(late, wu, wk)

        def k_slot(h, w, kh):
            u = jnp.maximum(h - (H - HG), 0)
            lhs = lhs_v.at[jnp.where(h >= H - HG, 1 + u // NC, 0)]
            first = None
            for r in range(S // KS):
                rows = slice(r * KS, (r + 1) * KS)
                res = _dot(lhs[rows, :], _unpack(w))
                kh[r * KS // 2:(r + 1) * KS // 2, :] = _pack(res)
                part_v[u, rows, :] = res
                first = res if r == 0 else first
            return first

        def mod_tile(w):
            acc = _fold8(w.astype(F32) * scb_v[...], jnp.add)
            return jnp.broadcast_to(jnp.sum(acc, axis=0, keepdims=True), (8, LANES))

        def mod(i):
            if i < 2:
                return moda_v[0:8, i * M:(i + 1) * M]
            return jnp.concatenate(
                [modb_v[(i - 2) * NC + ct] for ct in range(NC)], axis=1)

        def zeros8():
            return jnp.full((8, LANES), z_s[1], jnp.int32).astype(U32)

        def k_chunk(r, nsub=1, ties=(), after=None, unpack=False):
            n = KC // nsub
            lhs = ckv_v[pl.ds(aligned(r, KC), KC), :]
            for h in range(HG):
                if unpack:
                    w32 = head_w32(wuk_p, h, Dc, PLK)
                    wk0_v[h] = w32
                else:
                    w32 = wk0_v[h]
                for j in range(nsub):
                    i = h * nsub + j
                    rows = pl.ds(aligned(r * nsub + j, n // 2), n // 2)
                    w = _tied(w32, ties[i]) if i in ties else w32
                    res = _dot(lhs[j * n:(j + 1) * n], pltpu.bitcast(w, BF16))
                    k_v[h, rows, :] = _pack(res)
                    if after is not None:
                        after(i, res)

        c_c.wait()
        cc = c_v[...].astype(F32)
        sc = (cc * jax.nn.sigmoid(cc)).astype(BF16).astype(F32)
        scb_v[...] = jnp.broadcast_to(sc, (LANES, M)).T
        zpad = jnp.zeros((PAD, LANES), F32)
        for cidx in range(NC):
            hh_v[cidx, 0:PAD, :] = zpad
            hh_v[cidx, PAD + S:PAD + S + PAD, :] = zpad
        wou_v[HG] = jnp.zeros((Dc, D), BF16)
        wmodb_v[4 * NC] = jnp.zeros((M, LANES), BF16)
        c_k0.wait()
        relayout(wuk_r, wuk_p, 0, Dc, PLK)

        def ka_body(r, carry):
            c_ckv(r).wait()
            k_chunk(r, unpack=True)
            return carry

        jax.lax.fori_loop(0, NK - RCH - 1, ka_body, 0)

        c_ckv(NK - RCH - 1).wait()
        c_moda.wait()
        zero8 = zeros8()
        ties = {}
        for ct in range(2 * NC):
            cols = slice(ct * LANES, (ct + 1) * LANES)
            tile = mod_tile(wmoda_v[:, cols])
            moda_v[0:8, cols] = tile
            ties[2 + (ct * (2 * HG - 2)) // (2 * NC)] = pltpu.bitcast(tile, U32) & zero8
        k_chunk(NK - RCH - 1, 2, ties)

        def kb_body(j, carry):
            c_ckv(NK - RCH + j).wait()
            c_x(j).wait()
            c_q0(j).wait()
            zero8 = zeros8()
            lr = XC // HG
            ties = {}
            scale, shift = 1.0 + mod(1), mod(0)
            for i in range(HG):
                rows = pl.ds(pl.multiple_of(j * XC + i * lr, lr), lr)
                hn = _modulate(_ln(x_v[rows, :].astype(F32)), scale, shift)
                hn_v[rows, :] = hn.astype(BF16)
                ties[i + 2] = pltpu.bitcast(_fold8(hn[:, 0:LANES], jnp.maximum), U32) & zero8
            steps = relayout_steps(wq_r, wq_p, 0, j, M, PLQ)
            per = len(steps) // HG

            def side(i, res):
                for k, step in enumerate(steps[i * per:(i + 1) * per]):
                    step(pltpu.bitcast(res[k * 8:(k + 1) * 8], U32) & zero8)

            k_chunk(NK - RCH + j, 1, ties, side)
            return carry

        jax.lax.fori_loop(0, RCH, kb_body, 0)

        q_weight(0)
        c_v0.wait()
        relayout(wuv_r, wuv_p, 0, Dc, PLK)

        def attention(h, par, kh, side):
            HT = TQ // 2
            key_i = jax.lax.broadcasted_iota(jnp.int32, (HT, TQ), 0)
            qry_i = jax.lax.broadcasted_iota(jnp.int32, (HT, TQ), 1)
            causal_lo = key_i <= qry_i
            causal_hi = key_i + HT <= qry_i
            z_st = z_s[0]
            z_ld = z_s[1]
            zero8 = zeros8()

            m8 = {}
            seq = []

            def keys(*halves):
                ks = [kh[a * HT // 2:b * HT // 2, :] for a, b in halves]
                return _unpack(ks[0] if len(ks) == 1 else jnp.concatenate(ks, axis=0))

            def put(i, half, val):
                for k in range(val.shape[0] // HT):
                    t, off = (half + k) // 2, (half + k) % 2 * HT
                    s_v[i % NSB][z_st + t, off:off + HT, :] = val[k * HT:(k + 1) * HT]
                tm = _fold8(val, jnp.maximum)
                m8[i] = jnp.maximum(m8[i], tm) if i in m8 else tm

            def mm(a, b):
                res = _dot_nt(a, b)
                seq.append(res[0:8])
                return res

            def qk(i):
                qi = q_v[i * TQ:(i + 1) * TQ, :]
                if i % 2 == 0:
                    j = i + 1
                    strip = mm(q_v[j * TQ + HT:(j + 1) * TQ, :],
                               keys((2 * i + 1, 2 * i + 2), (2 * j + 1, 2 * j + 2)))
                    yield
                    qmix = jnp.concatenate(
                        [q_v[j * TQ:j * TQ + HT, :], q_v[i * TQ + HT:(i + 1) * TQ, :]], axis=0)
                    mix = mm(keys((2 * i + 1, 2 * i + 2)), qmix)
                    put(i, 2 * i + 1, jnp.where(causal_hi, mix, NEG))
                    st = jnp.concatenate([strip, strip], axis=0).T
                    put(j, 2 * i + 1, jnp.where(qry_i < HT, mix, st[0:HT]))
                    put(j, 2 * j + 1, jnp.where(causal_hi, st[HT:TQ], NEG))
                    yield
                for t in range(i - 1):
                    put(i, 2 * t, mm(keys((2 * t, 2 * t + 2)), qi))
                    yield
                if i % 2 == 0:
                    lo = max(2 * i - 2, 0)
                    res = mm(keys((lo, 2 * i + 1)), qi)
                    if i > 0:
                        put(i, lo, res[0:TQ])
                else:
                    res = mm(keys((2 * i - 2, 2 * i - 1), (2 * i, 2 * i + 1)), qi)
                    put(i, 2 * i - 2, res[0:HT])
                put(i, 2 * i, jnp.where(causal_lo, res[res.shape[0] - HT:], NEG))
                yield

            def pv(i):
                sb = s_v[i % NSB]
                mb = jnp.broadcast_to(jnp.max(m8[i], axis=0, keepdims=True), (8, TQ))
                l8 = None
                ot = None
                for t in range(i + 1):
                    tie = pltpu.bitcast(seq[-DIST], U32) & zero8
                    mt = pltpu.bitcast(pltpu.bitcast(mb, U32) | tie, F32)
                    tile = sb[z_ld + t].reshape(TQ // 8, 8, TQ)
                    p = jnp.exp2(tile - mt[None]).reshape(TQ, TQ)
                    part = _fold8(p, jnp.add)
                    l8 = part if l8 is None else l8 + part
                    o = _dot(_unpack(vt_v[z_ld, :, t * TQ:(t + 1) * TQ]), p.astype(BF16))
                    seq.append(o[0:8])
                    ot = o if ot is None else ot + o
                    if t == i:
                        l = jnp.sum(l8, axis=0, keepdims=True)
                        ot = ot * (1.0 / l)
                        ctx_v[h, i * TQ:(i + 1) * TQ, :] = ot.T.astype(BF16)
                    yield

            for i in range(LOOK):
                _run(qk(i))
            vt = _dot_nt(_unpack(head_w32(wuv_p, h, Dc, PLK, par)).T, ckv_v[...])
            vt_v[z_st] = _pack(vt)
            prev = vt[0:8, S - TQ:S]
            for res in q_rows(S - QT, S):
                seq.extend([prev] * NC)
                prev = res[0:8]
            per = max(1, -(-len(side) // NQ))
            for j, step in enumerate(side):
                ct, rg = j // per, (j % per) * (D // 8) // per
                src = vt[rg * 8:(rg + 1) * 8, ct * TQ:(ct + 1) * TQ]
                step(pltpu.bitcast(src, U32) & zero8)
            for i in range(NQ):
                j = i + AHEAD
                if LOOK <= j < NQ:
                    _run(qk(j), pv(i))
                else:
                    _run(pv(i))

        def side_work(h):
            g = jnp.minimum(h // HG + ((h % HG) >= RCH).astype(jnp.int32), NG - 1)
            ch = h % RCH
            steps = (relayout_steps(wq_r, wq_p, g, ch, M, PLQ)
                     + relayout_steps(wuv_r, wuv_p, g, ch, Dc, PLK))
            gk = jnp.minimum(h // HG + 1, NG - 1)
            for c in range(RCH):
                steps += relayout_steps(wuk_r, wuk_p, gk, c, Dc, PLK)
            return steps

        c_up = [cp(ctx_v.at[h], slab_hbm.at[h // HS, :, pl.ds(h % HS * D, D)], 1)
                for h in range(NSL * HS)]
        c_down = cp(slab_hbm, lhs_v.at[pl.ds(1, NSL)], 2)

        def head(h, par):
            ct = jnp.where(jnp.logical_and(h >= RCH, h < RCH + 4 * NC), h - RCH, 4 * NC)
            tile = mod_tile(wmodb_v[ct])
            modb_v[ct] = tile
            kh = k_v.at[h % HG]
            q_rows(0, S - QT, {4: pltpu.bitcast(tile, U32) & zeros8()})
            attention(h, par, kh, side_work(h))
            tie = k_slot(h, slot_weight(h, par), kh)
            q_weight(jnp.minimum(h + 1, H - 2 + (1 - par)), 1 - par, tie)

        def pair_body(j, carry):
            h = 2 * j

            @pl.when(h == 0)
            def _():
                c_k1.wait()

            @pl.when(h == RCH)
            def _():
                for d in c_late:
                    d.wait()

            @pl.when(h == NSL * HS + 2)
            def _():
                for d in c_up:
                    d.wait()

            @pl.when(h == H - HG)
            def _():
                c_down.wait()

            @pl.when(h == NSL * HS)
            def _():
                for d in c_up:
                    d.start()

            @pl.when(h == NSL * HS + 2)
            def _():
                c_down.start()

            head(h, 0)
            head(h + 1, 1)
            return carry

        jax.lax.fori_loop(0, H // 2, pair_body, 0)

        def sub_rows(r):
            out = []
            for j in range(TR // HB):
                r0 = r * TR + j * HB
                if not isinstance(r0, int):
                    r0 = pl.multiple_of(r0, HB)
                out.append(r0)
            return out

        def stage1(r):
            atts = []
            for r0 in sub_rows(r):
                rows = pl.ds(r0, HB)
                ctx = [ctx_v[h, rows, :] for h in range(H)]
                cols = []
                for ct in range(NC):
                    units = list(range(ct, HG, NC))
                    h0 = len(units) * HS
                    col = _dot(jnp.concatenate(ctx[h0:], axis=1),
                               wo_v[h0 * D:H * D, ct * LANES:(ct + 1) * LANES])
                    for u in units:
                        col = col + part_v[u, rows, :]
                    cols.append(col)
                atts.append(jnp.concatenate(cols, axis=1))
            lns = []
            for r0, att in zip(sub_rows(r), atts):
                rows = pl.ds(r0, HB)
                x1 = x_v[rows, :].astype(F32) + _rows_op(jnp.multiply, att, mod(2))
                x1_v[rows, :] = x1
                h2 = _modulate(_ln(x1), 1.0 + mod(4), mod(3))
                h2_v[rows, :] = h2
                lns.append(_ln(h2).astype(BF16))
            for r0, ln in zip(sub_rows(r), lns):
                u = _gelu(_dot(ln, w1_v[...]))
                for cidx in range(NC):
                    hh_v[cidx, pl.ds(r0 + PAD, HB), :] = u[:, cidx * LANES:(cidx + 1) * LANES]

        shifts = (1, -1, 2, -2)

        def stage2(r, last):
            lane_i = jax.lax.broadcasted_iota(jnp.int32, (HB, LANES), 1)
            y1s = []
            for r0 in sub_rows(r):
                tiles = []
                for cidx in range(NC):
                    lo, hi = cidx * LANES, (cidx + 1) * LANES
                    g_lo, g_hi = lo // C4, (hi - 1) // C4
                    t = hh_v[cidx, pl.ds(r0 + PAD - shifts[g_hi], HB), :]
                    for g in range(g_hi - 1, g_lo - 1, -1):
                        tg = hh_v[cidx, pl.ds(r0 + PAD - shifts[g], HB), :]
                        t = jnp.where(lane_i < (g + 1) * C4 - lo, tg, t)
                    tiles.append(t)
                hs = _dot(jnp.concatenate(tiles, axis=1).astype(BF16), w2_v[...])
                y1s.append(h2_v[pl.ds(r0, HB), :] + hs)
            gls = []
            f0 = Fh // LANES * LANES
            for y1 in y1s:
                ln = _ln(y1).astype(BF16)
                parts = [_gelu(_dot_nt(ln, w3_v[0:f0 // 2 // LANES * LANES, :]))]
                if f0 < Fh:
                    tail = _gelu(_dot_nt(w3_v[f0:Fh, :], ln)).T
                parts.append(_gelu(_dot_nt(ln, w3_v[f0 // 2 // LANES * LANES:f0, :])))
                if f0 < Fh:
                    parts.append(tail)
                gls.append(jnp.concatenate(parts, axis=1).astype(BF16))
            for k, (r0, y1, gl) in enumerate(zip(sub_rows(r), y1s, gls)):
                rows = pl.ds(r0, HB)
                h3 = _dot(gl, w4_v[...])
                out = x1_v[rows, :] + _rows_op(jnp.multiply, y1 + h3, mod(5))
                split = last and k == len(gls) - 1
                for lo, hi in ((0, M - LANES), (M - LANES, M)) if split else ((0, M),):
                    cols = pl.ds(lo, hi - lo)
                    o_v[rows, cols] = out[:, lo:hi].astype(BF16)
                    cp(o_v.at[rows, cols], out_hbm.at[rows, cols], 0).start()

        def s1_body(r, carry):
            stage1(r)
            return carry

        def s2_body(r, carry):
            for u in range(U2):
                stage2(r * U2 + u, u == U2 - 1)
            return carry

        jax.lax.fori_loop(0, NR, s1_body, 0)
        jax.lax.fori_loop(0, NR // U2, s2_body, 0)
        cp(o_v, out_hbm, 0).wait()

    hbm_spec = pl.BlockSpec(memory_space=pltpu.HBM)
    V = pltpu.VMEM
    scratch = [
        V((S, M), BF16),
        V((1 + NSL, S, Dc), BF16),
        V((NG, M, HG, D), BF16),
        V((NG, Dc, HG, D), BF16),
        V((NG, Dc, HG, D), BF16),
        V((NG * _gstride(PLQ), D), U32),
        V((NG * _gstride(PLK), D), U32),
        V((NG * _gstride(PLK), D), U32),
        V((H * D, M), BF16),
        V((HG + 1, Dc, D), BF16),
        V((M, M), BF16),
        V((M, M), BF16),
        V((Fh, M), BF16),
        V((Fh, M), BF16),
        V((M, 2 * M), BF16),
        V((4 * NC + 1, M, LANES), BF16),
        V((16, 2 * M), F32),
        V((4 * NC + 4, 8, LANES), F32),
        V((M, LANES), F32),
        V((S, M), BF16),
        V((M // 2, D), U32),
        V((HG, Dc // 2, D), U32),
        V((S, D), BF16),
        V((HG, S // 2, D), U32),
        V((1, D // 2, S), U32),
        [V((NQ, TQ, TQ), F32)] * NSB,
        pltpu.SMEM((2,), jnp.int32),
        V((H, S, D), BF16),
        V((HG, S, D), F32),
        V((S, M), F32),
        V((S, M), F32),
        V((NC, S + 2 * PAD, LANES), F32),
        V((S, M), BF16),
        V((1, M), BF16),
        pltpu.SemaphoreType.DMA((NSEM,)),
    ]
    out, _ = pl.pallas_call(
        kernel,
        out_shape=(jax.ShapeDtypeStruct((S, M), BF16),
                   jax.ShapeDtypeStruct((NSL, S, Dc), BF16)),
        in_specs=[hbm_spec] * 12,
        out_specs=(hbm_spec, hbm_spec),
        scratch_shapes=scratch,
        compiler_params=pltpu.CompilerParams(
            vmem_limit_bytes=120 * 1024 * 1024,
            disable_bounds_checks=True,
            disable_semaphore_checks=True,
        ),
        name="adaln_cla_mixer",
    )(x2, ckv2, A_w_q, A_w_uk, A_w_uv, wo2, B_w1, B_w2, B_w3.T, B_w4, c, w_mod)
    return out.reshape(B, S, M)
```

```python
import functools
import math
import os

import jax
import jax.numpy as jnp
import jax.experimental.pallas as pl
import jax.experimental.pallas.tpu as pltpu

BF16 = jnp.bfloat16
F32 = jnp.float32
U32 = jnp.uint32

LANES = 128
TQ = 128
TR = 256
HB = 128
HG = 8
RCH = 4
G = int(os.environ.get('G', 4))
CL = int(os.environ.get('CL', 0))
LOOK = int(os.environ.get('LOOK', 4))
AHEAD = 2
NSB = int(os.environ.get('NSB', 8))
DIST = int(os.environ.get('DIST', 11))
KC = 256
KS = int(os.environ.get('KS', 512))
QC = 128
QT = int(os.environ.get('QT', 384))
U2 = 2
QX = int(os.environ.get('QX', 2))
CSX = int(os.environ.get('CSX', 1))
PAD = 16
EPS = 1e-5
LOG2E = math.log2(math.e)
NEG = -1000000000.0 * LOG2E

_NT = (((1,), (1,)), ((), ()))


def _ln(x):
    m = jnp.mean(x, axis=-1, keepdims=True)
    xc = x - m
    v = jnp.mean(xc * xc, axis=-1, keepdims=True)
    return xc * jax.lax.rsqrt(v + EPS)


def _gelu(x):
    return jax.nn.gelu(x, approximate=True)


def _dot(a, b):
    return jnp.dot(a, b, preferred_element_type=F32)


def _dot_nt(a, b):
    return jax.lax.dot_general(a, b, _NT, preferred_element_type=F32)


def _fold8(x, op):
    parts = [op(x[j:j + 8], x[j + 8:j + 16]) for j in range(0, x.shape[0], 16)]
    acc = parts[0]
    for p in parts[1:]:
        acc = op(acc, p)
    return acc


def _rows_op(op, x, v8):
    r, m = x.shape
    return op(x.reshape(r // 8, 8, m), v8[None]).reshape(r, m)


def _modulate(x, scale8, shift8):
    r, m = x.shape
    return (x.reshape(r // 8, 8, m) * scale8[None] + shift8[None]).reshape(r, m)


def _pack(x):
    return pltpu.bitcast(x.astype(BF16), U32)


def _unpack(w):
    return pltpu.bitcast(w, BF16)


def _gstride(plane):
    return -(-8 * plane // 32) * 32


def _tied(w, tie):
    return jnp.concatenate([w[0:8] | tie, w[8:]], axis=0)


class _Mxus:
    def __init__(self):
        self.load = [0] * 4
        self.last = [TQ] * 4

    def next(self):
        return self.load.index(min(self.load))

    def issue(self, rows, count=1):
        for _ in range(count):
            j = self.next()
            self.load[j] += rows
            self.last[j] = rows

    def after_short(self):
        return self.last[self.next()] < TQ // 2

    def to_grid(self):
        rows = TQ - self.load[self.next()] % TQ
        return rows if rows >= TQ // 2 else rows + TQ


def _round_robin(gens):
    gens = list(gens)
    while gens:
        for g in list(gens):
            v = next(g, gens)
            if v is gens:
                gens.remove(g)
            else:
                yield v


def _run(gen):
    for _ in gen:
        pass


def _chain_gens(gens):
    for g in gens:
        yield from g


@jax.jit
def pallas_adaLN_cond__compressed_kv_cla__mixer_s_mlp__prompt_kernel(
    A_x: jax.Array,
    A_c_kv: jax.Array,
    A_w_q: jax.Array,
    A_w_uk: jax.Array,
    A_w_uv: jax.Array,
    A_w_o: jax.Array,
    B_x: jax.Array,
    B_w1: jax.Array,
    B_w2: jax.Array,
    B_w3: jax.Array,
    B_w4: jax.Array,
    c: jax.Array,
    w_mod: jax.Array,
):
    del B_x
    B, S, M = A_x.shape
    _, Sk, Dc = A_c_kv.shape
    _, H, D = A_w_q.shape
    Fh = B_w3.shape[1]
    assert B == 1 and Sk == S and D == LANES and H % HG == 0 and HG == 8
    assert S % TQ == 0 and S % (TR * U2) == 0 and TR % HB == 0 and S % KS == 0
    assert QT % QC == 0 and LOOK * TQ <= S - QT and KS >= M // 2
    assert M % LANES == 0 and M % 64 == 0 and Dc % 64 == 0
    NG = H // HG
    NQ = S // TQ
    NR = S // TR
    NC = M // LANES
    C4 = M // 4
    PLQ = M // 2 + 1
    PLK = Dc // 2 + 1
    NK = S // KC
    XC = S // RCH
    NSEM = NK + 5
    assert NK > RCH + 1 and NQ % G == 0 and NSB >= max(-(-LOOK // G) * G, AHEAD + CL + G)
    HS = Dc // D
    NSL = -(-HG // NC)
    assert H % 2 == 0 and RCH % 2 == 0 and RCH + 4 * NC <= H and NSL * HS + 2 < H - HG
    qscale = float(D) ** -0.5 * LOG2E

    x2 = A_x.reshape(S, M)
    ckv2 = A_c_kv.reshape(S, Dc)
    wo2 = A_w_o.reshape(H * D, M)

    def kernel(x_hbm, ckv_hbm, wq_hbm, wuk_hbm, wuv_hbm, wo_hbm, w1_hbm, w2_hbm,
               w3_hbm, w4_hbm, c_hbm, wmod_hbm, out_hbm, slab_hbm,
               x_v, lhs_v, wq_r, wuk_r, wuv_r, wq_p, wuk_p, wuv_p, wo_v, wou_v, w1_v,
               w2_v, w3_v, w4_v, wmoda_v, wmodb_v, moda_v, modb_v, scb_v, hn_v, wqc_v, wk0_v, q_v, k_v,
               vt_v, s_v, z_s, ctx_v, part_v, x1_v, h2_v, hh_v, o_v, c_v,
               sems):

        ckv_v = lhs_v.at[0]
        z_s[0] = 0
        z_s[1] = 0

        def aligned(i, n):
            return i * n if isinstance(i, int) else pl.multiple_of(i * n, n)

        def cp(src, dst, i):
            return pltpu.make_async_copy(src, dst, sems.at[i])

        def c_ckv(r):
            rows = pl.ds(aligned(r, KC), KC)
            return cp(ckv_hbm.at[rows, :], ckv_v.at[rows, :], r)

        def c_x(j):
            rows = pl.ds(aligned(j, XC), XC)
            return cp(x_hbm.at[rows, :], x_v.at[rows, :], NK - RCH + j)

        def c_q0(j):
            rows = pl.ds(aligned(j, M // RCH), M // RCH)
            return cp(wq_hbm.at[rows, pl.ds(0, HG), :], wq_r.at[0, rows], NK - RCH + j)

        def gcp(src, dst, g, i):
            return cp(src.at[:, pl.ds(g * HG, HG), :], dst.at[g], i)

        c_moda = cp(wmod_hbm.at[:, pl.ds(0, 2 * M)], wmoda_v, NK - RCH - 1)
        c_c = cp(c_hbm, c_v, NK)
        c_k0 = gcp(wuk_hbm, wuk_r, 0, NK + 1)
        c_v0 = gcp(wuv_hbm, wuv_r, 0, NK + 2)
        c_k1 = gcp(wuk_hbm, wuk_r, 1, NK + 3)
        c_late = []
        for g in range(1, NG):
            for src, dst, gg in ((wq_hbm, wq_r, g), (wuv_hbm, wuv_r, g), (wuk_hbm, wuk_r, g + 1)):
                if gg < NG:
                    c_late.append(gcp(src, dst, gg, NSEM - 1))
        for ct in range(4 * NC):
            c_late.append(cp(wmod_hbm.at[:, pl.ds(2 * M + ct * LANES, LANES)],
                             wmodb_v.at[ct], NSEM - 1))
        for u in range(HG):
            c_late.append(cp(wo_hbm.at[pl.ds(u // NC * Dc, Dc), pl.ds(u % NC * D, D)],
                             wou_v.at[u], NSEM - 1))
        for src, dst in ((wo_hbm, wo_v), (w1_hbm, w1_v), (w2_hbm, w2_v),
                         (w3_hbm, w3_v), (w4_hbm, w4_v)):
            c_late.append(cp(src, dst, NSEM - 1))
        order = [c_c, c_k0] + [c_ckv(r) for r in range(NK - RCH)] + [c_moda]
        for j in range(RCH):
            order += [c_ckv(NK - RCH + j), c_x(j), c_q0(j)]
        order += [c_v0, c_k1] + c_late
        for d in order:
            d.start()

        def relayout_steps(raw, dst, g, chunk, rows, plane):
            n = rows // RCH // 2
            base = g * _gstride(plane) + chunk * n
            if not isinstance(base, int):
                base = pl.multiple_of(base, 8)
            view = dst.at[pl.ds(base, 7 * plane + n), :]

            def step(j, tie):
                val = raw[g, pl.ds(chunk * (2 * n) + 2 * j, 2)].reshape(2 * HG, D)
                val = pltpu.bitcast(val, U32)
                if tie is not None:
                    val = val | tie
                view[pl.ds(j, 8, stride=plane), :] = val

            return [functools.partial(step, j) for j in range(n)]

        def relayout(raw, dst, g, rows, plane):
            for ch in range(RCH):
                for step in relayout_steps(raw, dst, g, ch, rows, plane):
                    step(None)

        def head_w32(src, h, rows, plane, par=None):
            base = (h // HG) * _gstride(plane) + ((h % HG) // 2) * plane
            ev = src[pl.ds(base, rows // 2), :]
            od = src[pl.ds(base + 4 * plane, rows // 2), :]
            par = h % 2 if par is None else par
            if par == 0:
                return (ev & U32(0xFFFF)) | (od << 16)
            return (ev >> 16) | (od & U32(0xFFFF0000))

        def q_weight(h, par=None, tie=None):
            wq = head_w32(wq_p, h, M, PLQ, par)
            if tie is not None:
                wq = wq | _rows_op(jnp.bitwise_and, pltpu.bitcast(tie[0:M // 2], U32), zeros8())
            wqc_v[...] = wq

        def q_rows(mx, lo, hi, ties=()):
            wq = wqc_v[...]
            res = []
            for r0 in range(lo, hi, QC):
                rows = slice(r0, r0 + QC)
                w = _tied(wq, ties[len(res)]) if len(res) in ties else wq
                res.append(_dot(hn_v[rows, :], _unpack(w)))
                mx.issue(QC, NC)
                q_v[rows, :] = (res[-1] * qscale).astype(BF16)
            return res

        def slot_weight(h, par):
            late = h >= H - HG
            wk = head_w32(wuk_p, jnp.where(late, h, h + HG), Dc, PLK, par)
            wu = pltpu.bitcast(wou_v[jnp.where(late, h - (H - HG), HG)], U32)
            return jnp.where(late, wu, wk)

        def k_slot(mx, h, w, kh):
            u = jnp.maximum(h - (H - HG), 0)
            lhs = lhs_v.at[jnp.where(h >= H - HG, 1 + u // NC, 0)]
            first = None
            for r in range(S // KS):
                rows = slice(r * KS, (r + 1) * KS)
                res = _dot(lhs[rows, :], _unpack(w))
                mx.issue(KS, HS)
                kh[r * KS // 2:(r + 1) * KS // 2, :] = _pack(res)
                part_v[u, rows, :] = res
                first = res if r == 0 else first
            return first

        def mod_tile(w):
            acc = _fold8(w.astype(F32) * scb_v[...], jnp.add)
            return jnp.broadcast_to(jnp.sum(acc, axis=0, keepdims=True), (8, LANES))

        def mod(i):
            if i < 2:
                return moda_v[0:8, i * M:(i + 1) * M]
            return jnp.concatenate(
                [modb_v[(i - 2) * NC + ct] for ct in range(NC)], axis=1)

        def zeros8():
            return jnp.full((8, LANES), z_s[1], jnp.int32).astype(U32)

        def k_chunk(r, nsub=1, ties=(), after=None, unpack=False):
            n = KC // nsub
            lhs = ckv_v[pl.ds(aligned(r, KC), KC), :]
            for h in range(HG):
                if unpack:
                    w32 = head_w32(wuk_p, h, Dc, PLK)
                    wk0_v[h] = w32
                else:
                    w32 = wk0_v[h]
                for j in range(nsub):
                    i = h * nsub + j
                    rows = pl.ds(aligned(r * nsub + j, n // 2), n // 2)
                    w = _tied(w32, ties[i]) if i in ties else w32
                    res = _dot(lhs[j * n:(j + 1) * n], pltpu.bitcast(w, BF16))
                    k_v[h, rows, :] = _pack(res)
                    if after is not None:
                        after(i, res)

        c_c.wait()
        cc = c_v[...].astype(F32)
        sc = (cc * jax.nn.sigmoid(cc)).astype(BF16).astype(F32)
        scb_v[...] = jnp.broadcast_to(sc, (LANES, M)).T
        zpad = jnp.zeros((PAD, LANES), F32)
        for cidx in range(NC):
            hh_v[cidx, 0:PAD, :] = zpad
            hh_v[cidx, PAD + S:PAD + S + PAD, :] = zpad
        wou_v[HG] = jnp.zeros((Dc, D), BF16)
        wmodb_v[4 * NC] = jnp.zeros((M, LANES), BF16)
        c_k0.wait()
        relayout(wuk_r, wuk_p, 0, Dc, PLK)

        def ka_body(r, carry):
            c_ckv(r).wait()
            k_chunk(r, unpack=True)
            return carry

        jax.lax.fori_loop(0, NK - RCH - 1, ka_body, 0)

        c_ckv(NK - RCH - 1).wait()
        c_moda.wait()
        zero8 = zeros8()
        ties = {}
        for ct in range(2 * NC):
            cols = slice(ct * LANES, (ct + 1) * LANES)
            tile = mod_tile(wmoda_v[:, cols])
            moda_v[0:8, cols] = tile
            ties[2 + (ct * (2 * HG - 2)) // (2 * NC)] = pltpu.bitcast(tile, U32) & zero8
        k_chunk(NK - RCH - 1, 2, ties)

        def kb_body(j, carry):
            c_ckv(NK - RCH + j).wait()
            c_x(j).wait()
            c_q0(j).wait()
            zero8 = zeros8()
            lr = XC // HG
            ties = {}
            scale, shift = 1.0 + mod(1), mod(0)
            for i in range(HG):
                rows = pl.ds(pl.multiple_of(j * XC + i * lr, lr), lr)
                hn = _modulate(_ln(x_v[rows, :].astype(F32)), scale, shift)
                hn_v[rows, :] = hn.astype(BF16)
                ties[i + 2] = pltpu.bitcast(_fold8(hn[:, 0:LANES], jnp.maximum), U32) & zero8
            steps = relayout_steps(wq_r, wq_p, 0, j, M, PLQ)
            per = len(steps) // HG

            def side(i, res):
                for k, step in enumerate(steps[i * per:(i + 1) * per]):
                    step(pltpu.bitcast(res[k * 8:(k + 1) * 8], U32) & zero8)

            k_chunk(NK - RCH + j, 1, ties, side)
            return carry

        jax.lax.fori_loop(0, RCH, kb_body, 0)

        q_weight(0)
        c_v0.wait()
        relayout(wuv_r, wuv_p, 0, Dc, PLK)

        def attention(mx, h, par, kh, side, mod_tie):
            PT = TQ // G
            key_i = jax.lax.broadcasted_iota(jnp.int32, (PT, TQ), 0)
            qry_i = jax.lax.broadcasted_iota(jnp.int32, (PT, TQ), 1)
            z_st = z_s[0]
            z_ld = z_s[1]
            zero8 = zeros8()

            m8 = {}
            seq = []

            def cat(xs):
                return xs[0] if len(xs) == 1 else jnp.concatenate(xs, axis=0)

            def keys(*parts):
                return _unpack(cat([kh[a * PT // 2:b * PT // 2, :] for a, b in parts]))

            def queries(*parts):
                return cat([q_v[a * PT:b * PT, :] for a, b in parts])

            def put(i, t, a, val):
                s_v[i % NSB][z_st + t, a * PT:a * PT + val.shape[0], :] = val
                tm = _fold8(val, jnp.maximum)
                m8[i] = jnp.maximum(m8[i], tm) if i in m8 else tm

            def causal(a, val):
                return jnp.where(key_i + a * PT <= qry_i, val, NEG)

            def mm(a, b):
                res = _dot_nt(a, b)
                mx.issue(a.shape[0])
                seq.append(res[0:8])
                return res

            def corner(g0):
                for a in range(1, G):
                    part = [((g0 + kb) * G + a, (g0 + kb) * G + a + 1) for kb in range(G)]
                    last = (g0 + G - 1) * G
                    strip = mm(queries((last + a, last + G)), keys(*part))
                    yield strip.shape[0]
                    ms = []
                    for b in range(G - 1):
                        i0, i1 = (g0 + b) * G, (g0 + b + 1) * G
                        ms.append(mm(keys(*part[:b + 1]),
                                     queries((i1, i1 + a), (i0 + a, i0 + G))))
                        if b < G - 2:
                            yield ms[-1].shape[0]
                    ms.append(cat([strip[0:PT]] * a + [strip]).T)
                    for b in range(G):
                        for kb in range(b + 1):
                            val = ms[b][kb * PT:(kb + 1) * PT]
                            if kb == b:
                                val = causal(a, val)
                            else:
                                val = jnp.where(qry_i < a * PT,
                                                ms[b - 1][kb * PT:(kb + 1) * PT], val)
                            put(g0 + b, g0 + kb, a, val)
                    yield (G - 1) * PT

            def qk(i):
                g0 = i // G * G
                qi = queries((i * G, (i + 1) * G))
                todo = list(range(g0 * G)) + [t * G for t in range(g0, i + 1)]
                while todo:
                    n = mx.to_grid() // PT
                    n = len(todo) if len(todo) - n < G // 2 else n
                    runs = []
                    for a in todo[:n]:
                        if runs and runs[-1][1] == a and a % G:
                            runs[-1][1] = a + 1
                        else:
                            runs.append([a, a + 1])
                    todo = todo[n:]
                    res = mm(keys(*runs), qi)
                    for a, b in runs:
                        val, res = res[:(b - a) * PT], res[(b - a) * PT:]
                        put(i, a // G, a % G, causal(0, val) if a == i * G else val)
                    yield n * PT

            def pv(i):
                sb = s_v[i % NSB]
                mb = jnp.broadcast_to(jnp.max(m8[i], axis=0, keepdims=True), (8, TQ))
                l8 = None
                ot = None
                for t in range(i + 1):
                    tie = pltpu.bitcast(seq[-DIST], U32) & zero8
                    mt = pltpu.bitcast(pltpu.bitcast(mb, U32) | tie, F32)
                    tile = sb[z_ld + t].reshape(TQ // 8, 8, TQ)
                    p = jnp.exp2(tile - mt[None]).reshape(TQ, TQ)
                    part = _fold8(p, jnp.add)
                    l8 = part if l8 is None else l8 + part
                    o = _dot(_unpack(vt_v[z_ld, :, t * TQ:(t + 1) * TQ]), p.astype(BF16))
                    mx.issue(D)
                    seq.append(o[0:8])
                    o = o.reshape(D // 8, 8, TQ)
                    ot = o if ot is None else ot + o
                    if t == i:
                        l = jnp.sum(l8, axis=0, keepdims=True)
                        ot = ot.reshape(D, TQ) * (1.0 / l)
                        ctx_v[h, i * TQ:(i + 1) * TQ, :] = ot.T.astype(BF16)
                    yield

            def q_gen(lo, hi, prev=None):
                for r0 in range(lo, hi, QC):
                    if prev is not None:
                        seq.extend([prev] * NC)
                    prev = q_rows(mx, r0, r0 + QC)[0][0:8]
                    yield

            def merge(scores, nscore, fill, nspare):
                acc = 0
                while True:
                    while mx.after_short() and next(fill, fill) is not fill:
                        pass
                    if next(scores, None) is None:
                        break
                    acc += max(nspare, 0)
                    while acc >= nscore:
                        acc -= nscore
                        next(fill, None)
                _run(fill)

            CS = G + CSX if G > 2 else 0
            CN = G * (G - 1)
            qrows = -(-LOOK // G) * G * TQ + QX * QC
            q_rows(mx, 0, qrows, mod_tie)
            early = []
            for g0 in range(0, LOOK, G):
                early += [corner(g0)] + [qk(i) for i in range(g0, min(g0 + G, LOOK))]
            merge(_chain_gens(early), 1, q_gen(qrows, S - QT), 0)
            vt = _dot_nt(_unpack(head_w32(wuv_p, h, Dc, PLK, par)).T, ckv_v[...])
            mx.issue(D, NQ * HS)
            vt_v[z_st] = _pack(vt)
            tail = q_gen(S - QT, S, vt[0:8, S - TQ:S])
            merge(corner(G) if LOOK <= G else iter(()), 1, tail, 0)
            per = max(1, -(-len(side) // NQ))
            for j, step in enumerate(side):
                ct, rg = j // per, (j % per) * (D // 8) // per
                src = vt[rg * 8:(rg + 1) * 8, ct * TQ:(ct + 1) * TQ]
                step(pltpu.bitcast(src, U32) & zero8)
            for i in range(NQ):
                j = i + AHEAD
                gens, nscore, nspare = [], 0, i + 1
                if (j + CL) % G == 0 and max(LOOK, G + 1) <= j + CL < NQ:
                    gens.append(corner(j + CL))
                    nscore, nspare = CN, nspare - CS
                if LOOK <= j < NQ:
                    gens.append(qk(j))
                    nscore += j // G * G
                merge(_round_robin(gens), max(nscore, 1), pv(i), nspare)

        def side_work(h):
            g = jnp.minimum(h // HG + ((h % HG) >= RCH).astype(jnp.int32), NG - 1)
            ch = h % RCH
            steps = (relayout_steps(wq_r, wq_p, g, ch, M, PLQ)
                     + relayout_steps(wuv_r, wuv_p, g, ch, Dc, PLK))
            gk = jnp.minimum(h // HG + 1, NG - 1)
            for c in range(RCH):
                steps += relayout_steps(wuk_r, wuk_p, gk, c, Dc, PLK)
            return steps

        c_up = [cp(ctx_v.at[h], slab_hbm.at[h // HS, :, pl.ds(h % HS * D, D)], 1)
                for h in range(NSL * HS)]
        c_down = cp(slab_hbm, lhs_v.at[pl.ds(1, NSL)], 2)

        def head(mx, h, par):
            ct = jnp.where(jnp.logical_and(h >= RCH, h < RCH + 4 * NC), h - RCH, 4 * NC)
            tile = mod_tile(wmodb_v[ct])
            modb_v[ct] = tile
            kh = k_v.at[h % HG]
            attention(mx, h, par, kh, side_work(h), {3: pltpu.bitcast(tile, U32) & zeros8()})
            tie = k_slot(mx, h, slot_weight(h, par), kh)
            q_weight(jnp.minimum(h + 1, H - 2 + (1 - par)), 1 - par, tie)

        def pair_body(j, carry):
            h = 2 * j

            @pl.when(h == 0)
            def _():
                c_k1.wait()

            @pl.when(h == RCH)
            def _():
                for d in c_late:
                    d.wait()

            @pl.when(h == NSL * HS + 2)
            def _():
                for d in c_up:
                    d.wait()

            @pl.when(h == H - HG)
            def _():
                c_down.wait()

            @pl.when(h == NSL * HS)
            def _():
                for d in c_up:
                    d.start()

            @pl.when(h == NSL * HS + 2)
            def _():
                c_down.start()

            mx = _Mxus()
            head(mx, h, 0)
            head(mx, h + 1, 1)
            if os.environ.get('DBG'):
                print('mxu loads', mx.load)
            return carry

        jax.lax.fori_loop(0, H // 2, pair_body, 0)

        def sub_rows(r):
            out = []
            for j in range(TR // HB):
                r0 = r * TR + j * HB
                if not isinstance(r0, int):
                    r0 = pl.multiple_of(r0, HB)
                out.append(r0)
            return out

        def stage1(r):
            atts = []
            for r0 in sub_rows(r):
                rows = pl.ds(r0, HB)
                ctx = [ctx_v[h, rows, :] for h in range(H)]
                cols = []
                for ct in range(NC):
                    units = list(range(ct, HG, NC))
                    h0 = len(units) * HS
                    col = _dot(jnp.concatenate(ctx[h0:], axis=1),
                               wo_v[h0 * D:H * D, ct * LANES:(ct + 1) * LANES])
                    for u in units:
                        col = col + part_v[u, rows, :]
                    cols.append(col)
                atts.append(jnp.concatenate(cols, axis=1))
            lns = []
            for r0, att in zip(sub_rows(r), atts):
                rows = pl.ds(r0, HB)
                x1 = x_v[rows, :].astype(F32) + _rows_op(jnp.multiply, att, mod(2))
                x1_v[rows, :] = x1
                h2 = _modulate(_ln(x1), 1.0 + mod(4), mod(3))
                h2_v[rows, :] = h2
                lns.append(_ln(h2).astype(BF16))
            for r0, ln in zip(sub_rows(r), lns):
                u = _gelu(_dot(ln, w1_v[...]))
                for cidx in range(NC):
                    hh_v[cidx, pl.ds(r0 + PAD, HB), :] = u[:, cidx * LANES:(cidx + 1) * LANES]

        shifts = (1, -1, 2, -2)

        def stage2(r, last):
            lane_i = jax.lax.broadcasted_iota(jnp.int32, (HB, LANES), 1)
            y1s = []
            for r0 in sub_rows(r):
                tiles = []
                for cidx in range(NC):
                    lo, hi = cidx * LANES, (cidx + 1) * LANES
                    g_lo, g_hi = lo // C4, (hi - 1) // C4
                    t = hh_v[cidx, pl.ds(r0 + PAD - shifts[g_hi], HB), :]
                    for g in range(g_hi - 1, g_lo - 1, -1):
                        tg = hh_v[cidx, pl.ds(r0 + PAD - shifts[g], HB), :]
                        t = jnp.where(lane_i < (g + 1) * C4 - lo, tg, t)
                    tiles.append(t)
                hs = _dot(jnp.concatenate(tiles, axis=1).astype(BF16), w2_v[...])
                y1s.append(h2_v[pl.ds(r0, HB), :] + hs)
            gls = []
            f0 = Fh // LANES * LANES
            for y1 in y1s:
                ln = _ln(y1).astype(BF16)
                parts = [_gelu(_dot_nt(ln, w3_v[0:f0 // 2 // LANES * LANES, :]))]
                if f0 < Fh:
                    tail = _gelu(_dot_nt(w3_v[f0:Fh, :], ln)).T
                parts.append(_gelu(_dot_nt(ln, w3_v[f0 // 2 // LANES * LANES:f0, :])))
                if f0 < Fh:
                    parts.append(tail)
                gls.append(jnp.concatenate(parts, axis=1).astype(BF16))
            for k, (r0, y1, gl) in enumerate(zip(sub_rows(r), y1s, gls)):
                rows = pl.ds(r0, HB)
                h3 = _dot(gl, w4_v[...])
                out = x1_v[rows, :] + _rows_op(jnp.multiply, y1 + h3, mod(5))
                split = last and k == len(gls) - 1
                for lo, hi in ((0, M - LANES), (M - LANES, M)) if split else ((0, M),):
                    cols = pl.ds(lo, hi - lo)
                    o_v[rows, cols] = out[:, lo:hi].astype(BF16)
                    cp(o_v.at[rows, cols], out_hbm.at[rows, cols], 0).start()

        def s1_body(r, carry):
            stage1(r)
            return carry

        def s2_body(r, carry):
            for u in range(U2):
                stage2(r * U2 + u, u == U2 - 1)
            return carry

        jax.lax.fori_loop(0, NR, s1_body, 0)
        jax.lax.fori_loop(0, NR // U2, s2_body, 0)
        cp(o_v, out_hbm, 0).wait()

    hbm_spec = pl.BlockSpec(memory_space=pltpu.HBM)
    V = pltpu.VMEM
    scratch = [
        V((S, M), BF16),
        V((1 + NSL, S, Dc), BF16),
        V((NG, M, HG, D), BF16),
        V((NG, Dc, HG, D), BF16),
        V((NG, Dc, HG, D), BF16),
        V((NG * _gstride(PLQ), D), U32),
        V((NG * _gstride(PLK), D), U32),
        V((NG * _gstride(PLK), D), U32),
        V((H * D, M), BF16),
        V((HG + 1, Dc, D), BF16),
        V((M, M), BF16),
        V((M, M), BF16),
        V((Fh, M), BF16),
        V((Fh, M), BF16),
        V((M, 2 * M), BF16),
        V((4 * NC + 1, M, LANES), BF16),
        V((16, 2 * M), F32),
        V((4 * NC + 4, 8, LANES), F32),
        V((M, LANES), F32),
        V((S, M), BF16),
        V((M // 2, D), U32),
        V((HG, Dc // 2, D), U32),
        V((S, D), BF16),
        V((HG, S // 2, D), U32),
        V((1, D // 2, S), U32),
        [V((NQ, TQ, TQ), F32)] * NSB,
        pltpu.SMEM((2,), jnp.int32),
        V((H, S, D), BF16),
        V((HG, S, D), F32),
        V((S, M), F32),
        V((S, M), F32),
        V((NC, S + 2 * PAD, LANES), F32),
        V((S, M), BF16),
        V((1, M), BF16),
        pltpu.SemaphoreType.DMA((NSEM,)),
    ]
    out, _ = pl.pallas_call(
        kernel,
        out_shape=(jax.ShapeDtypeStruct((S, M), BF16),
                   jax.ShapeDtypeStruct((NSL, S, Dc), BF16)),
        in_specs=[hbm_spec] * 12,
        out_specs=(hbm_spec, hbm_spec),
        scratch_shapes=scratch,
        compiler_params=pltpu.CompilerParams(
            vmem_limit_bytes=120 * 1024 * 1024,
            disable_bounds_checks=True,
            disable_semaphore_checks=True,
        ),
        name="adaln_cla_mixer",
    )(x2, ckv2, A_w_q, A_w_uk, A_w_uv, wo2, B_w1, B_w2, B_w3.T, B_w4, c, w_mod)
    return out.reshape(B, S, M)
```

```python
import functools
import math

import jax
import jax.numpy as jnp
import jax.experimental.pallas as pl
import jax.experimental.pallas.tpu as pltpu

BF16 = jnp.bfloat16
F32 = jnp.float32
U32 = jnp.uint32

LANES = 128
TQ = 128
G = 4
TR = 256
HB = 128
HG = 8
RCH = 4
AHEAD = 2
NSB = 8
DIST = 11
KC = 256
KS = 512
QC = 128
QT = 384
U2 = 2
PAD = 16
EPS = 1e-5
LOG2E = math.log2(math.e)
NEG = -1000000000.0 * LOG2E

_NT = (((1,), (1,)), ((), ()))


def _ln(x):
    m = jnp.mean(x, axis=-1, keepdims=True)
    xc = x - m
    v = jnp.mean(xc * xc, axis=-1, keepdims=True)
    return xc * jax.lax.rsqrt(v + EPS)


def _gelu(x):
    return jax.nn.gelu(x, approximate=True)


def _dot(a, b):
    return jnp.dot(a, b, preferred_element_type=F32)


def _dot_nt(a, b):
    return jax.lax.dot_general(a, b, _NT, preferred_element_type=F32)


def _fold8(x, op):
    parts = [op(x[j:j + 8], x[j + 8:j + 16]) for j in range(0, x.shape[0], 16)]
    acc = parts[0]
    for p in parts[1:]:
        acc = op(acc, p)
    return acc


def _rows_op(op, x, v8):
    r, m = x.shape
    return op(x.reshape(r // 8, 8, m), v8[None]).reshape(r, m)


def _modulate(x, scale8, shift8):
    r, m = x.shape
    return (x.reshape(r // 8, 8, m) * scale8[None] + shift8[None]).reshape(r, m)


def _pack(x):
    return pltpu.bitcast(x.astype(BF16), U32)


def _unpack(w):
    return pltpu.bitcast(w, BF16)


def _gstride(plane):
    return -(-8 * plane // 32) * 32


def _tied(w, tie):
    return jnp.concatenate([w[0:8] | tie, w[8:]], axis=0)


class _Mxus:
    def __init__(self):
        self.load = [0] * 4
        self.last = [TQ] * 4

    def next(self):
        return self.load.index(min(self.load))

    def issue(self, rows, count=1):
        for _ in range(count):
            j = self.next()
            self.load[j] += rows
            self.last[j] = rows

    def after_short(self):
        return self.last[self.next()] < TQ // 2

    def to_grid(self):
        rows = TQ - self.load[self.next()] % TQ
        return rows if rows >= TQ // 2 else rows + TQ


def _round_robin(gens):
    gens = list(gens)
    while gens:
        for g in list(gens):
            v = next(g, gens)
            if v is gens:
                gens.remove(g)
            else:
                yield v


def _run(gen):
    for _ in gen:
        pass


def _chain_gens(gens):
    for g in gens:
        yield from g


@jax.jit
def pallas_adaLN_cond__compressed_kv_cla__mixer_s_mlp__prompt_kernel(
    A_x: jax.Array,
    A_c_kv: jax.Array,
    A_w_q: jax.Array,
    A_w_uk: jax.Array,
    A_w_uv: jax.Array,
    A_w_o: jax.Array,
    B_x: jax.Array,
    B_w1: jax.Array,
    B_w2: jax.Array,
    B_w3: jax.Array,
    B_w4: jax.Array,
    c: jax.Array,
    w_mod: jax.Array,
):
    del B_x
    B, S, M = A_x.shape
    _, Sk, Dc = A_c_kv.shape
    _, H, D = A_w_q.shape
    Fh = B_w3.shape[1]
    assert B == 1 and Sk == S and D == LANES and H % HG == 0 and HG == 8
    assert S % TQ == 0 and S % (TR * U2) == 0 and TR % HB == 0 and S % KS == 0
    assert QT % QC == 0 and 2 * G * TQ <= S - QT and KS >= M // 2
    assert M % LANES == 0 and M % 64 == 0 and Dc % 64 == 0
    NG = H // HG
    NQ = S // TQ
    NR = S // TR
    NC = M // LANES
    C4 = M // 4
    PLQ = M // 2 + 1
    PLK = Dc // 2 + 1
    NK = S // KC
    XC = S // RCH
    NSEM = NK + 5
    assert NK > RCH + 1 and NQ % G == 0 and NSB >= max(2 * G, AHEAD + G)
    HS = Dc // D
    NSL = -(-HG // NC)
    assert H % 2 == 0 and RCH % 2 == 0 and RCH + 4 * NC <= H and NSL * HS + 2 < H - HG
    qscale = float(D) ** -0.5 * LOG2E

    x2 = A_x.reshape(S, M)
    ckv2 = A_c_kv.reshape(S, Dc)
    wo2 = A_w_o.reshape(H * D, M)

    def kernel(x_hbm, ckv_hbm, wq_hbm, wuk_hbm, wuv_hbm, wo_hbm, w1_hbm, w2_hbm,
               w3_hbm, w4_hbm, c_hbm, wmod_hbm, out_hbm, slab_hbm,
               x_v, lhs_v, wq_r, wuk_r, wuv_r, wq_p, wuk_p, wuv_p, wo_v, wou_v, w1_v,
               w2_v, w3_v, w4_v, wmoda_v, wmodb_v, moda_v, modb_v, scb_v, hn_v, wqc_v, wk0_v, q_v, k_v,
               vt_v, s_v, z_s, ctx_v, part_v, x1_v, h2_v, hh_v, o_v, c_v,
               sems):

        ckv_v = lhs_v.at[0]
        z_s[0] = 0
        z_s[1] = 0

        def aligned(i, n):
            return i * n if isinstance(i, int) else pl.multiple_of(i * n, n)

        def cp(src, dst, i):
            return pltpu.make_async_copy(src, dst, sems.at[i])

        def c_ckv(r):
            rows = pl.ds(aligned(r, KC), KC)
            return cp(ckv_hbm.at[rows, :], ckv_v.at[rows, :], r)

        def c_x(j):
            rows = pl.ds(aligned(j, XC), XC)
            return cp(x_hbm.at[rows, :], x_v.at[rows, :], NK - RCH + j)

        def c_q0(j):
            rows = pl.ds(aligned(j, M // RCH), M // RCH)
            return cp(wq_hbm.at[rows, pl.ds(0, HG), :], wq_r.at[0, rows], NK - RCH + j)

        def gcp(src, dst, g, i):
            return cp(src.at[:, pl.ds(g * HG, HG), :], dst.at[g], i)

        c_moda = cp(wmod_hbm.at[:, pl.ds(0, 2 * M)], wmoda_v, NK - RCH - 1)
        c_c = cp(c_hbm, c_v, NK)
        c_k0 = gcp(wuk_hbm, wuk_r, 0, NK + 1)
        c_v0 = gcp(wuv_hbm, wuv_r, 0, NK + 2)
        c_k1 = gcp(wuk_hbm, wuk_r, 1, NK + 3)
        c_late = []
        for g in range(1, NG):
            for src, dst, gg in ((wq_hbm, wq_r, g), (wuv_hbm, wuv_r, g), (wuk_hbm, wuk_r, g + 1)):
                if gg < NG:
                    c_late.append(gcp(src, dst, gg, NSEM - 1))
        for ct in range(4 * NC):
            c_late.append(cp(wmod_hbm.at[:, pl.ds(2 * M + ct * LANES, LANES)],
                             wmodb_v.at[ct], NSEM - 1))
        for u in range(HG):
            c_late.append(cp(wo_hbm.at[pl.ds(u // NC * Dc, Dc), pl.ds(u % NC * D, D)],
                             wou_v.at[u], NSEM - 1))
        for src, dst in ((wo_hbm, wo_v), (w1_hbm, w1_v), (w2_hbm, w2_v),
                         (w3_hbm, w3_v), (w4_hbm, w4_v)):
            c_late.append(cp(src, dst, NSEM - 1))
        order = [c_c, c_k0] + [c_ckv(r) for r in range(NK - RCH)] + [c_moda]
        for j in range(RCH):
            order += [c_ckv(NK - RCH + j), c_x(j), c_q0(j)]
        order += [c_v0, c_k1] + c_late
        for d in order:
            d.start()

        def relayout_steps(raw, dst, g, chunk, rows, plane):
            n = rows // RCH // 2
            base = g * _gstride(plane) + chunk * n
            if not isinstance(base, int):
                base = pl.multiple_of(base, 8)
            view = dst.at[pl.ds(base, 7 * plane + n), :]

            def step(j, tie):
                val = raw[g, pl.ds(chunk * (2 * n) + 2 * j, 2)].reshape(2 * HG, D)
                val = pltpu.bitcast(val, U32)
                if tie is not None:
                    val = val | tie
                view[pl.ds(j, 8, stride=plane), :] = val

            return [functools.partial(step, j) for j in range(n)]

        def relayout(raw, dst, g, rows, plane):
            for ch in range(RCH):
                for step in relayout_steps(raw, dst, g, ch, rows, plane):
                    step(None)

        def head_w32(src, h, rows, plane, par=None):
            base = (h // HG) * _gstride(plane) + ((h % HG) // 2) * plane
            ev = src[pl.ds(base, rows // 2), :]
            od = src[pl.ds(base + 4 * plane, rows // 2), :]
            par = h % 2 if par is None else par
            if par == 0:
                return (ev & U32(0xFFFF)) | (od << 16)
            return (ev >> 16) | (od & U32(0xFFFF0000))

        def q_weight(h, par=None, tie=None):
            wq = head_w32(wq_p, h, M, PLQ, par)
            if tie is not None:
                wq = wq | _rows_op(jnp.bitwise_and, pltpu.bitcast(tie[0:M // 2], U32), zeros8())
            wqc_v[...] = wq

        def q_rows(mx, lo, hi, ties=()):
            wq = wqc_v[...]
            res = []
            for r0 in range(lo, hi, QC):
                rows = slice(r0, r0 + QC)
                w = _tied(wq, ties[len(res)]) if len(res) in ties else wq
                res.append(_dot(hn_v[rows, :], _unpack(w)))
                mx.issue(QC, NC)
                q_v[rows, :] = (res[-1] * qscale).astype(BF16)
            return res

        def slot_weight(h, par):
            late = h >= H - HG
            wk = head_w32(wuk_p, jnp.where(late, h, h + HG), Dc, PLK, par)
            wu = pltpu.bitcast(wou_v[jnp.where(late, h - (H - HG), HG)], U32)
            return jnp.where(late, wu, wk)

        def k_slot(mx, h, w, kh):
            u = jnp.maximum(h - (H - HG), 0)
            lhs = lhs_v.at[jnp.where(h >= H - HG, 1 + u // NC, 0)]
            first = None
            for r in range(S // KS):
                rows = slice(r * KS, (r + 1) * KS)
                res = _dot(lhs[rows, :], _unpack(w))
                mx.issue(KS, HS)
                kh[r * KS // 2:(r + 1) * KS // 2, :] = _pack(res)
                part_v[u, rows, :] = res
                first = res if r == 0 else first
            return first

        def mod_tile(w):
            acc = _fold8(w.astype(F32) * scb_v[...], jnp.add)
            return jnp.broadcast_to(jnp.sum(acc, axis=0, keepdims=True), (8, LANES))

        def mod(i):
            if i < 2:
                return moda_v[0:8, i * M:(i + 1) * M]
            return jnp.concatenate(
                [modb_v[(i - 2) * NC + ct] for ct in range(NC)], axis=1)

        def zeros8():
            return jnp.full((8, LANES), z_s[1], jnp.int32).astype(U32)

        def k_chunk(r, nsub=1, ties=(), after=None, unpack=False):
            n = KC // nsub
            lhs = ckv_v[pl.ds(aligned(r, KC), KC), :]
            for h in range(HG):
                if unpack:
                    w32 = head_w32(wuk_p, h, Dc, PLK)
                    wk0_v[h] = w32
                else:
                    w32 = wk0_v[h]
                for j in range(nsub):
                    i = h * nsub + j
                    rows = pl.ds(aligned(r * nsub + j, n // 2), n // 2)
                    w = _tied(w32, ties[i]) if i in ties else w32
                    res = _dot(lhs[j * n:(j + 1) * n], pltpu.bitcast(w, BF16))
                    k_v[h, rows, :] = _pack(res)
                    if after is not None:
                        after(i, res)

        c_c.wait()
        cc = c_v[...].astype(F32)
        sc = (cc * jax.nn.sigmoid(cc)).astype(BF16).astype(F32)
        scb_v[...] = jnp.broadcast_to(sc, (LANES, M)).T
        zpad = jnp.zeros((PAD, LANES), F32)
        for cidx in range(NC):
            hh_v[cidx, 0:PAD, :] = zpad
            hh_v[cidx, PAD + S:PAD + S + PAD, :] = zpad
        wou_v[HG] = jnp.zeros((Dc, D), BF16)
        wmodb_v[4 * NC] = jnp.zeros((M, LANES), BF16)
        c_k0.wait()
        relayout(wuk_r, wuk_p, 0, Dc, PLK)

        def ka_body(r, carry):
            c_ckv(r).wait()
            k_chunk(r, unpack=True)
            return carry

        jax.lax.fori_loop(0, NK - RCH - 1, ka_body, 0)

        c_ckv(NK - RCH - 1).wait()
        c_moda.wait()
        zero8 = zeros8()
        ties = {}
        for ct in range(2 * NC):
            cols = slice(ct * LANES, (ct + 1) * LANES)
            tile = mod_tile(wmoda_v[:, cols])
            moda_v[0:8, cols] = tile
            ties[2 + (ct * (2 * HG - 2)) // (2 * NC)] = pltpu.bitcast(tile, U32) & zero8
        k_chunk(NK - RCH - 1, 2, ties)

        def kb_body(j, carry):
            c_ckv(NK - RCH + j).wait()
            c_x(j).wait()
            c_q0(j).wait()
            zero8 = zeros8()
            lr = XC // HG
            ties = {}
            scale, shift = 1.0 + mod(1), mod(0)
            for i in range(HG):
                rows = pl.ds(pl.multiple_of(j * XC + i * lr, lr), lr)
                hn = _modulate(_ln(x_v[rows, :].astype(F32)), scale, shift)
                hn_v[rows, :] = hn.astype(BF16)
                ties[i + 2] = pltpu.bitcast(_fold8(hn[:, 0:LANES], jnp.maximum), U32) & zero8
            steps = relayout_steps(wq_r, wq_p, 0, j, M, PLQ)
            per = len(steps) // HG

            def side(i, res):
                for k, step in enumerate(steps[i * per:(i + 1) * per]):
                    step(pltpu.bitcast(res[k * 8:(k + 1) * 8], U32) & zero8)

            k_chunk(NK - RCH + j, 1, ties, side)
            return carry

        jax.lax.fori_loop(0, RCH, kb_body, 0)

        q_weight(0)
        c_v0.wait()
        relayout(wuv_r, wuv_p, 0, Dc, PLK)

        def attention(mx, h, par, kh, side, mod_tie):
            PT = TQ // G
            key_i = jax.lax.broadcasted_iota(jnp.int32, (PT, TQ), 0)
            qry_i = jax.lax.broadcasted_iota(jnp.int32, (PT, TQ), 1)
            z_st = z_s[0]
            z_ld = z_s[1]
            zero8 = zeros8()

            m8 = {}
            seq = []

            def cat(xs):
                return xs[0] if len(xs) == 1 else jnp.concatenate(xs, axis=0)

            def keys(*parts):
                return _unpack(cat([kh[a * PT // 2:b * PT // 2, :] for a, b in parts]))

            def queries(*parts):
                return cat([q_v[a * PT:b * PT, :] for a, b in parts])

            def put(i, t, a, val):
                s_v[i % NSB][z_st + t, a * PT:a * PT + val.shape[0], :] = val
                tm = _fold8(val, jnp.maximum)
                m8[i] = jnp.maximum(m8[i], tm) if i in m8 else tm

            def causal(a, val):
                return jnp.where(key_i + a * PT <= qry_i, val, NEG)

            def mm(a, b):
                res = _dot_nt(a, b)
                mx.issue(a.shape[0])
                seq.append(res[0:8])
                return res

            def corner(g0):
                for a in range(1, G):
                    part = [((g0 + kb) * G + a, (g0 + kb) * G + a + 1) for kb in range(G)]
                    last = (g0 + G - 1) * G
                    strip = mm(queries((last + a, last + G)), keys(*part))
                    yield strip.shape[0]
                    ms = []
                    for b in range(G - 1):
                        i0, i1 = (g0 + b) * G, (g0 + b + 1) * G
                        ms.append(mm(keys(*part[:b + 1]),
                                     queries((i1, i1 + a), (i0 + a, i0 + G))))
                        if b < G - 2:
                            yield ms[-1].shape[0]
                    ms.append(cat([strip[0:PT]] * a + [strip]).T)
                    for b in range(G):
                        for kb in range(b + 1):
                            val = ms[b][kb * PT:(kb + 1) * PT]
                            if kb == b:
                                val = causal(a, val)
                            else:
                                val = jnp.where(qry_i < a * PT,
                                                ms[b - 1][kb * PT:(kb + 1) * PT], val)
                            put(g0 + b, g0 + kb, a, val)
                    yield (G - 1) * PT

            def qk(i):
                g0 = i // G * G
                qi = queries((i * G, (i + 1) * G))
                todo = list(range(g0 * G)) + [t * G for t in range(g0, i + 1)]
                while todo:
                    n = mx.to_grid() // PT
                    n = len(todo) if len(todo) - n < G // 2 else n
                    runs = []
                    for a in todo[:n]:
                        if runs and runs[-1][1] == a and a % G:
                            runs[-1][1] = a + 1
                        else:
                            runs.append([a, a + 1])
                    todo = todo[n:]
                    res = mm(keys(*runs), qi)
                    for a, b in runs:
                        val, res = res[:(b - a) * PT], res[(b - a) * PT:]
                        put(i, a // G, a % G, causal(0, val) if a == i * G else val)
                    yield n * PT

            def pv(i):
                sb = s_v[i % NSB]
                mb = jnp.broadcast_to(jnp.max(m8[i], axis=0, keepdims=True), (8, TQ))
                l8 = None
                ot = None
                for t in range(i + 1):
                    tie = pltpu.bitcast(seq[-DIST], U32) & zero8
                    mt = pltpu.bitcast(pltpu.bitcast(mb, U32) | tie, F32)
                    tile = sb[z_ld + t].reshape(TQ // 8, 8, TQ)
                    p = jnp.exp2(tile - mt[None]).reshape(TQ, TQ)
                    part = _fold8(p, jnp.add)
                    l8 = part if l8 is None else l8 + part
                    o = _dot(_unpack(vt_v[z_ld, :, t * TQ:(t + 1) * TQ]), p.astype(BF16))
                    mx.issue(D)
                    seq.append(o[0:8])
                    o = o.reshape(D // 8, 8, TQ)
                    ot = o if ot is None else ot + o
                    if t == i:
                        l = jnp.sum(l8, axis=0, keepdims=True)
                        ot = ot.reshape(D, TQ) * (1.0 / l)
                        ctx_v[h, i * TQ:(i + 1) * TQ, :] = ot.T.astype(BF16)
                    yield

            def q_gen(lo, hi, prev=None):
                for r0 in range(lo, hi, QC):
                    if prev is not None:
                        seq.extend([prev] * NC)
                    prev = q_rows(mx, r0, r0 + QC)[0][0:8]
                    yield

            def merge(scores, nscore, fill, nspare):
                acc = 0
                while True:
                    while mx.after_short() and next(fill, fill) is not fill:
                        pass
                    if next(scores, None) is None:
                        break
                    acc += max(nspare, 0)
                    while acc >= nscore:
                        acc -= nscore
                        next(fill, None)
                _run(fill)

            qrows = G * TQ + 2 * QC
            q_rows(mx, 0, qrows, mod_tie)
            early = [corner(0)] + [qk(i) for i in range(G)]
            merge(_chain_gens(early), 1, q_gen(qrows, S - QT), 0)
            vt = _dot_nt(_unpack(head_w32(wuv_p, h, Dc, PLK, par)).T, ckv_v[...])
            mx.issue(D, NQ * HS)
            vt_v[z_st] = _pack(vt)
            tail = q_gen(S - QT, S, vt[0:8, S - TQ:S])
            merge(corner(G), 1, tail, 0)
            per = max(1, -(-len(side) // NQ))
            for j, step in enumerate(side):
                ct, rg = j // per, (j % per) * (D // 8) // per
                src = vt[rg * 8:(rg + 1) * 8, ct * TQ:(ct + 1) * TQ]
                step(pltpu.bitcast(src, U32) & zero8)
            for i in range(NQ):
                j = i + AHEAD
                gens, nscore, nspare = [], 0, i + 1
                if j % G == 0 and G < j < NQ:
                    gens.append(corner(j))
                    nscore, nspare = G * (G - 1), nspare - G
                if G <= j < NQ:
                    gens.append(qk(j))
                    nscore += j // G * G
                merge(_round_robin(gens), max(nscore, 1), pv(i), nspare)

        def side_work(h):
            g = jnp.minimum(h // HG + ((h % HG) >= RCH).astype(jnp.int32), NG - 1)
            ch = h % RCH
            steps = (relayout_steps(wq_r, wq_p, g, ch, M, PLQ)
                     + relayout_steps(wuv_r, wuv_p, g, ch, Dc, PLK))
            gk = jnp.minimum(h // HG + 1, NG - 1)
            for c in range(RCH):
                steps += relayout_steps(wuk_r, wuk_p, gk, c, Dc, PLK)
            return steps

        c_up = [cp(ctx_v.at[h], slab_hbm.at[h // HS, :, pl.ds(h % HS * D, D)], 1)
                for h in range(NSL * HS)]
        c_down = cp(slab_hbm, lhs_v.at[pl.ds(1, NSL)], 2)

        def head(mx, h, par):
            ct = jnp.where(jnp.logical_and(h >= RCH, h < RCH + 4 * NC), h - RCH, 4 * NC)
            tile = mod_tile(wmodb_v[ct])
            modb_v[ct] = tile
            kh = k_v.at[h % HG]
            attention(mx, h, par, kh, side_work(h), {3: pltpu.bitcast(tile, U32) & zeros8()})
            tie = k_slot(mx, h, slot_weight(h, par), kh)
            q_weight(jnp.minimum(h + 1, H - 2 + (1 - par)), 1 - par, tie)

        def pair_body(j, carry):
            h = 2 * j

            @pl.when(h == 0)
            def _():
                c_k1.wait()

            @pl.when(h == RCH)
            def _():
                for d in c_late:
                    d.wait()

            @pl.when(h == NSL * HS + 2)
            def _():
                for d in c_up:
                    d.wait()

            @pl.when(h == H - HG)
            def _():
                c_down.wait()

            @pl.when(h == NSL * HS)
            def _():
                for d in c_up:
                    d.start()

            @pl.when(h == NSL * HS + 2)
            def _():
                c_down.start()

            mx = _Mxus()
            head(mx, h, 0)
            head(mx, h + 1, 1)
            return carry

        jax.lax.fori_loop(0, H // 2, pair_body, 0)

        def sub_rows(r):
            out = []
            for j in range(TR // HB):
                r0 = r * TR + j * HB
                if not isinstance(r0, int):
                    r0 = pl.multiple_of(r0, HB)
                out.append(r0)
            return out

        def stage1(r):
            atts = []
            for r0 in sub_rows(r):
                rows = pl.ds(r0, HB)
                ctx = [ctx_v[h, rows, :] for h in range(H)]
                cols = []
                for ct in range(NC):
                    units = list(range(ct, HG, NC))
                    h0 = len(units) * HS
                    col = _dot(jnp.concatenate(ctx[h0:], axis=1),
                               wo_v[h0 * D:H * D, ct * LANES:(ct + 1) * LANES])
                    for u in units:
                        col = col + part_v[u, rows, :]
                    cols.append(col)
                atts.append(jnp.concatenate(cols, axis=1))
            lns = []
            for r0, att in zip(sub_rows(r), atts):
                rows = pl.ds(r0, HB)
                x1 = x_v[rows, :].astype(F32) + _rows_op(jnp.multiply, att, mod(2))
                x1_v[rows, :] = x1
                h2 = _modulate(_ln(x1), 1.0 + mod(4), mod(3))
                h2_v[rows, :] = h2
                lns.append(_ln(h2).astype(BF16))
            for r0, ln in zip(sub_rows(r), lns):
                u = _gelu(_dot(ln, w1_v[...]))
                for cidx in range(NC):
                    hh_v[cidx, pl.ds(r0 + PAD, HB), :] = u[:, cidx * LANES:(cidx + 1) * LANES]

        shifts = (1, -1, 2, -2)

        def stage2(r, last):
            lane_i = jax.lax.broadcasted_iota(jnp.int32, (HB, LANES), 1)
            y1s = []
            for r0 in sub_rows(r):
                tiles = []
                for cidx in range(NC):
                    lo, hi = cidx * LANES, (cidx + 1) * LANES
                    g_lo, g_hi = lo // C4, (hi - 1) // C4
                    t = hh_v[cidx, pl.ds(r0 + PAD - shifts[g_hi], HB), :]
                    for g in range(g_hi - 1, g_lo - 1, -1):
                        tg = hh_v[cidx, pl.ds(r0 + PAD - shifts[g], HB), :]
                        t = jnp.where(lane_i < (g + 1) * C4 - lo, tg, t)
                    tiles.append(t)
                hs = _dot(jnp.concatenate(tiles, axis=1).astype(BF16), w2_v[...])
                y1s.append(h2_v[pl.ds(r0, HB), :] + hs)
            gls = []
            f0 = Fh // LANES * LANES
            for y1 in y1s:
                ln = _ln(y1).astype(BF16)
                parts = [_gelu(_dot_nt(ln, w3_v[0:f0 // 2 // LANES * LANES, :]))]
                if f0 < Fh:
                    tail = _gelu(_dot_nt(w3_v[f0:Fh, :], ln)).T
                parts.append(_gelu(_dot_nt(ln, w3_v[f0 // 2 // LANES * LANES:f0, :])))
                if f0 < Fh:
                    parts.append(tail)
                gls.append(jnp.concatenate(parts, axis=1).astype(BF16))
            for k, (r0, y1, gl) in enumerate(zip(sub_rows(r), y1s, gls)):
                rows = pl.ds(r0, HB)
                h3 = _dot(gl, w4_v[...])
                out = x1_v[rows, :] + _rows_op(jnp.multiply, y1 + h3, mod(5))
                split = last and k == len(gls) - 1
                for lo, hi in ((0, M - LANES), (M - LANES, M)) if split else ((0, M),):
                    cols = pl.ds(lo, hi - lo)
                    o_v[rows, cols] = out[:, lo:hi].astype(BF16)
                    cp(o_v.at[rows, cols], out_hbm.at[rows, cols], 0).start()

        def s1_body(r, carry):
            stage1(r)
            return carry

        def s2_body(r, carry):
            for u in range(U2):
                stage2(r * U2 + u, u == U2 - 1)
            return carry

        jax.lax.fori_loop(0, NR, s1_body, 0)
        jax.lax.fori_loop(0, NR // U2, s2_body, 0)
        cp(o_v, out_hbm, 0).wait()

    hbm_spec = pl.BlockSpec(memory_space=pltpu.HBM)
    V = pltpu.VMEM
    scratch = [
        V((S, M), BF16),
        V((1 + NSL, S, Dc), BF16),
        V((NG, M, HG, D), BF16),
        V((NG, Dc, HG, D), BF16),
        V((NG, Dc, HG, D), BF16),
        V((NG * _gstride(PLQ), D), U32),
        V((NG * _gstride(PLK), D), U32),
        V((NG * _gstride(PLK), D), U32),
        V((H * D, M), BF16),
        V((HG + 1, Dc, D), BF16),
        V((M, M), BF16),
        V((M, M), BF16),
        V((Fh, M), BF16),
        V((Fh, M), BF16),
        V((M, 2 * M), BF16),
        V((4 * NC + 1, M, LANES), BF16),
        V((16, 2 * M), F32),
        V((4 * NC + 4, 8, LANES), F32),
        V((M, LANES), F32),
        V((S, M), BF16),
        V((M // 2, D), U32),
        V((HG, Dc // 2, D), U32),
        V((S, D), BF16),
        V((HG, S // 2, D), U32),
        V((1, D // 2, S), U32),
        [V((NQ, TQ, TQ), F32)] * NSB,
        pltpu.SMEM((2,), jnp.int32),
        V((H, S, D), BF16),
        V((HG, S, D), F32),
        V((S, M), F32),
        V((S, M), F32),
        V((NC, S + 2 * PAD, LANES), F32),
        V((S, M), BF16),
        V((1, M), BF16),
        pltpu.SemaphoreType.DMA((NSEM,)),
    ]
    out, _ = pl.pallas_call(
        kernel,
        out_shape=(jax.ShapeDtypeStruct((S, M), BF16),
                   jax.ShapeDtypeStruct((NSL, S, Dc), BF16)),
        in_specs=[hbm_spec] * 12,
        out_specs=(hbm_spec, hbm_spec),
        scratch_shapes=scratch,
        compiler_params=pltpu.CompilerParams(
            vmem_limit_bytes=120 * 1024 * 1024,
            disable_bounds_checks=True,
            disable_semaphore_checks=True,
        ),
        name="adaln_cla_mixer",
    )(x2, ckv2, A_w_q, A_w_uk, A_w_uv, wo2, B_w1, B_w2, B_w3.T, B_w4, c, w_mod)
    return out.reshape(B, S, M)
```

```python
import functools
import math

import jax
import jax.numpy as jnp
import jax.experimental.pallas as pl
import jax.experimental.pallas.tpu as pltpu

BF16 = jnp.bfloat16
F32 = jnp.float32
U32 = jnp.uint32

LANES = 128
TQ = 128
G = 4
TR = 256
HB = 128
HG = 8
RCH = 4
AHEAD = 2
NSB = 8
DIST = 11
KC = 256
KS = 512
QC = 128
QT = 384
U2 = 2
NZ = 8
PAD = 16
EPS = 1e-5
LOG2E = math.log2(math.e)
NEG = -1000000000.0 * LOG2E

_NT = (((1,), (1,)), ((), ()))


def _ln(x):
    m = jnp.mean(x, axis=-1, keepdims=True)
    xc = x - m
    v = jnp.mean(xc * xc, axis=-1, keepdims=True)
    return xc * jax.lax.rsqrt(v + EPS)


def _gelu(x):
    return jax.nn.gelu(x, approximate=True)


def _dot(a, b):
    return jnp.dot(a, b, preferred_element_type=F32)


def _dot_nt(a, b):
    return jax.lax.dot_general(a, b, _NT, preferred_element_type=F32)


def _fold8(x, op):
    parts = [op(x[j:j + 8], x[j + 8:j + 16]) for j in range(0, x.shape[0], 16)]
    acc = parts[0]
    for p in parts[1:]:
        acc = op(acc, p)
    return acc


def _rows_op(op, x, v8):
    r, m = x.shape
    return op(x.reshape(r // 8, 8, m), v8[None]).reshape(r, m)


def _modulate(x, scale8, shift8):
    r, m = x.shape
    return (x.reshape(r // 8, 8, m) * scale8[None] + shift8[None]).reshape(r, m)


def _pack(x):
    return pltpu.bitcast(x.astype(BF16), U32)


def _unpack(w):
    return pltpu.bitcast(w, BF16)


def _gstride(plane):
    return -(-8 * plane // 32) * 32


def _tied(w, tie):
    return jnp.concatenate([w[0:8] | tie, w[8:]], axis=0)


class _Mxus:
    def __init__(self):
        self.load = [0] * 4
        self.last = [TQ] * 4

    def next(self):
        return self.load.index(min(self.load))

    def issue(self, rows, count=1):
        for _ in range(count):
            j = self.next()
            self.load[j] += rows
            self.last[j] = rows

    def after_short(self):
        return self.last[self.next()] < TQ // 2

    def to_grid(self):
        rows = TQ - self.load[self.next()] % TQ
        return rows if rows >= TQ // 2 else rows + TQ


def _round_robin(gens):
    gens = list(gens)
    while gens:
        for g in list(gens):
            v = next(g, gens)
            if v is gens:
                gens.remove(g)
            else:
                yield v


def _run(gen):
    for _ in gen:
        pass


def _chain_gens(gens):
    for g in gens:
        yield from g


@jax.jit
def pallas_adaLN_cond__compressed_kv_cla__mixer_s_mlp__prompt_kernel(
    A_x: jax.Array,
    A_c_kv: jax.Array,
    A_w_q: jax.Array,
    A_w_uk: jax.Array,
    A_w_uv: jax.Array,
    A_w_o: jax.Array,
    B_x: jax.Array,
    B_w1: jax.Array,
    B_w2: jax.Array,
    B_w3: jax.Array,
    B_w4: jax.Array,
    c: jax.Array,
    w_mod: jax.Array,
):
    del B_x
    B, S, M = A_x.shape
    _, Sk, Dc = A_c_kv.shape
    _, H, D = A_w_q.shape
    Fh = B_w3.shape[1]
    assert B == 1 and Sk == S and D == LANES and H % HG == 0 and HG == 8
    assert S % TQ == 0 and S % (TR * U2) == 0 and TR % HB == 0 and S % KS == 0
    assert QT % QC == 0 and 2 * G * TQ <= S - QT and KS >= M // 2
    assert M % LANES == 0 and M % 64 == 0 and Dc % 64 == 0
    NG = H // HG
    NQ = S // TQ
    NR = S // TR
    NC = M // LANES
    C4 = M // 4
    PLQ = M // 2 + 1
    PLK = Dc // 2 + 1
    NK = S // KC
    XC = S // RCH
    NSEM = NK + 5
    assert NK > RCH + 1 and NQ % G == 0 and NSB >= max(2 * G, AHEAD + G)
    HS = Dc // D
    NSL = -(-HG // NC)
    assert H % 2 == 0 and RCH % 2 == 0 and RCH + 4 * NC <= H and NSL * HS + 2 < H - HG
    qscale = float(D) ** -0.5 * LOG2E

    x2 = A_x.reshape(S, M)
    ckv2 = A_c_kv.reshape(S, Dc)
    wo2 = A_w_o.reshape(H * D, M)

    def kernel(x_hbm, ckv_hbm, wq_hbm, wuk_hbm, wuv_hbm, wo_hbm, w1_hbm, w2_hbm,
               w3_hbm, w4_hbm, c_hbm, wmod_hbm, out_hbm, slab_hbm,
               x_v, lhs_v, wq_r, wuk_r, wuv_r, wq_p, wuk_p, wuv_p, wo_v, wou_v, w1_v,
               w2_v, w3_v, w4_v, wmoda_v, wmodb_v, moda_v, modb_v, scb_v, hn_v, wqc_v, wk0_v, q_v, k_v,
               vt_v, s_v, z_s, ctx_v, part_v, x1_v, h2_v, hh_v, o_v, c_v,
               sems):

        ckv_v = lhs_v.at[0]
        for k in range(NZ):
            z_s[k] = 0

        def fresh(ref, k):
            if not k:
                return ref
            return ref.at[pl.ds(pl.multiple_of(z_s[k], 256), ref.shape[0])]

        def aligned(i, n):
            return i * n if isinstance(i, int) else pl.multiple_of(i * n, n)

        def cp(src, dst, i):
            return pltpu.make_async_copy(src, dst, sems.at[i])

        def c_ckv(r):
            rows = pl.ds(aligned(r, KC), KC)
            return cp(ckv_hbm.at[rows, :], ckv_v.at[rows, :], r)

        def c_x(j):
            rows = pl.ds(aligned(j, XC), XC)
            return cp(x_hbm.at[rows, :], x_v.at[rows, :], NK - RCH + j)

        def c_q0(j):
            rows = pl.ds(aligned(j, M // RCH), M // RCH)
            return cp(wq_hbm.at[rows, pl.ds(0, HG), :], wq_r.at[0, rows], NK - RCH + j)

        def gcp(src, dst, g, i):
            return cp(src.at[:, pl.ds(g * HG, HG), :], dst.at[g], i)

        c_moda = cp(wmod_hbm.at[:, pl.ds(0, 2 * M)], wmoda_v, NK - RCH - 1)
        c_c = cp(c_hbm, c_v, NK)
        c_k0 = gcp(wuk_hbm, wuk_r, 0, NK + 1)
        c_v0 = gcp(wuv_hbm, wuv_r, 0, NK + 2)
        c_k1 = gcp(wuk_hbm, wuk_r, 1, NK + 3)
        c_late = []
        for g in range(1, NG):
            for src, dst, gg in ((wq_hbm, wq_r, g), (wuv_hbm, wuv_r, g), (wuk_hbm, wuk_r, g + 1)):
                if gg < NG:
                    c_late.append(gcp(src, dst, gg, NSEM - 1))
        for ct in range(4 * NC):
            c_late.append(cp(wmod_hbm.at[:, pl.ds(2 * M + ct * LANES, LANES)],
                             wmodb_v.at[ct], NSEM - 1))
        for u in range(HG):
            c_late.append(cp(wo_hbm.at[pl.ds(u // NC * Dc, Dc), pl.ds(u % NC * D, D)],
                             wou_v.at[u], NSEM - 1))
        for src, dst in ((wo_hbm, wo_v), (w1_hbm, w1_v), (w2_hbm, w2_v),
                         (w3_hbm, w3_v), (w4_hbm, w4_v)):
            c_late.append(cp(src, dst, NSEM - 1))
        order = [c_c, c_k0] + [c_ckv(r) for r in range(NK - RCH)] + [c_moda]
        for j in range(RCH):
            order += [c_ckv(NK - RCH + j), c_x(j), c_q0(j)]
        order += [c_v0, c_k1] + c_late
        for d in order:
            d.start()

        def relayout_steps(raw, dst, g, chunk, rows, plane):
            n = rows // RCH // 2
            base = g * _gstride(plane) + chunk * n
            if not isinstance(base, int):
                base = pl.multiple_of(base, 8)
            view = dst.at[pl.ds(base, 7 * plane + n), :]

            def step(j, tie):
                val = raw[g, pl.ds(chunk * (2 * n) + 2 * j, 2)].reshape(2 * HG, D)
                val = pltpu.bitcast(val, U32)
                if tie is not None:
                    val = val | tie
                view[pl.ds(j, 8, stride=plane), :] = val

            return [functools.partial(step, j) for j in range(n)]

        def relayout(raw, dst, g, rows, plane):
            for ch in range(RCH):
                for step in relayout_steps(raw, dst, g, ch, rows, plane):
                    step(None)

        def head_w32(src, h, rows, plane, par=None):
            base = (h // HG) * _gstride(plane) + ((h % HG) // 2) * plane
            ev = src[pl.ds(base, rows // 2), :]
            od = src[pl.ds(base + 4 * plane, rows // 2), :]
            par = h % 2 if par is None else par
            if par == 0:
                return (ev & U32(0xFFFF)) | (od << 16)
            return (ev >> 16) | (od & U32(0xFFFF0000))

        def q_weight(h, par=None, tie=None):
            wq = head_w32(wq_p, h, M, PLQ, par)
            if tie is not None:
                wq = wq | _rows_op(jnp.bitwise_and, pltpu.bitcast(tie[0:M // 2], U32), zeros8())
            wqc_v[...] = wq

        def q_rows(mx, lo, hi, ties=()):
            wq = wqc_v[...]
            res = []
            for r0 in range(lo, hi, QC):
                rows = slice(r0, r0 + QC)
                w = _tied(wq, ties[len(res)]) if len(res) in ties else wq
                res.append(_dot(hn_v[rows, :], _unpack(w)))
                mx.issue(QC, NC)
                q_v[rows, :] = (res[-1] * qscale).astype(BF16)
            return res

        def slot_weight(h, par):
            late = h >= H - HG
            wk = head_w32(wuk_p, jnp.where(late, h, h + HG), Dc, PLK, par)
            wu = pltpu.bitcast(wou_v[jnp.where(late, h - (H - HG), HG)], U32)
            return jnp.where(late, wu, wk)

        def k_slot(mx, h, w, kh):
            u = jnp.maximum(h - (H - HG), 0)
            lhs = lhs_v.at[jnp.where(h >= H - HG, 1 + u // NC, 0)]
            first = None
            for r in range(S // KS):
                rows = slice(r * KS, (r + 1) * KS)
                res = _dot(lhs[rows, :], _unpack(w))
                mx.issue(KS, HS)
                kh[r * KS // 2:(r + 1) * KS // 2, :] = _pack(res)
                part_v[u, rows, :] = res
                first = res if r == 0 else first
            return first

        def mod_tile(w):
            acc = _fold8(w.astype(F32) * scb_v[...], jnp.add)
            return jnp.broadcast_to(jnp.sum(acc, axis=0, keepdims=True), (8, LANES))

        def mod(i):
            if i < 2:
                return moda_v[0:8, i * M:(i + 1) * M]
            return jnp.concatenate(
                [modb_v[(i - 2) * NC + ct] for ct in range(NC)], axis=1)

        def zeros8():
            return jnp.full((8, LANES), z_s[1], jnp.int32).astype(U32)

        def k_chunk(r, nsub=1, ties=(), after=None, unpack=False):
            n = KC // nsub
            lhs = ckv_v[pl.ds(aligned(r, KC), KC), :]
            for h in range(HG):
                if unpack:
                    w32 = head_w32(wuk_p, h, Dc, PLK)
                    wk0_v[h] = w32
                else:
                    w32 = wk0_v[h]
                for j in range(nsub):
                    i = h * nsub + j
                    rows = pl.ds(aligned(r * nsub + j, n // 2), n // 2)
                    w = _tied(w32, ties[i]) if i in ties else w32
                    res = _dot(lhs[j * n:(j + 1) * n], pltpu.bitcast(w, BF16))
                    k_v[h, rows, :] = _pack(res)
                    if after is not None:
                        after(i, res)

        c_c.wait()
        cc = c_v[...].astype(F32)
        sc = (cc * jax.nn.sigmoid(cc)).astype(BF16).astype(F32)
        scb_v[...] = jnp.broadcast_to(sc, (LANES, M)).T
        zpad = jnp.zeros((PAD, LANES), F32)
        for cidx in range(NC):
            hh_v[cidx, 0:PAD, :] = zpad
            hh_v[cidx, PAD + S:PAD + S + PAD, :] = zpad
        wou_v[HG] = jnp.zeros((Dc, D), BF16)
        wmodb_v[4 * NC] = jnp.zeros((M, LANES), BF16)
        c_k0.wait()
        relayout(wuk_r, wuk_p, 0, Dc, PLK)

        def ka_body(r, carry):
            c_ckv(r).wait()
            k_chunk(r, unpack=True)
            return carry

        jax.lax.fori_loop(0, NK - RCH - 1, ka_body, 0)

        c_ckv(NK - RCH - 1).wait()
        c_moda.wait()
        zero8 = zeros8()
        ties = {}
        for ct in range(2 * NC):
            cols = slice(ct * LANES, (ct + 1) * LANES)
            tile = mod_tile(wmoda_v[:, cols])
            moda_v[0:8, cols] = tile
            ties[2 + (ct * (2 * HG - 2)) // (2 * NC)] = pltpu.bitcast(tile, U32) & zero8
        k_chunk(NK - RCH - 1, 2, ties)

        def kb_body(j, carry):
            c_ckv(NK - RCH + j).wait()
            c_x(j).wait()
            c_q0(j).wait()
            zero8 = zeros8()
            lr = XC // HG
            ties = {}
            scale, shift = 1.0 + mod(1), mod(0)
            for i in range(HG):
                rows = pl.ds(pl.multiple_of(j * XC + i * lr, lr), lr)
                hn = _modulate(_ln(x_v[rows, :].astype(F32)), scale, shift)
                hn_v[rows, :] = hn.astype(BF16)
                ties[i + 2] = pltpu.bitcast(_fold8(hn[:, 0:LANES], jnp.maximum), U32) & zero8
            steps = relayout_steps(wq_r, wq_p, 0, j, M, PLQ)
            per = len(steps) // HG

            def side(i, res):
                for k, step in enumerate(steps[i * per:(i + 1) * per]):
                    step(pltpu.bitcast(res[k * 8:(k + 1) * 8], U32) & zero8)

            k_chunk(NK - RCH + j, 1, ties, side)
            return carry

        jax.lax.fori_loop(0, RCH, kb_body, 0)

        q_weight(0)
        c_v0.wait()
        relayout(wuv_r, wuv_p, 0, Dc, PLK)

        def attention(mx, h, par, kh, side, mod_tie):
            PT = TQ // G
            key_i = jax.lax.broadcasted_iota(jnp.int32, (PT, TQ), 0)
            qry_i = jax.lax.broadcasted_iota(jnp.int32, (PT, TQ), 1)
            z_st = z_s[0]
            z_ld = z_s[1]
            zero8 = zeros8()

            m8 = {}
            seq = []

            def cat(xs):
                return xs[0] if len(xs) == 1 else jnp.concatenate(xs, axis=0)

            def keys(*parts):
                return _unpack(cat([kh[a * PT // 2:b * PT // 2, :] for a, b in parts]))

            def queries(*parts):
                return cat([q_v[a * PT:b * PT, :] for a, b in parts])

            def put(i, t, a, val):
                s_v[i % NSB][z_st + t, a * PT:a * PT + val.shape[0], :] = val
                tm = _fold8(val, jnp.maximum)
                m8[i] = jnp.maximum(m8[i], tm) if i in m8 else tm

            def causal(a, val):
                return jnp.where(key_i + a * PT <= qry_i, val, NEG)

            def mm(a, b):
                res = _dot_nt(a, b)
                mx.issue(a.shape[0])
                seq.append(res[0:8])
                return res

            def corner(g0):
                for a in range(1, G):
                    part = [((g0 + kb) * G + a, (g0 + kb) * G + a + 1) for kb in range(G)]
                    last = (g0 + G - 1) * G
                    strip = mm(queries((last + a, last + G)), keys(*part))
                    yield strip.shape[0]
                    ms = []
                    for b in range(G - 1):
                        i0, i1 = (g0 + b) * G, (g0 + b + 1) * G
                        ms.append(mm(keys(*part[:b + 1]),
                                     queries((i1, i1 + a), (i0 + a, i0 + G))))
                        if b < G - 2:
                            yield ms[-1].shape[0]
                    ms.append(cat([strip[0:PT]] * a + [strip]).T)
                    for b in range(G):
                        for kb in range(b + 1):
                            val = ms[b][kb * PT:(kb + 1) * PT]
                            if kb == b:
                                val = causal(a, val)
                            else:
                                val = jnp.where(qry_i < a * PT,
                                                ms[b - 1][kb * PT:(kb + 1) * PT], val)
                            put(g0 + b, g0 + kb, a, val)
                    yield (G - 1) * PT

            def qk(i):
                g0 = i // G * G
                qi = queries((i * G, (i + 1) * G))
                todo = list(range(g0 * G)) + [t * G for t in range(g0, i + 1)]
                while todo:
                    n = mx.to_grid() // PT
                    n = len(todo) if len(todo) - n < G // 2 else n
                    runs = []
                    for a in todo[:n]:
                        if runs and runs[-1][1] == a and a % G:
                            runs[-1][1] = a + 1
                        else:
                            runs.append([a, a + 1])
                    todo = todo[n:]
                    res = mm(keys(*runs), qi)
                    off = 0
                    for a, b in runs:
                        val = res[off:off + (b - a) * PT]
                        off += (b - a) * PT
                        put(i, a // G, a % G, causal(0, val) if a == i * G else val)
                    yield n * PT

            def pv(i):
                sb = s_v[i % NSB]
                mb = jnp.broadcast_to(jnp.max(m8[i], axis=0, keepdims=True), (8, TQ))
                l8 = None
                ot = None
                for t in range(i + 1):
                    tie = pltpu.bitcast(seq[-DIST], U32) & zero8
                    mt = pltpu.bitcast(pltpu.bitcast(mb, U32) | tie, F32)
                    tile = sb[z_ld + t].reshape(TQ // 8, 8, TQ)
                    p = jnp.exp2(tile - mt[None]).reshape(TQ, TQ)
                    part = _fold8(p, jnp.add)
                    l8 = part if l8 is None else l8 + part
                    o = _dot(_unpack(vt_v[z_ld, :, t * TQ:(t + 1) * TQ]), p.astype(BF16))
                    mx.issue(D)
                    seq.append(o[0:8])
                    o = o.reshape(D // 8, 8, TQ)
                    ot = o if ot is None else ot + o
                    if t == i:
                        l = jnp.sum(l8, axis=0, keepdims=True)
                        ot = ot.reshape(D, TQ) * (1.0 / l)
                        ctx_v[h, i * TQ:(i + 1) * TQ, :] = ot.T.astype(BF16)
                    yield

            def q_gen(lo, hi, prev=None):
                for r0 in range(lo, hi, QC):
                    if prev is not None:
                        seq.extend([prev] * NC)
                    prev = q_rows(mx, r0, r0 + QC)[0][0:8]
                    yield

            def merge(scores, nscore, fill, nspare):
                acc = 0
                while True:
                    while mx.after_short() and next(fill, fill) is not fill:
                        pass
                    if next(scores, None) is None:
                        break
                    acc += max(nspare, 0)
                    while acc >= nscore:
                        acc -= nscore
                        next(fill, None)
                _run(fill)

            qrows = G * TQ + 2 * QC
            q_rows(mx, 0, qrows, mod_tie)
            early = [corner(0)] + [qk(i) for i in range(G)]
            merge(_chain_gens(early), 1, q_gen(qrows, S - QT), 0)
            vt = _dot_nt(_unpack(head_w32(wuv_p, h, Dc, PLK, par)).T, ckv_v[...])
            mx.issue(D, NQ * HS)
            vt_v[z_st] = _pack(vt)
            tail = q_gen(S - QT, S, vt[0:8, S - TQ:S])
            merge(corner(G), 1, tail, 0)
            per = max(1, -(-len(side) // NQ))
            for j, step in enumerate(side):
                ct, rg = j // per, (j % per) * (D // 8) // per
                src = vt[rg * 8:(rg + 1) * 8, ct * TQ:(ct + 1) * TQ]
                step(pltpu.bitcast(src, U32) & zero8)
            for i in range(NQ):
                j = i + AHEAD
                gens, nscore, nspare = [], 0, i + 1
                if j % G == 0 and G < j < NQ:
                    gens.append(corner(j))
                    nscore, nspare = G * (G - 1), nspare - G
                if G <= j < NQ:
                    gens.append(qk(j))
                    nscore += j // G * G
                merge(_round_robin(gens), max(nscore, 1), pv(i), nspare)

        def side_work(h):
            g = jnp.minimum(h // HG + ((h % HG) >= RCH).astype(jnp.int32), NG - 1)
            ch = h % RCH
            steps = (relayout_steps(wq_r, wq_p, g, ch, M, PLQ)
                     + relayout_steps(wuv_r, wuv_p, g, ch, Dc, PLK))
            gk = jnp.minimum(h // HG + 1, NG - 1)
            for c in range(RCH):
                steps += relayout_steps(wuk_r, wuk_p, gk, c, Dc, PLK)
            return steps

        c_up = [cp(ctx_v.at[h], slab_hbm.at[h // HS, :, pl.ds(h % HS * D, D)], 1)
                for h in range(NSL * HS)]
        c_down = cp(slab_hbm, lhs_v.at[pl.ds(1, NSL)], 2)

        def head(mx, h, par):
            ct = jnp.where(jnp.logical_and(h >= RCH, h < RCH + 4 * NC), h - RCH, 4 * NC)
            tile = mod_tile(wmodb_v[ct])
            modb_v[ct] = tile
            kh = k_v.at[h % HG]
            attention(mx, h, par, kh, side_work(h), {3: pltpu.bitcast(tile, U32) & zeros8()})
            tie = k_slot(mx, h, slot_weight(h, par), kh)
            q_weight(jnp.minimum(h + 1, H - 2 + (1 - par)), 1 - par, tie)

        def pair_body(j, carry):
            h = 2 * j

            @pl.when(h == 0)
            def _():
                c_k1.wait()

            @pl.when(h == RCH)
            def _():
                for d in c_late:
                    d.wait()

            @pl.when(h == NSL * HS + 2)
            def _():
                for d in c_up:
                    d.wait()

            @pl.when(h == H - HG)
            def _():
                c_down.wait()

            @pl.when(h == NSL * HS)
            def _():
                for d in c_up:
                    d.start()

            @pl.when(h == NSL * HS + 2)
            def _():
                c_down.start()

            mx = _Mxus()
            head(mx, h, 0)
            head(mx, h + 1, 1)
            return carry

        jax.lax.fori_loop(0, H // 2, pair_body, 0)

        def sub_rows(r):
            out = []
            for j in range(TR // HB):
                r0 = r * TR + j * HB
                if not isinstance(r0, int):
                    r0 = pl.multiple_of(r0, HB)
                out.append(r0)
            return out

        def stage1(r):
            atts = []
            for k, r0 in enumerate(sub_rows(r)):
                rows = pl.ds(r0, HB)
                cols = []
                for ct in range(NC):
                    units = list(range(ct, HG, NC))
                    h0 = len(units) * HS
                    ctx = fresh(ctx_v, ct)
                    lhs = jnp.concatenate([ctx[h, rows, :] for h in range(h0, H)], axis=1)
                    w = wo_v[h0 * D:H * D, ct * LANES:(ct + 1) * LANES]
                    if ct == NC - 1 and k == TR // HB - 1:
                        col = jnp.concatenate(
                            [_dot(lhs[0:HB // 2], w), _dot(lhs[HB // 2:HB], w)], axis=0)
                    else:
                        col = _dot(lhs, w)
                    for u in units:
                        col = col + part_v[u, rows, :]
                    cols.append(col)
                atts.append(jnp.concatenate(cols, axis=1))
            lns = []
            for k, (r0, att) in enumerate(zip(sub_rows(r), atts)):
                rows = pl.ds(r0, HB)
                x1 = x_v[rows, :].astype(F32) + _rows_op(jnp.multiply, att, mod(2))
                x1_v[rows, :] = x1
                h2 = _modulate(_ln(x1), 1.0 + mod(4), mod(3))
                h2_v[rows, :] = h2
                if k == 0:
                    h2 = fresh(h2_v, 1)[rows, :]
                lns.append(_ln(h2).astype(BF16))
            for r0, ln in zip(sub_rows(r), lns):
                u = _gelu(_dot(ln, w1_v[...]))
                for cidx in range(NC):
                    hh_v[cidx, pl.ds(r0 + PAD, HB), :] = u[:, cidx * LANES:(cidx + 1) * LANES]

        shifts = (1, -1, 2, -2)

        def stage2(r, last, k0):
            lane_i = jax.lax.broadcasted_iota(jnp.int32, (HB, LANES), 1)
            y1s = []
            for k, r0 in enumerate(sub_rows(r)):
                tiles = []
                for cidx in range(NC):
                    lo, hi = cidx * LANES, (cidx + 1) * LANES
                    g_lo, g_hi = lo // C4, (hi - 1) // C4
                    t = hh_v[cidx, pl.ds(r0 + PAD - shifts[g_hi], HB), :]
                    for g in range(g_hi - 1, g_lo - 1, -1):
                        tg = hh_v[cidx, pl.ds(r0 + PAD - shifts[g], HB), :]
                        t = jnp.where(lane_i < (g + 1) * C4 - lo, tg, t)
                    tiles.append(t)
                hs = _dot(jnp.concatenate(tiles, axis=1).astype(BF16),
                          fresh(w2_v, k0 + k)[...])
                y1s.append(h2_v[pl.ds(r0, HB), :] + hs)
            gls = []
            f0 = Fh // LANES * LANES
            for k, y1 in enumerate(y1s):
                ln = _ln(y1).astype(BF16)
                w3 = fresh(w3_v, k0 + k)
                parts = [_gelu(_dot_nt(ln, w3[0:f0 // 2 // LANES * LANES, :]))]
                if f0 < Fh:
                    tail = _gelu(_dot_nt(w3[f0:Fh, :], ln)).T
                parts.append(_gelu(_dot_nt(ln, w3[f0 // 2 // LANES * LANES:f0, :])))
                if f0 < Fh:
                    parts.append(tail)
                gls.append(jnp.concatenate(parts, axis=1).astype(BF16))
            for k, (r0, y1, gl) in enumerate(zip(sub_rows(r), y1s, gls)):
                rows = pl.ds(r0, HB)
                h3 = _dot(gl, fresh(w4_v, k0 + k)[...])
                out = x1_v[rows, :] + _rows_op(jnp.multiply, y1 + h3, mod(5))
                split = last and k == len(gls) - 1
                for lo, hi in ((0, M - LANES), (M - LANES, M)) if split else ((0, M),):
                    cols = pl.ds(lo, hi - lo)
                    o_v[rows, cols] = out[:, lo:hi].astype(BF16)
                    cp(o_v.at[rows, cols], out_hbm.at[rows, cols], 0).start()

        def s1_body(r, carry):
            stage1(r)
            return carry

        def s2_body(r, carry):
            for u in range(U2):
                stage2(r * U2 + u, u == U2 - 1, u * (TR // HB))
            return carry

        jax.lax.fori_loop(0, NR, s1_body, 0)
        jax.lax.fori_loop(0, NR // U2, s2_body, 0)
        cp(o_v, out_hbm, 0).wait()

    hbm_spec = pl.BlockSpec(memory_space=pltpu.HBM)
    V = pltpu.VMEM
    scratch = [
        V((S, M), BF16),
        V((1 + NSL, S, Dc), BF16),
        V((NG, M, HG, D), BF16),
        V((NG, Dc, HG, D), BF16),
        V((NG, Dc, HG, D), BF16),
        V((NG * _gstride(PLQ), D), U32),
        V((NG * _gstride(PLK), D), U32),
        V((NG * _gstride(PLK), D), U32),
        V((H * D, M), BF16),
        V((HG + 1, Dc, D), BF16),
        V((M, M), BF16),
        V((M, M), BF16),
        V((Fh, M), BF16),
        V((Fh, M), BF16),
        V((M, 2 * M), BF16),
        V((4 * NC + 1, M, LANES), BF16),
        V((16, 2 * M), F32),
        V((4 * NC + 4, 8, LANES), F32),
        V((M, LANES), F32),
        V((S, M), BF16),
        V((M // 2, D), U32),
        V((HG, Dc // 2, D), U32),
        V((S, D), BF16),
        V((HG, S // 2, D), U32),
        V((1, D // 2, S), U32),
        [V((NQ, TQ, TQ), F32)] * NSB,
        pltpu.SMEM((NZ,), jnp.int32),
        V((H, S, D), BF16),
        V((HG, S, D), F32),
        V((S, M), F32),
        V((S, M), F32),
        V((NC, S + 2 * PAD, LANES), F32),
        V((S, M), BF16),
        V((1, M), BF16),
        pltpu.SemaphoreType.DMA((NSEM,)),
    ]
    out, _ = pl.pallas_call(
        kernel,
        out_shape=(jax.ShapeDtypeStruct((S, M), BF16),
                   jax.ShapeDtypeStruct((NSL, S, Dc), BF16)),
        in_specs=[hbm_spec] * 12,
        out_specs=(hbm_spec, hbm_spec),
        scratch_shapes=scratch,
        compiler_params=pltpu.CompilerParams(
            vmem_limit_bytes=120 * 1024 * 1024,
            disable_bounds_checks=True,
            disable_semaphore_checks=True,
        ),
        name="adaln_cla_mixer",
    )(x2, ckv2, A_w_q, A_w_uk, A_w_uv, wo2, B_w1, B_w2, B_w3.T, B_w4, c, w_mod)
    return out.reshape(B, S, M)
```
